```python
import os as _os
_os.environ.setdefault("JAX_PLATFORMS", "cpu")
import jax
import jax.numpy as jnp

def _softmax(x, axis=-1):
    return jax.nn.softmax(x, axis=axis)
def _gelu(x):
    return jax.nn.gelu(x, approximate=True)
def _silu(x):
    return jax.nn.silu(x)
def _sigmoid(x):
    return jax.nn.sigmoid(x)
def _layernorm(x, axis=-1, eps=1e-5):
    m = jnp.mean(x, axis=axis, keepdims=True)
    v = jnp.var(x, axis=axis, keepdims=True)
    return (x - m) / jnp.sqrt(v + eps)
def _scatter_add(tgt, idx, src, axis=0):
    return tgt.at[idx].add(src)
def _segment_sum(src, seg, n):
    return jax.ops.segment_sum(src, seg, n)
class _Rng:
    def __init__(self, key):
        self._k = key
    def _next(self):
        self._k, sub = jax.random.split(self._k)
        return sub
    def normal(self, shape):
        return jax.random.normal(self._next(), shape, dtype=jnp.bfloat16)
    def randint(self, lo, hi, shape):
        return jax.random.randint(self._next(), shape, lo, hi, dtype=jnp.int32)
    def uniform(self, shape, lo=0.0, hi=1.0):
        return jax.random.uniform(self._next(), shape, jnp.bfloat16, lo, hi)
    def permutation(self, n):
        return jax.random.permutation(self._next(), n)


kernel_name = 'recurrent_scan__ssm_conv_s4__mixer_s_mlp__prompt'

def setup_inputs():
    _rng = _Rng(jax.random.key(int.from_bytes(__import__("os").urandom(4), "little")))
    _w = (lambda a: (lambda t: t.astype(jnp.bfloat16) if jnp.issubdtype(t.dtype, jnp.floating) else t)(jnp.asarray(a)))
    def _A_setup():
        B, L, D, N = 1, 2048, 512, 128
        A_re = -jnp.exp((lambda *s: _rng.normal(s) * 0.1)(D, N))
        A_im = jnp.pi * (lambda *s: _rng.normal(s) * 0.1)(D, N)
        B_re = (lambda *s: _rng.normal(s) * 0.1)(D, N)
        B_im = (lambda *s: _rng.normal(s) * 0.1)(D, N)
        C_re = (lambda *s: _rng.normal(s) * 0.1)(D, N)
        C_im = (lambda *s: _rng.normal(s) * 0.1)(D, N)
        log_dt = (lambda *s: _rng.normal(s) * 0.1)(D) * 0.5 - 4.0
        Dskip = (lambda *s: _rng.normal(s) * 0.05)(D)
        return {
            "u": _w((lambda *s: _rng.normal(s) * 0.05)(B, L, D)),
            "A_re": _w(A_re),
            "A_im": _w(A_im),
            "B_re": _w(B_re),
            "B_im": _w(B_im),
            "C_re": _w(C_re),
            "C_im": _w(C_im),
            "log_dt": _w(log_dt),
            "Dskip": _w(Dskip),
        }
    _A_in = _A_setup()

    def _B_setup():
        B, S, D, F = 1, 2048, 512, 1376
        return {
            "x":  _w((lambda *s: _rng.normal(s) * 0.05)(B, S, D)),
            "w1": _w((lambda *s: _rng.normal(s) * 0.8)(D, D) * (D ** -0.5)),
            "w2": _w((lambda *s: _rng.normal(s) * 0.8)(D, D) * (D ** -0.5)),
            "w3": _w((lambda *s: _rng.normal(s) * 0.8)(D, F) * (D ** -0.5)),
            "w4": _w((lambda *s: _rng.normal(s) * 0.8)(F, D) * (F ** -0.5)),
        }
    _B_in = _B_setup()

    return {
        "A_u": _A_in["u"],
        "A_A_re": _A_in["A_re"],
        "A_A_im": _A_in["A_im"],
        "A_B_re": _A_in["B_re"],
        "A_B_im": _A_in["B_im"],
        "A_C_re": _A_in["C_re"],
        "A_C_im": _A_in["C_im"],
        "A_log_dt": _A_in["log_dt"],
        "A_Dskip": _A_in["Dskip"],
        "B_x": _B_in["x"],
        "B_w1": _B_in["w1"],
        "B_w2": _B_in["w2"],
        "B_w3": _B_in["w3"],
        "B_w4": _B_in["w4"],
    }

def reference(A_u, A_A_re, A_A_im, A_B_re, A_B_im, A_C_re, A_C_im, A_log_dt, A_Dskip, B_x, B_w1, B_w2, B_w3, B_w4):
    def _A_ref(u, A_re, A_im, B_re, B_im, C_re, C_im, log_dt, Dskip):
        Bsz, L, D = u.shape
        dt = jnp.exp(log_dt)[:, None]
        A = A_re + 1j * A_im
        Bc = B_re + 1j * B_im
        Cc = C_re + 1j * C_im
        logdA = dt * A
        dB = dt * Bc
        l = (lambda x, dt: x.astype(dt))(jnp.arange(L), A_re.dtype)
        P = jnp.exp(logdA[:, :, None] * l[None, None, :])
        K = jnp.einsum("dn,dnl,dn->dl", Cc, P, dB).real
        L2 = 2 * L
        Kp = jnp.pad(K, ((0, 0), (0, L)))
        up = (lambda x, *d: x.transpose(*d))(u, 0, 2, 1)
        up = jnp.pad(up, ((0, 0), (0, 0), (0, L)))
        Kf = (lambda x, axes=(-2,-1): jnp.fft.rfft2(x.astype(jnp.float32), axes=axes))(Kp[:, None, :], axes=(-2, -1))
        Uf = (lambda x, axes=(-2,-1): jnp.fft.rfft2(x.astype(jnp.float32), axes=axes))(up[:, :, None, :], axes=(-2, -1))
        Yf = Uf * Kf[None, :, :, :]
        y = (lambda x, s, axes=(-2,-1): jnp.fft.irfft2(x, s=s, axes=axes).astype(jnp.bfloat16))(Yf, (1, L2), axes=(-2, -1))[:, :, 0, :L]
        y = (lambda x, *d: x.transpose(*d))(y, 0, 2, 1) + u * Dskip[None, None, :]
        return y

    def _B_ref(x, w1, w2, w3, w4):
        B, S, D = x.shape
        h = _gelu(_layernorm(x, axis=-1) @ w1)
        c = D // 4
        g0 = jnp.pad(h[:, :, 0*c:1*c], ((0, 0), (1, 0), (0, 0)))[:, :S, :]
        g1 = jnp.pad(h[:, :, 1*c:2*c], ((0, 0), (0, 1), (0, 0)))[:, 1:, :]
        g2 = jnp.pad(h[:, :, 2*c:3*c], ((0, 0), (2, 0), (0, 0)))[:, :S, :]
        g3 = jnp.pad(h[:, :, 3*c:   ], ((0, 0), (0, 2), (0, 0)))[:, 2:, :]
        hs = jnp.concatenate([g0, g1, g2, g3], axis=-1) @ w2
        x1 = x + hs
        h2 = _gelu(_layernorm(x1, axis=-1) @ w3) @ w4
        return x1 + h2

    x = A_u
    xn = _layernorm(x, axis=-1)
    s = _A_ref(xn, A_A_re, A_A_im, A_B_re, A_B_im, A_C_re, A_C_im, A_log_dt, A_Dskip)
    g = _silu(_B_ref(xn, B_w1, B_w2, B_w3, B_w4))
    return x + s * g
```

```python
import numpy as np
import jax
import jax.numpy as jnp
from jax import lax
import jax.experimental.pallas as pl
import jax.experimental.pallas.tpu as pltpu

L = 2048
D = 512
N = 128
FF = 1376
J = 128
NB = L // J
NQ = 672
HI = (0, 1, 2, 3, 4, 5, 6, 7, 256, 258, 260, 262, 512, 516, 768, 772,
      1024, 1280, 1536, 1792, 2048)
NHI = len(HI)
XR = 24
CH = 32
RB = 256
WIN = ((0, 128), (0, 256), (128, 256), (256, 256), (320, 128), (384, 128),
       (384, 128), (448, 128), (448, 128), (512, 128), (512, 128), (512, 128),
       (512, 128), (512, 128), (512, 128), (520, 128))
GW = sum(w[1] for w in WIN)


def _q_of_m(m):
    if m < 256:
        return m
    if m < 512:
        return 256 + (m - 256) // 2
    if m < 1024:
        return 384 + (m - 512) // 4
    if m < 2048:
        return 512 + (m - 1024) // 8
    return 640


def _build_tables():
    pos = np.arange(L, dtype=np.int64)
    rr = np.zeros(L, np.int64)
    for l in range(L):
        if l < 256:
            rr[l] = l
        else:
            step = 1 << (int(l).bit_length() - 8)
            lo = (l // step) * step
            rem = l - lo
            if rem * 2 < step or (rem * 2 == step and (lo // step) % 2 == 0):
                rr[l] = lo
            else:
                rr[l] = lo + step
    w = np.pi * (2 * np.arange(J) + 1) / (2 * J)
    n = np.arange(J)
    f_fwd = np.concatenate([np.cos(np.outer(w, n)), -np.sin(np.outer(w, n))], 0)
    f_inv = np.concatenate([np.cos(np.outer(n, w)), -np.sin(np.outer(n, w))], 1) / J
    g_all = np.zeros((2 * J, GW))
    off = 0
    for dl in range(NB):
        s0, ln = WIN[dl]
        for p in range(-J, J):
            l = dl * J + p
            if 0 <= l < L:
                q = _q_of_m(int(rr[l])) - s0
                assert 0 <= q < ln
                g_all[:J, off + q] += np.cos(w * p)
                g_all[J:, off + q] += -np.sin(w * p)
        off += ln
    sel = np.zeros((32, 128))
    for dd in range(4):
        sel[np.arange(32), dd * 32 + np.arange(32)] = 1.0
    del pos
    return (f_fwd.astype(np.float32), f_inv.astype(np.float32),
            g_all.astype(np.float32), sel.astype(np.float32))


_F_FWD, _F_INV, _G_ALL, _SEL = _build_tables()


def _bf(x):
    return x.astype(jnp.bfloat16)


def _rb(x):
    return x.astype(jnp.bfloat16).astype(jnp.float32)


def _cmul(a, b):
    return (a[0] * b[0] - a[1] * b[1], a[0] * b[1] + a[1] * b[0])


def _gelu(x):
    c = 0.7978845608028654
    return 0.5 * x * (1.0 + jnp.tanh(c * (x + 0.044715 * (x * x * x))))


def _layernorm(x):
    m = jnp.mean(x, axis=-1, keepdims=True)
    xc = x - m
    v = jnp.mean(xc * xc, axis=-1, keepdims=True)
    den = _rb(jnp.sqrt(_rb(_rb(v) + 1e-5)))
    return _rb(_rb(x - _rb(m)) / den)


def _dot(a, b):
    return jnp.dot(a, b, preferred_element_type=jnp.float32)


def _dot_nt(a, b):
    return lax.dot_general(a, b, (((1,), (1,)), ((), ())),
                           preferred_element_type=jnp.float32)


def _kernel(are_ref, aim_ref, bre_ref, bim_ref, cre_ref, cim_ref, ldt_ref, dsk_ref,
            ffwd_ref, finv_ref, sel_ref,
            x_hbm, w1_hbm, w2_hbm, w3_hbm, w4_hbm, g_hbm,
            out_hbm,
            x_v, w1_v, w2_v, w3_v, w4_v, g_v, out_v,
            xn_v, h_v, u_v, kt_v, z_v,
            yr_v, yi_v, xr_v, xi_v, o_v, kd_v,
            sem_in, sem_out):
    copies = [pltpu.make_async_copy(s, d, sem_in.at[k]) for k, (s, d) in enumerate(
        [(x_hbm, x_v), (w1_hbm, w1_v), (g_hbm, g_v), (w2_hbm, w2_v), (w3_hbm, w3_v),
         (w4_hbm, w4_v)])]
    for c in copies:
        c.start()

    def kgen(c, carry):
        r0 = pl.multiple_of(c * CH, CH)
        rows = pl.ds(r0, CH)
        f32 = jnp.float32
        dt = _rb(jnp.exp(ldt_ref[rows, :].astype(f32)))
        lr = dt * are_ref[rows, :].astype(f32)
        li = dt * aim_ref[rows, :].astype(f32)
        dbr = dt * bre_ref[rows, :].astype(f32)
        dbi = dt * bim_ref[rows, :].astype(f32)
        w = _cmul((cre_ref[rows, :].astype(f32), cim_ref[rows, :].astype(f32)), (dbr, dbi))

        def cexp(m):
            e = jnp.exp(lr * m)
            a = li * m
            return (e * jnp.cos(a), e * jnp.sin(a))

        z1 = cexp(1.0)
        z8 = cexp(8.0)
        z256 = cexp(256.0)
        z1024 = cexp(1024.0)
        z2 = _cmul(z1, z1)
        z4 = _cmul(z2, z2)

        def put_y(j, v):
            yr_v[pl.ds(j, CH, stride=32), :] = v[0]
            yi_v[pl.ds(j, CH, stride=32), :] = v[1]

        def put_x(i, v):
            xr_v[pl.ds(i, CH, stride=XR), :] = v[0]
            xi_v[pl.ds(i, CH, stride=XR), :] = -v[1]

        put_y(0, (jnp.ones_like(lr), jnp.zeros_like(lr)))
        y = z8
        put_y(1, y)
        for j in range(2, 32):
            y = _cmul(y, z8)
            put_y(j, y)
        v = w
        put_x(0, v)
        for i in range(1, 8):
            v = _cmul(v, z1)
            put_x(i, v)
        x8 = _cmul(w, z256)
        v = x8
        put_x(8, v)
        for i in range(9, 12):
            v = _cmul(v, z2)
            put_x(i, v)
        x12 = _cmul(x8, z256)
        put_x(12, x12)
        put_x(13, _cmul(x12, z4))
        x14 = _cmul(x12, z256)
        put_x(14, x14)
        put_x(15, _cmul(x14, z4))
        v = _cmul(w, z1024)
        put_x(16, v)
        for i in range(17, 21):
            v = _cmul(v, z256)
            put_x(i, v)
        zero = jnp.zeros_like(lr)
        for i in range(21, XR):
            put_x(i, (zero, zero))
        for g in range(CH // 4):
            xr = _bf(xr_v[g * 4 * XR:(g + 1) * 4 * XR, :])
            xi = _bf(xi_v[g * 4 * XR:(g + 1) * 4 * XR, :])
            yr = _bf(yr_v[g * 128:(g + 1) * 128, :])
            yi = _bf(yi_v[g * 128:(g + 1) * 128, :])
            o = _dot_nt(xr, yr) + _dot_nt(xi, yi)
            o_v[pl.ds(pl.multiple_of(c * (CH * XR) + g * 4 * XR, 8), 4 * XR), :] = o
        return carry

    lax.fori_loop(0, D // CH, kgen, 0)

    rid = lax.broadcasted_iota(jnp.int32, (D, 128), 0)
    lid = lax.broadcasted_iota(jnp.int32, (D, 128), 1)
    keep = (rid % 4) == (lid // 32)
    keep_last = keep & ((lid % 32) == 0)
    sel = sel_ref[...]
    for i in range(NHI):
        oi = o_v[pl.ds(i, D, stride=XR), :]
        oi = jnp.where(keep_last if HI[i] == 2048 else keep, oi, 0.0)
        kt = _dot_nt(sel, _bf(oi))
        q0 = _q_of_m(HI[i])
        st = _q_of_m(HI[i] + 8) - q0 if HI[i] < 2048 else 1
        for c in range(4):
            if st == 1:
                kd_v[c, q0:q0 + 32, :] = kt[:, c * 128:(c + 1) * 128]
            else:
                kd_v[c, pl.ds(q0, 32, stride=st), :] = kt[:, c * 128:(c + 1) * 128]

    copies[2].wait()
    off = 0
    for dl in range(NB):
        s0, ln = WIN[dl]
        kw = jnp.concatenate([_bf(kd_v[c, s0:s0 + ln, :]) for c in range(4)], axis=1)
        kt_v[dl] = _dot(g_v[:, off:off + ln], kw)
        off += ln

    copies[0].wait()
    copies[1].wait()
    h_v[0:8, :] = jnp.zeros((8, D), jnp.float32)
    h_v[8 + L:16 + L, :] = jnp.zeros((8, D), jnp.float32)

    def phase1(b, carry):
        r0 = pl.multiple_of(b * RB, RB)
        x = x_v[pl.ds(r0, RB), :].astype(jnp.float32)
        xn = _bf(_layernorm(x))
        xn_v[pl.ds(r0, RB), :] = xn
        h = _rb(_gelu(_rb(_dot(xn, w1_v[...]))))
        h_v[pl.ds(pl.multiple_of(r0 + 8, 8), RB), :] = h
        for k in range(RB // J):
            u_v[b * (RB // J) + k] = _dot(ffwd_ref[...], xn[k * J:(k + 1) * J, :])
        return carry

    lax.fori_loop(0, L // RB, phase1, 0)

    def zphase(t, carry):
        f0 = pl.multiple_of((t // 4) * 16, 16)
        c0 = pl.multiple_of((t % 4) * 128, 128)
        re = pl.ds(f0, 16)
        im = pl.ds(pl.multiple_of(f0 + J, 16), 16)
        cs = pl.ds(c0, 128)
        for i in range(NB):
            zr = None
            zi = None
            for dl in range(i + 1):
                kr = kt_v[dl, re, cs]
                ki = kt_v[dl, im, cs]
                ur = u_v[i - dl, re, cs]
                ui = u_v[i - dl, im, cs]
                pr = kr * ur - ki * ui
                pi = kr * ui + ki * ur
                zr = pr if zr is None else zr + pr
                zi = pi if zi is None else zi + pi
            z_v[i, re, cs] = _bf(zr)
            z_v[i, im, cs] = _bf(zi)
        return carry

    lax.fori_loop(0, 32, zphase, 0)

    copies[3].wait()
    copies[4].wait()
    copies[5].wait()
    dsk = dsk_ref[...].astype(jnp.float32)

    def out_copy(b):
        r0 = pl.multiple_of(b * RB, RB)
        return pltpu.make_async_copy(out_v.at[pl.ds(r0, RB), :],
                                     out_hbm.at[pl.ds(r0, RB), :], sem_out.at[b])

    def phase2(b, carry):
        r0 = pl.multiple_of(b * RB, RB)
        ext = RB + 16
        parts = []
        for gi, sh in enumerate((1, -1, 2, -2)):
            hv = h_v[pl.ds(r0, ext), gi * 128:(gi + 1) * 128]
            hv = pltpu.roll(hv, sh % ext, 0)
            parts.append(_bf(hv[8:8 + RB, :]))
        hs = _rb(_dot(jnp.concatenate(parts, axis=1), w2_v[...]))
        xn = xn_v[pl.ds(r0, RB), :].astype(jnp.float32)
        x1 = _rb(xn + hs)
        a = _rb(_dot(_bf(_layernorm(x1)), w3_v[...]))
        h2 = _rb(_dot(_bf(_gelu(a)), w4_v[...]))
        bb = _rb(x1 + h2)
        gate = _rb(bb * jax.nn.sigmoid(bb))
        ys = [_dot(finv_ref[...], z_v[b * (RB // J) + k]) for k in range(RB // J)]
        y = _rb(jnp.concatenate(ys, axis=0))
        s = _rb(y + _rb(xn * dsk))
        x = x_v[pl.ds(r0, RB), :].astype(jnp.float32)
        out_v[pl.ds(r0, RB), :] = _bf(x + _rb(s * gate))
        out_copy(b).start()
        return carry

    lax.fori_loop(0, L // RB, phase2, 0)
    for b in range(L // RB):
        out_copy(b).wait()


@jax.jit
def pallas_recurrent_scan__ssm_conv_s4__mixer_s_mlp__prompt_kernel(
    A_u: jax.Array,
    A_A_re: jax.Array,
    A_A_im: jax.Array,
    A_B_re: jax.Array,
    A_B_im: jax.Array,
    A_C_re: jax.Array,
    A_C_im: jax.Array,
    A_log_dt: jax.Array,
    A_Dskip: jax.Array,
    B_x: jax.Array,
    B_w1: jax.Array,
    B_w2: jax.Array,
    B_w3: jax.Array,
    B_w4: jax.Array,
):
    bf16 = jnp.bfloat16
    f32 = jnp.float32
    x = A_u.reshape(L, D)
    vm = pl.BlockSpec(memory_space=pltpu.VMEM)
    hbm = pl.BlockSpec(memory_space=pl.ANY)
    out = pl.pallas_call(
        _kernel,
        out_shape=jax.ShapeDtypeStruct((L, D), bf16),
        in_specs=[vm] * 11 + [hbm] * 6,
        out_specs=hbm,
        scratch_shapes=[
            pltpu.VMEM((L, D), bf16),
            pltpu.VMEM((D, D), bf16),
            pltpu.VMEM((D, D), bf16),
            pltpu.VMEM((D, FF), bf16),
            pltpu.VMEM((FF, D), bf16),
            pltpu.VMEM((2 * J, GW), bf16),
            pltpu.VMEM((L, D), bf16),
            pltpu.VMEM((L, D), bf16),
            pltpu.VMEM((L + 16, D), f32),
            pltpu.VMEM((NB, 2 * J, D), f32),
            pltpu.VMEM((NB, 2 * J, D), f32),
            pltpu.VMEM((NB, 2 * J, D), bf16),
            pltpu.VMEM((CH * 32, N), f32),
            pltpu.VMEM((CH * 32, N), f32),
            pltpu.VMEM((CH * XR, N), f32),
            pltpu.VMEM((CH * XR, N), f32),
            pltpu.VMEM((D * XR, 128), f32),
            pltpu.VMEM((4, NQ, 128), f32),
            pltpu.SemaphoreType.DMA((6,)),
            pltpu.SemaphoreType.DMA((L // RB,)),
        ],
        compiler_params=pltpu.CompilerParams(vmem_limit_bytes=100 * 1024 * 1024),
    )(A_A_re, A_A_im, A_B_re, A_B_im, A_C_re, A_C_im,
      A_log_dt.reshape(D, 1), A_Dskip.reshape(1, D),
      jnp.asarray(_F_FWD, bf16), jnp.asarray(_F_INV, bf16), jnp.asarray(_SEL, bf16),
      x, B_w1, B_w2, B_w3, B_w4, jnp.asarray(_G_ALL, bf16))
    return out.reshape(1, L, D)
```

```python
import numpy as np
import jax
import jax.numpy as jnp
from jax import lax
import jax.experimental.pallas as pl
import jax.experimental.pallas.tpu as pltpu

L = 2048
D = 512
N = 128
FF = 1376
J = 128
NB = L // J
NQ = 656
_STEP = (1, 1, 2, 2, 4, 4, 4, 4, 8, 8, 8, 8, 8, 8, 8, 8)
HI = tuple(128 * k + b for k in range(16) for b in range(0, 8, _STEP[k])) + (2048,)
NHI = len(HI)
CH = 32
RB = 256
WIN = ((0, 128), (0, 256), (128, 256), (256, 256), (320, 128), (384, 128),
       (384, 128), (448, 128), (448, 128), (512, 128), (512, 128), (512, 128),
       (512, 128), (512, 128), (512, 128), (528, 128))
GW = sum(w[1] for w in WIN)


def _q_of_m(m):
    hi = (m // 128) * 128 + (m % 8)
    return 16 * HI.index(hi) + (m % 128) // 8


def _build_tables():
    pos = np.arange(L, dtype=np.int64)
    rr = np.zeros(L, np.int64)
    for l in range(L):
        if l < 256:
            rr[l] = l
        else:
            step = 1 << (int(l).bit_length() - 8)
            lo = (l // step) * step
            rem = l - lo
            if rem * 2 < step or (rem * 2 == step and (lo // step) % 2 == 0):
                rr[l] = lo
            else:
                rr[l] = lo + step
    w = np.pi * (2 * np.arange(J) + 1) / (2 * J)
    n = np.arange(J)
    f_fwd = np.concatenate([np.cos(np.outer(w, n)), -np.sin(np.outer(w, n))], 0)
    f_inv = np.concatenate([np.cos(np.outer(n, w)), -np.sin(np.outer(n, w))], 1) / J
    g_all = np.zeros((2 * J, GW))
    off = 0
    for dl in range(NB):
        s0, ln = WIN[dl]
        for p in range(-J, J):
            l = dl * J + p
            if 0 <= l < L:
                q = _q_of_m(int(rr[l])) - s0
                assert 0 <= q < ln
                g_all[:J, off + q] += np.cos(w * p)
                g_all[J:, off + q] += -np.sin(w * p)
        off += ln
    sel = np.zeros((16, 128))
    for dd in range(8):
        sel[np.arange(16), np.arange(16) * 8 + dd] = 1.0
    del pos
    return (f_fwd.astype(np.float32), f_inv.astype(np.float32),
            g_all.astype(np.float32), sel.astype(np.float32))


_F_FWD, _F_INV, _G_ALL, _SEL = _build_tables()


def _bf(x):
    return x.astype(jnp.bfloat16)


def _rb(x):
    return x.astype(jnp.bfloat16).astype(jnp.float32)


def _cmul(a, b):
    return (a[0] * b[0] - a[1] * b[1], a[0] * b[1] + a[1] * b[0])


def _gelu(x):
    c = 0.7978845608028654
    return 0.5 * x * (1.0 + jnp.tanh(c * (x + 0.044715 * (x * x * x))))


def _layernorm(x):
    m = jnp.mean(x, axis=-1, keepdims=True)
    xc = x - m
    v = jnp.mean(xc * xc, axis=-1, keepdims=True)
    den = _rb(jnp.sqrt(_rb(_rb(v) + 1e-5)))
    return _rb(_rb(x - _rb(m)) / den)


def _dot(a, b):
    return jnp.dot(a, b, preferred_element_type=jnp.float32)


def _dot_nt(a, b):
    return lax.dot_general(a, b, (((1,), (1,)), ((), ())),
                           preferred_element_type=jnp.float32)


def _kernel(are_ref, aim_ref, bre_ref, bim_ref, cre_ref, cim_ref, ldt_ref, dsk_ref,
            ffwd_ref, finv_ref, sel_ref,
            x_hbm, w1_hbm, w2_hbm, w3_hbm, w4_hbm, g_hbm,
            out_hbm,
            x_v, w1_v, w2_v, w3_v, w4_v, g_v, out_v,
            xn_v, h_v, u_v, kt_v, z_v,
            yr_v, yi_v, xr_v, xi_v, o_v, kd_v, dt_v,
            sem_in, sem_out):
    copies = [pltpu.make_async_copy(s, d, sem_in.at[k]) for k, (s, d) in enumerate(
        [(x_hbm, x_v), (w1_hbm, w1_v), (g_hbm, g_v), (w2_hbm, w2_v), (w3_hbm, w3_v),
         (w4_hbm, w4_v)])]
    for c in copies:
        c.start()

    dt_row = _rb(jnp.exp(ldt_ref[...].astype(jnp.float32))).reshape(1, D)
    dt_v[...] = jnp.transpose(jnp.broadcast_to(dt_row, (N, D)))

    def kgen(c, carry):
        r0 = pl.multiple_of(c * CH, CH)
        rows = pl.ds(r0, CH)
        f32 = jnp.float32
        dt = dt_v[rows, :]
        lr = dt * are_ref[rows, :].astype(f32)
        li = dt * aim_ref[rows, :].astype(f32)
        dbr = dt * bre_ref[rows, :].astype(f32)
        dbi = dt * bim_ref[rows, :].astype(f32)
        w = _cmul((cre_ref[rows, :].astype(f32), cim_ref[rows, :].astype(f32)), (dbr, dbi))

        def cexp(m):
            e = jnp.exp(lr * m)
            a = li * m
            return (e * jnp.cos(a), e * jnp.sin(a))

        z1 = cexp(1.0)
        z8 = cexp(8.0)
        z128 = cexp(128.0)
        z1024 = cexp(1024.0)

        def put_y(j, v):
            for g in range(CH // 8):
                yr_v[g, 8 * j:8 * j + 8, :] = v[0][8 * g:8 * g + 8, :]
                yi_v[g, 8 * j:8 * j + 8, :] = v[1][8 * g:8 * g + 8, :]

        def put_x(i, v):
            nvi = -v[1]
            for g in range(CH // 8):
                xr_v[g, 8 * i:8 * i + 8, :] = v[0][8 * g:8 * g + 8, :]
                xi_v[g, 8 * i:8 * i + 8, :] = nvi[8 * g:8 * g + 8, :]

        put_y(0, (jnp.ones_like(lr), jnp.zeros_like(lr)))
        y = z8
        put_y(1, y)
        for j in range(2, 16):
            y = _cmul(y, z8)
            put_y(j, y)
        v = w
        for b in range(8):
            if b:
                v = _cmul(v, z1)
            t = v
            for k in range(8):
                if (128 * k + b) in HI:
                    if k:
                        t = _cmul(t, z128)
                    put_x(HI.index(128 * k + b), t)
        t = _cmul(w, z1024)
        for k in range(8, 17):
            if k > 8:
                t = _cmul(t, z128)
            put_x(HI.index(128 * k), t)
        for g in range(CH // 8):
            o = (_dot_nt(_bf(xr_v[g]), _bf(yr_v[g])) + _dot_nt(_bf(xi_v[g]), _bf(yi_v[g])))
            for i in range(NHI):
                o_v[i, pl.ds(pl.multiple_of(r0 + 8 * g, 8), 8), :] = o[8 * i:8 * i + 8, :]
        return carry

    with jax.named_scope('p_kgen'):
        lax.fori_loop(0, D // CH, kgen, 0)

    rid = lax.broadcasted_iota(jnp.int32, (D, 128), 0)
    lid = lax.broadcasted_iota(jnp.int32, (D, 128), 1)
    keep = (rid % 8) == (lid % 8)
    keep_last = keep & (lid < 8)
    sel = sel_ref[...]
    with jax.named_scope('p_sel'):
        for i in range(NHI):
            oi = jnp.where(keep_last if HI[i] == 2048 else keep, o_v[i], 0.0)
            kd_v[16 * i:16 * i + 16, :] = _dot_nt(sel, _bf(oi))

    copies[2].wait()
    off = 0
    for dl in range(NB):
        s0, ln = WIN[dl]
        kt_v[dl] = _dot(g_v[:, off:off + ln], _bf(kd_v[s0:s0 + ln, :]))
        off += ln

    copies[0].wait()
    copies[1].wait()
    h_v[0:8, :] = jnp.zeros((8, D), jnp.float32)
    h_v[8 + L:16 + L, :] = jnp.zeros((8, D), jnp.float32)

    def phase1(b, carry):
        r0 = pl.multiple_of(b * RB, RB)
        x = x_v[pl.ds(r0, RB), :].astype(jnp.float32)
        xn = _bf(_layernorm(x))
        xn_v[pl.ds(r0, RB), :] = xn
        h = _rb(_gelu(_rb(_dot(xn, w1_v[...]))))
        h_v[pl.ds(pl.multiple_of(r0 + 8, 8), RB), :] = h
        for k in range(RB // J):
            u_v[b * (RB // J) + k] = _dot(ffwd_ref[...], xn[k * J:(k + 1) * J, :])
        return carry

    with jax.named_scope('p_phase1'):
        lax.fori_loop(0, L // RB, phase1, 0)

    def zphase(t, carry):
        f0 = pl.multiple_of((t // 4) * 16, 16)
        c0 = pl.multiple_of((t % 4) * 128, 128)
        re = pl.ds(f0, 16)
        im = pl.ds(pl.multiple_of(f0 + J, 16), 16)
        cs = pl.ds(c0, 128)
        for i in range(NB):
            zr = None
            zi = None
            for dl in range(i + 1):
                kr = kt_v[dl, re, cs]
                ki = kt_v[dl, im, cs]
                ur = u_v[i - dl, re, cs]
                ui = u_v[i - dl, im, cs]
                pr = kr * ur - ki * ui
                pi = kr * ui + ki * ur
                zr = pr if zr is None else zr + pr
                zi = pi if zi is None else zi + pi
            z_v[i, re, cs] = _bf(zr)
            z_v[i, im, cs] = _bf(zi)
        return carry

    with jax.named_scope('p_z'):
        lax.fori_loop(0, 32, zphase, 0)

    copies[3].wait()
    copies[4].wait()
    copies[5].wait()
    dsk = dsk_ref[...].astype(jnp.float32).reshape(1, D)

    def out_copy(b):
        r0 = pl.multiple_of(b * RB, RB)
        return pltpu.make_async_copy(out_v.at[pl.ds(r0, RB), :],
                                     out_hbm.at[pl.ds(r0, RB), :], sem_out.at[b])

    def phase2(b, carry):
        r0 = pl.multiple_of(b * RB, RB)
        ext = RB + 16
        parts = []
        for gi, sh in enumerate((1, -1, 2, -2)):
            hv = h_v[pl.ds(r0, ext), gi * 128:(gi + 1) * 128]
            hv = pltpu.roll(hv, sh % ext, 0)
            parts.append(_bf(hv[8:8 + RB, :]))
        hs = _rb(_dot(jnp.concatenate(parts, axis=1), w2_v[...]))
        xn = xn_v[pl.ds(r0, RB), :].astype(jnp.float32)
        x1 = _rb(xn + hs)
        a = _rb(_dot_nt(_bf(_layernorm(x1)), w3_v[...]))
        h2 = _rb(_dot(_bf(_gelu(a)), w4_v[...]))
        bb = _rb(x1 + h2)
        gate = _rb(bb * jax.nn.sigmoid(bb))
        ys = [_dot(finv_ref[...], z_v[b * (RB // J) + k]) for k in range(RB // J)]
        y = _rb(jnp.concatenate(ys, axis=0))
        s = _rb(y + _rb(xn * dsk))
        x = x_v[pl.ds(r0, RB), :].astype(jnp.float32)
        out_v[pl.ds(r0, RB), :] = _bf(x + _rb(s * gate))
        out_copy(b).start()
        return carry

    with jax.named_scope('p_phase2'):
        lax.fori_loop(0, L // RB, phase2, 0)
    for b in range(L // RB):
        out_copy(b).wait()


@jax.jit
def pallas_recurrent_scan__ssm_conv_s4__mixer_s_mlp__prompt_kernel(
    A_u: jax.Array,
    A_A_re: jax.Array,
    A_A_im: jax.Array,
    A_B_re: jax.Array,
    A_B_im: jax.Array,
    A_C_re: jax.Array,
    A_C_im: jax.Array,
    A_log_dt: jax.Array,
    A_Dskip: jax.Array,
    B_x: jax.Array,
    B_w1: jax.Array,
    B_w2: jax.Array,
    B_w3: jax.Array,
    B_w4: jax.Array,
):
    bf16 = jnp.bfloat16
    f32 = jnp.float32
    x = A_u.reshape(L, D)
    vm = pl.BlockSpec(memory_space=pltpu.VMEM)
    hbm = pl.BlockSpec(memory_space=pltpu.HBM)
    out = pl.pallas_call(
        _kernel,
        out_shape=jax.ShapeDtypeStruct((L, D), bf16),
        in_specs=[vm] * 11 + [hbm] * 6,
        out_specs=hbm,
        scratch_shapes=[
            pltpu.VMEM((L, D), bf16),
            pltpu.VMEM((D, D), bf16),
            pltpu.VMEM((D, D), bf16),
            pltpu.VMEM((FF, D), bf16),
            pltpu.VMEM((FF, D), bf16),
            pltpu.VMEM((2 * J, GW), bf16),
            pltpu.VMEM((L, D), bf16),
            pltpu.VMEM((L, D), bf16),
            pltpu.VMEM((L + 16, D), f32),
            pltpu.VMEM((NB, 2 * J, D), f32),
            pltpu.VMEM((NB, 2 * J, D), f32),
            pltpu.VMEM((NB, 2 * J, D), bf16),
            pltpu.VMEM((CH // 8, 128, N), f32),
            pltpu.VMEM((CH // 8, 128, N), f32),
            pltpu.VMEM((CH // 8, 8 * NHI, N), f32),
            pltpu.VMEM((CH // 8, 8 * NHI, N), f32),
            pltpu.VMEM((NHI, D, 128), f32),
            pltpu.VMEM((NQ, D), f32),
            pltpu.VMEM((D, N), f32),
            pltpu.SemaphoreType.DMA((6,)),
            pltpu.SemaphoreType.DMA((L // RB,)),
        ],
        compiler_params=pltpu.CompilerParams(vmem_limit_bytes=100 * 1024 * 1024),
    )(A_A_re, A_A_im, A_B_re, A_B_im, A_C_re, A_C_im,
      A_log_dt, A_Dskip,
      jnp.asarray(_F_FWD, bf16), jnp.asarray(_F_INV, bf16), jnp.asarray(_SEL, bf16),
      *[pltpu.with_memory_space_constraint(t, pltpu.HBM)
        for t in (x, B_w1, B_w2, B_w3.T, B_w4, jnp.asarray(_G_ALL, bf16))])
    return out.reshape(1, L, D)
```

```python
import functools
import numpy as np
import jax
import jax.numpy as jnp
from jax import lax
import jax.experimental.pallas as pl
import jax.experimental.pallas.tpu as pltpu

L = 2048
D = 512
N = 128
FF = 1376
J = 128
NB = L // J
NQ = 656
_STEP = (1, 1, 2, 2, 4, 4, 4, 4, 8, 8, 8, 8, 8, 8, 8, 8)
HI = tuple(128 * k + b for k in range(16) for b in range(0, 8, _STEP[k])) + (2048,)
NHI = len(HI)
CH = 32
RB = 256
WIN = ((0, 128), (0, 256), (128, 256), (256, 256), (320, 128), (384, 128),
       (384, 128), (448, 128), (448, 128), (512, 128), (512, 128), (512, 128),
       (512, 128), (512, 128), (512, 128), (528, 128))
GW = sum(w[1] for w in WIN)


def _q_of_m(m):
    hi = (m // 128) * 128 + (m % 8)
    return 16 * HI.index(hi) + (m % 128) // 8


def _build_tables():
    pos = np.arange(L, dtype=np.int64)
    rr = np.zeros(L, np.int64)
    for l in range(L):
        if l < 256:
            rr[l] = l
        else:
            step = 1 << (int(l).bit_length() - 8)
            lo = (l // step) * step
            rem = l - lo
            if rem * 2 < step or (rem * 2 == step and (lo // step) % 2 == 0):
                rr[l] = lo
            else:
                rr[l] = lo + step
    w = np.pi * (2 * np.arange(J) + 1) / (2 * J)
    n = np.arange(J)
    f_fwd = np.concatenate([np.cos(np.outer(w, n)), -np.sin(np.outer(w, n))], 0)
    f_inv = np.concatenate([np.cos(np.outer(n, w)), -np.sin(np.outer(n, w))], 1) / J
    g_all = np.zeros((2 * J, GW))
    off = 0
    for dl in range(NB):
        s0, ln = WIN[dl]
        for p in range(-J, J):
            l = dl * J + p
            if 0 <= l < L:
                q = _q_of_m(int(rr[l])) - s0
                assert 0 <= q < ln
                g_all[:J, off + q] += np.cos(w * p)
                g_all[J:, off + q] += -np.sin(w * p)
        off += ln
    sel = np.zeros((16, 128))
    for dd in range(8):
        sel[np.arange(16), np.arange(16) * 8 + dd] = 1.0
    del pos
    return (f_fwd.astype(np.float32), f_inv.astype(np.float32),
            g_all.astype(np.float32), sel.astype(np.float32))


_F_FWD, _F_INV, _G_ALL, _SEL = _build_tables()


def _bf(x):
    return x.astype(jnp.bfloat16)


def _rb(x):
    return x.astype(jnp.bfloat16).astype(jnp.float32)


def _cmul(a, b):
    return (a[0] * b[0] - a[1] * b[1], a[0] * b[1] + a[1] * b[0])


def _gelu(x):
    c = 0.7978845608028654
    return 0.5 * x * (1.0 + jnp.tanh(c * (x + 0.044715 * (x * x * x))))


def _layernorm(x):
    m = jnp.mean(x, axis=-1, keepdims=True)
    xc = x - m
    v = jnp.mean(xc * xc, axis=-1, keepdims=True)
    den = _rb(jnp.sqrt(_rb(_rb(v) + 1e-5)))
    return _rb(_rb(x - _rb(m)) / den)


def _dot(a, b):
    return jnp.dot(a, b, preferred_element_type=jnp.float32)


def _dot_nt(a, b):
    return lax.dot_general(a, b, (((1,), (1,)), ((), ())),
                           preferred_element_type=jnp.float32)


def _kernel(are_ref, aim_ref, bre_ref, bim_ref, cre_ref, cim_ref, ldt_ref, dsk_ref,
            ffwd_ref, finv_ref, sel_ref,
            x_hbm, w1_hbm, w2_hbm, w3_hbm, w4_hbm, g_hbm,
            out_hbm,
            x_v, w1_v, w2_v, w3_v, w4_v, g_v, out_v,
            xn_v, h_v, u_v, kt_v, z_v,
            yr_v, yi_v, xr_v, xi_v, o_v, kd_v, dt_v,
            sem_in, sem_out):
    copies = [pltpu.make_async_copy(s, d, sem_in.at[k]) for k, (s, d) in enumerate(
        [(x_hbm, x_v), (w1_hbm, w1_v), (g_hbm, g_v), (w2_hbm, w2_v), (w3_hbm, w3_v),
         (w4_hbm, w4_v)])]
    for c in copies:
        c.start()

    dt_row = _rb(jnp.exp(ldt_ref[...].astype(jnp.float32))).reshape(1, D)
    dt_v[...] = jnp.transpose(jnp.broadcast_to(dt_row, (N, D)))

    def kgen(c, carry):
        r0 = pl.multiple_of(c * CH, CH)
        rows = pl.ds(r0, CH)
        f32 = jnp.float32
        dt = dt_v[rows, :]
        lr = dt * are_ref[rows, :].astype(f32)
        li = dt * aim_ref[rows, :].astype(f32)
        dbr = dt * bre_ref[rows, :].astype(f32)
        dbi = dt * bim_ref[rows, :].astype(f32)
        w = _cmul((cre_ref[rows, :].astype(f32), cim_ref[rows, :].astype(f32)), (dbr, dbi))

        def cexp(m):
            e = jnp.exp(lr * m)
            a = li * m
            return (e * jnp.cos(a), e * jnp.sin(a))

        z1 = cexp(1.0)
        z8 = cexp(8.0)
        z128 = cexp(128.0)
        z1024 = cexp(1024.0)

        def put_y(j, v):
            for g in range(CH // 8):
                yr_v[g, 8 * j:8 * j + 8, :] = v[0][8 * g:8 * g + 8, :]
                yi_v[g, 8 * j:8 * j + 8, :] = v[1][8 * g:8 * g + 8, :]

        def put_x(i, v):
            nvi = -v[1]
            for g in range(CH // 8):
                xr_v[g, 8 * i:8 * i + 8, :] = v[0][8 * g:8 * g + 8, :]
                xi_v[g, 8 * i:8 * i + 8, :] = nvi[8 * g:8 * g + 8, :]

        put_y(0, (jnp.ones_like(lr), jnp.zeros_like(lr)))
        y = z8
        put_y(1, y)
        for j in range(2, 16):
            y = _cmul(y, z8)
            put_y(j, y)
        v = w
        for b in range(8):
            if b:
                v = _cmul(v, z1)
            t = v
            for k in range(8):
                if (128 * k + b) in HI:
                    if k:
                        t = _cmul(t, z128)
                    put_x(HI.index(128 * k + b), t)
        t = _cmul(w, z1024)
        for k in range(8, 17):
            if k > 8:
                t = _cmul(t, z128)
            put_x(HI.index(128 * k), t)
        for g in range(CH // 8):
            o = (_dot_nt(_bf(xr_v[g]), _bf(yr_v[g])) + _dot_nt(_bf(xi_v[g]), _bf(yi_v[g])))
            for i in range(NHI):
                o_v[i, pl.ds(pl.multiple_of(r0 + 8 * g, 8), 8), :] = o[8 * i:8 * i + 8, :]
        return carry

    with jax.named_scope('p_kgen'):
        lax.fori_loop(0, D // CH, kgen, 0)

    rid = lax.broadcasted_iota(jnp.int32, (D, 128), 0)
    lid = lax.broadcasted_iota(jnp.int32, (D, 128), 1)
    keep = (rid % 8) == (lid % 8)
    keep_last = keep & (lid < 8)
    sel = sel_ref[...]
    with jax.named_scope('p_sel'):
        for i in range(NHI):
            oi = jnp.where(keep_last if HI[i] == 2048 else keep, o_v[i], 0.0)
            kd_v[16 * i:16 * i + 16, :] = _dot_nt(sel, _bf(oi))

    copies[2].wait()
    off = 0
    for dl in range(NB):
        s0, ln = WIN[dl]
        kt_v[dl] = _dot(g_v[:, off:off + ln], _bf(kd_v[s0:s0 + ln, :]))
        off += ln

    copies[0].wait()
    copies[1].wait()
    h_v[0:8, :] = jnp.zeros((8, D), jnp.float32)
    h_v[8 + L:16 + L, :] = jnp.zeros((8, D), jnp.float32)

    def phase1(b, carry):
        r0 = pl.multiple_of(b * RB, RB)
        x = x_v[pl.ds(r0, RB), :].astype(jnp.float32)
        xn = _bf(_layernorm(x))
        xn_v[pl.ds(r0, RB), :] = xn
        h = _rb(_gelu(_rb(_dot(xn, w1_v[...]))))
        h_v[pl.ds(pl.multiple_of(r0 + 8, 8), RB), :] = h
        for k in range(RB // J):
            u_v[b * (RB // J) + k] = _dot(ffwd_ref[...], xn[k * J:(k + 1) * J, :])
        return carry

    with jax.named_scope('p_phase1'):
        lax.fori_loop(0, L // RB, phase1, 0)

    def zpair(p):
        for ft in range(J // 16):
            re = pl.ds(ft * 16, 16)
            im = pl.ds(J + ft * 16, 16)
            for ct in range(D // 128):
                cs = pl.ds(ct * 128, 128)
                sr = si = ar = ai = None
                for t in range(NB + 1):
                    first = t <= p
                    dl = jnp.where(first, t, t - p - 1)
                    src = jnp.where(first, p - t, NB - t)
                    kr = kt_v[dl, re, cs]
                    ki = kt_v[dl, im, cs]
                    ur = u_v[src, re, cs]
                    ui = u_v[src, im, cs]
                    pr = kr * ur - ki * ui
                    pi = kr * ui + ki * ur
                    sr = pr if sr is None else sr + pr
                    si = pi if si is None else si + pi
                    if t == 0:
                        ar, ai = sr, si
                    elif t < NB // 2:
                        ar = jnp.where(first, sr, ar)
                        ai = jnp.where(first, si, ai)
                z_v[p, re, cs] = _bf(ar)
                z_v[p, im, cs] = _bf(ai)
                z_v[NB - 1 - p, re, cs] = _bf(sr - ar)
                z_v[NB - 1 - p, im, cs] = _bf(si - ai)

    def zpro(p, carry):
        zpair(p)
        return carry

    with jax.named_scope('p_z'):
        lax.fori_loop(0, 2, zpro, 0)

    copies[3].wait()
    copies[4].wait()
    copies[5].wait()
    dsk = dsk_ref[...].astype(jnp.float32).reshape(1, D)

    def out_copy(b):
        r0 = pl.multiple_of(b * RB, RB)
        return pltpu.make_async_copy(out_v.at[pl.ds(r0, RB), :],
                                     out_hbm.at[pl.ds(r0, RB), :], sem_out.at[b])

    def phase2(e, carry, with_pair):
        b = jnp.where(e % 2 == 0, e // 2, 7 - e // 2)
        r0 = pl.multiple_of(b * RB, RB)
        if with_pair:
            zpair(e + 2)
        ext = RB + 16
        parts = []
        for gi, sh in enumerate((1, -1, 2, -2)):
            hv = h_v[pl.ds(r0, ext), gi * 128:(gi + 1) * 128]
            hv = pltpu.roll(hv, sh % ext, 0)
            parts.append(_bf(hv[8:8 + RB, :]))
        hs = _rb(_dot(jnp.concatenate(parts, axis=1), w2_v[...]))
        xn = xn_v[pl.ds(r0, RB), :].astype(jnp.float32)
        x1 = _rb(xn + hs)
        a = _rb(_dot_nt(_bf(_layernorm(x1)), w3_v[...]))
        h2 = _rb(_dot(_bf(_gelu(a)), w4_v[...]))
        bb = _rb(x1 + h2)
        gate = _rb(bb * jax.nn.sigmoid(bb))
        ys = [_dot(finv_ref[...], z_v[b * (RB // J) + k]) for k in range(RB // J)]
        y = _rb(jnp.concatenate(ys, axis=0))
        s = _rb(y + _rb(xn * dsk))
        x = x_v[pl.ds(r0, RB), :].astype(jnp.float32)
        out_v[pl.ds(r0, RB), :] = _bf(x + _rb(s * gate))
        out_copy(b).start()
        return carry

    with jax.named_scope('p_phase2'):
        lax.fori_loop(0, 6, functools.partial(phase2, with_pair=True), 0)
        lax.fori_loop(6, 8, functools.partial(phase2, with_pair=False), 0)
    for b in range(L // RB):
        out_copy(b).wait()


@jax.jit
def pallas_recurrent_scan__ssm_conv_s4__mixer_s_mlp__prompt_kernel(
    A_u: jax.Array,
    A_A_re: jax.Array,
    A_A_im: jax.Array,
    A_B_re: jax.Array,
    A_B_im: jax.Array,
    A_C_re: jax.Array,
    A_C_im: jax.Array,
    A_log_dt: jax.Array,
    A_Dskip: jax.Array,
    B_x: jax.Array,
    B_w1: jax.Array,
    B_w2: jax.Array,
    B_w3: jax.Array,
    B_w4: jax.Array,
):
    bf16 = jnp.bfloat16
    f32 = jnp.float32
    x = A_u.reshape(L, D)
    vm = pl.BlockSpec(memory_space=pltpu.VMEM)
    hbm = pl.BlockSpec(memory_space=pltpu.HBM)
    out = pl.pallas_call(
        _kernel,
        out_shape=jax.ShapeDtypeStruct((L, D), bf16),
        in_specs=[vm] * 11 + [hbm] * 6,
        out_specs=hbm,
        scratch_shapes=[
            pltpu.VMEM((L, D), bf16),
            pltpu.VMEM((D, D), bf16),
            pltpu.VMEM((D, D), bf16),
            pltpu.VMEM((FF, D), bf16),
            pltpu.VMEM((FF, D), bf16),
            pltpu.VMEM((2 * J, GW), bf16),
            pltpu.VMEM((L, D), bf16),
            pltpu.VMEM((L, D), bf16),
            pltpu.VMEM((L + 16, D), f32),
            pltpu.VMEM((NB, 2 * J, D), f32),
            pltpu.VMEM((NB, 2 * J, D), f32),
            pltpu.VMEM((NB, 2 * J, D), bf16),
            pltpu.VMEM((CH // 8, 128, N), f32),
            pltpu.VMEM((CH // 8, 128, N), f32),
            pltpu.VMEM((CH // 8, 8 * NHI, N), f32),
            pltpu.VMEM((CH // 8, 8 * NHI, N), f32),
            pltpu.VMEM((NHI, D, 128), f32),
            pltpu.VMEM((NQ, D), f32),
            pltpu.VMEM((D, N), f32),
            pltpu.SemaphoreType.DMA((6,)),
            pltpu.SemaphoreType.DMA((L // RB,)),
        ],
        compiler_params=pltpu.CompilerParams(vmem_limit_bytes=100 * 1024 * 1024),
    )(A_A_re, A_A_im, A_B_re, A_B_im, A_C_re, A_C_im,
      A_log_dt, A_Dskip,
      jnp.asarray(_F_FWD, bf16), jnp.asarray(_F_INV, bf16), jnp.asarray(_SEL, bf16),
      *[pltpu.with_memory_space_constraint(t, pltpu.HBM)
        for t in (x, B_w1, B_w2, B_w3.T, B_w4, jnp.asarray(_G_ALL, bf16))])
    return out.reshape(1, L, D)
```

```python
import functools
import numpy as np
import jax
import jax.numpy as jnp
from jax import lax
import jax.experimental.pallas as pl
import jax.experimental.pallas.tpu as pltpu

L = 2048
D = 512
N = 128
FF = 1376
J = 128
NB = L // J
NQ = 656
_STEP = (1, 1, 2, 2, 4, 4, 4, 4, 8, 8, 8, 8, 8, 8, 8, 8)
HI = tuple(128 * k + b for k in range(16) for b in range(0, 8, _STEP[k])) + (2048,)
NHI = len(HI)
CH = 32
RB = 256
WIN = ((0, 128), (0, 256), (128, 256), (256, 256), (320, 128), (384, 128),
       (384, 128), (448, 128), (448, 128), (512, 128), (512, 128), (512, 128),
       (512, 128), (512, 128), (512, 128), (528, 128))
GW = sum(w[1] for w in WIN)


def _q_of_m(m):
    hi = (m // 128) * 128 + (m % 8)
    return 16 * HI.index(hi) + (m % 128) // 8


def _build_tables():
    pos = np.arange(L, dtype=np.int64)
    rr = np.zeros(L, np.int64)
    for l in range(L):
        if l < 256:
            rr[l] = l
        else:
            step = 1 << (int(l).bit_length() - 8)
            lo = (l // step) * step
            rem = l - lo
            if rem * 2 < step or (rem * 2 == step and (lo // step) % 2 == 0):
                rr[l] = lo
            else:
                rr[l] = lo + step
    w = np.pi * (2 * np.arange(J) + 1) / (2 * J)
    n = np.arange(J)
    f_fwd = np.concatenate([np.cos(np.outer(w, n)), -np.sin(np.outer(w, n))], 0)
    f_inv = np.concatenate([np.cos(np.outer(n, w)), -np.sin(np.outer(n, w))], 1) / J
    g_all = np.zeros((2 * J, GW))
    off = 0
    for dl in range(NB):
        s0, ln = WIN[dl]
        for p in range(-J, J):
            l = dl * J + p
            if 0 <= l < L:
                q = _q_of_m(int(rr[l])) - s0
                assert 0 <= q < ln
                g_all[:J, off + q] += np.cos(w * p)
                g_all[J:, off + q] += -np.sin(w * p)
        off += ln
    sel = np.zeros((16, 128))
    for dd in range(8):
        sel[np.arange(16), np.arange(16) * 8 + dd] = 1.0
    del pos
    return (f_fwd.astype(np.float32), f_inv.astype(np.float32),
            g_all.astype(np.float32), sel.astype(np.float32))


_F_FWD, _F_INV, _G_ALL, _SEL = _build_tables()


def _bf(x):
    return x.astype(jnp.bfloat16)


def _rb(x):
    return x.astype(jnp.bfloat16).astype(jnp.float32)


def _cmul(a, b):
    return (a[0] * b[0] - a[1] * b[1], a[0] * b[1] + a[1] * b[0])


def _gelu(x):
    c = 0.7978845608028654
    return 0.5 * x * (1.0 + jnp.tanh(c * (x + 0.044715 * (x * x * x))))


def _layernorm(x):
    m = jnp.mean(x, axis=-1, keepdims=True)
    xc = x - m
    v = jnp.mean(xc * xc, axis=-1, keepdims=True)
    den = _rb(jnp.sqrt(_rb(_rb(v) + 1e-5)))
    return _rb(_rb(x - _rb(m)) / den)


def _dot(a, b):
    return jnp.dot(a, b, preferred_element_type=jnp.float32)


def _dot_nt(a, b):
    return lax.dot_general(a, b, (((1,), (1,)), ((), ())),
                           preferred_element_type=jnp.float32)


def _kernel(are_ref, aim_ref, bre_ref, bim_ref, cre_ref, cim_ref, ldt_ref, dsk_ref,
            ffwd_ref, finv_ref, sel_ref,
            x_hbm, w1_hbm, w2_hbm, w3_hbm, w4_hbm, g_hbm,
            out_hbm,
            x_v, w1_v, w2_v, w3_v, w4_v, g_v, out_v,
            xn_v, h_v, u_v, kt_v, z_v,
            yr_v, yi_v, xr_v, xi_v, o_v, kd_v, dt_v,
            sem_in, sem_out):
    copies = [pltpu.make_async_copy(s, d, sem_in.at[k]) for k, (s, d) in enumerate(
        [(x_hbm, x_v), (w1_hbm, w1_v), (g_hbm, g_v), (w2_hbm, w2_v), (w3_hbm, w3_v),
         (w4_hbm, w4_v)])]
    for c in copies:
        c.start()

    dt_row = _rb(jnp.exp(ldt_ref[...].astype(jnp.float32))).reshape(1, D)
    dt_v[...] = jnp.transpose(jnp.broadcast_to(dt_row, (N, D)))

    def kgen(c, carry):
        r0 = pl.multiple_of(c * CH, CH)
        rows = pl.ds(r0, CH)
        f32 = jnp.float32
        dt = dt_v[rows, :]
        lr = dt * are_ref[rows, :].astype(f32)
        li = dt * aim_ref[rows, :].astype(f32)
        dbr = dt * bre_ref[rows, :].astype(f32)
        dbi = dt * bim_ref[rows, :].astype(f32)
        w = _cmul((cre_ref[rows, :].astype(f32), cim_ref[rows, :].astype(f32)), (dbr, dbi))

        def cexp(m):
            e = jnp.exp(lr * m)
            a = li * m
            return (e * jnp.cos(a), e * jnp.sin(a))

        z1 = cexp(1.0)
        z8 = cexp(8.0)
        z128 = cexp(128.0)
        z1024 = cexp(1024.0)

        def put_y(j, v):
            for g in range(CH // 8):
                yr_v[g, 8 * j:8 * j + 8, :] = v[0][8 * g:8 * g + 8, :]
                yi_v[g, 8 * j:8 * j + 8, :] = v[1][8 * g:8 * g + 8, :]

        def put_x(i, v):
            nvi = -v[1]
            for g in range(CH // 8):
                xr_v[g, 8 * i:8 * i + 8, :] = v[0][8 * g:8 * g + 8, :]
                xi_v[g, 8 * i:8 * i + 8, :] = nvi[8 * g:8 * g + 8, :]

        put_y(0, (jnp.ones_like(lr), jnp.zeros_like(lr)))
        y = z8
        put_y(1, y)
        for j in range(2, 16):
            y = _cmul(y, z8)
            put_y(j, y)
        v = w
        for b in range(8):
            if b:
                v = _cmul(v, z1)
            t = v
            for k in range(8):
                if (128 * k + b) in HI:
                    if k:
                        t = _cmul(t, z128)
                    put_x(HI.index(128 * k + b), t)
        t = _cmul(w, z1024)
        for k in range(8, 17):
            if k > 8:
                t = _cmul(t, z128)
            put_x(HI.index(128 * k), t)
        for g in range(CH // 8):
            o = (_dot_nt(_bf(xr_v[g]), _bf(yr_v[g])) + _dot_nt(_bf(xi_v[g]), _bf(yi_v[g])))
            for i in range(NHI):
                o_v[i, pl.ds(pl.multiple_of(r0 + 8 * g, 8), 8), :] = o[8 * i:8 * i + 8, :]
        return carry

    with jax.named_scope('p_kgen'):
        lax.fori_loop(0, D // CH, kgen, 0)

    rid = lax.broadcasted_iota(jnp.int32, (D, 128), 0)
    lid = lax.broadcasted_iota(jnp.int32, (D, 128), 1)
    keep = (rid % 8) == (lid % 8)
    keep_last = keep & (lid < 8)
    sel = sel_ref[...]
    with jax.named_scope('p_sel'):
        for i in range(NHI):
            oi = jnp.where(keep_last if HI[i] == 2048 else keep, o_v[i], 0.0)
            kd_v[16 * i:16 * i + 16, :] = _dot_nt(sel, _bf(oi))

    copies[2].wait()
    off = 0
    for dl in range(NB):
        s0, ln = WIN[dl]
        kt_v[dl] = _dot(g_v[:, off:off + ln], _bf(kd_v[s0:s0 + ln, :]))
        off += ln

    copies[0].wait()
    copies[1].wait()
    h_v[0:8, :] = jnp.zeros((8, D), jnp.float32)
    h_v[8 + L:16 + L, :] = jnp.zeros((8, D), jnp.float32)

    def phase1(b, carry):
        r0 = pl.multiple_of(b * RB, RB)
        x = x_v[pl.ds(r0, RB), :].astype(jnp.float32)
        xn = _bf(_layernorm(x))
        xn_v[pl.ds(r0, RB), :] = xn
        h = _rb(_gelu(_rb(_dot(xn, w1_v[...]))))
        h_v[pl.ds(pl.multiple_of(r0 + 8, 8), RB), :] = h
        for k in range(RB // J):
            u_v[b * (RB // J) + k] = _dot(ffwd_ref[...], xn[k * J:(k + 1) * J, :])
        return carry

    with jax.named_scope('p_phase1'):
        lax.fori_loop(0, L // RB, phase1, 0)

    def zblock(i):
        for ft in range(J // 16):
            re = pl.ds(ft * 16, 16)
            im = pl.ds(J + ft * 16, 16)
            for ct in range(D // 128):
                cs = pl.ds(ct * 128, 128)
                sr = si = None
                for dl in range(i + 1):
                    kr = kt_v[dl, re, cs]
                    ki = kt_v[dl, im, cs]
                    ur = u_v[i - dl, re, cs]
                    ui = u_v[i - dl, im, cs]
                    pr = kr * ur - ki * ui
                    pi = kr * ui + ki * ur
                    sr = pr if sr is None else sr + pr
                    si = pi if si is None else si + pi
                z_v[i, re, cs] = _bf(sr)
                z_v[i, im, cs] = _bf(si)

    with jax.named_scope('p_z'):
        zblock(0)
        zblock(1)

    copies[3].wait()
    copies[4].wait()
    copies[5].wait()
    dsk = dsk_ref[...].astype(jnp.float32).reshape(1, D)

    def out_copy(b):
        r0 = b * RB
        return pltpu.make_async_copy(out_v.at[pl.ds(r0, RB), :],
                                     out_hbm.at[pl.ds(r0, RB), :], sem_out.at[b])

    def phase2(b):
        r0 = b * RB
        if b + 1 < L // RB:
            zblock(2 * b + 2)
            zblock(2 * b + 3)
        ext = RB + 16
        parts = []
        for gi, sh in enumerate((1, -1, 2, -2)):
            hv = h_v[pl.ds(r0, ext), gi * 128:(gi + 1) * 128]
            hv = pltpu.roll(hv, sh % ext, 0)
            parts.append(_bf(hv[8:8 + RB, :]))
        hs = _rb(_dot(jnp.concatenate(parts, axis=1), w2_v[...]))
        xn = xn_v[pl.ds(r0, RB), :].astype(jnp.float32)
        x1 = _rb(xn + hs)
        a = _rb(_dot_nt(_bf(_layernorm(x1)), w3_v[...]))
        h2 = _rb(_dot(_bf(_gelu(a)), w4_v[...]))
        bb = _rb(x1 + h2)
        gate = _rb(bb * jax.nn.sigmoid(bb))
        ys = [_dot(finv_ref[...], z_v[b * (RB // J) + k]) for k in range(RB // J)]
        y = _rb(jnp.concatenate(ys, axis=0))
        s = _rb(y + _rb(xn * dsk))
        x = x_v[pl.ds(r0, RB), :].astype(jnp.float32)
        out_v[pl.ds(r0, RB), :] = _bf(x + _rb(s * gate))
        out_copy(b).start()

    with jax.named_scope('p_phase2'):
        for b in range(L // RB):
            phase2(b)
    for b in range(L // RB):
        out_copy(b).wait()


@jax.jit
def pallas_recurrent_scan__ssm_conv_s4__mixer_s_mlp__prompt_kernel(
    A_u: jax.Array,
    A_A_re: jax.Array,
    A_A_im: jax.Array,
    A_B_re: jax.Array,
    A_B_im: jax.Array,
    A_C_re: jax.Array,
    A_C_im: jax.Array,
    A_log_dt: jax.Array,
    A_Dskip: jax.Array,
    B_x: jax.Array,
    B_w1: jax.Array,
    B_w2: jax.Array,
    B_w3: jax.Array,
    B_w4: jax.Array,
):
    bf16 = jnp.bfloat16
    f32 = jnp.float32
    x = A_u.reshape(L, D)
    vm = pl.BlockSpec(memory_space=pltpu.VMEM)
    hbm = pl.BlockSpec(memory_space=pltpu.HBM)
    out = pl.pallas_call(
        _kernel,
        out_shape=jax.ShapeDtypeStruct((L, D), bf16),
        in_specs=[vm] * 11 + [hbm] * 6,
        out_specs=hbm,
        scratch_shapes=[
            pltpu.VMEM((L, D), bf16),
            pltpu.VMEM((D, D), bf16),
            pltpu.VMEM((D, D), bf16),
            pltpu.VMEM((FF, D), bf16),
            pltpu.VMEM((FF, D), bf16),
            pltpu.VMEM((2 * J, GW), bf16),
            pltpu.VMEM((L, D), bf16),
            pltpu.VMEM((L, D), bf16),
            pltpu.VMEM((L + 16, D), f32),
            pltpu.VMEM((NB, 2 * J, D), f32),
            pltpu.VMEM((NB, 2 * J, D), f32),
            pltpu.VMEM((NB, 2 * J, D), bf16),
            pltpu.VMEM((CH // 8, 128, N), f32),
            pltpu.VMEM((CH // 8, 128, N), f32),
            pltpu.VMEM((CH // 8, 8 * NHI, N), f32),
            pltpu.VMEM((CH // 8, 8 * NHI, N), f32),
            pltpu.VMEM((NHI, D, 128), f32),
            pltpu.VMEM((NQ, D), f32),
            pltpu.VMEM((D, N), f32),
            pltpu.SemaphoreType.DMA((6,)),
            pltpu.SemaphoreType.DMA((L // RB,)),
        ],
        compiler_params=pltpu.CompilerParams(vmem_limit_bytes=100 * 1024 * 1024),
    )(A_A_re, A_A_im, A_B_re, A_B_im, A_C_re, A_C_im,
      A_log_dt, A_Dskip,
      jnp.asarray(_F_FWD, bf16), jnp.asarray(_F_INV, bf16), jnp.asarray(_SEL, bf16),
      *[pltpu.with_memory_space_constraint(t, pltpu.HBM)
        for t in (x, B_w1, B_w2, B_w3.T, B_w4, jnp.asarray(_G_ALL, bf16))])
    return out.reshape(1, L, D)
```

```python
import functools
import numpy as np
import jax
import jax.numpy as jnp
from jax import lax
import jax.experimental.pallas as pl
import jax.experimental.pallas.tpu as pltpu

L = 2048
D = 512
N = 128
FF = 1376
J = 128
NB = L // J
NQ = 656
_STEP = (1, 1, 2, 2, 4, 4, 4, 4, 8, 8, 8, 8, 8, 8, 8, 8)
HI = tuple(128 * k + b for k in range(16) for b in range(0, 8, _STEP[k])) + (2048,)
NHI = len(HI)
CH = 32
RB = 256
WIN = ((0, 128), (0, 256), (128, 256), (256, 256), (320, 128), (384, 128),
       (384, 128), (448, 128), (448, 128), (512, 128), (512, 128), (512, 128),
       (512, 128), (512, 128), (512, 128), (528, 128))
GW = sum(w[1] for w in WIN)


def _q_of_m(m):
    hi = (m // 128) * 128 + (m % 8)
    return 16 * HI.index(hi) + (m % 128) // 8


def _build_tables():
    pos = np.arange(L, dtype=np.int64)
    rr = np.zeros(L, np.int64)
    for l in range(L):
        if l < 256:
            rr[l] = l
        else:
            step = 1 << (int(l).bit_length() - 8)
            lo = (l // step) * step
            rem = l - lo
            if rem * 2 < step or (rem * 2 == step and (lo // step) % 2 == 0):
                rr[l] = lo
            else:
                rr[l] = lo + step
    w = np.pi * (2 * np.arange(J) + 1) / (2 * J)
    n = np.arange(J)
    f_fwd = np.concatenate([np.cos(np.outer(w, n)), -np.sin(np.outer(w, n))], 0)
    f_inv = np.concatenate([np.cos(np.outer(n, w)), -np.sin(np.outer(n, w))], 1) / J
    g_all = np.zeros((2 * J, GW))
    off = 0
    for dl in range(NB):
        s0, ln = WIN[dl]
        for p in range(-J, J):
            l = dl * J + p
            if 0 <= l < L:
                q = _q_of_m(int(rr[l])) - s0
                assert 0 <= q < ln
                g_all[:J, off + q] += np.cos(w * p)
                g_all[J:, off + q] += -np.sin(w * p)
        off += ln
    sel = np.zeros((16, 128))
    for dd in range(8):
        sel[np.arange(16), np.arange(16) * 8 + dd] = 1.0
    del pos
    return (f_fwd.astype(np.float32), f_inv.astype(np.float32),
            g_all.astype(np.float32), sel.astype(np.float32))


_F_FWD, _F_INV, _G_ALL, _SEL = _build_tables()


def _bf(x):
    return x.astype(jnp.bfloat16)


def _rb(x):
    return x.astype(jnp.bfloat16).astype(jnp.float32)


def _cmul(a, b):
    return (a[0] * b[0] - a[1] * b[1], a[0] * b[1] + a[1] * b[0])


def _gelu(x):
    c = 0.7978845608028654
    return 0.5 * x * (1.0 + jnp.tanh(c * (x + 0.044715 * (x * x * x))))


def _layernorm(x):
    m = jnp.mean(x, axis=-1, keepdims=True)
    xc = x - m
    v = jnp.mean(xc * xc, axis=-1, keepdims=True)
    den = _rb(jnp.sqrt(_rb(_rb(v) + 1e-5)))
    return _rb(_rb(x - _rb(m)) / den)


def _dot(a, b):
    return jnp.dot(a, b, preferred_element_type=jnp.float32)


def _dot_nt(a, b):
    return lax.dot_general(a, b, (((1,), (1,)), ((), ())),
                           preferred_element_type=jnp.float32)


def _kernel(are_ref, aim_ref, bre_ref, bim_ref, cre_ref, cim_ref, ldt_ref, dsk_ref,
            ffwd_ref, finv_ref, sel_ref,
            x_hbm, w1_hbm, w2_hbm, w3_hbm, w4_hbm, g_hbm,
            out_hbm,
            x_v, w1_v, w2_v, w3_v, w4_v, g_v, out_v,
            xn_v, h_v, u_v, kt_v, z_v,
            yr_v, yi_v, xr_v, xi_v, o_v, kd_v, dt_v,
            sem_in, sem_out):
    copies = [pltpu.make_async_copy(s, d, sem_in.at[k]) for k, (s, d) in enumerate(
        [(x_hbm, x_v), (w1_hbm, w1_v), (g_hbm, g_v), (w2_hbm, w2_v), (w3_hbm, w3_v),
         (w4_hbm, w4_v)])]
    for c in copies:
        c.start()

    dt_row = _rb(jnp.exp(ldt_ref[...].astype(jnp.float32))).reshape(1, D)
    dt_v[...] = jnp.transpose(jnp.broadcast_to(dt_row, (N, D)))

    def kgen(c, carry):
        r0 = pl.multiple_of(c * CH, CH)
        rows = pl.ds(r0, CH)
        f32 = jnp.float32
        dt = dt_v[rows, :]
        lr = dt * are_ref[rows, :].astype(f32)
        li = dt * aim_ref[rows, :].astype(f32)
        dbr = dt * bre_ref[rows, :].astype(f32)
        dbi = dt * bim_ref[rows, :].astype(f32)
        w = _cmul((cre_ref[rows, :].astype(f32), cim_ref[rows, :].astype(f32)), (dbr, dbi))

        def csq(a):
            ab = a[0] * a[1]
            return (a[0] * a[0] - a[1] * a[1], ab + ab)

        e1 = jnp.exp(lr)
        z1 = (e1 * jnp.cos(li), e1 * jnp.sin(li))
        z8 = csq(csq(csq(z1)))
        z128 = csq(csq(csq(csq(z8))))
        z1024 = csq(csq(csq(z128)))

        def put_y(j, v):
            for g in range(CH // 8):
                yr_v[g, 8 * j:8 * j + 8, :] = v[0][8 * g:8 * g + 8, :]
                yi_v[g, 8 * j:8 * j + 8, :] = v[1][8 * g:8 * g + 8, :]

        def put_x(i, v):
            nvi = -v[1]
            for g in range(CH // 8):
                xr_v[g, 8 * i:8 * i + 8, :] = v[0][8 * g:8 * g + 8, :]
                xi_v[g, 8 * i:8 * i + 8, :] = nvi[8 * g:8 * g + 8, :]

        put_y(0, (jnp.ones_like(lr), jnp.zeros_like(lr)))
        y = z8
        put_y(1, y)
        for j in range(2, 16):
            y = _cmul(y, z8)
            put_y(j, y)
        v = w
        for b in range(8):
            if b:
                v = _cmul(v, z1)
            t = v
            for k in range(8):
                if (128 * k + b) in HI:
                    if k:
                        t = _cmul(t, z128)
                    put_x(HI.index(128 * k + b), t)
        t = _cmul(w, z1024)
        for k in range(8, 17):
            if k > 8:
                t = _cmul(t, z128)
            put_x(HI.index(128 * k), t)
        for g in range(CH // 8):
            o = (_dot_nt(_bf(xr_v[g]), _bf(yr_v[g])) + _dot_nt(_bf(xi_v[g]), _bf(yi_v[g])))
            for i in range(NHI):
                o_v[i, pl.ds(pl.multiple_of(r0 + 8 * g, 8), 8), :] = o[8 * i:8 * i + 8, :]
        return carry

    with jax.named_scope('p_kgen'):
        lax.fori_loop(0, D // CH, kgen, 0)

    rid = lax.broadcasted_iota(jnp.int32, (D, 128), 0)
    lid = lax.broadcasted_iota(jnp.int32, (D, 128), 1)
    keep = (rid % 8) == (lid % 8)
    keep_last = keep & (lid < 8)
    sel = sel_ref[...]
    with jax.named_scope('p_sel'):
        for i in range(NHI):
            oi = jnp.where(keep_last if HI[i] == 2048 else keep, o_v[i], 0.0)
            kd_v[16 * i:16 * i + 16, :] = _dot_nt(sel, _bf(oi))

    copies[2].wait()
    off = 0
    for dl in range(NB):
        s0, ln = WIN[dl]
        kt_v[dl] = _dot(g_v[:, off:off + ln], _bf(kd_v[s0:s0 + ln, :]))
        off += ln

    copies[0].wait()
    copies[1].wait()
    h_v[0:8, :] = jnp.zeros((8, D), jnp.float32)
    h_v[8 + L:16 + L, :] = jnp.zeros((8, D), jnp.float32)

    def phase1(b, carry):
        r0 = pl.multiple_of(b * RB, RB)
        x = x_v[pl.ds(r0, RB), :].astype(jnp.float32)
        xn = _bf(_layernorm(x))
        xn_v[pl.ds(r0, RB), :] = xn
        h = _rb(_gelu(_rb(_dot(xn, w1_v[...]))))
        h_v[pl.ds(pl.multiple_of(r0 + 8, 8), RB), :] = h
        for k in range(RB // J):
            u_v[b * (RB // J) + k] = _dot(ffwd_ref[...], xn[k * J:(k + 1) * J, :])
        return carry

    with jax.named_scope('p_phase1'):
        lax.fori_loop(0, L // RB, phase1, 0)

    def zphase(t, carry):
        f0 = pl.multiple_of((t // 4) * 16, 16)
        c0 = pl.multiple_of((t % 4) * 128, 128)
        re = pl.ds(f0, 16)
        im = pl.ds(pl.multiple_of(f0 + J, 16), 16)
        cs = pl.ds(c0, 128)
        for i in range(NB):
            zr = None
            zi = None
            for dl in range(i + 1):
                kr = kt_v[dl, re, cs]
                ki = kt_v[dl, im, cs]
                ur = u_v[i - dl, re, cs]
                ui = u_v[i - dl, im, cs]
                pr = kr * ur - ki * ui
                pi = kr * ui + ki * ur
                zr = pr if zr is None else zr + pr
                zi = pi if zi is None else zi + pi
            z_v[i, re, cs] = _bf(zr)
            z_v[i, im, cs] = _bf(zi)
        return carry

    with jax.named_scope('p_z'):
        lax.fori_loop(0, 32, zphase, 0)

    copies[3].wait()
    copies[4].wait()
    copies[5].wait()
    dsk = dsk_ref[...].astype(jnp.float32).reshape(1, D)

    def out_copy(b):
        r0 = pl.multiple_of(b * RB, RB)
        return pltpu.make_async_copy(out_v.at[pl.ds(r0, RB), :],
                                     out_hbm.at[pl.ds(r0, RB), :], sem_out.at[b])

    def phase2(b, carry):
        r0 = pl.multiple_of(b * RB, RB)
        ext = RB + 16
        parts = []
        for gi, sh in enumerate((1, -1, 2, -2)):
            hv = h_v[pl.ds(r0, ext), gi * 128:(gi + 1) * 128]
            hv = pltpu.roll(hv, sh % ext, 0)
            parts.append(_bf(hv[8:8 + RB, :]))
        hs = _rb(_dot(jnp.concatenate(parts, axis=1), w2_v[...]))
        xn = xn_v[pl.ds(r0, RB), :].astype(jnp.float32)
        x1 = _rb(xn + hs)
        a = _rb(_dot_nt(_bf(_layernorm(x1)), w3_v[...]))
        h2 = _rb(_dot(_bf(_gelu(a)), w4_v[...]))
        bb = _rb(x1 + h2)
        gate = _rb(bb * jax.nn.sigmoid(bb))
        ys = [_dot(finv_ref[...], z_v[b * (RB // J) + k]) for k in range(RB // J)]
        y = _rb(jnp.concatenate(ys, axis=0))
        s = _rb(y + _rb(xn * dsk))
        x = x_v[pl.ds(r0, RB), :].astype(jnp.float32)
        out_v[pl.ds(r0, RB), :] = _bf(x + _rb(s * gate))
        out_copy(b).start()
        return carry

    with jax.named_scope('p_phase2'):
        lax.fori_loop(0, L // RB, phase2, 0)
    for b in range(L // RB):
        out_copy(b).wait()


@jax.jit
def pallas_recurrent_scan__ssm_conv_s4__mixer_s_mlp__prompt_kernel(
    A_u: jax.Array,
    A_A_re: jax.Array,
    A_A_im: jax.Array,
    A_B_re: jax.Array,
    A_B_im: jax.Array,
    A_C_re: jax.Array,
    A_C_im: jax.Array,
    A_log_dt: jax.Array,
    A_Dskip: jax.Array,
    B_x: jax.Array,
    B_w1: jax.Array,
    B_w2: jax.Array,
    B_w3: jax.Array,
    B_w4: jax.Array,
):
    bf16 = jnp.bfloat16
    f32 = jnp.float32
    x = A_u.reshape(L, D)
    vm = pl.BlockSpec(memory_space=pltpu.VMEM)
    hbm = pl.BlockSpec(memory_space=pltpu.HBM)
    out = pl.pallas_call(
        _kernel,
        out_shape=jax.ShapeDtypeStruct((L, D), bf16),
        in_specs=[vm] * 11 + [hbm] * 6,
        out_specs=hbm,
        scratch_shapes=[
            pltpu.VMEM((L, D), bf16),
            pltpu.VMEM((D, D), bf16),
            pltpu.VMEM((D, D), bf16),
            pltpu.VMEM((FF, D), bf16),
            pltpu.VMEM((FF, D), bf16),
            pltpu.VMEM((2 * J, GW), bf16),
            pltpu.VMEM((L, D), bf16),
            pltpu.VMEM((L, D), bf16),
            pltpu.VMEM((L + 16, D), f32),
            pltpu.VMEM((NB, 2 * J, D), f32),
            pltpu.VMEM((NB, 2 * J, D), f32),
            pltpu.VMEM((NB, 2 * J, D), bf16),
            pltpu.VMEM((CH // 8, 128, N), f32),
            pltpu.VMEM((CH // 8, 128, N), f32),
            pltpu.VMEM((CH // 8, 8 * NHI, N), f32),
            pltpu.VMEM((CH // 8, 8 * NHI, N), f32),
            pltpu.VMEM((NHI, D, 128), f32),
            pltpu.VMEM((NQ, D), f32),
            pltpu.VMEM((D, N), f32),
            pltpu.SemaphoreType.DMA((6,)),
            pltpu.SemaphoreType.DMA((L // RB,)),
        ],
        compiler_params=pltpu.CompilerParams(vmem_limit_bytes=100 * 1024 * 1024),
    )(A_A_re, A_A_im, A_B_re, A_B_im, A_C_re, A_C_im,
      A_log_dt, A_Dskip,
      jnp.asarray(_F_FWD, bf16), jnp.asarray(_F_INV, bf16), jnp.asarray(_SEL, bf16),
      *[pltpu.with_memory_space_constraint(t, pltpu.HBM)
        for t in (x, B_w1, B_w2, B_w3.T, B_w4, jnp.asarray(_G_ALL, bf16))])
    return out.reshape(1, L, D)
```

```python
import functools
import numpy as np
import jax
import jax.numpy as jnp
from jax import lax
import jax.experimental.pallas as pl
import jax.experimental.pallas.tpu as pltpu

L = 2048
D = 512
N = 128
FF = 1376
J = 128
NB = L // J
NQ = 656
_STEP = (1, 1, 2, 2, 4, 4, 4, 4, 8, 8, 8, 8, 8, 8, 8, 8)
HI = tuple(128 * k + b for k in range(16) for b in range(0, 8, _STEP[k])) + (2048,)
NHI = len(HI)
CH = 32
RB = 256
WIN = ((0, 128), (0, 256), (128, 256), (256, 256), (320, 128), (384, 128),
       (384, 128), (448, 128), (448, 128), (512, 128), (512, 128), (512, 128),
       (512, 128), (512, 128), (512, 128), (528, 128))
GW = sum(w[1] for w in WIN)


def _q_of_m(m):
    hi = (m // 128) * 128 + (m % 8)
    return 16 * HI.index(hi) + (m % 128) // 8


def _build_tables():
    pos = np.arange(L, dtype=np.int64)
    rr = np.zeros(L, np.int64)
    for l in range(L):
        if l < 256:
            rr[l] = l
        else:
            step = 1 << (int(l).bit_length() - 8)
            lo = (l // step) * step
            rem = l - lo
            if rem * 2 < step or (rem * 2 == step and (lo // step) % 2 == 0):
                rr[l] = lo
            else:
                rr[l] = lo + step
    w = np.pi * (2 * np.arange(J) + 1) / (2 * J)
    n = np.arange(J)
    f_fwd = np.concatenate([np.cos(np.outer(w, n)), -np.sin(np.outer(w, n))], 0)
    f_inv = np.concatenate([np.cos(np.outer(n, w)), -np.sin(np.outer(n, w))], 1) / J
    g_all = np.zeros((2 * J, GW))
    off = 0
    for dl in range(NB):
        s0, ln = WIN[dl]
        for p in range(-J, J):
            l = dl * J + p
            if 0 <= l < L:
                q = _q_of_m(int(rr[l])) - s0
                assert 0 <= q < ln
                g_all[:J, off + q] += np.cos(w * p)
                g_all[J:, off + q] += -np.sin(w * p)
        off += ln
    sel = np.zeros((16, 128))
    for dd in range(8):
        sel[np.arange(16), np.arange(16) * 8 + dd] = 1.0
    del pos
    return (f_fwd.astype(np.float32), f_inv.astype(np.float32),
            g_all.astype(np.float32), sel.astype(np.float32))


_F_FWD, _F_INV, _G_ALL, _SEL = _build_tables()


def _bf(x):
    return x.astype(jnp.bfloat16)


def _rb(x):
    return x.astype(jnp.bfloat16).astype(jnp.float32)


def _cmul(a, b):
    return (a[0] * b[0] - a[1] * b[1], a[0] * b[1] + a[1] * b[0])


def _gelu(x):
    c = 0.7978845608028654
    return 0.5 * x * (1.0 + jnp.tanh(c * (x + 0.044715 * (x * x * x))))


def _layernorm(x):
    m = jnp.mean(x, axis=-1, keepdims=True)
    xc = x - m
    v = jnp.mean(xc * xc, axis=-1, keepdims=True)
    den = _rb(jnp.sqrt(_rb(_rb(v) + 1e-5)))
    return _rb(_rb(x - _rb(m)) / den)


def _dot(a, b):
    return jnp.dot(a, b, preferred_element_type=jnp.float32)


def _dot_nt(a, b):
    return lax.dot_general(a, b, (((1,), (1,)), ((), ())),
                           preferred_element_type=jnp.float32)


def _kernel(are_ref, aim_ref, bre_ref, bim_ref, cre_ref, cim_ref, ldt_ref, dsk_ref,
            ffwd_ref, finv_ref, sel_ref,
            x_hbm, w1_hbm, w2_hbm, w3_hbm, w4_hbm, g_hbm,
            out_hbm,
            x_v, w1_v, w2_v, w3_v, w4_v, g_v, out_v,
            xn_v, h_v, u_v, kt_v, z_v,
            yr_v, yi_v, xr_v, xi_v, o_v, kd_v, dt_v,
            sem_in, sem_out):
    copies = [pltpu.make_async_copy(s, d, sem_in.at[k]) for k, (s, d) in enumerate(
        [(x_hbm, x_v), (w1_hbm, w1_v), (g_hbm, g_v), (w2_hbm, w2_v), (w3_hbm, w3_v),
         (w4_hbm, w4_v)])]
    for c in copies:
        c.start()

    dt_row = _rb(jnp.exp(ldt_ref[...].astype(jnp.float32))).reshape(1, D)
    dt_v[...] = jnp.transpose(jnp.broadcast_to(dt_row, (N, D)))

    def kgen(c, carry):
        r0 = pl.multiple_of(c * CH, CH)
        rows = pl.ds(r0, CH)
        f32 = jnp.float32
        dt = dt_v[rows, :]
        lr = dt * are_ref[rows, :].astype(f32)
        li = dt * aim_ref[rows, :].astype(f32)
        dbr = dt * bre_ref[rows, :].astype(f32)
        dbi = dt * bim_ref[rows, :].astype(f32)
        w = _cmul((cre_ref[rows, :].astype(f32), cim_ref[rows, :].astype(f32)), (dbr, dbi))

        def csq(a):
            ab = a[0] * a[1]
            return (a[0] * a[0] - a[1] * a[1], ab + ab)

        e1 = jnp.exp(lr)
        z1 = (e1 * jnp.cos(li), e1 * jnp.sin(li))
        z8 = csq(csq(csq(z1)))
        z128 = csq(csq(csq(csq(z8))))
        z1024 = csq(csq(csq(z128)))

        def put_y(j, v):
            for g in range(CH // 8):
                yr_v[g, 8 * j:8 * j + 8, :] = v[0][8 * g:8 * g + 8, :]
                yi_v[g, 8 * j:8 * j + 8, :] = v[1][8 * g:8 * g + 8, :]

        def put_x(i, v):
            nvi = -v[1]
            for g in range(CH // 8):
                xr_v[g, 8 * i:8 * i + 8, :] = v[0][8 * g:8 * g + 8, :]
                xi_v[g, 8 * i:8 * i + 8, :] = nvi[8 * g:8 * g + 8, :]

        put_y(0, (jnp.ones_like(lr), jnp.zeros_like(lr)))
        y = z8
        put_y(1, y)
        for j in range(2, 16):
            y = _cmul(y, z8)
            put_y(j, y)
        v = w
        for b in range(8):
            if b:
                v = _cmul(v, z1)
            t = v
            for k in range(8):
                if (128 * k + b) in HI:
                    if k:
                        t = _cmul(t, z128)
                    put_x(HI.index(128 * k + b), t)
        t = _cmul(w, z1024)
        for k in range(8, 17):
            if k > 8:
                t = _cmul(t, z128)
            put_x(HI.index(128 * k), t)
        for g in range(CH // 8):
            o = (_dot_nt(_bf(xr_v[g]), _bf(yr_v[g])) + _dot_nt(_bf(xi_v[g]), _bf(yi_v[g])))
            for i in range(NHI):
                o_v[i, pl.ds(pl.multiple_of(r0 + 8 * g, 8), 8), :] = o[8 * i:8 * i + 8, :]
        return carry

    with jax.named_scope('p_kgen'):
        lax.fori_loop(0, D // CH, kgen, 0)

    rid = lax.broadcasted_iota(jnp.int32, (D, 128), 0)
    lid = lax.broadcasted_iota(jnp.int32, (D, 128), 1)
    keep = (rid % 8) == (lid % 8)
    keep_last = keep & (lid < 8)
    sel = sel_ref[...]
    with jax.named_scope('p_sel'):
        for i in range(NHI):
            oi = jnp.where(keep_last if HI[i] == 2048 else keep, o_v[i], 0.0)
            kd_v[16 * i:16 * i + 16, :] = _dot_nt(sel, _bf(oi))

    copies[2].wait()
    off = 0
    for dl in range(NB):
        s0, ln = WIN[dl]
        kt_v[dl] = _dot(g_v[:, off:off + ln], _bf(kd_v[s0:s0 + ln, :]))
        off += ln

    copies[0].wait()
    copies[1].wait()
    h_v[0:8, :] = jnp.zeros((8, D), jnp.float32)
    h_v[8 + L:16 + L, :] = jnp.zeros((8, D), jnp.float32)

    def phase1(b, carry):
        r0 = pl.multiple_of(b * RB, RB)
        x = x_v[pl.ds(r0, RB), :].astype(jnp.float32)
        xn = _bf(_layernorm(x))
        xn_v[pl.ds(r0, RB), :] = xn
        h = _rb(_gelu(_rb(_dot(xn, w1_v[...]))))
        h_v[pl.ds(pl.multiple_of(r0 + 8, 8), RB), :] = h
        for k in range(RB // J):
            u_v[b * (RB // J) + k] = _dot(ffwd_ref[...], xn[k * J:(k + 1) * J, :])
        return carry

    with jax.named_scope('p_phase1'):
        lax.fori_loop(0, L // RB, phase1, 0)

    def ztile(i, ft, ct):
        re = pl.ds(ft * 16, 16)
        im = pl.ds(J + ft * 16, 16)
        cs = pl.ds(ct * 128, 128)
        zr = zi = None
        for dl in range(i + 1):
            kr = kt_v[dl, re, cs]
            ki = kt_v[dl, im, cs]
            ur = u_v[i - dl, re, cs]
            ui = u_v[i - dl, im, cs]
            pr = kr * ur - ki * ui
            pi = kr * ui + ki * ur
            zr = pr if zr is None else zr + pr
            zi = pi if zi is None else zi + pi
        z_v[i, re, cs] = _bf(zr)
        z_v[i, im, cs] = _bf(zi)

    copies[3].wait()
    copies[4].wait()
    copies[5].wait()
    dsk = dsk_ref[...].astype(jnp.float32).reshape(1, D)

    def out_copy(b):
        return pltpu.make_async_copy(out_v.at[pl.ds(b * RB, RB), :],
                                     out_hbm.at[pl.ds(b * RB, RB), :], sem_out.at[b])

    ZSCHED = ((0, 1, 2, 3, 6), (4, 11), (5, 10), (7, 8), (9, 12), (13,), (14,), (15,))
    FCH = tuple((c, min(128, FF - c)) for c in range(0, FF, 128))

    def phase2(b):
        r0 = b * RB
        tiles = [(i, ft, ct) for i in ZSCHED[b] for ft in range(J // 16) for ct in range(D // 128)]
        nslots = 4 + 2 * len(FCH)
        per = -(-len(tiles) // nslots)

        def fill():
            for _ in range(per):
                if tiles:
                    ztile(*tiles.pop(0))

        ext = RB + 16
        parts = []
        for gi, sh in enumerate((1, -1, 2, -2)):
            hv = h_v[pl.ds(r0, ext), gi * 128:(gi + 1) * 128]
            hv = pltpu.roll(hv, sh % ext, 0)
            parts.append(_bf(hv[8:8 + RB, :]))
        hcat = jnp.concatenate(parts, axis=1)
        hs = []
        for n in range(4):
            hs.append(_rb(_dot(hcat, w2_v[:, n * 128:(n + 1) * 128])))
            fill()
        xn = xn_v[pl.ds(r0, RB), :].astype(jnp.float32)
        x1 = _rb(xn + jnp.concatenate(hs, axis=1))
        ln2 = _bf(_layernorm(x1))
        h2 = None
        for c, n in FCH:
            a = _rb(_dot_nt(ln2, w3_v[c:c + n, :]))
            fill()
            t = _dot(_bf(_gelu(a)), w4_v[c:c + n, :])
            h2 = t if h2 is None else h2 + t
            fill()
        while tiles:
            fill()
        bb = _rb(x1 + _rb(h2))
        gate = _rb(bb * jax.nn.sigmoid(bb))
        ys = [_dot(finv_ref[...], z_v[b * (RB // J) + k]) for k in range(RB // J)]
        y = _rb(jnp.concatenate(ys, axis=0))
        s = _rb(y + _rb(xn * dsk))
        x = x_v[pl.ds(r0, RB), :].astype(jnp.float32)
        out_v[pl.ds(r0, RB), :] = _bf(x + _rb(s * gate))
        out_copy(b).start()

    with jax.named_scope('p_phase2'):
        for b in range(L // RB):
            phase2(b)
    for b in range(L // RB):
        out_copy(b).wait()


@jax.jit
def pallas_recurrent_scan__ssm_conv_s4__mixer_s_mlp__prompt_kernel(
    A_u: jax.Array,
    A_A_re: jax.Array,
    A_A_im: jax.Array,
    A_B_re: jax.Array,
    A_B_im: jax.Array,
    A_C_re: jax.Array,
    A_C_im: jax.Array,
    A_log_dt: jax.Array,
    A_Dskip: jax.Array,
    B_x: jax.Array,
    B_w1: jax.Array,
    B_w2: jax.Array,
    B_w3: jax.Array,
    B_w4: jax.Array,
):
    bf16 = jnp.bfloat16
    f32 = jnp.float32
    x = A_u.reshape(L, D)
    vm = pl.BlockSpec(memory_space=pltpu.VMEM)
    hbm = pl.BlockSpec(memory_space=pltpu.HBM)
    out = pl.pallas_call(
        _kernel,
        out_shape=jax.ShapeDtypeStruct((L, D), bf16),
        in_specs=[vm] * 11 + [hbm] * 6,
        out_specs=hbm,
        scratch_shapes=[
            pltpu.VMEM((L, D), bf16),
            pltpu.VMEM((D, D), bf16),
            pltpu.VMEM((D, D), bf16),
            pltpu.VMEM((FF, D), bf16),
            pltpu.VMEM((FF, D), bf16),
            pltpu.VMEM((2 * J, GW), bf16),
            pltpu.VMEM((L, D), bf16),
            pltpu.VMEM((L, D), bf16),
            pltpu.VMEM((L + 16, D), f32),
            pltpu.VMEM((NB, 2 * J, D), f32),
            pltpu.VMEM((NB, 2 * J, D), f32),
            pltpu.VMEM((NB, 2 * J, D), bf16),
            pltpu.VMEM((CH // 8, 128, N), f32),
            pltpu.VMEM((CH // 8, 128, N), f32),
            pltpu.VMEM((CH // 8, 8 * NHI, N), f32),
            pltpu.VMEM((CH // 8, 8 * NHI, N), f32),
            pltpu.VMEM((NHI, D, 128), f32),
            pltpu.VMEM((NQ, D), f32),
            pltpu.VMEM((D, N), f32),
            pltpu.SemaphoreType.DMA((6,)),
            pltpu.SemaphoreType.DMA((L // RB,)),
        ],
        compiler_params=pltpu.CompilerParams(vmem_limit_bytes=100 * 1024 * 1024),
    )(A_A_re, A_A_im, A_B_re, A_B_im, A_C_re, A_C_im,
      A_log_dt, A_Dskip,
      jnp.asarray(_F_FWD, bf16), jnp.asarray(_F_INV, bf16), jnp.asarray(_SEL, bf16),
      *[pltpu.with_memory_space_constraint(t, pltpu.HBM)
        for t in (x, B_w1, B_w2, B_w3.T, B_w4, jnp.asarray(_G_ALL, bf16))])
    return out.reshape(1, L, D)
```

```python
import functools
import numpy as np
import jax
import jax.numpy as jnp
from jax import lax
import jax.experimental.pallas as pl
import jax.experimental.pallas.tpu as pltpu

L = 2048
D = 512
N = 128
FF = 1376
FP = 1408
J = 128
NB = L // J
NQ = 656
_STEP = (1, 1, 2, 2, 4, 4, 4, 4, 8, 8, 8, 8, 8, 8, 8, 8)
HI = tuple(128 * k + b for k in range(16) for b in range(0, 8, _STEP[k])) + (2048,)
NHI = len(HI)
CH = 32
RB = 256
WIN = ((0, 128), (0, 256), (128, 256), (256, 256), (320, 128), (384, 128),
       (384, 128), (448, 128), (448, 128), (512, 128), (512, 128), (512, 128),
       (512, 128), (512, 128), (512, 128), (528, 128))
GW = sum(w[1] for w in WIN)


def _q_of_m(m):
    hi = (m // 128) * 128 + (m % 8)
    return 16 * HI.index(hi) + (m % 128) // 8


def _build_tables():
    pos = np.arange(L, dtype=np.int64)
    rr = np.zeros(L, np.int64)
    for l in range(L):
        if l < 256:
            rr[l] = l
        else:
            step = 1 << (int(l).bit_length() - 8)
            lo = (l // step) * step
            rem = l - lo
            if rem * 2 < step or (rem * 2 == step and (lo // step) % 2 == 0):
                rr[l] = lo
            else:
                rr[l] = lo + step
    w = np.pi * (2 * np.arange(J) + 1) / (2 * J)
    n = np.arange(J)
    f_fwd = np.concatenate([np.cos(np.outer(w, n)), -np.sin(np.outer(w, n))], 0)
    f_inv = np.concatenate([np.cos(np.outer(n, w)), -np.sin(np.outer(n, w))], 1) / J
    g_all = np.zeros((2 * J, GW))
    off = 0
    for dl in range(NB):
        s0, ln = WIN[dl]
        for p in range(-J, J):
            l = dl * J + p
            if 0 <= l < L:
                q = _q_of_m(int(rr[l])) - s0
                assert 0 <= q < ln
                g_all[:J, off + q] += np.cos(w * p)
                g_all[J:, off + q] += -np.sin(w * p)
        off += ln
    sel = np.zeros((16, 128))
    for dd in range(8):
        sel[np.arange(16), np.arange(16) * 8 + dd] = 1.0
    del pos
    return (f_fwd.astype(np.float32), f_inv.astype(np.float32),
            g_all.astype(np.float32), sel.astype(np.float32))


_F_FWD, _F_INV, _G_ALL, _SEL = _build_tables()


def _bf(x):
    return x.astype(jnp.bfloat16)


def _rb(x):
    return x.astype(jnp.bfloat16).astype(jnp.float32)


def _cmul(a, b):
    return (a[0] * b[0] - a[1] * b[1], a[0] * b[1] + a[1] * b[0])


def _gelu(x):
    c = 0.7978845608028654
    return 0.5 * x * (1.0 + jnp.tanh(c * (x + 0.044715 * (x * x * x))))


def _layernorm(x):
    m = jnp.mean(x, axis=-1, keepdims=True)
    xc = x - m
    v = jnp.mean(xc * xc, axis=-1, keepdims=True)
    den = _rb(jnp.sqrt(_rb(_rb(v) + 1e-5)))
    return _rb(_rb(x - _rb(m)) / den)


def _dot(a, b):
    return jnp.dot(a, b, preferred_element_type=jnp.float32)


def _dot_nt(a, b):
    return lax.dot_general(a, b, (((1,), (1,)), ((), ())),
                           preferred_element_type=jnp.float32)


def _kernel(are_ref, aim_ref, bre_ref, bim_ref, cre_ref, cim_ref, ldt_ref, dsk_ref,
            ffwd_ref, finv_ref, sel_ref,
            x_hbm, w1_hbm, w2_hbm, w3_hbm, w4_hbm, g_hbm,
            out_hbm,
            x_v, w1_v, w2_v, w3_v, w4_v, g_v, out_v,
            xn_v, h_v, u_v, kt_v, z_v,
            yr_v, yi_v, xr_v, xi_v, o_v, kd_v, dt_v, x1_v, ln2_v, h2_v,
            sem_in, sem_out):
    copies = [pltpu.make_async_copy(s, d, sem_in.at[k]) for k, (s, d) in enumerate(
        [(x_hbm, x_v), (w1_hbm, w1_v), (g_hbm, g_v), (w2_hbm, w2_v),
         (w3_hbm, w3_v.at[0:FF, :]), (w4_hbm, w4_v.at[0:FF, :])])]
    for c in copies:
        c.start()

    dt_row = _rb(jnp.exp(ldt_ref[...].astype(jnp.float32))).reshape(1, D)
    dt_v[...] = jnp.transpose(jnp.broadcast_to(dt_row, (N, D)))

    def kgen(c, carry):
        r0 = pl.multiple_of(c * CH, CH)
        rows = pl.ds(r0, CH)
        f32 = jnp.float32
        dt = dt_v[rows, :]
        lr = dt * are_ref[rows, :].astype(f32)
        li = dt * aim_ref[rows, :].astype(f32)
        dbr = dt * bre_ref[rows, :].astype(f32)
        dbi = dt * bim_ref[rows, :].astype(f32)
        w = _cmul((cre_ref[rows, :].astype(f32), cim_ref[rows, :].astype(f32)), (dbr, dbi))

        def csq(a):
            ab = a[0] * a[1]
            return (a[0] * a[0] - a[1] * a[1], ab + ab)

        e1 = jnp.exp(lr)
        z1 = (e1 * jnp.cos(li), e1 * jnp.sin(li))
        z8 = csq(csq(csq(z1)))
        z128 = csq(csq(csq(csq(z8))))
        z1024 = csq(csq(csq(z128)))

        def put_y(j, v):
            for g in range(CH // 8):
                yr_v[g, 8 * j:8 * j + 8, :] = v[0][8 * g:8 * g + 8, :]
                yi_v[g, 8 * j:8 * j + 8, :] = v[1][8 * g:8 * g + 8, :]

        def put_x(i, v):
            nvi = -v[1]
            for g in range(CH // 8):
                xr_v[g, 8 * i:8 * i + 8, :] = v[0][8 * g:8 * g + 8, :]
                xi_v[g, 8 * i:8 * i + 8, :] = nvi[8 * g:8 * g + 8, :]

        put_y(0, (jnp.ones_like(lr), jnp.zeros_like(lr)))
        y = z8
        put_y(1, y)
        for j in range(2, 16):
            y = _cmul(y, z8)
            put_y(j, y)
        v = w
        for b in range(8):
            if b:
                v = _cmul(v, z1)
            t = v
            for k in range(8):
                if (128 * k + b) in HI:
                    if k:
                        t = _cmul(t, z128)
                    put_x(HI.index(128 * k + b), t)
        t = _cmul(w, z1024)
        for k in range(8, 17):
            if k > 8:
                t = _cmul(t, z128)
            put_x(HI.index(128 * k), t)
        for g in range(CH // 8):
            o = (_dot_nt(_bf(xr_v[g]), _bf(yr_v[g])) + _dot_nt(_bf(xi_v[g]), _bf(yi_v[g])))
            for i in range(NHI):
                o_v[i, pl.ds(pl.multiple_of(r0 + 8 * g, 8), 8), :] = o[8 * i:8 * i + 8, :]
        return carry

    with jax.named_scope('p_kgen'):
        lax.fori_loop(0, D // CH, kgen, 0)

    rid = lax.broadcasted_iota(jnp.int32, (D, 128), 0)
    lid = lax.broadcasted_iota(jnp.int32, (D, 128), 1)
    keep = (rid % 8) == (lid % 8)
    keep_last = keep & (lid < 8)
    sel = sel_ref[...]
    with jax.named_scope('p_sel'):
        for i in range(NHI):
            oi = jnp.where(keep_last if HI[i] == 2048 else keep, o_v[i], 0.0)
            kd_v[16 * i:16 * i + 16, :] = _dot_nt(sel, _bf(oi))

    copies[2].wait()
    off = 0
    for dl in range(NB):
        s0, ln = WIN[dl]
        kt_v[dl] = _dot(g_v[:, off:off + ln], _bf(kd_v[s0:s0 + ln, :]))
        off += ln

    copies[0].wait()
    copies[1].wait()
    h_v[0:8, :] = jnp.zeros((8, D), jnp.float32)
    h_v[8 + L:16 + L, :] = jnp.zeros((8, D), jnp.float32)

    def phase1(b, carry):
        r0 = pl.multiple_of(b * RB, RB)
        x = x_v[pl.ds(r0, RB), :].astype(jnp.float32)
        xn = _bf(_layernorm(x))
        xn_v[pl.ds(r0, RB), :] = xn
        h = _rb(_gelu(_rb(_dot(xn, w1_v[...]))))
        h_v[pl.ds(pl.multiple_of(r0 + 8, 8), RB), :] = h
        for k in range(RB // J):
            u_v[b * (RB // J) + k] = _dot(ffwd_ref[...], xn[k * J:(k + 1) * J, :])
        return carry

    with jax.named_scope('p_phase1'):
        lax.fori_loop(0, L // RB, phase1, 0)

    def ztile(i, t):
        f0 = pl.multiple_of((t // 4) * 16, 16)
        re = pl.ds(f0, 16)
        im = pl.ds(pl.multiple_of(f0 + J, 16), 16)
        cs = pl.ds(pl.multiple_of((t % 4) * 128, 128), 128)
        zr = zi = None
        for dl in range(i + 1):
            kr = kt_v[dl, re, cs]
            ki = kt_v[dl, im, cs]
            ur = u_v[i - dl, re, cs]
            ui = u_v[i - dl, im, cs]
            pr = kr * ur - ki * ui
            pi = kr * ui + ki * ur
            zr = pr if zr is None else zr + pr
            zi = pi if zi is None else zi + pi
        z_v[i, re, cs] = _bf(zr)
        z_v[i, im, cs] = _bf(zi)

    copies[3].wait()
    copies[4].wait()
    copies[5].wait()
    w3_v[FF:FP, :] = jnp.zeros((FP - FF, D), jnp.bfloat16)
    w4_v[FF:FP, :] = jnp.zeros((FP - FF, D), jnp.bfloat16)
    dsk = dsk_ref[...].astype(jnp.float32).reshape(1, D)

    def out_copy(b):
        return pltpu.make_async_copy(out_v.at[pl.ds(b * RB, RB), :],
                                     out_hbm.at[pl.ds(b * RB, RB), :], sem_out.at[b])

    ZSCHED = ((0, 1, 2, 3, 6), (4, 11), (5, 10), (7, 8), (9, 12), (13,), (14,), (15,))
    NFC = FP // 128

    def phase2(b):
        r0 = b * RB
        ext = RB + 16
        parts = []
        for gi, sh in enumerate((1, -1, 2, -2)):
            hv = h_v[pl.ds(r0, ext), gi * 128:(gi + 1) * 128]
            hv = pltpu.roll(hv, sh % ext, 0)
            parts.append(_bf(hv[8:8 + RB, :]))
        hs = _rb(_dot(jnp.concatenate(parts, axis=1), w2_v[...]))
        xn = xn_v[pl.ds(r0, RB), :].astype(jnp.float32)
        x1 = _rb(xn + hs)
        x1_v[...] = x1
        ln2_v[...] = _bf(_layernorm(x1))
        h2_v[...] = jnp.zeros((RB, D), jnp.float32)

        def fchunk(c, carry):
            rows = pl.ds(pl.multiple_of(c * 128, 128), 128)
            a = _rb(_dot_nt(ln2_v[...], w3_v[rows, :]))
            h2_v[...] += _dot(_bf(_gelu(a)), w4_v[rows, :])
            for i in ZSCHED[b]:
                for k in range(3):
                    ztile(i, jnp.minimum(3 * c + k, 31))
            return carry

        lax.fori_loop(0, NFC, fchunk, 0)
        bb = _rb(x1_v[...] + _rb(h2_v[...]))
        gate = _rb(bb * jax.nn.sigmoid(bb))
        ys = [_dot(finv_ref[...], z_v[b * (RB // J) + k]) for k in range(RB // J)]
        y = _rb(jnp.concatenate(ys, axis=0))
        xn = xn_v[pl.ds(r0, RB), :].astype(jnp.float32)
        s = _rb(y + _rb(xn * dsk))
        x = x_v[pl.ds(r0, RB), :].astype(jnp.float32)
        out_v[pl.ds(r0, RB), :] = _bf(x + _rb(s * gate))
        out_copy(b).start()

    with jax.named_scope('p_phase2'):
        for b in range(L // RB):
            phase2(b)
    for b in range(L // RB):
        out_copy(b).wait()


@jax.jit
def pallas_recurrent_scan__ssm_conv_s4__mixer_s_mlp__prompt_kernel(
    A_u: jax.Array,
    A_A_re: jax.Array,
    A_A_im: jax.Array,
    A_B_re: jax.Array,
    A_B_im: jax.Array,
    A_C_re: jax.Array,
    A_C_im: jax.Array,
    A_log_dt: jax.Array,
    A_Dskip: jax.Array,
    B_x: jax.Array,
    B_w1: jax.Array,
    B_w2: jax.Array,
    B_w3: jax.Array,
    B_w4: jax.Array,
):
    bf16 = jnp.bfloat16
    f32 = jnp.float32
    x = A_u.reshape(L, D)
    vm = pl.BlockSpec(memory_space=pltpu.VMEM)
    hbm = pl.BlockSpec(memory_space=pltpu.HBM)
    out = pl.pallas_call(
        _kernel,
        out_shape=jax.ShapeDtypeStruct((L, D), bf16),
        in_specs=[vm] * 11 + [hbm] * 6,
        out_specs=hbm,
        scratch_shapes=[
            pltpu.VMEM((L, D), bf16),
            pltpu.VMEM((D, D), bf16),
            pltpu.VMEM((D, D), bf16),
            pltpu.VMEM((FP, D), bf16),
            pltpu.VMEM((FP, D), bf16),
            pltpu.VMEM((2 * J, GW), bf16),
            pltpu.VMEM((L, D), bf16),
            pltpu.VMEM((L, D), bf16),
            pltpu.VMEM((L + 16, D), f32),
            pltpu.VMEM((NB, 2 * J, D), f32),
            pltpu.VMEM((NB, 2 * J, D), f32),
            pltpu.VMEM((NB, 2 * J, D), bf16),
            pltpu.VMEM((CH // 8, 128, N), f32),
            pltpu.VMEM((CH // 8, 128, N), f32),
            pltpu.VMEM((CH // 8, 8 * NHI, N), f32),
            pltpu.VMEM((CH // 8, 8 * NHI, N), f32),
            pltpu.VMEM((NHI, D, 128), f32),
            pltpu.VMEM((NQ, D), f32),
            pltpu.VMEM((D, N), f32),
            pltpu.VMEM((RB, D), f32),
            pltpu.VMEM((RB, D), bf16),
            pltpu.VMEM((RB, D), f32),
            pltpu.SemaphoreType.DMA((6,)),
            pltpu.SemaphoreType.DMA((L // RB,)),
        ],
        compiler_params=pltpu.CompilerParams(vmem_limit_bytes=100 * 1024 * 1024),
    )(A_A_re, A_A_im, A_B_re, A_B_im, A_C_re, A_C_im,
      A_log_dt, A_Dskip,
      jnp.asarray(_F_FWD, bf16), jnp.asarray(_F_INV, bf16), jnp.asarray(_SEL, bf16),
      *[pltpu.with_memory_space_constraint(t, pltpu.HBM)
        for t in (x, B_w1, B_w2, B_w3.T, B_w4, jnp.asarray(_G_ALL, bf16))])
    return out.reshape(1, L, D)
```

```python
import functools
import numpy as np
import jax
import jax.numpy as jnp
from jax import lax
import jax.experimental.pallas as pl
import jax.experimental.pallas.tpu as pltpu

L = 2048
D = 512
N = 128
FF = 1376
FP = 1408
J = 128
NB = L // J
NQ = 656
_STEP = (1, 1, 2, 2, 4, 4, 4, 4, 8, 8, 8, 8, 8, 8, 8, 8)
HI = tuple(128 * k + b for k in range(16) for b in range(0, 8, _STEP[k])) + (2048,)
NHI = len(HI)
CH = 32
RB = 256
WIN = ((0, 128), (0, 256), (128, 256), (256, 256), (320, 128), (384, 128),
       (384, 128), (448, 128), (448, 128), (512, 128), (512, 128), (512, 128),
       (512, 128), (512, 128), (512, 128), (528, 128))
GW = sum(w[1] for w in WIN)


def _q_of_m(m):
    hi = (m // 128) * 128 + (m % 8)
    return 16 * HI.index(hi) + (m % 128) // 8


def _build_tables():
    pos = np.arange(L, dtype=np.int64)
    rr = np.zeros(L, np.int64)
    for l in range(L):
        if l < 256:
            rr[l] = l
        else:
            step = 1 << (int(l).bit_length() - 8)
            lo = (l // step) * step
            rem = l - lo
            if rem * 2 < step or (rem * 2 == step and (lo // step) % 2 == 0):
                rr[l] = lo
            else:
                rr[l] = lo + step
    w = np.pi * (2 * np.arange(J) + 1) / (2 * J)
    n = np.arange(J)
    f_fwd = np.concatenate([np.cos(np.outer(w, n)), -np.sin(np.outer(w, n))], 0)
    f_inv = np.concatenate([np.cos(np.outer(n, w)), -np.sin(np.outer(n, w))], 1) / J
    g_all = np.zeros((2 * J, GW))
    off = 0
    for dl in range(NB):
        s0, ln = WIN[dl]
        for p in range(-J, J):
            l = dl * J + p
            if 0 <= l < L:
                q = _q_of_m(int(rr[l])) - s0
                assert 0 <= q < ln
                g_all[:J, off + q] += np.cos(w * p)
                g_all[J:, off + q] += -np.sin(w * p)
        off += ln
    sel = np.zeros((16, 128))
    for dd in range(8):
        sel[np.arange(16), np.arange(16) * 8 + dd] = 1.0
    del pos
    return (f_fwd.astype(np.float32), f_inv.astype(np.float32),
            g_all.astype(np.float32), sel.astype(np.float32))


_F_FWD, _F_INV, _G_ALL, _SEL = _build_tables()


def _bf(x):
    return x.astype(jnp.bfloat16)


def _rb(x):
    return x.astype(jnp.bfloat16).astype(jnp.float32)


def _cmul(a, b):
    return (a[0] * b[0] - a[1] * b[1], a[0] * b[1] + a[1] * b[0])


def _gelu(x):
    c = 0.7978845608028654
    return 0.5 * x * (1.0 + jnp.tanh(c * (x + 0.044715 * (x * x * x))))


def _layernorm(x):
    m = jnp.mean(x, axis=-1, keepdims=True)
    xc = x - m
    v = jnp.mean(xc * xc, axis=-1, keepdims=True)
    den = _rb(jnp.sqrt(_rb(_rb(v) + 1e-5)))
    return _rb(_rb(x - _rb(m)) / den)


def _dot(a, b):
    return jnp.dot(a, b, preferred_element_type=jnp.float32)


def _dot_nt(a, b):
    return lax.dot_general(a, b, (((1,), (1,)), ((), ())),
                           preferred_element_type=jnp.float32)


def _kernel(are_ref, aim_ref, bre_ref, bim_ref, cre_ref, cim_ref, ldt_ref, dsk_ref,
            ffwd_ref, finv_ref, sel_ref,
            x_hbm, w1_hbm, w2_hbm, w3_hbm, w4_hbm, g_hbm,
            out_hbm,
            x_v, w1_v, w2_v, w3_v, w4_v, g_v, out_v,
            xn_v, h_v, u_v, kt_v, z_v,
            yr_v, yi_v, xr_v, xi_v, o_v, kd_v, dt_v, x1_v, ln2_v, h2_v, ga_v,
            sem_in, sem_out):
    copies = [pltpu.make_async_copy(s, d, sem_in.at[k]) for k, (s, d) in enumerate(
        [(x_hbm, x_v), (w1_hbm, w1_v), (g_hbm, g_v), (w2_hbm, w2_v),
         (w3_hbm, w3_v.at[0:FF, :]), (w4_hbm, w4_v.at[0:FF, :])])]
    for c in copies:
        c.start()

    dt_row = _rb(jnp.exp(ldt_ref[...].astype(jnp.float32))).reshape(1, D)
    dt_v[...] = jnp.transpose(jnp.broadcast_to(dt_row, (N, D)))

    def kgen(c, carry):
        r0 = pl.multiple_of(c * CH, CH)
        rows = pl.ds(r0, CH)
        f32 = jnp.float32
        dt = dt_v[rows, :]
        lr = dt * are_ref[rows, :].astype(f32)
        li = dt * aim_ref[rows, :].astype(f32)
        dbr = dt * bre_ref[rows, :].astype(f32)
        dbi = dt * bim_ref[rows, :].astype(f32)
        w = _cmul((cre_ref[rows, :].astype(f32), cim_ref[rows, :].astype(f32)), (dbr, dbi))

        def csq(a):
            ab = a[0] * a[1]
            return (a[0] * a[0] - a[1] * a[1], ab + ab)

        e1 = jnp.exp(lr)
        z1 = (e1 * jnp.cos(li), e1 * jnp.sin(li))
        z8 = csq(csq(csq(z1)))
        z128 = csq(csq(csq(csq(z8))))
        z1024 = csq(csq(csq(z128)))

        def put_y(j, v):
            for g in range(CH // 8):
                yr_v[g, 8 * j:8 * j + 8, :] = v[0][8 * g:8 * g + 8, :]
                yi_v[g, 8 * j:8 * j + 8, :] = v[1][8 * g:8 * g + 8, :]

        def put_x(i, v):
            nvi = -v[1]
            for g in range(CH // 8):
                xr_v[g, 8 * i:8 * i + 8, :] = v[0][8 * g:8 * g + 8, :]
                xi_v[g, 8 * i:8 * i + 8, :] = nvi[8 * g:8 * g + 8, :]

        put_y(0, (jnp.ones_like(lr), jnp.zeros_like(lr)))
        y = z8
        put_y(1, y)
        for j in range(2, 16):
            y = _cmul(y, z8)
            put_y(j, y)
        v = w
        for b in range(8):
            if b:
                v = _cmul(v, z1)
            t = v
            for k in range(8):
                if (128 * k + b) in HI:
                    if k:
                        t = _cmul(t, z128)
                    put_x(HI.index(128 * k + b), t)
        t = _cmul(w, z1024)
        for k in range(8, 17):
            if k > 8:
                t = _cmul(t, z128)
            put_x(HI.index(128 * k), t)
        for g in range(CH // 8):
            o = (_dot_nt(_bf(xr_v[g]), _bf(yr_v[g])) + _dot_nt(_bf(xi_v[g]), _bf(yi_v[g])))
            for i in range(NHI):
                o_v[i, pl.ds(pl.multiple_of(r0 + 8 * g, 8), 8), :] = o[8 * i:8 * i + 8, :]
        return carry

    with jax.named_scope('p_kgen'):
        lax.fori_loop(0, D // CH, kgen, 0)

    rid = lax.broadcasted_iota(jnp.int32, (D, 128), 0)
    lid = lax.broadcasted_iota(jnp.int32, (D, 128), 1)
    keep = (rid % 8) == (lid % 8)
    keep_last = keep & (lid < 8)
    sel = sel_ref[...]
    with jax.named_scope('p_sel'):
        for i in range(NHI):
            oi = jnp.where(keep_last if HI[i] == 2048 else keep, o_v[i], 0.0)
            kd_v[16 * i:16 * i + 16, :] = _dot_nt(sel, _bf(oi))

    copies[2].wait()
    off = 0
    for dl in range(NB):
        s0, ln = WIN[dl]
        kt_v[dl] = _dot(g_v[:, off:off + ln], _bf(kd_v[s0:s0 + ln, :]))
        off += ln

    copies[0].wait()
    copies[1].wait()
    h_v[0:8, :] = jnp.zeros((8, D), jnp.float32)
    h_v[8 + L:16 + L, :] = jnp.zeros((8, D), jnp.float32)

    def phase1(b, carry):
        r0 = pl.multiple_of(b * RB, RB)
        x = x_v[pl.ds(r0, RB), :].astype(jnp.float32)
        xn = _bf(_layernorm(x))
        xn_v[pl.ds(r0, RB), :] = xn
        h = _rb(_gelu(_rb(_dot(xn, w1_v[...]))))
        h_v[pl.ds(pl.multiple_of(r0 + 8, 8), RB), :] = h
        for k in range(RB // J):
            u_v[b * (RB // J) + k] = _dot(ffwd_ref[...], xn[k * J:(k + 1) * J, :])
        return carry

    with jax.named_scope('p_phase1'):
        lax.fori_loop(0, L // RB, phase1, 0)

    def ztile(i, t):
        if isinstance(t, int):
            re = pl.ds((t // 4) * 16, 16)
            im = pl.ds((t // 4) * 16 + J, 16)
            cs = pl.ds((t % 4) * 128, 128)
        else:
            f0 = pl.multiple_of((t // 4) * 16, 16)
            re = pl.ds(f0, 16)
            im = pl.ds(pl.multiple_of(f0 + J, 16), 16)
            cs = pl.ds(pl.multiple_of((t % 4) * 128, 128), 128)
        zr = zi = None
        for dl in range(i + 1):
            kr = kt_v[dl, re, cs]
            ki = kt_v[dl, im, cs]
            ur = u_v[i - dl, re, cs]
            ui = u_v[i - dl, im, cs]
            pr = kr * ur - ki * ui
            pi = kr * ui + ki * ur
            zr = pr if zr is None else zr + pr
            zi = pi if zi is None else zi + pi
        z_v[i, re, cs] = _bf(zr)
        z_v[i, im, cs] = _bf(zi)

    copies[3].wait()
    copies[4].wait()
    copies[5].wait()
    w3_v[FF:FP, :] = jnp.zeros((FP - FF, D), jnp.bfloat16)
    w4_v[FF:FP, :] = jnp.zeros((FP - FF, D), jnp.bfloat16)
    dsk = dsk_ref[...].astype(jnp.float32).reshape(1, D)

    def out_copy(b):
        return pltpu.make_async_copy(out_v.at[pl.ds(b * RB, RB), :],
                                     out_hbm.at[pl.ds(b * RB, RB), :], sem_out.at[b])

    ZSCHED = ((0, 1, 2, 3, 6), (4, 11), (5, 10), (7, 8), (9, 12), (13,), (14,), (15,))
    NFC = FP // 128

    def phase2(b):
        r0 = b * RB
        ext = RB + 16
        parts = []
        for gi, sh in enumerate((1, -1, 2, -2)):
            hv = h_v[pl.ds(r0, ext), gi * 128:(gi + 1) * 128]
            hv = pltpu.roll(hv, sh % ext, 0)
            parts.append(_bf(hv[8:8 + RB, :]))
        hs = _rb(_dot(jnp.concatenate(parts, axis=1), w2_v[...]))
        xn = xn_v[pl.ds(r0, RB), :].astype(jnp.float32)
        x1 = _rb(xn + hs)
        x1_v[...] = x1
        ln2_v[...] = _bf(_layernorm(x1))
        h2_v[...] = jnp.zeros((RB, D), jnp.float32)

        def up(c):
            rows = pl.ds(pl.multiple_of(c * 128, 128), 128)
            return _bf(_gelu(_rb(_dot_nt(ln2_v[...], w3_v[rows, :]))))

        ga_v[0] = up(0)

        def fchunk(c, carry):
            rows = pl.ds(pl.multiple_of(c * 128, 128), 128)
            h2_v[...] += _dot(ga_v[c % 2], w4_v[rows, :])
            ga_v[(c + 1) % 2] = up(c + 1)
            for i in ZSCHED[b]:
                for k in range(3):
                    ztile(i, 3 * c + k)
            return carry

        lax.fori_loop(0, NFC - 1, fchunk, 0)
        h2_v[...] += _dot(ga_v[(NFC - 1) % 2], w4_v[(NFC - 1) * 128:NFC * 128, :])
        for i in ZSCHED[b]:
            for t in range(3 * (NFC - 1), 32):
                ztile(i, t)
        bb = _rb(x1_v[...] + _rb(h2_v[...]))
        gate = _rb(bb * jax.nn.sigmoid(bb))
        ys = [_dot(finv_ref[...], z_v[b * (RB // J) + k]) for k in range(RB // J)]
        y = _rb(jnp.concatenate(ys, axis=0))
        xn = xn_v[pl.ds(r0, RB), :].astype(jnp.float32)
        s = _rb(y + _rb(xn * dsk))
        x = x_v[pl.ds(r0, RB), :].astype(jnp.float32)
        out_v[pl.ds(r0, RB), :] = _bf(x + _rb(s * gate))
        out_copy(b).start()

    with jax.named_scope('p_phase2'):
        for b in range(L // RB):
            phase2(b)
    for b in range(L // RB):
        out_copy(b).wait()


@jax.jit
def pallas_recurrent_scan__ssm_conv_s4__mixer_s_mlp__prompt_kernel(
    A_u: jax.Array,
    A_A_re: jax.Array,
    A_A_im: jax.Array,
    A_B_re: jax.Array,
    A_B_im: jax.Array,
    A_C_re: jax.Array,
    A_C_im: jax.Array,
    A_log_dt: jax.Array,
    A_Dskip: jax.Array,
    B_x: jax.Array,
    B_w1: jax.Array,
    B_w2: jax.Array,
    B_w3: jax.Array,
    B_w4: jax.Array,
):
    bf16 = jnp.bfloat16
    f32 = jnp.float32
    x = A_u.reshape(L, D)
    vm = pl.BlockSpec(memory_space=pltpu.VMEM)
    hbm = pl.BlockSpec(memory_space=pltpu.HBM)
    out = pl.pallas_call(
        _kernel,
        out_shape=jax.ShapeDtypeStruct((L, D), bf16),
        in_specs=[vm] * 11 + [hbm] * 6,
        out_specs=hbm,
        scratch_shapes=[
            pltpu.VMEM((L, D), bf16),
            pltpu.VMEM((D, D), bf16),
            pltpu.VMEM((D, D), bf16),
            pltpu.VMEM((FP, D), bf16),
            pltpu.VMEM((FP, D), bf16),
            pltpu.VMEM((2 * J, GW), bf16),
            pltpu.VMEM((L, D), bf16),
            pltpu.VMEM((L, D), bf16),
            pltpu.VMEM((L + 16, D), f32),
            pltpu.VMEM((NB, 2 * J, D), f32),
            pltpu.VMEM((NB, 2 * J, D), f32),
            pltpu.VMEM((NB, 2 * J, D), bf16),
            pltpu.VMEM((CH // 8, 128, N), f32),
            pltpu.VMEM((CH // 8, 128, N), f32),
            pltpu.VMEM((CH // 8, 8 * NHI, N), f32),
            pltpu.VMEM((CH // 8, 8 * NHI, N), f32),
            pltpu.VMEM((NHI, D, 128), f32),
            pltpu.VMEM((NQ, D), f32),
            pltpu.VMEM((D, N), f32),
            pltpu.VMEM((RB, D), f32),
            pltpu.VMEM((RB, D), bf16),
            pltpu.VMEM((RB, D), f32),
            pltpu.VMEM((2, RB, 128), bf16),
            pltpu.SemaphoreType.DMA((6,)),
            pltpu.SemaphoreType.DMA((L // RB,)),
        ],
        compiler_params=pltpu.CompilerParams(vmem_limit_bytes=100 * 1024 * 1024),
    )(A_A_re, A_A_im, A_B_re, A_B_im, A_C_re, A_C_im,
      A_log_dt, A_Dskip,
      jnp.asarray(_F_FWD, bf16), jnp.asarray(_F_INV, bf16), jnp.asarray(_SEL, bf16),
      *[pltpu.with_memory_space_constraint(t, pltpu.HBM)
        for t in (x, B_w1, B_w2, B_w3.T, B_w4, jnp.asarray(_G_ALL, bf16))])
    return out.reshape(1, L, D)
```

```python
import functools
import numpy as np
import jax
import jax.numpy as jnp
from jax import lax
import jax.experimental.pallas as pl
import jax.experimental.pallas.tpu as pltpu

L = 2048
D = 512
N = 128
FF = 1376
FP = 1408
J = 128
NB = L // J
NQ = 656
_STEP = (1, 1, 2, 2, 4, 4, 4, 4, 8, 8, 8, 8, 8, 8, 8, 8)
HI = tuple(128 * k + b for k in range(16) for b in range(0, 8, _STEP[k])) + (2048,)
NHI = len(HI)
CH = 32
RB = 256
WIN = ((0, 128), (0, 256), (128, 256), (256, 256), (320, 128), (384, 128),
       (384, 128), (448, 128), (448, 128), (512, 128), (512, 128), (512, 128),
       (512, 128), (512, 128), (512, 128), (528, 128))
GW = sum(w[1] for w in WIN)


def _q_of_m(m):
    hi = (m // 128) * 128 + (m % 8)
    return 16 * HI.index(hi) + (m % 128) // 8


def _build_tables():
    pos = np.arange(L, dtype=np.int64)
    rr = np.zeros(L, np.int64)
    for l in range(L):
        if l < 256:
            rr[l] = l
        else:
            step = 1 << (int(l).bit_length() - 8)
            lo = (l // step) * step
            rem = l - lo
            if rem * 2 < step or (rem * 2 == step and (lo // step) % 2 == 0):
                rr[l] = lo
            else:
                rr[l] = lo + step
    w = np.pi * (2 * np.arange(J) + 1) / (2 * J)
    n = np.arange(J)
    f_fwd = np.concatenate([np.cos(np.outer(w, n)), -np.sin(np.outer(w, n))], 0)
    f_inv = np.concatenate([np.cos(np.outer(n, w)), -np.sin(np.outer(n, w))], 1) / J
    g_all = np.zeros((2 * J, GW))
    off = 0
    for dl in range(NB):
        s0, ln = WIN[dl]
        for p in range(-J, J):
            l = dl * J + p
            if 0 <= l < L:
                q = _q_of_m(int(rr[l])) - s0
                assert 0 <= q < ln
                g_all[:J, off + q] += np.cos(w * p)
                g_all[J:, off + q] += -np.sin(w * p)
        off += ln
    sel = np.zeros((16, 128))
    for dd in range(8):
        sel[np.arange(16), np.arange(16) * 8 + dd] = 1.0
    del pos
    return (f_fwd.astype(np.float32), f_inv.astype(np.float32),
            g_all.astype(np.float32), sel.astype(np.float32))


_F_FWD, _F_INV, _G_ALL, _SEL = _build_tables()


def _bf(x):
    return x.astype(jnp.bfloat16)


def _rb(x):
    return x.astype(jnp.bfloat16).astype(jnp.float32)


def _cmul(a, b):
    return (a[0] * b[0] - a[1] * b[1], a[0] * b[1] + a[1] * b[0])


def _gelu(x):
    c = 0.7978845608028654
    return 0.5 * x * (1.0 + jnp.tanh(c * (x + 0.044715 * (x * x * x))))


def _layernorm(x):
    m = jnp.mean(x, axis=-1, keepdims=True)
    xc = x - m
    v = jnp.mean(xc * xc, axis=-1, keepdims=True)
    den = _rb(jnp.sqrt(_rb(_rb(v) + 1e-5)))
    return _rb(_rb(x - _rb(m)) / den)


def _dot(a, b):
    return jnp.dot(a, b, preferred_element_type=jnp.float32)


def _dot_nt(a, b):
    return lax.dot_general(a, b, (((1,), (1,)), ((), ())),
                           preferred_element_type=jnp.float32)


def _kernel(are_ref, aim_ref, bre_ref, bim_ref, cre_ref, cim_ref, ldt_ref, dsk_ref,
            ffwd_ref, finv_ref, sel_ref,
            x_hbm, w1_hbm, w2_hbm, w3_hbm, w4_hbm, g_hbm,
            out_hbm,
            x_v, w1_v, w2_v, w3_v, w4_v, g_v, out_v,
            xn_v, h_v, u_v, kt_v, z_v,
            yr_v, yi_v, xr_v, xi_v, o_v, kd_v, dt_v, x1_v, ln2_v, h2_v, ga_v, gate_v,
            sem_in, sem_out):
    copies = [pltpu.make_async_copy(s, d, sem_in.at[k]) for k, (s, d) in enumerate(
        [(x_hbm, x_v), (w1_hbm, w1_v), (g_hbm, g_v), (w2_hbm, w2_v),
         (w3_hbm, w3_v.at[0:FF, :]), (w4_hbm, w4_v.at[0:FF, :])])]
    for c in copies:
        c.start()

    dt_row = _rb(jnp.exp(ldt_ref[...].astype(jnp.float32))).reshape(1, D)
    dt_v[...] = jnp.transpose(jnp.broadcast_to(dt_row, (N, D)))

    def kgen(c, carry):
        r0 = pl.multiple_of(c * CH, CH)
        rows = pl.ds(r0, CH)
        f32 = jnp.float32
        dt = dt_v[rows, :]
        lr = dt * are_ref[rows, :].astype(f32)
        li = dt * aim_ref[rows, :].astype(f32)
        dbr = dt * bre_ref[rows, :].astype(f32)
        dbi = dt * bim_ref[rows, :].astype(f32)
        w = _cmul((cre_ref[rows, :].astype(f32), cim_ref[rows, :].astype(f32)), (dbr, dbi))

        def csq(a):
            ab = a[0] * a[1]
            return (a[0] * a[0] - a[1] * a[1], ab + ab)

        e1 = jnp.exp(lr)
        z1 = (e1 * jnp.cos(li), e1 * jnp.sin(li))
        z8 = csq(csq(csq(z1)))
        z128 = csq(csq(csq(csq(z8))))
        z1024 = csq(csq(csq(z128)))

        def put_y(j, v):
            for g in range(CH // 8):
                yr_v[g, 8 * j:8 * j + 8, :] = v[0][8 * g:8 * g + 8, :]
                yi_v[g, 8 * j:8 * j + 8, :] = v[1][8 * g:8 * g + 8, :]

        def put_x(i, v):
            nvi = -v[1]
            for g in range(CH // 8):
                xr_v[g, 8 * i:8 * i + 8, :] = v[0][8 * g:8 * g + 8, :]
                xi_v[g, 8 * i:8 * i + 8, :] = nvi[8 * g:8 * g + 8, :]

        put_y(0, (jnp.ones_like(lr), jnp.zeros_like(lr)))
        y = z8
        put_y(1, y)
        for j in range(2, 16):
            y = _cmul(y, z8)
            put_y(j, y)
        v = w
        for b in range(8):
            if b:
                v = _cmul(v, z1)
            t = v
            for k in range(8):
                if (128 * k + b) in HI:
                    if k:
                        t = _cmul(t, z128)
                    put_x(HI.index(128 * k + b), t)
        t = _cmul(w, z1024)
        for k in range(8, 17):
            if k > 8:
                t = _cmul(t, z128)
            put_x(HI.index(128 * k), t)
        for g in range(CH // 8):
            o = (_dot_nt(_bf(xr_v[g]), _bf(yr_v[g])) + _dot_nt(_bf(xi_v[g]), _bf(yi_v[g])))
            for i in range(NHI):
                o_v[i, pl.ds(pl.multiple_of(r0 + 8 * g, 8), 8), :] = o[8 * i:8 * i + 8, :]
        return carry

    with jax.named_scope('p_kgen'):
        lax.fori_loop(0, D // CH, kgen, 0)

    rid = lax.broadcasted_iota(jnp.int32, (D, 128), 0)
    lid = lax.broadcasted_iota(jnp.int32, (D, 128), 1)
    keep = (rid % 8) == (lid % 8)
    keep_last = keep & (lid < 8)
    sel = sel_ref[...]
    with jax.named_scope('p_sel'):
        for i in range(NHI):
            oi = jnp.where(keep_last if HI[i] == 2048 else keep, o_v[i], 0.0)
            kd_v[16 * i:16 * i + 16, :] = _dot_nt(sel, _bf(oi))

    copies[2].wait()
    off = 0
    for dl in range(NB):
        s0, ln = WIN[dl]
        kt_v[dl] = _dot(g_v[:, off:off + ln], _bf(kd_v[s0:s0 + ln, :]))
        off += ln

    copies[0].wait()
    copies[1].wait()
    h_v[0:8, :] = jnp.zeros((8, D), jnp.float32)
    h_v[8 + L:16 + L, :] = jnp.zeros((8, D), jnp.float32)

    def phase1(b, carry):
        r0 = pl.multiple_of(b * RB, RB)
        x = x_v[pl.ds(r0, RB), :].astype(jnp.float32)
        xn = _bf(_layernorm(x))
        xn_v[pl.ds(r0, RB), :] = xn
        h = _rb(_gelu(_rb(_dot(xn, w1_v[...]))))
        h_v[pl.ds(pl.multiple_of(r0 + 8, 8), RB), :] = h
        for k in range(RB // J):
            u_v[b * (RB // J) + k] = _dot(ffwd_ref[...], xn[k * J:(k + 1) * J, :])
        return carry

    with jax.named_scope('p_phase1'):
        lax.fori_loop(0, L // RB, phase1, 0)

    def ztile(t):
        f0 = pl.multiple_of((t // 4) * 16, 16)
        re = pl.ds(f0, 16)
        im = pl.ds(pl.multiple_of(f0 + J, 16), 16)
        cs = pl.ds(pl.multiple_of((t % 4) * 128, 128), 128)
        for i in range(NB):
            zr = zi = None
            for dl in range(i + 1):
                kr = kt_v[dl, re, cs]
                ki = kt_v[dl, im, cs]
                ur = u_v[i - dl, re, cs]
                ui = u_v[i - dl, im, cs]
                pr = kr * ur - ki * ui
                pi = kr * ui + ki * ur
                zr = pr if zr is None else zr + pr
                zi = pi if zi is None else zi + pi
            z_v[i, re, cs] = _bf(zr)
            z_v[i, im, cs] = _bf(zi)

    copies[3].wait()
    copies[4].wait()
    copies[5].wait()
    w3_v[FF:FP, :] = jnp.zeros((FP - FF, D), jnp.bfloat16)
    w4_v[FF:FP, :] = jnp.zeros((FP - FF, D), jnp.bfloat16)
    NFC = FP // 128

    def phase2(b, carry):
        r0 = pl.multiple_of(b * RB, RB)
        ext = RB + 16
        parts = []
        for gi, sh in enumerate((1, -1, 2, -2)):
            hv = h_v[pl.ds(r0, ext), gi * 128:(gi + 1) * 128]
            hv = pltpu.roll(hv, sh % ext, 0)
            parts.append(_bf(hv[8:8 + RB, :]))
        hs = _rb(_dot(jnp.concatenate(parts, axis=1), w2_v[...]))
        xn = xn_v[pl.ds(r0, RB), :].astype(jnp.float32)
        x1 = _rb(xn + hs)
        x1_v[...] = x1
        ln2_v[...] = _bf(_layernorm(x1))
        h2_v[...] = jnp.zeros((RB, D), jnp.float32)
        ga_v[...] = jnp.zeros((RB, 128), jnp.bfloat16)

        def frows(c):
            return pl.ds(pl.multiple_of(jnp.clip(c, 0, NFC - 1) * 128, 128), 128)

        def up(c):
            return _bf(_gelu(_rb(_dot_nt(ln2_v[...], w3_v[frows(c), :]))))

        def fgroup(k, cc):
            c = 3 * k
            g0 = up(c)
            d = _dot(ga_v[...], w4_v[frows(c - 1), :])
            g1 = up(c + 1)
            d = d + _dot(g0, w4_v[frows(c), :])
            ga_v[...] = up(c + 2)
            d = d + _dot(g1, w4_v[frows(c + 1), :])
            h2_v[...] += d
            ztile(4 * b + k)
            return cc

        lax.fori_loop(0, 4, fgroup, 0)
        bb = _rb(x1_v[...] + _rb(h2_v[...]))
        gate_v[pl.ds(r0, RB), :] = _bf(bb * jax.nn.sigmoid(bb))
        return carry

    with jax.named_scope('p_phase2'):
        lax.fori_loop(0, L // RB, phase2, 0)

    dsk = dsk_ref[...].astype(jnp.float32).reshape(1, D)

    def out_copy(b):
        r0 = pl.multiple_of(b * RB, RB)
        return pltpu.make_async_copy(out_v.at[pl.ds(r0, RB), :],
                                     out_hbm.at[pl.ds(r0, RB), :], sem_out.at[b])

    def phase3(b, carry):
        r0 = pl.multiple_of(b * RB, RB)
        ys = [_dot(finv_ref[...], z_v[b * (RB // J) + k]) for k in range(RB // J)]
        y = _rb(jnp.concatenate(ys, axis=0))
        xn = xn_v[pl.ds(r0, RB), :].astype(jnp.float32)
        s = _rb(y + _rb(xn * dsk))
        x = x_v[pl.ds(r0, RB), :].astype(jnp.float32)
        gate = gate_v[pl.ds(r0, RB), :].astype(jnp.float32)
        out_v[pl.ds(r0, RB), :] = _bf(x + _rb(s * gate))
        out_copy(b).start()
        return carry

    with jax.named_scope('p_phase3'):
        lax.fori_loop(0, L // RB, phase3, 0)
    for b in range(L // RB):
        out_copy(b).wait()


@jax.jit
def pallas_recurrent_scan__ssm_conv_s4__mixer_s_mlp__prompt_kernel(
    A_u: jax.Array,
    A_A_re: jax.Array,
    A_A_im: jax.Array,
    A_B_re: jax.Array,
    A_B_im: jax.Array,
    A_C_re: jax.Array,
    A_C_im: jax.Array,
    A_log_dt: jax.Array,
    A_Dskip: jax.Array,
    B_x: jax.Array,
    B_w1: jax.Array,
    B_w2: jax.Array,
    B_w3: jax.Array,
    B_w4: jax.Array,
):
    bf16 = jnp.bfloat16
    f32 = jnp.float32
    x = A_u.reshape(L, D)
    vm = pl.BlockSpec(memory_space=pltpu.VMEM)
    hbm = pl.BlockSpec(memory_space=pltpu.HBM)
    out = pl.pallas_call(
        _kernel,
        out_shape=jax.ShapeDtypeStruct((L, D), bf16),
        in_specs=[vm] * 11 + [hbm] * 6,
        out_specs=hbm,
        scratch_shapes=[
            pltpu.VMEM((L, D), bf16),
            pltpu.VMEM((D, D), bf16),
            pltpu.VMEM((D, D), bf16),
            pltpu.VMEM((FP, D), bf16),
            pltpu.VMEM((FP, D), bf16),
            pltpu.VMEM((2 * J, GW), bf16),
            pltpu.VMEM((L, D), bf16),
            pltpu.VMEM((L, D), bf16),
            pltpu.VMEM((L + 16, D), f32),
            pltpu.VMEM((NB, 2 * J, D), f32),
            pltpu.VMEM((NB, 2 * J, D), f32),
            pltpu.VMEM((NB, 2 * J, D), bf16),
            pltpu.VMEM((CH // 8, 128, N), f32),
            pltpu.VMEM((CH // 8, 128, N), f32),
            pltpu.VMEM((CH // 8, 8 * NHI, N), f32),
            pltpu.VMEM((CH // 8, 8 * NHI, N), f32),
            pltpu.VMEM((NHI, D, 128), f32),
            pltpu.VMEM((NQ, D), f32),
            pltpu.VMEM((D, N), f32),
            pltpu.VMEM((RB, D), f32),
            pltpu.VMEM((RB, D), bf16),
            pltpu.VMEM((RB, D), f32),
            pltpu.VMEM((RB, 128), bf16),
            pltpu.VMEM((L, D), bf16),
            pltpu.SemaphoreType.DMA((6,)),
            pltpu.SemaphoreType.DMA((L // RB,)),
        ],
        compiler_params=pltpu.CompilerParams(vmem_limit_bytes=100 * 1024 * 1024),
    )(A_A_re, A_A_im, A_B_re, A_B_im, A_C_re, A_C_im,
      A_log_dt, A_Dskip,
      jnp.asarray(_F_FWD, bf16), jnp.asarray(_F_INV, bf16), jnp.asarray(_SEL, bf16),
      *[pltpu.with_memory_space_constraint(t, pltpu.HBM)
        for t in (x, B_w1, B_w2, B_w3.T, B_w4, jnp.asarray(_G_ALL, bf16))])
    return out.reshape(1, L, D)
```

```python
import functools
import numpy as np
import jax
import jax.numpy as jnp
from jax import lax
import jax.experimental.pallas as pl
import jax.experimental.pallas.tpu as pltpu

L = 2048
D = 512
N = 128
FF = 1376
FP = 1408
J = 128
NB = L // J
NQ = 656
_STEP = (1, 1, 2, 2, 4, 4, 4, 4, 8, 8, 8, 8, 8, 8, 8, 8)
HI = tuple(128 * k + b for k in range(16) for b in range(0, 8, _STEP[k])) + (2048,)
NHI = len(HI)
CH = 32
RB = 256
WIN = ((0, 128), (0, 256), (128, 256), (256, 256), (320, 128), (384, 128),
       (384, 128), (448, 128), (448, 128), (512, 128), (512, 128), (512, 128),
       (512, 128), (512, 128), (512, 128), (528, 128))
GW = sum(w[1] for w in WIN)


def _q_of_m(m):
    hi = (m // 128) * 128 + (m % 8)
    return 16 * HI.index(hi) + (m % 128) // 8


def _build_tables():
    pos = np.arange(L, dtype=np.int64)
    rr = np.zeros(L, np.int64)
    for l in range(L):
        if l < 256:
            rr[l] = l
        else:
            step = 1 << (int(l).bit_length() - 8)
            lo = (l // step) * step
            rem = l - lo
            if rem * 2 < step or (rem * 2 == step and (lo // step) % 2 == 0):
                rr[l] = lo
            else:
                rr[l] = lo + step
    w = np.pi * (2 * np.arange(J) + 1) / (2 * J)
    n = np.arange(J)
    f_fwd = np.concatenate([np.cos(np.outer(w, n)), -np.sin(np.outer(w, n))], 0)
    f_inv = np.concatenate([np.cos(np.outer(n, w)), -np.sin(np.outer(n, w))], 1) / J
    g_all = np.zeros((2 * J, GW))
    off = 0
    for dl in range(NB):
        s0, ln = WIN[dl]
        for p in range(-J, J):
            l = dl * J + p
            if 0 <= l < L:
                q = _q_of_m(int(rr[l])) - s0
                assert 0 <= q < ln
                g_all[:J, off + q] += np.cos(w * p)
                g_all[J:, off + q] += -np.sin(w * p)
        off += ln
    sel = np.zeros((16, 128))
    for dd in range(8):
        sel[np.arange(16), np.arange(16) * 8 + dd] = 1.0
    del pos
    return (f_fwd.astype(np.float32), f_inv.astype(np.float32),
            g_all.astype(np.float32), sel.astype(np.float32))


_F_FWD, _F_INV, _G_ALL, _SEL = _build_tables()


def _bf(x):
    return x.astype(jnp.bfloat16)


def _rb(x):
    return x.astype(jnp.bfloat16).astype(jnp.float32)


def _cmul(a, b):
    return (a[0] * b[0] - a[1] * b[1], a[0] * b[1] + a[1] * b[0])


def _gelu(x):
    c = 0.7978845608028654
    return 0.5 * x * (1.0 + jnp.tanh(c * (x + 0.044715 * (x * x * x))))


def _layernorm(x):
    m = jnp.mean(x, axis=-1, keepdims=True)
    xc = x - m
    v = jnp.mean(xc * xc, axis=-1, keepdims=True)
    den = _rb(jnp.sqrt(_rb(_rb(v) + 1e-5)))
    return _rb(_rb(x - _rb(m)) / den)


def _dot(a, b):
    return jnp.dot(a, b, preferred_element_type=jnp.float32)


def _dot_nt(a, b):
    return lax.dot_general(a, b, (((1,), (1,)), ((), ())),
                           preferred_element_type=jnp.float32)


def _kernel(are_ref, aim_ref, bre_ref, bim_ref, cre_ref, cim_ref, ldt_ref, dsk_ref,
            ffwd_ref, finv_ref, sel_ref,
            x_hbm, w1_hbm, w2_hbm, w3_hbm, w4_hbm, g_hbm,
            out_hbm,
            x_v, w1_v, w2_v, w3_v, w4_v, g_v, out_v,
            xn_v, h_v, u_v, kt_v, z_v,
            yr_v, yi_v, xr_v, xi_v, o_v, kd_v, dt_v, x1_v, ln2_v, ga_v, gate_v,
            sem_in, sem_out):
    copies = [pltpu.make_async_copy(s, d, sem_in.at[k]) for k, (s, d) in enumerate(
        [(x_hbm, x_v), (w1_hbm, w1_v), (g_hbm, g_v), (w2_hbm, w2_v),
         (w3_hbm, w3_v.at[0:FF, :]), (w4_hbm, w4_v.at[0:FF, :])])]
    for c in copies:
        c.start()

    dt_row = _rb(jnp.exp(ldt_ref[...].astype(jnp.float32))).reshape(1, D)
    dt_v[...] = jnp.transpose(jnp.broadcast_to(dt_row, (N, D)))

    def kgen(c, carry):
        r0 = pl.multiple_of(c * CH, CH)
        rows = pl.ds(r0, CH)
        f32 = jnp.float32
        dt = dt_v[rows, :]
        lr = dt * are_ref[rows, :].astype(f32)
        li = dt * aim_ref[rows, :].astype(f32)
        dbr = dt * bre_ref[rows, :].astype(f32)
        dbi = dt * bim_ref[rows, :].astype(f32)
        w = _cmul((cre_ref[rows, :].astype(f32), cim_ref[rows, :].astype(f32)), (dbr, dbi))

        def csq(a):
            ab = a[0] * a[1]
            return (a[0] * a[0] - a[1] * a[1], ab + ab)

        e1 = jnp.exp(lr)
        z1 = (e1 * jnp.cos(li), e1 * jnp.sin(li))
        z8 = csq(csq(csq(z1)))
        z128 = csq(csq(csq(csq(z8))))
        z1024 = csq(csq(csq(z128)))

        def put_y(j, v):
            for g in range(CH // 8):
                yr_v[g, 8 * j:8 * j + 8, :] = v[0][8 * g:8 * g + 8, :]
                yi_v[g, 8 * j:8 * j + 8, :] = v[1][8 * g:8 * g + 8, :]

        def put_x(i, v):
            nvi = -v[1]
            for g in range(CH // 8):
                xr_v[g, 8 * i:8 * i + 8, :] = v[0][8 * g:8 * g + 8, :]
                xi_v[g, 8 * i:8 * i + 8, :] = nvi[8 * g:8 * g + 8, :]

        put_y(0, (jnp.ones_like(lr), jnp.zeros_like(lr)))
        y = z8
        put_y(1, y)
        for j in range(2, 16):
            y = _cmul(y, z8)
            put_y(j, y)
        v = w
        for b in range(8):
            if b:
                v = _cmul(v, z1)
            t = v
            for k in range(8):
                if (128 * k + b) in HI:
                    if k:
                        t = _cmul(t, z128)
                    put_x(HI.index(128 * k + b), t)
        t = _cmul(w, z1024)
        for k in range(8, 17):
            if k > 8:
                t = _cmul(t, z128)
            put_x(HI.index(128 * k), t)
        for g in range(CH // 8):
            o = (_dot_nt(_bf(xr_v[g]), _bf(yr_v[g])) + _dot_nt(_bf(xi_v[g]), _bf(yi_v[g])))
            for i in range(NHI):
                o_v[i, pl.ds(pl.multiple_of(r0 + 8 * g, 8), 8), :] = o[8 * i:8 * i + 8, :]
        return carry

    with jax.named_scope('p_kgen'):
        lax.fori_loop(0, D // CH, kgen, 0)

    rid = lax.broadcasted_iota(jnp.int32, (D, 128), 0)
    lid = lax.broadcasted_iota(jnp.int32, (D, 128), 1)
    keep = (rid % 8) == (lid % 8)
    keep_last = keep & (lid < 8)
    sel = sel_ref[...]
    with jax.named_scope('p_sel'):
        for i in range(NHI):
            oi = jnp.where(keep_last if HI[i] == 2048 else keep, o_v[i], 0.0)
            kd_v[16 * i:16 * i + 16, :] = _dot_nt(sel, _bf(oi))

    copies[2].wait()
    off = 0
    for dl in range(NB):
        s0, ln = WIN[dl]
        kt_v[dl] = _dot(g_v[:, off:off + ln], _bf(kd_v[s0:s0 + ln, :]))
        off += ln

    copies[0].wait()
    copies[1].wait()
    h_v[0:8, :] = jnp.zeros((8, D), jnp.float32)
    h_v[8 + L:16 + L, :] = jnp.zeros((8, D), jnp.float32)

    def phase1(b, carry):
        r0 = pl.multiple_of(b * RB, RB)
        x = x_v[pl.ds(r0, RB), :].astype(jnp.float32)
        xn = _bf(_layernorm(x))
        xn_v[pl.ds(r0, RB), :] = xn
        h = _rb(_gelu(_rb(_dot(xn, w1_v[...]))))
        h_v[pl.ds(pl.multiple_of(r0 + 8, 8), RB), :] = h
        for k in range(RB // J):
            u_v[b * (RB // J) + k] = _dot(ffwd_ref[...], xn[k * J:(k + 1) * J, :])
        return carry

    with jax.named_scope('p_phase1'):
        lax.fori_loop(0, L // RB, phase1, 0)

    def ztile(t):
        f0 = pl.multiple_of((t // 4) * 16, 16)
        re = pl.ds(f0, 16)
        im = pl.ds(pl.multiple_of(f0 + J, 16), 16)
        cs = pl.ds(pl.multiple_of((t % 4) * 128, 128), 128)
        for i in range(NB):
            zr = zi = None
            for dl in range(i + 1):
                kr = kt_v[dl, re, cs]
                ki = kt_v[dl, im, cs]
                ur = u_v[i - dl, re, cs]
                ui = u_v[i - dl, im, cs]
                pr = kr * ur - ki * ui
                pi = kr * ui + ki * ur
                zr = pr if zr is None else zr + pr
                zi = pi if zi is None else zi + pi
            z_v[i, re, cs] = _bf(zr)
            z_v[i, im, cs] = _bf(zi)

    copies[3].wait()
    copies[4].wait()
    copies[5].wait()
    w3_v[FF:FP, :] = jnp.zeros((FP - FF, D), jnp.bfloat16)
    w4_v[FF:FP, :] = jnp.zeros((FP - FF, D), jnp.bfloat16)
    NFC = FP // 128

    def pre(b):
        r0 = pl.multiple_of(b * RB, RB)
        ext = RB + 16
        parts = []
        for gi, sh in enumerate((1, -1, 2, -2)):
            hv = h_v[pl.ds(r0, ext), gi * 128:(gi + 1) * 128]
            hv = pltpu.roll(hv, sh % ext, 0)
            parts.append(_bf(hv[8:8 + RB, :]))
        hs = _rb(_dot(jnp.concatenate(parts, axis=1), w2_v[...]))
        xn = xn_v[pl.ds(r0, RB), :].astype(jnp.float32)
        x1 = _rb(xn + hs)
        x1_v[pl.ds(r0, RB), :] = _bf(x1)
        ln2_v[...] = _bf(_layernorm(x1))

    def up(slot, c):
        c0 = pl.multiple_of(jnp.minimum(c, NFC - 1) * 128, 128)
        ga_v[slot, :, pl.ds(pl.multiple_of(c * 128, 128), 128)] = _bf(
            _gelu(_rb(_dot_nt(ln2_v[...], w3_v[pl.ds(c0, 128), :]))))

    def down(b, n):
        r0 = pl.multiple_of(b * RB, RB)
        cs = pl.ds(pl.multiple_of(n * 128, 128), 128)
        h2 = _rb(_dot(ga_v[b % 2, :, 0:FP], w4_v[:, cs]))
        bb = _rb(x1_v[pl.ds(r0, RB), cs].astype(jnp.float32) + h2)
        gate_v[pl.ds(r0, RB), cs] = _bf(bb * jax.nn.sigmoid(bb))

    def phase2(b, carry, with_up):
        if with_up:
            pre(b + 1)

        def inner(k, cc):
            down(b, k)
            if with_up:
                for q in range(3):
                    up((b + 1) % 2, 3 * k + q)
            ztile(4 * b + k)
            return cc

        lax.fori_loop(0, 4, inner, 0)
        return carry

    with jax.named_scope('p_phase2'):
        pre(0)

        def up0(c, cc):
            up(0, c)
            return cc

        lax.fori_loop(0, NFC, up0, 0)
        lax.fori_loop(0, L // RB - 1, functools.partial(phase2, with_up=True), 0)
        phase2(L // RB - 1, 0, with_up=False)

    dsk = dsk_ref[...].astype(jnp.float32).reshape(1, D)

    def out_copy(b):
        r0 = pl.multiple_of(b * RB, RB)
        return pltpu.make_async_copy(out_v.at[pl.ds(r0, RB), :],
                                     out_hbm.at[pl.ds(r0, RB), :], sem_out.at[b])

    def phase3(b, carry):
        r0 = pl.multiple_of(b * RB, RB)
        ys = [_dot(finv_ref[...], z_v[b * (RB // J) + k]) for k in range(RB // J)]
        y = _rb(jnp.concatenate(ys, axis=0))
        xn = xn_v[pl.ds(r0, RB), :].astype(jnp.float32)
        s = _rb(y + _rb(xn * dsk))
        x = x_v[pl.ds(r0, RB), :].astype(jnp.float32)
        gate = gate_v[pl.ds(r0, RB), :].astype(jnp.float32)
        out_v[pl.ds(r0, RB), :] = _bf(x + _rb(s * gate))
        out_copy(b).start()
        return carry

    with jax.named_scope('p_phase3'):
        lax.fori_loop(0, L // RB, phase3, 0)
    for b in range(L // RB):
        out_copy(b).wait()


@jax.jit
def pallas_recurrent_scan__ssm_conv_s4__mixer_s_mlp__prompt_kernel(
    A_u: jax.Array,
    A_A_re: jax.Array,
    A_A_im: jax.Array,
    A_B_re: jax.Array,
    A_B_im: jax.Array,
    A_C_re: jax.Array,
    A_C_im: jax.Array,
    A_log_dt: jax.Array,
    A_Dskip: jax.Array,
    B_x: jax.Array,
    B_w1: jax.Array,
    B_w2: jax.Array,
    B_w3: jax.Array,
    B_w4: jax.Array,
):
    bf16 = jnp.bfloat16
    f32 = jnp.float32
    x = A_u.reshape(L, D)
    vm = pl.BlockSpec(memory_space=pltpu.VMEM)
    hbm = pl.BlockSpec(memory_space=pltpu.HBM)
    out = pl.pallas_call(
        _kernel,
        out_shape=jax.ShapeDtypeStruct((L, D), bf16),
        in_specs=[vm] * 11 + [hbm] * 6,
        out_specs=hbm,
        scratch_shapes=[
            pltpu.VMEM((L, D), bf16),
            pltpu.VMEM((D, D), bf16),
            pltpu.VMEM((D, D), bf16),
            pltpu.VMEM((FP, D), bf16),
            pltpu.VMEM((FP, D), bf16),
            pltpu.VMEM((2 * J, GW), bf16),
            pltpu.VMEM((L, D), bf16),
            pltpu.VMEM((L, D), bf16),
            pltpu.VMEM((L + 16, D), f32),
            pltpu.VMEM((NB, 2 * J, D), f32),
            pltpu.VMEM((NB, 2 * J, D), f32),
            pltpu.VMEM((NB, 2 * J, D), bf16),
            pltpu.VMEM((CH // 8, 128, N), f32),
            pltpu.VMEM((CH // 8, 128, N), f32),
            pltpu.VMEM((CH // 8, 8 * NHI, N), f32),
            pltpu.VMEM((CH // 8, 8 * NHI, N), f32),
            pltpu.VMEM((NHI, D, 128), f32),
            pltpu.VMEM((NQ, D), f32),
            pltpu.VMEM((D, N), f32),
            pltpu.VMEM((L, D), bf16),
            pltpu.VMEM((RB, D), bf16),
            pltpu.VMEM((2, RB, FP + 128), bf16),
            pltpu.VMEM((L, D), bf16),
            pltpu.SemaphoreType.DMA((6,)),
            pltpu.SemaphoreType.DMA((L // RB,)),
        ],
        compiler_params=pltpu.CompilerParams(vmem_limit_bytes=100 * 1024 * 1024),
    )(A_A_re, A_A_im, A_B_re, A_B_im, A_C_re, A_C_im,
      A_log_dt, A_Dskip,
      jnp.asarray(_F_FWD, bf16), jnp.asarray(_F_INV, bf16), jnp.asarray(_SEL, bf16),
      *[pltpu.with_memory_space_constraint(t, pltpu.HBM)
        for t in (x, B_w1, B_w2, B_w3.T, B_w4, jnp.asarray(_G_ALL, bf16))])
    return out.reshape(1, L, D)
```

```python
import functools
import numpy as np
import jax
import jax.numpy as jnp
from jax import lax
import jax.experimental.pallas as pl
import jax.experimental.pallas.tpu as pltpu

L = 2048
D = 512
N = 128
FF = 1376
FP = 1408
J = 128
NB = L // J
NQ = 656
_STEP = (1, 1, 2, 2, 4, 4, 4, 4, 8, 8, 8, 8, 8, 8, 8, 8)
HI = tuple(128 * k + b for k in range(16) for b in range(0, 8, _STEP[k])) + (2048,)
NHI = len(HI)
CH = 32
RB = 256
WIN = ((0, 128), (0, 256), (128, 256), (256, 256), (320, 128), (384, 128),
       (384, 128), (448, 128), (448, 128), (512, 128), (512, 128), (512, 128),
       (512, 128), (512, 128), (512, 128), (528, 128))
GW = sum(w[1] for w in WIN)


def _q_of_m(m):
    hi = (m // 128) * 128 + (m % 8)
    return 16 * HI.index(hi) + (m % 128) // 8


def _build_tables():
    pos = np.arange(L, dtype=np.int64)
    rr = np.zeros(L, np.int64)
    for l in range(L):
        if l < 256:
            rr[l] = l
        else:
            step = 1 << (int(l).bit_length() - 8)
            lo = (l // step) * step
            rem = l - lo
            if rem * 2 < step or (rem * 2 == step and (lo // step) % 2 == 0):
                rr[l] = lo
            else:
                rr[l] = lo + step
    w = np.pi * (2 * np.arange(J) + 1) / (2 * J)
    n = np.arange(J)
    f_fwd = np.concatenate([np.cos(np.outer(w, n)), -np.sin(np.outer(w, n))], 0)
    f_inv = np.concatenate([np.cos(np.outer(n, w)), -np.sin(np.outer(n, w))], 1) / J
    g_all = np.zeros((2 * J, GW))
    off = 0
    for dl in range(NB):
        s0, ln = WIN[dl]
        for p in range(-J, J):
            l = dl * J + p
            if 0 <= l < L:
                q = _q_of_m(int(rr[l])) - s0
                assert 0 <= q < ln
                g_all[:J, off + q] += np.cos(w * p)
                g_all[J:, off + q] += -np.sin(w * p)
        off += ln
    sel = np.zeros((16, 128))
    for dd in range(8):
        sel[np.arange(16), np.arange(16) * 8 + dd] = 1.0
    del pos
    return (f_fwd.astype(np.float32), f_inv.astype(np.float32),
            g_all.astype(np.float32), sel.astype(np.float32))


_F_FWD, _F_INV, _G_ALL, _SEL = _build_tables()


def _bf(x):
    return x.astype(jnp.bfloat16)


def _rb(x):
    return x.astype(jnp.bfloat16).astype(jnp.float32)


def _cmul(a, b):
    return (a[0] * b[0] - a[1] * b[1], a[0] * b[1] + a[1] * b[0])


def _gelu(x):
    c = 0.7978845608028654
    return 0.5 * x * (1.0 + jnp.tanh(c * (x + 0.044715 * (x * x * x))))


def _layernorm(x):
    m = jnp.mean(x, axis=-1, keepdims=True)
    xc = x - m
    v = jnp.mean(xc * xc, axis=-1, keepdims=True)
    den = _rb(jnp.sqrt(_rb(_rb(v) + 1e-5)))
    return _rb(_rb(x - _rb(m)) / den)


def _dot(a, b):
    return jnp.dot(a, b, preferred_element_type=jnp.float32)


def _dot_nt(a, b):
    return lax.dot_general(a, b, (((1,), (1,)), ((), ())),
                           preferred_element_type=jnp.float32)


def _kernel(are_ref, aim_ref, bre_ref, bim_ref, cre_ref, cim_ref, ldt_ref, dsk_ref,
            ffwd_ref, finv_ref, sel_ref,
            x_hbm, w1_hbm, w2_hbm, w3_hbm, w4_hbm, g_hbm,
            out_hbm,
            x_v, w1_v, w2_v, w3_v, w4_v, g_v, out_v,
            xn_v, h_v, u_v, kt_v, z_v,
            yr_v, yi_v, xr_v, xi_v, o_v, kd_v, dt_v, x1_v, ln2_v, ga_v, gate_v,
            sem_in, sem_out):
    copies = [pltpu.make_async_copy(s, d, sem_in.at[k]) for k, (s, d) in enumerate(
        [(x_hbm, x_v), (w1_hbm, w1_v), (g_hbm, g_v), (w2_hbm, w2_v),
         (w3_hbm, w3_v.at[0:FF, :]), (w4_hbm, w4_v.at[0:FF, :])])]
    for c in copies:
        c.start()

    dt_row = _rb(jnp.exp(ldt_ref[...].astype(jnp.float32))).reshape(1, D)
    dt_v[...] = jnp.transpose(jnp.broadcast_to(dt_row, (N, D)))

    def kgen(c, carry):
        r0 = pl.multiple_of(c * CH, CH)
        rows = pl.ds(r0, CH)
        f32 = jnp.float32
        dt = dt_v[rows, :]
        lr = dt * are_ref[rows, :].astype(f32)
        li = dt * aim_ref[rows, :].astype(f32)
        dbr = dt * bre_ref[rows, :].astype(f32)
        dbi = dt * bim_ref[rows, :].astype(f32)
        w = _cmul((cre_ref[rows, :].astype(f32), cim_ref[rows, :].astype(f32)), (dbr, dbi))

        def csq(a):
            ab = a[0] * a[1]
            return (a[0] * a[0] - a[1] * a[1], ab + ab)

        e1 = jnp.exp(lr)
        z1 = (e1 * jnp.cos(li), e1 * jnp.sin(li))
        z8 = csq(csq(csq(z1)))
        z128 = csq(csq(csq(csq(z8))))
        z1024 = csq(csq(csq(z128)))

        def put_y(j, v):
            for g in range(CH // 8):
                yr_v[g, 8 * j:8 * j + 8, :] = v[0][8 * g:8 * g + 8, :]
                yi_v[g, 8 * j:8 * j + 8, :] = v[1][8 * g:8 * g + 8, :]

        def put_x(i, v):
            nvi = -v[1]
            for g in range(CH // 8):
                xr_v[g, 8 * i:8 * i + 8, :] = v[0][8 * g:8 * g + 8, :]
                xi_v[g, 8 * i:8 * i + 8, :] = nvi[8 * g:8 * g + 8, :]

        put_y(0, (jnp.ones_like(lr), jnp.zeros_like(lr)))
        y = z8
        put_y(1, y)
        for j in range(2, 16):
            y = _cmul(y, z8)
            put_y(j, y)
        v = w
        for b in range(8):
            if b:
                v = _cmul(v, z1)
            t = v
            for k in range(8):
                if (128 * k + b) in HI:
                    if k:
                        t = _cmul(t, z128)
                    put_x(HI.index(128 * k + b), t)
        t = _cmul(w, z1024)
        for k in range(8, 17):
            if k > 8:
                t = _cmul(t, z128)
            put_x(HI.index(128 * k), t)
        for g in range(CH // 8):
            o = (_dot_nt(_bf(xr_v[g]), _bf(yr_v[g])) + _dot_nt(_bf(xi_v[g]), _bf(yi_v[g])))
            for i in range(NHI):
                o_v[i, pl.ds(pl.multiple_of(r0 + 8 * g, 8), 8), :] = o[8 * i:8 * i + 8, :]
        return carry

    with jax.named_scope('p_kgen'):
        lax.fori_loop(0, D // CH, kgen, 0)

    rid = lax.broadcasted_iota(jnp.int32, (D, 128), 0)
    lid = lax.broadcasted_iota(jnp.int32, (D, 128), 1)
    keep = (rid % 8) == (lid % 8)
    keep_last = keep & (lid < 8)
    sel = sel_ref[...]
    with jax.named_scope('p_sel'):
        for i in range(NHI):
            oi = jnp.where(keep_last if HI[i] == 2048 else keep, o_v[i], 0.0)
            kd_v[16 * i:16 * i + 16, :] = _dot_nt(sel, _bf(oi))

    copies[2].wait()
    off = 0
    for dl in range(NB):
        s0, ln = WIN[dl]
        kt_v[dl] = _dot(g_v[:, off:off + ln], _bf(kd_v[s0:s0 + ln, :]))
        off += ln

    copies[0].wait()
    copies[1].wait()
    h_v[0:8, :] = jnp.zeros((8, D), jnp.float32)
    h_v[8 + L:16 + L, :] = jnp.zeros((8, D), jnp.float32)

    def phase1(b, carry):
        r0 = pl.multiple_of(b * RB, RB)
        x = x_v[pl.ds(r0, RB), :].astype(jnp.float32)
        xn = _bf(_layernorm(x))
        xn_v[pl.ds(r0, RB), :] = xn
        h = _rb(_gelu(_rb(_dot(xn, w1_v[...]))))
        h_v[pl.ds(pl.multiple_of(r0 + 8, 8), RB), :] = h
        for k in range(RB // J):
            u_v[b * (RB // J) + k] = _dot(ffwd_ref[...], xn[k * J:(k + 1) * J, :])
        return carry

    with jax.named_scope('p_phase1'):
        lax.fori_loop(0, L // RB, phase1, 0)

    def ztile(t, i0=0, i1=NB):
        f0 = pl.multiple_of((t // 4) * 16, 16)
        re = pl.ds(f0, 16)
        im = pl.ds(pl.multiple_of(f0 + J, 16), 16)
        cs = pl.ds(pl.multiple_of((t % 4) * 128, 128), 128)
        for i in range(i0, i1):
            zr = zi = None
            for dl in range(i + 1):
                kr = kt_v[dl, re, cs]
                ki = kt_v[dl, im, cs]
                ur = u_v[i - dl, re, cs]
                ui = u_v[i - dl, im, cs]
                pr = kr * ur - ki * ui
                pi = kr * ui + ki * ur
                zr = pr if zr is None else zr + pr
                zi = pi if zi is None else zi + pi
            z_v[i, re, cs] = _bf(zr)
            z_v[i, im, cs] = _bf(zi)

    copies[3].wait()
    copies[4].wait()
    copies[5].wait()
    w3_v[FF:FP, :] = jnp.zeros((FP - FF, D), jnp.bfloat16)
    w4_v[FF:FP, :] = jnp.zeros((FP - FF, D), jnp.bfloat16)
    NFC = FP // 128

    def pre(b):
        r0 = pl.multiple_of(b * RB, RB)
        ext = RB + 16
        parts = []
        for gi, sh in enumerate((1, -1, 2, -2)):
            hv = h_v[pl.ds(r0, ext), gi * 128:(gi + 1) * 128]
            hv = pltpu.roll(hv, sh % ext, 0)
            parts.append(_bf(hv[8:8 + RB, :]))
        hs = _rb(_dot(jnp.concatenate(parts, axis=1), w2_v[...]))
        xn = xn_v[pl.ds(r0, RB), :].astype(jnp.float32)
        x1 = _rb(xn + hs)
        x1_v[pl.ds(r0, RB), :] = _bf(x1)
        ln2_v[...] = _bf(_layernorm(x1))

    def up(slot, c):
        c0 = pl.multiple_of(jnp.minimum(c, NFC - 1) * 128, 128)
        ga_v[slot, :, pl.ds(pl.multiple_of(c * 128, 128), 128)] = _bf(
            _gelu(_rb(_dot_nt(ln2_v[...], w3_v[pl.ds(c0, 128), :]))))

    def down(b, n):
        r0 = pl.multiple_of(b * RB, RB)
        cs = pl.ds(pl.multiple_of(n * 128, 128), 128)
        h2 = _rb(_dot(ga_v[b % 2, :, 0:FP], w4_v[:, cs]))
        bb = _rb(x1_v[pl.ds(r0, RB), cs].astype(jnp.float32) + h2)
        gate_v[pl.ds(r0, RB), cs] = _bf(bb * jax.nn.sigmoid(bb))

    def phase2(b, carry, with_up):
        if with_up:
            pre(b + 1)

        def inner(k, cc):
            @pl.when(k >= 0)
            def _():
                down(b, k)
                ztile(4 * b + k, 11, NB)

            @pl.when(k >= 0)
            def _():
                if with_up:
                    for q in range(3):
                        up((b + 1) % 2, 3 * k + q)
                ztile(4 * b + k, 0, 11)

            return cc

        lax.fori_loop(0, 4, inner, 0)
        return carry

    with jax.named_scope('p_phase2'):
        pre(0)

        def up0(c, cc):
            up(0, c)
            return cc

        lax.fori_loop(0, NFC, up0, 0)
        lax.fori_loop(0, L // RB - 1, functools.partial(phase2, with_up=True), 0)
        phase2(L // RB - 1, 0, with_up=False)

    dsk = dsk_ref[...].astype(jnp.float32).reshape(1, D)

    def out_copy(b):
        r0 = pl.multiple_of(b * RB, RB)
        return pltpu.make_async_copy(out_v.at[pl.ds(r0, RB), :],
                                     out_hbm.at[pl.ds(r0, RB), :], sem_out.at[b])

    def phase3(b, carry):
        r0 = pl.multiple_of(b * RB, RB)
        ys = [_dot(finv_ref[...], z_v[b * (RB // J) + k]) for k in range(RB // J)]
        y = _rb(jnp.concatenate(ys, axis=0))
        xn = xn_v[pl.ds(r0, RB), :].astype(jnp.float32)
        s = _rb(y + _rb(xn * dsk))
        x = x_v[pl.ds(r0, RB), :].astype(jnp.float32)
        gate = gate_v[pl.ds(r0, RB), :].astype(jnp.float32)
        out_v[pl.ds(r0, RB), :] = _bf(x + _rb(s * gate))
        out_copy(b).start()
        return carry

    with jax.named_scope('p_phase3'):
        lax.fori_loop(0, L // RB, phase3, 0)
    for b in range(L // RB):
        out_copy(b).wait()


@jax.jit
def pallas_recurrent_scan__ssm_conv_s4__mixer_s_mlp__prompt_kernel(
    A_u: jax.Array,
    A_A_re: jax.Array,
    A_A_im: jax.Array,
    A_B_re: jax.Array,
    A_B_im: jax.Array,
    A_C_re: jax.Array,
    A_C_im: jax.Array,
    A_log_dt: jax.Array,
    A_Dskip: jax.Array,
    B_x: jax.Array,
    B_w1: jax.Array,
    B_w2: jax.Array,
    B_w3: jax.Array,
    B_w4: jax.Array,
):
    bf16 = jnp.bfloat16
    f32 = jnp.float32
    x = A_u.reshape(L, D)
    vm = pl.BlockSpec(memory_space=pltpu.VMEM)
    hbm = pl.BlockSpec(memory_space=pltpu.HBM)
    out = pl.pallas_call(
        _kernel,
        out_shape=jax.ShapeDtypeStruct((L, D), bf16),
        in_specs=[vm] * 11 + [hbm] * 6,
        out_specs=hbm,
        scratch_shapes=[
            pltpu.VMEM((L, D), bf16),
            pltpu.VMEM((D, D), bf16),
            pltpu.VMEM((D, D), bf16),
            pltpu.VMEM((FP, D), bf16),
            pltpu.VMEM((FP, D), bf16),
            pltpu.VMEM((2 * J, GW), bf16),
            pltpu.VMEM((L, D), bf16),
            pltpu.VMEM((L, D), bf16),
            pltpu.VMEM((L + 16, D), f32),
            pltpu.VMEM((NB, 2 * J, D), f32),
            pltpu.VMEM((NB, 2 * J, D), f32),
            pltpu.VMEM((NB, 2 * J, D), bf16),
            pltpu.VMEM((CH // 8, 128, N), f32),
            pltpu.VMEM((CH // 8, 128, N), f32),
            pltpu.VMEM((CH // 8, 8 * NHI, N), f32),
            pltpu.VMEM((CH // 8, 8 * NHI, N), f32),
            pltpu.VMEM((NHI, D, 128), f32),
            pltpu.VMEM((NQ, D), f32),
            pltpu.VMEM((D, N), f32),
            pltpu.VMEM((L, D), bf16),
            pltpu.VMEM((RB, D), bf16),
            pltpu.VMEM((2, RB, FP + 128), bf16),
            pltpu.VMEM((L, D), bf16),
            pltpu.SemaphoreType.DMA((6,)),
            pltpu.SemaphoreType.DMA((L // RB,)),
        ],
        compiler_params=pltpu.CompilerParams(vmem_limit_bytes=100 * 1024 * 1024),
    )(A_A_re, A_A_im, A_B_re, A_B_im, A_C_re, A_C_im,
      A_log_dt, A_Dskip,
      jnp.asarray(_F_FWD, bf16), jnp.asarray(_F_INV, bf16), jnp.asarray(_SEL, bf16),
      *[pltpu.with_memory_space_constraint(t, pltpu.HBM)
        for t in (x, B_w1, B_w2, B_w3.T, B_w4, jnp.asarray(_G_ALL, bf16))])
    return out.reshape(1, L, D)
```

```python
import functools
import numpy as np
import jax
import jax.numpy as jnp
from jax import lax
import jax.experimental.pallas as pl
import jax.experimental.pallas.tpu as pltpu

L = 2048
D = 512
N = 128
FF = 1376
FP = 1408
J = 128
NB = L // J
NQ = 656
_STEP = (1, 1, 2, 2, 4, 4, 4, 4, 8, 8, 8, 8, 8, 8, 8, 8)
HI = tuple(128 * k + b for k in range(16) for b in range(0, 8, _STEP[k])) + (2048,)
NHI = len(HI)
CH = 32
RB = 256
WIN = ((0, 128), (0, 256), (128, 256), (256, 256), (320, 128), (384, 128),
       (384, 128), (448, 128), (448, 128), (512, 128), (512, 128), (512, 128),
       (512, 128), (512, 128), (512, 128), (528, 128))
GW = sum(w[1] for w in WIN)


def _q_of_m(m):
    hi = (m // 128) * 128 + (m % 8)
    return 16 * HI.index(hi) + (m % 128) // 8


def _build_tables():
    pos = np.arange(L, dtype=np.int64)
    rr = np.zeros(L, np.int64)
    for l in range(L):
        if l < 256:
            rr[l] = l
        else:
            step = 1 << (int(l).bit_length() - 8)
            lo = (l // step) * step
            rem = l - lo
            if rem * 2 < step or (rem * 2 == step and (lo // step) % 2 == 0):
                rr[l] = lo
            else:
                rr[l] = lo + step
    w = np.pi * (2 * np.arange(J) + 1) / (2 * J)
    n = np.arange(J)
    f_fwd = np.concatenate([np.cos(np.outer(w, n)), -np.sin(np.outer(w, n))], 0)
    f_inv = np.concatenate([np.cos(np.outer(n, w)), -np.sin(np.outer(n, w))], 1) / J
    g_all = np.zeros((2 * J, GW))
    off = 0
    for dl in range(NB):
        s0, ln = WIN[dl]
        for p in range(-J, J):
            l = dl * J + p
            if 0 <= l < L:
                q = _q_of_m(int(rr[l])) - s0
                assert 0 <= q < ln
                g_all[:J, off + q] += np.cos(w * p)
                g_all[J:, off + q] += -np.sin(w * p)
        off += ln
    sel = np.zeros((16, 128))
    for dd in range(8):
        sel[np.arange(16), np.arange(16) * 8 + dd] = 1.0
    del pos
    return (f_fwd.astype(np.float32), f_inv.astype(np.float32),
            g_all.astype(np.float32), sel.astype(np.float32))


_F_FWD, _F_INV, _G_ALL, _SEL = _build_tables()


def _bf(x):
    return x.astype(jnp.bfloat16)


def _rb(x):
    return x.astype(jnp.bfloat16).astype(jnp.float32)


def _cmul(a, b):
    return (a[0] * b[0] - a[1] * b[1], a[0] * b[1] + a[1] * b[0])


def _gelu(x):
    c = 0.7978845608028654
    return 0.5 * x * (1.0 + jnp.tanh(c * (x + 0.044715 * (x * x * x))))


def _layernorm(x):
    m = jnp.mean(x, axis=-1, keepdims=True)
    xc = x - m
    v = jnp.mean(xc * xc, axis=-1, keepdims=True)
    den = _rb(jnp.sqrt(_rb(_rb(v) + 1e-5)))
    return _rb(_rb(x - _rb(m)) / den)


def _dot(a, b):
    return jnp.dot(a, b, preferred_element_type=jnp.float32)


def _dot_nt(a, b):
    return lax.dot_general(a, b, (((1,), (1,)), ((), ())),
                           preferred_element_type=jnp.float32)


def _kernel(are_ref, aim_ref, bre_ref, bim_ref, cre_ref, cim_ref, ldt_ref, dsk_ref,
            ffwd_ref, finv_ref, sel_ref,
            x_hbm, w1_hbm, w2_hbm, w3_hbm, w4_hbm, g_hbm,
            out_hbm,
            x_v, w1_v, w2_v, w3_v, w4_v, g_v, out_v,
            xn_v, h_v, u_v, kt_v, z_v,
            yr_v, yi_v, xr_v, xi_v, o_v, kd_v, dt_v, x1_v, ln2_v, ga_v, gate_v,
            sem_in, sem_out):
    copies = [pltpu.make_async_copy(s, d, sem_in.at[k]) for k, (s, d) in enumerate(
        [(x_hbm, x_v), (w1_hbm, w1_v), (g_hbm, g_v), (w2_hbm, w2_v),
         (w3_hbm, w3_v.at[0:FF, :]), (w4_hbm, w4_v.at[0:FF, :])])]
    for c in copies:
        c.start()

    dt_row = _rb(jnp.exp(ldt_ref[...].astype(jnp.float32))).reshape(1, D)
    dt_v[...] = jnp.transpose(jnp.broadcast_to(dt_row, (N, D)))

    def kgen(c, carry):
        r0 = pl.multiple_of(c * CH, CH)
        rows = pl.ds(r0, CH)
        f32 = jnp.float32
        dt = dt_v[rows, :]
        lr = dt * are_ref[rows, :].astype(f32)
        li = dt * aim_ref[rows, :].astype(f32)
        dbr = dt * bre_ref[rows, :].astype(f32)
        dbi = dt * bim_ref[rows, :].astype(f32)
        w = _cmul((cre_ref[rows, :].astype(f32), cim_ref[rows, :].astype(f32)), (dbr, dbi))

        def csq(a):
            ab = a[0] * a[1]
            return (a[0] * a[0] - a[1] * a[1], ab + ab)

        e1 = jnp.exp(lr)
        z1 = (e1 * jnp.cos(li), e1 * jnp.sin(li))
        z8 = csq(csq(csq(z1)))
        z128 = csq(csq(csq(csq(z8))))
        z1024 = csq(csq(csq(z128)))

        def put_y(j, v):
            for g in range(CH // 8):
                yr_v[g, 8 * j:8 * j + 8, :] = v[0][8 * g:8 * g + 8, :]
                yi_v[g, 8 * j:8 * j + 8, :] = v[1][8 * g:8 * g + 8, :]

        def put_x(i, v):
            nvi = -v[1]
            for g in range(CH // 8):
                xr_v[g, 8 * i:8 * i + 8, :] = v[0][8 * g:8 * g + 8, :]
                xi_v[g, 8 * i:8 * i + 8, :] = nvi[8 * g:8 * g + 8, :]

        put_y(0, (jnp.ones_like(lr), jnp.zeros_like(lr)))
        y = z8
        put_y(1, y)
        for j in range(2, 16):
            y = _cmul(y, z8)
            put_y(j, y)
        v = w
        for b in range(8):
            if b:
                v = _cmul(v, z1)
            t = v
            for k in range(8):
                if (128 * k + b) in HI:
                    if k:
                        t = _cmul(t, z128)
                    put_x(HI.index(128 * k + b), t)
        t = _cmul(w, z1024)
        for k in range(8, 17):
            if k > 8:
                t = _cmul(t, z128)
            put_x(HI.index(128 * k), t)
        for g in range(CH // 8):
            o = (_dot_nt(_bf(xr_v[g]), _bf(yr_v[g])) + _dot_nt(_bf(xi_v[g]), _bf(yi_v[g])))
            for i in range(NHI):
                o_v[i, pl.ds(pl.multiple_of(r0 + 8 * g, 8), 8), :] = o[8 * i:8 * i + 8, :]
        return carry

    with jax.named_scope('p_kgen'):
        lax.fori_loop(0, D // CH, kgen, 0)

    rid = lax.broadcasted_iota(jnp.int32, (D, 128), 0)
    lid = lax.broadcasted_iota(jnp.int32, (D, 128), 1)
    keep = (rid % 8) == (lid % 8)
    keep_last = keep & (lid < 8)
    sel = sel_ref[...]
    with jax.named_scope('p_sel'):
        for i in range(NHI):
            oi = jnp.where(keep_last if HI[i] == 2048 else keep, o_v[i], 0.0)
            kd_v[16 * i:16 * i + 16, :] = _dot_nt(sel, _bf(oi))

    copies[2].wait()
    off = 0
    for dl in range(NB):
        s0, ln = WIN[dl]
        kt_v[dl] = _dot(g_v[:, off:off + ln], _bf(kd_v[s0:s0 + ln, :]))
        off += ln

    copies[0].wait()
    copies[1].wait()
    h_v[0:8, :] = jnp.zeros((8, D), jnp.float32)
    h_v[8 + L:16 + L, :] = jnp.zeros((8, D), jnp.float32)

    def phase1(b, carry):
        r0 = pl.multiple_of(b * RB, RB)
        x = x_v[pl.ds(r0, RB), :].astype(jnp.float32)
        xn = _bf(_layernorm(x))
        xn_v[pl.ds(r0, RB), :] = xn
        h = _rb(_gelu(_rb(_dot(xn, w1_v[...]))))
        h_v[pl.ds(pl.multiple_of(r0 + 8, 8), RB), :] = h
        for k in range(RB // J):
            u_v[b * (RB // J) + k] = _dot(ffwd_ref[...], xn[k * J:(k + 1) * J, :])
        return carry

    with jax.named_scope('p_phase1'):
        lax.fori_loop(0, L // RB, phase1, 0)

    def zgroup(t, i0):
        cs = pl.ds(pl.multiple_of((t % 4) * 128, 128), 128)
        for hh in range(2):
            f0 = pl.multiple_of((t // 4) * 16 + 8 * hh, 8)
            re = pl.ds(f0, 8)
            im = pl.ds(pl.multiple_of(f0 + J, 8), 8)
            acc = {}
            uc = {}
            for dl in range(i0 + 4):
                kr = kt_v[dl, re, cs]
                ki = kt_v[dl, im, cs]
                for i in range(max(i0, dl), i0 + 4):
                    src = i - dl
                    if src not in uc:
                        uc[src] = (u_v[src, re, cs], u_v[src, im, cs])
                    ur, ui = uc[src]
                    pr = kr * ur - ki * ui
                    pi = kr * ui + ki * ur
                    acc[i] = (pr, pi) if i not in acc else (acc[i][0] + pr, acc[i][1] + pi)
            for i in range(i0, i0 + 4):
                z_v[i, re, cs] = acc[i][0]
                z_v[i, im, cs] = acc[i][1]

    copies[3].wait()
    copies[4].wait()
    copies[5].wait()
    w3_v[FF:FP, :] = jnp.zeros((FP - FF, D), jnp.bfloat16)
    w4_v[FF:FP, :] = jnp.zeros((FP - FF, D), jnp.bfloat16)
    NFC = FP // 128

    def pre(b):
        r0 = pl.multiple_of(b * RB, RB)
        ext = RB + 16
        parts = []
        for gi, sh in enumerate((1, -1, 2, -2)):
            hv = h_v[pl.ds(r0, ext), gi * 128:(gi + 1) * 128]
            hv = pltpu.roll(hv, sh % ext, 0)
            parts.append(_bf(hv[8:8 + RB, :]))
        hs = _rb(_dot(jnp.concatenate(parts, axis=1), w2_v[...]))
        xn = xn_v[pl.ds(r0, RB), :].astype(jnp.float32)
        x1 = _rb(xn + hs)
        x1_v[pl.ds(r0, RB), :] = _bf(x1)
        ln2_v[...] = _bf(_layernorm(x1))

    def up(slot, c):
        c0 = pl.multiple_of(jnp.minimum(c, NFC - 1) * 128, 128)
        ga_v[slot, :, pl.ds(pl.multiple_of(c * 128, 128), 128)] = _bf(
            _gelu(_rb(_dot_nt(ln2_v[...], w3_v[pl.ds(c0, 128), :]))))

    def down(b, n):
        r0 = pl.multiple_of(b * RB, RB)
        cs = pl.ds(pl.multiple_of(n * 128, 128), 128)
        h2 = _rb(_dot(ga_v[b % 2, :, 0:FP], w4_v[:, cs]))
        bb = _rb(x1_v[pl.ds(r0, RB), cs].astype(jnp.float32) + h2)
        gate_v[pl.ds(r0, RB), cs] = _bf(bb * jax.nn.sigmoid(bb))

    def phase2(b, carry, with_up):
        if with_up:
            pre(b + 1)

        def inner(k, cc):
            t = 4 * b + k
            zgroup(t, 12)
            down(b, k)
            for q in range(3):
                zgroup(t, 8 - 4 * q)
                if with_up:
                    up((b + 1) % 2, 3 * k + q)
            return cc

        lax.fori_loop(0, 4, inner, 0)
        return carry

    with jax.named_scope('p_phase2'):
        pre(0)

        def up0(c, cc):
            up(0, c)
            return cc

        lax.fori_loop(0, NFC, up0, 0)
        lax.fori_loop(0, L // RB - 1, functools.partial(phase2, with_up=True), 0)
        phase2(L // RB - 1, 0, with_up=False)

    dsk = dsk_ref[...].astype(jnp.float32).reshape(1, D)

    def out_copy(b):
        r0 = pl.multiple_of(b * RB, RB)
        return pltpu.make_async_copy(out_v.at[pl.ds(r0, RB), :],
                                     out_hbm.at[pl.ds(r0, RB), :], sem_out.at[b])

    def phase3(b, carry):
        r0 = pl.multiple_of(b * RB, RB)
        ys = [_dot(finv_ref[...], _bf(z_v[b * (RB // J) + k])) for k in range(RB // J)]
        y = _rb(jnp.concatenate(ys, axis=0))
        xn = xn_v[pl.ds(r0, RB), :].astype(jnp.float32)
        s = _rb(y + _rb(xn * dsk))
        x = x_v[pl.ds(r0, RB), :].astype(jnp.float32)
        gate = gate_v[pl.ds(r0, RB), :].astype(jnp.float32)
        out_v[pl.ds(r0, RB), :] = _bf(x + _rb(s * gate))
        out_copy(b).start()
        return carry

    with jax.named_scope('p_phase3'):
        lax.fori_loop(0, L // RB, phase3, 0)
    for b in range(L // RB):
        out_copy(b).wait()


@jax.jit
def pallas_recurrent_scan__ssm_conv_s4__mixer_s_mlp__prompt_kernel(
    A_u: jax.Array,
    A_A_re: jax.Array,
    A_A_im: jax.Array,
    A_B_re: jax.Array,
    A_B_im: jax.Array,
    A_C_re: jax.Array,
    A_C_im: jax.Array,
    A_log_dt: jax.Array,
    A_Dskip: jax.Array,
    B_x: jax.Array,
    B_w1: jax.Array,
    B_w2: jax.Array,
    B_w3: jax.Array,
    B_w4: jax.Array,
):
    bf16 = jnp.bfloat16
    f32 = jnp.float32
    x = A_u.reshape(L, D)
    vm = pl.BlockSpec(memory_space=pltpu.VMEM)
    hbm = pl.BlockSpec(memory_space=pltpu.HBM)
    out = pl.pallas_call(
        _kernel,
        out_shape=jax.ShapeDtypeStruct((L, D), bf16),
        in_specs=[vm] * 11 + [hbm] * 6,
        out_specs=hbm,
        scratch_shapes=[
            pltpu.VMEM((L, D), bf16),
            pltpu.VMEM((D, D), bf16),
            pltpu.VMEM((D, D), bf16),
            pltpu.VMEM((FP, D), bf16),
            pltpu.VMEM((FP, D), bf16),
            pltpu.VMEM((2 * J, GW), bf16),
            pltpu.VMEM((L, D), bf16),
            pltpu.VMEM((L, D), bf16),
            pltpu.VMEM((L + 16, D), f32),
            pltpu.VMEM((NB, 2 * J, D), f32),
            pltpu.VMEM((NB, 2 * J, D), f32),
            pltpu.VMEM((NB, 2 * J, D), f32),
            pltpu.VMEM((CH // 8, 128, N), f32),
            pltpu.VMEM((CH // 8, 128, N), f32),
            pltpu.VMEM((CH // 8, 8 * NHI, N), f32),
            pltpu.VMEM((CH // 8, 8 * NHI, N), f32),
            pltpu.VMEM((NHI, D, 128), f32),
            pltpu.VMEM((NQ, D), f32),
            pltpu.VMEM((D, N), f32),
            pltpu.VMEM((L, D), bf16),
            pltpu.VMEM((RB, D), bf16),
            pltpu.VMEM((2, RB, FP + 128), bf16),
            pltpu.VMEM((L, D), bf16),
            pltpu.SemaphoreType.DMA((6,)),
            pltpu.SemaphoreType.DMA((L // RB,)),
        ],
        compiler_params=pltpu.CompilerParams(vmem_limit_bytes=100 * 1024 * 1024),
    )(A_A_re, A_A_im, A_B_re, A_B_im, A_C_re, A_C_im,
      A_log_dt, A_Dskip,
      jnp.asarray(_F_FWD, bf16), jnp.asarray(_F_INV, bf16), jnp.asarray(_SEL, bf16),
      *[pltpu.with_memory_space_constraint(t, pltpu.HBM)
        for t in (x, B_w1, B_w2, B_w3.T, B_w4, jnp.asarray(_G_ALL, bf16))])
    return out.reshape(1, L, D)
```

```python
import functools
import numpy as np
import jax
import jax.numpy as jnp
from jax import lax
import jax.experimental.pallas as pl
import jax.experimental.pallas.tpu as pltpu

L = 2048
D = 512
N = 128
FF = 1376
J = 128
NB = L // J
NQ = 656
_STEP = (1, 1, 2, 2, 4, 4, 4, 4, 8, 8, 8, 8, 8, 8, 8, 8)
HI = tuple(128 * k + b for k in range(16) for b in range(0, 8, _STEP[k])) + (2048,)
NHI = len(HI)
CH = 32
RB = 512
WIN = ((0, 128), (0, 256), (128, 256), (256, 256), (320, 128), (384, 128),
       (384, 128), (448, 128), (448, 128), (512, 128), (512, 128), (512, 128),
       (512, 128), (512, 128), (512, 128), (528, 128))
GW = sum(w[1] for w in WIN)


def _q_of_m(m):
    hi = (m // 128) * 128 + (m % 8)
    return 16 * HI.index(hi) + (m % 128) // 8


def _build_tables():
    pos = np.arange(L, dtype=np.int64)
    rr = np.zeros(L, np.int64)
    for l in range(L):
        if l < 256:
            rr[l] = l
        else:
            step = 1 << (int(l).bit_length() - 8)
            lo = (l // step) * step
            rem = l - lo
            if rem * 2 < step or (rem * 2 == step and (lo // step) % 2 == 0):
                rr[l] = lo
            else:
                rr[l] = lo + step
    w = np.pi * (2 * np.arange(J) + 1) / (2 * J)
    n = np.arange(J)
    f_fwd = np.concatenate([np.cos(np.outer(w, n)), -np.sin(np.outer(w, n))], 0)
    f_inv = np.concatenate([np.cos(np.outer(n, w)), -np.sin(np.outer(n, w))], 1) / J
    g_all = np.zeros((2 * J, GW))
    off = 0
    for dl in range(NB):
        s0, ln = WIN[dl]
        for p in range(-J, J):
            l = dl * J + p
            if 0 <= l < L:
                q = _q_of_m(int(rr[l])) - s0
                assert 0 <= q < ln
                g_all[:J, off + q] += np.cos(w * p)
                g_all[J:, off + q] += -np.sin(w * p)
        off += ln
    sel = np.zeros((16, 128))
    for dd in range(8):
        sel[np.arange(16), np.arange(16) * 8 + dd] = 1.0
    del pos
    return (f_fwd.astype(np.float32), f_inv.astype(np.float32),
            g_all.astype(np.float32), sel.astype(np.float32))


_F_FWD, _F_INV, _G_ALL, _SEL = _build_tables()


def _bf(x):
    return x.astype(jnp.bfloat16)


def _rb(x):
    return x.astype(jnp.bfloat16).astype(jnp.float32)


def _cmul(a, b):
    return (a[0] * b[0] - a[1] * b[1], a[0] * b[1] + a[1] * b[0])


def _gelu(x):
    c = 0.7978845608028654
    return 0.5 * x * (1.0 + jnp.tanh(c * (x + 0.044715 * (x * x * x))))


def _layernorm(x):
    m = jnp.mean(x, axis=-1, keepdims=True)
    xc = x - m
    v = jnp.mean(xc * xc, axis=-1, keepdims=True)
    den = _rb(jnp.sqrt(_rb(_rb(v) + 1e-5)))
    return _rb(_rb(x - _rb(m)) / den)


def _layernorm2(x):
    m = jnp.mean(x, axis=-1, keepdims=True)
    xc = x - m
    v = jnp.mean(xc * xc, axis=-1, keepdims=True)
    return xc / jnp.sqrt(v + 1e-5)


def _dot(a, b):
    return jnp.dot(a, b, preferred_element_type=jnp.float32)


def _dot_nt(a, b):
    return lax.dot_general(a, b, (((1,), (1,)), ((), ())),
                           preferred_element_type=jnp.float32)


def _kernel(are_ref, aim_ref, bre_ref, bim_ref, cre_ref, cim_ref, ldt_ref, dsk_ref,
            ffwd_ref, finv_ref, sel_ref,
            x_hbm, w1_hbm, w2_hbm, w3_hbm, w4_hbm, g_hbm,
            out_hbm,
            x_v, w1_v, w2_v, w3_v, w4_v, g_v, out_v,
            xn_v, h_v, u_v, kt_v, z_v,
            yr_v, yi_v, xr_v, xi_v, o_v, kd_v, dt_v,
            sem_in, sem_out):
    copies = [pltpu.make_async_copy(s, d, sem_in.at[k]) for k, (s, d) in enumerate(
        [(x_hbm, x_v), (w1_hbm, w1_v), (g_hbm, g_v), (w2_hbm, w2_v), (w3_hbm, w3_v),
         (w4_hbm, w4_v)])]
    for c in copies:
        c.start()

    dt_row = _rb(jnp.exp(ldt_ref[...].astype(jnp.float32))).reshape(1, D)
    dt_v[...] = jnp.transpose(jnp.broadcast_to(dt_row, (N, D)))

    def kgen(c, carry):
        r0 = pl.multiple_of(c * CH, CH)
        rows = pl.ds(r0, CH)
        f32 = jnp.float32
        dt = dt_v[rows, :]
        lr = dt * are_ref[rows, :].astype(f32)
        li = dt * aim_ref[rows, :].astype(f32)
        dbr = dt * bre_ref[rows, :].astype(f32)
        dbi = dt * bim_ref[rows, :].astype(f32)
        w = _cmul((cre_ref[rows, :].astype(f32), cim_ref[rows, :].astype(f32)), (dbr, dbi))

        def csq(a):
            ab = a[0] * a[1]
            return (a[0] * a[0] - a[1] * a[1], ab + ab)

        e1 = jnp.exp(lr)
        z1 = (e1 * jnp.cos(li), e1 * jnp.sin(li))
        z8 = csq(csq(csq(z1)))
        z128 = csq(csq(csq(csq(z8))))
        z1024 = csq(csq(csq(z128)))

        def put_y(j, v):
            for g in range(CH // 8):
                yr_v[g, 8 * j:8 * j + 8, :] = v[0][8 * g:8 * g + 8, :]
                yi_v[g, 8 * j:8 * j + 8, :] = v[1][8 * g:8 * g + 8, :]

        def put_x(i, v):
            nvi = -v[1]
            for g in range(CH // 8):
                xr_v[g, 8 * i:8 * i + 8, :] = v[0][8 * g:8 * g + 8, :]
                xi_v[g, 8 * i:8 * i + 8, :] = nvi[8 * g:8 * g + 8, :]

        put_y(0, (jnp.ones_like(lr), jnp.zeros_like(lr)))
        y = z8
        put_y(1, y)
        for j in range(2, 16):
            y = _cmul(y, z8)
            put_y(j, y)
        v = w
        for b in range(8):
            if b:
                v = _cmul(v, z1)
            t = v
            for k in range(8):
                if (128 * k + b) in HI:
                    if k:
                        t = _cmul(t, z128)
                    put_x(HI.index(128 * k + b), t)
        t = _cmul(w, z1024)
        for k in range(8, 17):
            if k > 8:
                t = _cmul(t, z128)
            put_x(HI.index(128 * k), t)
        for g in range(CH // 8):
            o = (_dot_nt(_bf(xr_v[g]), _bf(yr_v[g])) + _dot_nt(_bf(xi_v[g]), _bf(yi_v[g])))
            for i in range(NHI):
                o_v[i, pl.ds(pl.multiple_of(r0 + 8 * g, 8), 8), :] = o[8 * i:8 * i + 8, :]
        return carry

    with jax.named_scope('p_kgen'):
        lax.fori_loop(0, D // CH, kgen, 0)

    rid = lax.broadcasted_iota(jnp.int32, (D, 128), 0)
    lid = lax.broadcasted_iota(jnp.int32, (D, 128), 1)
    keep = (rid % 8) == (lid % 8)
    keep_last = keep & (lid < 8)
    sel = sel_ref[...]
    with jax.named_scope('p_sel'):
        for i in range(NHI):
            oi = jnp.where(keep_last if HI[i] == 2048 else keep, o_v[i], 0.0)
            kd_v[16 * i:16 * i + 16, :] = _dot_nt(sel, _bf(oi))

    copies[2].wait()
    off = 0
    for dl in range(NB):
        s0, ln = WIN[dl]
        kt_v[dl] = _dot(g_v[:, off:off + ln], _bf(kd_v[s0:s0 + ln, :]))
        off += ln

    copies[0].wait()
    copies[1].wait()
    h_v[0:8, :] = jnp.zeros((8, D), jnp.float32)
    h_v[8 + L:16 + L, :] = jnp.zeros((8, D), jnp.float32)

    def phase1(b, carry):
        r0 = pl.multiple_of(b * RB, RB)
        x = x_v[pl.ds(r0, RB), :].astype(jnp.float32)
        xn = _bf(_layernorm(x))
        xn_v[pl.ds(r0, RB), :] = xn
        h = _gelu(_dot(xn, w1_v[...]))
        h_v[pl.ds(pl.multiple_of(r0 + 8, 8), RB), :] = h
        for k in range(RB // J):
            u_v[b * (RB // J) + k] = _dot(ffwd_ref[...], xn[k * J:(k + 1) * J, :])
        return carry

    with jax.named_scope('p_phase1'):
        lax.fori_loop(0, L // RB, phase1, 0)

    def zphase(t, carry):
        f0 = pl.multiple_of((t // 4) * 16, 16)
        c0 = pl.multiple_of((t % 4) * 128, 128)
        re = pl.ds(f0, 16)
        im = pl.ds(pl.multiple_of(f0 + J, 16), 16)
        cs = pl.ds(c0, 128)
        for i in range(NB):
            zr = None
            zi = None
            for dl in range(i + 1):
                kr = kt_v[dl, re, cs]
                ki = kt_v[dl, im, cs]
                ur = u_v[i - dl, re, cs]
                ui = u_v[i - dl, im, cs]
                pr = kr * ur - ki * ui
                pi = kr * ui + ki * ur
                zr = pr if zr is None else zr + pr
                zi = pi if zi is None else zi + pi
            z_v[i, re, cs] = _bf(zr)
            z_v[i, im, cs] = _bf(zi)
        return carry

    with jax.named_scope('p_z'):
        lax.fori_loop(0, 32, zphase, 0)

    copies[3].wait()
    copies[4].wait()
    copies[5].wait()
    dsk = dsk_ref[...].astype(jnp.float32).reshape(1, D)

    def out_copy(b):
        r0 = pl.multiple_of(b * RB, RB)
        return pltpu.make_async_copy(out_v.at[pl.ds(r0, RB), :],
                                     out_hbm.at[pl.ds(r0, RB), :], sem_out.at[b])

    def phase2(b, carry):
        r0 = pl.multiple_of(b * RB, RB)
        ext = RB + 16
        parts = []
        for gi, sh in enumerate((1, -1, 2, -2)):
            hv = h_v[pl.ds(r0, ext), gi * 128:(gi + 1) * 128]
            hv = pltpu.roll(hv, sh % ext, 0)
            parts.append(_bf(hv[8:8 + RB, :]))
        hs = _dot(jnp.concatenate(parts, axis=1), w2_v[...])
        xn = xn_v[pl.ds(r0, RB), :].astype(jnp.float32)
        x1 = xn + hs
        a = _dot_nt(_bf(_layernorm2(x1)), w3_v[...])
        h2 = _dot(_bf(_gelu(a)), w4_v[...])
        bb = x1 + h2
        gate = bb * jax.nn.sigmoid(bb)
        ys = [_dot(finv_ref[...], z_v[b * (RB // J) + k]) for k in range(RB // J)]
        y = jnp.concatenate(ys, axis=0)
        s = y + xn * dsk
        x = x_v[pl.ds(r0, RB), :].astype(jnp.float32)
        out_v[pl.ds(r0, RB), :] = _bf(x + s * gate)
        out_copy(b).start()
        return carry

    with jax.named_scope('p_phase2'):
        lax.fori_loop(0, L // RB, phase2, 0)
    for b in range(L // RB):
        out_copy(b).wait()


@jax.jit
def pallas_recurrent_scan__ssm_conv_s4__mixer_s_mlp__prompt_kernel(
    A_u: jax.Array,
    A_A_re: jax.Array,
    A_A_im: jax.Array,
    A_B_re: jax.Array,
    A_B_im: jax.Array,
    A_C_re: jax.Array,
    A_C_im: jax.Array,
    A_log_dt: jax.Array,
    A_Dskip: jax.Array,
    B_x: jax.Array,
    B_w1: jax.Array,
    B_w2: jax.Array,
    B_w3: jax.Array,
    B_w4: jax.Array,
):
    bf16 = jnp.bfloat16
    f32 = jnp.float32
    x = A_u.reshape(L, D)
    vm = pl.BlockSpec(memory_space=pltpu.VMEM)
    hbm = pl.BlockSpec(memory_space=pltpu.HBM)
    out = pl.pallas_call(
        _kernel,
        out_shape=jax.ShapeDtypeStruct((L, D), bf16),
        in_specs=[vm] * 11 + [hbm] * 6,
        out_specs=hbm,
        scratch_shapes=[
            pltpu.VMEM((L, D), bf16),
            pltpu.VMEM((D, D), bf16),
            pltpu.VMEM((D, D), bf16),
            pltpu.VMEM((FF, D), bf16),
            pltpu.VMEM((FF, D), bf16),
            pltpu.VMEM((2 * J, GW), bf16),
            pltpu.VMEM((L, D), bf16),
            pltpu.VMEM((L, D), bf16),
            pltpu.VMEM((L + 16, D), f32),
            pltpu.VMEM((NB, 2 * J, D), f32),
            pltpu.VMEM((NB, 2 * J, D), f32),
            pltpu.VMEM((NB, 2 * J, D), bf16),
            pltpu.VMEM((CH // 8, 128, N), f32),
            pltpu.VMEM((CH // 8, 128, N), f32),
            pltpu.VMEM((CH // 8, 8 * NHI, N), f32),
            pltpu.VMEM((CH // 8, 8 * NHI, N), f32),
            pltpu.VMEM((NHI, D, 128), f32),
            pltpu.VMEM((NQ, D), f32),
            pltpu.VMEM((D, N), f32),
            pltpu.SemaphoreType.DMA((6,)),
            pltpu.SemaphoreType.DMA((L // RB,)),
        ],
        compiler_params=pltpu.CompilerParams(vmem_limit_bytes=100 * 1024 * 1024),
    )(A_A_re, A_A_im, A_B_re, A_B_im, A_C_re, A_C_im,
      A_log_dt, A_Dskip,
      jnp.asarray(_F_FWD, bf16), jnp.asarray(_F_INV, bf16), jnp.asarray(_SEL, bf16),
      *[pltpu.with_memory_space_constraint(t, pltpu.HBM)
        for t in (x, B_w1, B_w2, B_w3.T, B_w4, jnp.asarray(_G_ALL, bf16))])
    return out.reshape(1, L, D)
```

```python
import functools
import numpy as np
import jax
import jax.numpy as jnp
from jax import lax
import jax.experimental.pallas as pl
import jax.experimental.pallas.tpu as pltpu

L = 2048
D = 512
N = 128
FF = 1376
J = 128
NB = L // J
NQ = 656
_STEP = (1, 1, 2, 2, 4, 4, 4, 4, 8, 8, 8, 8, 8, 8, 8, 8)
HI = tuple(128 * k + b for k in range(16) for b in range(0, 8, _STEP[k])) + (2048,)
NHI = len(HI)
CH = 32
RB = 512
WIN = ((0, 128), (0, 256), (128, 256), (256, 256), (320, 128), (384, 128),
       (384, 128), (448, 128), (448, 128), (512, 128), (512, 128), (512, 128),
       (512, 128), (512, 128), (512, 128), (528, 128))
GW = sum(w[1] for w in WIN)


def _q_of_m(m):
    hi = (m // 128) * 128 + (m % 8)
    return 16 * HI.index(hi) + (m % 128) // 8


def _build_tables():
    pos = np.arange(L, dtype=np.int64)
    rr = np.zeros(L, np.int64)
    for l in range(L):
        if l < 256:
            rr[l] = l
        else:
            step = 1 << (int(l).bit_length() - 8)
            lo = (l // step) * step
            rem = l - lo
            if rem * 2 < step or (rem * 2 == step and (lo // step) % 2 == 0):
                rr[l] = lo
            else:
                rr[l] = lo + step
    w = np.pi * (2 * np.arange(J) + 1) / (2 * J)
    n = np.arange(J)
    f_fwd = np.concatenate([np.cos(np.outer(w, n)), -np.sin(np.outer(w, n))], 0)
    f_inv = np.concatenate([np.cos(np.outer(n, w)), -np.sin(np.outer(n, w))], 1) / J
    g_all = np.zeros((2 * J, GW))
    off = 0
    for dl in range(NB):
        s0, ln = WIN[dl]
        for p in range(-J, J):
            l = dl * J + p
            if 0 <= l < L:
                q = _q_of_m(int(rr[l])) - s0
                assert 0 <= q < ln
                g_all[:J, off + q] += np.cos(w * p)
                g_all[J:, off + q] += -np.sin(w * p)
        off += ln
    sel = np.zeros((16, 128))
    for dd in range(8):
        sel[np.arange(16), np.arange(16) * 8 + dd] = 1.0
    del pos
    return (f_fwd.astype(np.float32), f_inv.astype(np.float32),
            g_all.astype(np.float32), sel.astype(np.float32))


_F_FWD, _F_INV, _G_ALL, _SEL = _build_tables()


def _bf(x):
    return x.astype(jnp.bfloat16)


def _rb(x):
    return x.astype(jnp.bfloat16).astype(jnp.float32)


def _cmul(a, b):
    return (a[0] * b[0] - a[1] * b[1], a[0] * b[1] + a[1] * b[0])


def _gelu(x):
    c = 0.7978845608028654
    return 0.5 * x * (1.0 + jnp.tanh(c * (x + 0.044715 * (x * x * x))))


def _layernorm(x):
    m = jnp.mean(x, axis=-1, keepdims=True)
    xc = x - m
    v = jnp.mean(xc * xc, axis=-1, keepdims=True)
    den = _rb(jnp.sqrt(_rb(_rb(v) + 1e-5)))
    return _rb(_rb(x - _rb(m)) / den)


def _layernorm2(x):
    m = jnp.mean(x, axis=-1, keepdims=True)
    xc = x - m
    v = jnp.mean(xc * xc, axis=-1, keepdims=True)
    return xc / jnp.sqrt(v + 1e-5)


def _dot(a, b):
    return jnp.dot(a, b, preferred_element_type=jnp.float32)


def _dot_nt(a, b):
    return lax.dot_general(a, b, (((1,), (1,)), ((), ())),
                           preferred_element_type=jnp.float32)


def _kernel(are_ref, aim_ref, bre_ref, bim_ref, cre_ref, cim_ref, ldt_ref, dsk_ref,
            ffwd_ref, finv_ref, sel_ref,
            x_hbm, w1_hbm, w2_hbm, w3_hbm, w4_hbm, g_hbm,
            out_hbm,
            x_v, w1_v, w2_v, w3_v, w4_v, g_v, out_v,
            xn_v, h_v, u_v, kt_v, z_v,
            yr_v, yi_v, xr_v, xi_v, o_v, kd_v, dt_v,
            sem_in, sem_out):
    copies = [pltpu.make_async_copy(s, d, sem_in.at[k]) for k, (s, d) in enumerate(
        [(x_hbm, x_v), (w1_hbm, w1_v), (g_hbm, g_v), (w2_hbm, w2_v), (w3_hbm, w3_v),
         (w4_hbm, w4_v)])]
    for c in copies:
        c.start()

    dt_row = _rb(jnp.exp(ldt_ref[...].astype(jnp.float32))).reshape(1, D)
    dt_v[...] = jnp.transpose(jnp.broadcast_to(dt_row, (N, D)))

    def kgen(c, carry):
        r0 = pl.multiple_of(c * CH, CH)
        rows = pl.ds(r0, CH)
        f32 = jnp.float32
        dt = dt_v[rows, :]
        lr = dt * are_ref[rows, :].astype(f32)
        li = dt * aim_ref[rows, :].astype(f32)
        dbr = dt * bre_ref[rows, :].astype(f32)
        dbi = dt * bim_ref[rows, :].astype(f32)
        w = _cmul((cre_ref[rows, :].astype(f32), cim_ref[rows, :].astype(f32)), (dbr, dbi))

        def csq(a):
            ab = a[0] * a[1]
            return (a[0] * a[0] - a[1] * a[1], ab + ab)

        e1 = jnp.exp(lr)
        z1 = (e1 * jnp.cos(li), e1 * jnp.sin(li))
        z8 = csq(csq(csq(z1)))
        z128 = csq(csq(csq(csq(z8))))
        z1024 = csq(csq(csq(z128)))

        def put_y(j, v):
            for g in range(CH // 8):
                yr_v[g, 8 * j:8 * j + 8, :] = v[0][8 * g:8 * g + 8, :]
                yi_v[g, 8 * j:8 * j + 8, :] = v[1][8 * g:8 * g + 8, :]

        def put_x(i, v):
            nvi = -v[1]
            for g in range(CH // 8):
                xr_v[g, 8 * i:8 * i + 8, :] = v[0][8 * g:8 * g + 8, :]
                xi_v[g, 8 * i:8 * i + 8, :] = nvi[8 * g:8 * g + 8, :]

        put_y(0, (jnp.ones_like(lr), jnp.zeros_like(lr)))
        y = z8
        put_y(1, y)
        for j in range(2, 16):
            y = _cmul(y, z8)
            put_y(j, y)
        v = w
        for b in range(8):
            if b:
                v = _cmul(v, z1)
            t = v
            for k in range(8):
                if (128 * k + b) in HI:
                    if k:
                        t = _cmul(t, z128)
                    put_x(HI.index(128 * k + b), t)
        t = _cmul(w, z1024)
        for k in range(8, 17):
            if k > 8:
                t = _cmul(t, z128)
            put_x(HI.index(128 * k), t)
        for g in range(CH // 8):
            o = (_dot_nt(_bf(xr_v[g]), _bf(yr_v[g])) + _dot_nt(_bf(xi_v[g]), _bf(yi_v[g])))
            for i in range(NHI):
                o_v[i, pl.ds(pl.multiple_of(r0 + 8 * g, 8), 8), :] = o[8 * i:8 * i + 8, :]
        return carry

    with jax.named_scope('p_kgen'):
        lax.fori_loop(0, D // CH, kgen, 0)

    rid = lax.broadcasted_iota(jnp.int32, (D, 128), 0)
    lid = lax.broadcasted_iota(jnp.int32, (D, 128), 1)
    keep = (rid % 8) == (lid % 8)
    keep_last = keep & (lid < 8)
    sel = sel_ref[...]
    with jax.named_scope('p_sel'):
        for i in range(NHI):
            oi = jnp.where(keep_last if HI[i] == 2048 else keep, o_v[i], 0.0)
            kd_v[16 * i:16 * i + 16, :] = _dot_nt(sel, _bf(oi))

    copies[2].wait()
    off = 0
    for dl in range(NB):
        s0, ln = WIN[dl]
        kt_v[dl] = _dot(g_v[:, off:off + ln], _bf(kd_v[s0:s0 + ln, :]))
        off += ln

    copies[0].wait()
    copies[1].wait()
    h_v[0:8, :] = jnp.zeros((8, D), jnp.float32)
    h_v[8 + L:16 + L, :] = jnp.zeros((8, D), jnp.float32)

    def phase1(b, carry):
        r0 = pl.multiple_of(b * RB, RB)
        x = x_v[pl.ds(r0, RB), :].astype(jnp.float32)
        xn = _bf(_layernorm(x))
        xn_v[pl.ds(r0, RB), :] = xn
        h = _gelu(_dot(xn, w1_v[...]))
        h_v[pl.ds(pl.multiple_of(r0 + 8, 8), RB), :] = h
        for k in range(RB // J):
            u_v[b * (RB // J) + k] = _dot(ffwd_ref[...], xn[k * J:(k + 1) * J, :])
        return carry

    with jax.named_scope('p_phase1'):
        lax.fori_loop(0, L // RB, phase1, 0)

    def zphase(t, carry):
        f0 = pl.multiple_of((t // 4) * 8, 8)
        re = pl.ds(f0, 8)
        im = pl.ds(pl.multiple_of(f0 + J, 8), 8)
        cs = pl.ds(pl.multiple_of((t % 4) * 128, 128), 128)
        GZ = 4
        for i0 in range(0, NB, GZ):
            acc = {}
            uc = {}
            for dl in range(i0 + GZ):
                kr = kt_v[dl, re, cs]
                ki = kt_v[dl, im, cs]
                ks = kr + ki
                for i in range(max(i0, dl), i0 + GZ):
                    src = i - dl
                    if src not in uc:
                        ur = u_v[src, re, cs]
                        ui = u_v[src, im, cs]
                        uc[src] = (ur, ui, ur + ui)
                    ur, ui, us = uc[src]
                    p = (kr * ur, ki * ui, ks * us)
                    acc[i] = p if i not in acc else tuple(x + y for x, y in zip(acc[i], p))
            for i in range(i0, i0 + GZ):
                s1, s2, s3 = acc[i]
                z_v[i, re, cs] = s1 - s2
                z_v[i, im, cs] = s3 - (s1 + s2)
        return carry

    with jax.named_scope('p_z'):
        lax.fori_loop(0, 64, zphase, 0)

    copies[3].wait()
    copies[4].wait()
    copies[5].wait()
    dsk = dsk_ref[...].astype(jnp.float32).reshape(1, D)

    def out_copy(b):
        r0 = pl.multiple_of(b * RB, RB)
        return pltpu.make_async_copy(out_v.at[pl.ds(r0, RB), :],
                                     out_hbm.at[pl.ds(r0, RB), :], sem_out.at[b])

    def phase2(b, carry):
        r0 = pl.multiple_of(b * RB, RB)
        ext = RB + 16
        parts = []
        for gi, sh in enumerate((1, -1, 2, -2)):
            hv = h_v[pl.ds(r0, ext), gi * 128:(gi + 1) * 128]
            hv = pltpu.roll(hv, sh % ext, 0)
            parts.append(_bf(hv[8:8 + RB, :]))
        hs = _dot(jnp.concatenate(parts, axis=1), w2_v[...])
        xn = xn_v[pl.ds(r0, RB), :].astype(jnp.float32)
        x1 = xn + hs
        a = _dot_nt(_bf(_layernorm2(x1)), w3_v[...])
        h2 = _dot(_bf(_gelu(a)), w4_v[...])
        bb = x1 + h2
        gate = bb * jax.nn.sigmoid(bb)
        ys = [_dot(finv_ref[...], _bf(z_v[b * (RB // J) + k])) for k in range(RB // J)]
        y = jnp.concatenate(ys, axis=0)
        s = y + xn * dsk
        x = x_v[pl.ds(r0, RB), :].astype(jnp.float32)
        out_v[pl.ds(r0, RB), :] = _bf(x + s * gate)
        out_copy(b).start()
        return carry

    with jax.named_scope('p_phase2'):
        lax.fori_loop(0, L // RB, phase2, 0)
    for b in range(L // RB):
        out_copy(b).wait()


@jax.jit
def pallas_recurrent_scan__ssm_conv_s4__mixer_s_mlp__prompt_kernel(
    A_u: jax.Array,
    A_A_re: jax.Array,
    A_A_im: jax.Array,
    A_B_re: jax.Array,
    A_B_im: jax.Array,
    A_C_re: jax.Array,
    A_C_im: jax.Array,
    A_log_dt: jax.Array,
    A_Dskip: jax.Array,
    B_x: jax.Array,
    B_w1: jax.Array,
    B_w2: jax.Array,
    B_w3: jax.Array,
    B_w4: jax.Array,
):
    bf16 = jnp.bfloat16
    f32 = jnp.float32
    x = A_u.reshape(L, D)
    vm = pl.BlockSpec(memory_space=pltpu.VMEM)
    hbm = pl.BlockSpec(memory_space=pltpu.HBM)
    out = pl.pallas_call(
        _kernel,
        out_shape=jax.ShapeDtypeStruct((L, D), bf16),
        in_specs=[vm] * 11 + [hbm] * 6,
        out_specs=hbm,
        scratch_shapes=[
            pltpu.VMEM((L, D), bf16),
            pltpu.VMEM((D, D), bf16),
            pltpu.VMEM((D, D), bf16),
            pltpu.VMEM((FF, D), bf16),
            pltpu.VMEM((FF, D), bf16),
            pltpu.VMEM((2 * J, GW), bf16),
            pltpu.VMEM((L, D), bf16),
            pltpu.VMEM((L, D), bf16),
            pltpu.VMEM((L + 16, D), f32),
            pltpu.VMEM((NB, 2 * J, D), f32),
            pltpu.VMEM((NB, 2 * J, D), f32),
            pltpu.VMEM((NB, 2 * J, D), f32),
            pltpu.VMEM((CH // 8, 128, N), f32),
            pltpu.VMEM((CH // 8, 128, N), f32),
            pltpu.VMEM((CH // 8, 8 * NHI, N), f32),
            pltpu.VMEM((CH // 8, 8 * NHI, N), f32),
            pltpu.VMEM((NHI, D, 128), f32),
            pltpu.VMEM((NQ, D), f32),
            pltpu.VMEM((D, N), f32),
            pltpu.SemaphoreType.DMA((6,)),
            pltpu.SemaphoreType.DMA((L // RB,)),
        ],
        compiler_params=pltpu.CompilerParams(vmem_limit_bytes=100 * 1024 * 1024),
    )(A_A_re, A_A_im, A_B_re, A_B_im, A_C_re, A_C_im,
      A_log_dt, A_Dskip,
      jnp.asarray(_F_FWD, bf16), jnp.asarray(_F_INV, bf16), jnp.asarray(_SEL, bf16),
      *[pltpu.with_memory_space_constraint(t, pltpu.HBM)
        for t in (x, B_w1, B_w2, B_w3.T, B_w4, jnp.asarray(_G_ALL, bf16))])
    return out.reshape(1, L, D)
```

```python
import functools
import numpy as np
import jax
import jax.numpy as jnp
from jax import lax
import jax.experimental.pallas as pl
import jax.experimental.pallas.tpu as pltpu

L = 2048
D = 512
N = 128
FF = 1376
J = 128
NB = L // J
NQ = 656
_STEP = (1, 1, 2, 2, 4, 4, 4, 4, 8, 8, 8, 8, 8, 8, 8, 8)
HI = tuple(128 * k + b for k in range(16) for b in range(0, 8, _STEP[k])) + (2048,)
NHI = len(HI)
CH = 32
RB = 512
WIN = ((0, 128), (0, 256), (128, 256), (256, 256), (320, 128), (384, 128),
       (384, 128), (448, 128), (448, 128), (512, 128), (512, 128), (512, 128),
       (512, 128), (512, 128), (512, 128), (528, 128))
GW = sum(w[1] for w in WIN)


def _q_of_m(m):
    hi = (m // 128) * 128 + (m % 8)
    return 16 * HI.index(hi) + (m % 128) // 8


def _build_tables():
    pos = np.arange(L, dtype=np.int64)
    rr = np.zeros(L, np.int64)
    for l in range(L):
        if l < 256:
            rr[l] = l
        else:
            step = 1 << (int(l).bit_length() - 8)
            lo = (l // step) * step
            rem = l - lo
            if rem * 2 < step or (rem * 2 == step and (lo // step) % 2 == 0):
                rr[l] = lo
            else:
                rr[l] = lo + step
    w = np.pi * (2 * np.arange(J) + 1) / (2 * J)
    n = np.arange(J)
    f_fwd = np.concatenate([np.cos(np.outer(w, n)), -np.sin(np.outer(w, n))], 0)
    f_inv = np.concatenate([np.cos(np.outer(n, w)), -np.sin(np.outer(n, w))], 1) / J
    g_all = np.zeros((2 * J, GW))
    off = 0
    for dl in range(NB):
        s0, ln = WIN[dl]
        for p in range(-J, J):
            l = dl * J + p
            if 0 <= l < L:
                q = _q_of_m(int(rr[l])) - s0
                assert 0 <= q < ln
                g_all[:J, off + q] += np.cos(w * p)
                g_all[J:, off + q] += -np.sin(w * p)
        off += ln
    sel = np.zeros((16, 128))
    for dd in range(8):
        sel[np.arange(16), np.arange(16) * 8 + dd] = 1.0
    del pos
    return (f_fwd.astype(np.float32), f_inv.astype(np.float32),
            g_all.astype(np.float32), sel.astype(np.float32))


_F_FWD, _F_INV, _G_ALL, _SEL = _build_tables()


def _bf(x):
    return x.astype(jnp.bfloat16)


def _rb(x):
    return x.astype(jnp.bfloat16).astype(jnp.float32)


def _cmul(a, b):
    return (a[0] * b[0] - a[1] * b[1], a[0] * b[1] + a[1] * b[0])


def _sincos(x):
    k = jnp.floor(x * 0.6366197723675814 + 0.5)
    r = x - k * 1.5703125
    r = r - k * 4.837512969970703125e-4
    r = r - k * 7.549789954891882e-8
    r2 = r * r
    sn = r + r * r2 * (-1.6666654611e-1 + r2 * (8.3321608736e-3 + r2 * -1.9515295891e-4))
    cs = 1.0 + r2 * (-0.5 + r2 * (4.166664568298827e-2 + r2 * (-1.388731625493765e-3
                                                             + r2 * 2.443315711809948e-5)))
    q = k - 4.0 * jnp.floor(k * 0.25)
    odd = (q == 1.0) | (q == 3.0)
    s0 = jnp.where(odd, cs, sn)
    c0 = jnp.where(odd, sn, cs)
    s1 = jnp.where(q >= 2.0, -s0, s0)
    c1 = jnp.where((q == 1.0) | (q == 2.0), -c0, c0)
    return s1, c1


def _gelu(x):
    c = 0.7978845608028654
    return 0.5 * x * (1.0 + jnp.tanh(c * (x + 0.044715 * (x * x * x))))


def _layernorm(x):
    m = jnp.mean(x, axis=-1, keepdims=True)
    xc = x - m
    v = jnp.mean(xc * xc, axis=-1, keepdims=True)
    den = _rb(jnp.sqrt(_rb(_rb(v) + 1e-5)))
    return _rb(_rb(x - _rb(m)) / den)


def _layernorm2(x):
    m = jnp.mean(x, axis=-1, keepdims=True)
    xc = x - m
    v = jnp.mean(xc * xc, axis=-1, keepdims=True)
    return xc / jnp.sqrt(v + 1e-5)


def _dot(a, b):
    return jnp.dot(a, b, preferred_element_type=jnp.float32)


def _dot_nt(a, b):
    return lax.dot_general(a, b, (((1,), (1,)), ((), ())),
                           preferred_element_type=jnp.float32)


def _kernel(are_ref, aim_ref, bre_ref, bim_ref, cre_ref, cim_ref, ldt_ref, dsk_ref,
            ffwd_ref, finv_ref, sel_ref,
            x_hbm, w1_hbm, w2_hbm, w3_hbm, w4_hbm, g_hbm,
            out_hbm,
            x_v, w1_v, w2_v, w3_v, w4_v, g_v, out_v,
            xn_v, h_v, u_v, kt_v, z_v,
            yr_v, yi_v, xr_v, xi_v, o_v, kd_v, dt_v,
            sem_in, sem_out):
    copies = [pltpu.make_async_copy(s, d, sem_in.at[k]) for k, (s, d) in enumerate(
        [(x_hbm, x_v), (w1_hbm, w1_v), (g_hbm, g_v), (w2_hbm, w2_v), (w3_hbm, w3_v),
         (w4_hbm, w4_v)])]
    for c in copies:
        c.start()

    dt_row = _rb(jnp.exp(ldt_ref[...].astype(jnp.float32))).reshape(1, D)
    dt_v[...] = jnp.transpose(jnp.broadcast_to(dt_row, (N, D)))

    def kgen(c, carry):
        r0 = pl.multiple_of(c * CH, CH)
        rows = pl.ds(r0, CH)
        f32 = jnp.float32
        dt = dt_v[rows, :]
        lr = dt * are_ref[rows, :].astype(f32)
        li = dt * aim_ref[rows, :].astype(f32)
        dbr = dt * bre_ref[rows, :].astype(f32)
        dbi = dt * bim_ref[rows, :].astype(f32)
        w = _cmul((cre_ref[rows, :].astype(f32), cim_ref[rows, :].astype(f32)), (dbr, dbi))

        def csq(a):
            ab = a[0] * a[1]
            return (a[0] * a[0] - a[1] * a[1], ab + ab)

        e1 = jnp.exp(lr)
        sn, cs = _sincos(li)
        z1 = (e1 * cs, e1 * sn)
        z8 = csq(csq(csq(z1)))
        z128 = csq(csq(csq(csq(z8))))
        z1024 = csq(csq(csq(z128)))

        def put_y(j, v):
            for g in range(CH // 8):
                yr_v[g, 8 * j:8 * j + 8, :] = v[0][8 * g:8 * g + 8, :]
                yi_v[g, 8 * j:8 * j + 8, :] = v[1][8 * g:8 * g + 8, :]

        def put_x(i, v):
            nvi = -v[1]
            for g in range(CH // 8):
                xr_v[g, 8 * i:8 * i + 8, :] = v[0][8 * g:8 * g + 8, :]
                xi_v[g, 8 * i:8 * i + 8, :] = nvi[8 * g:8 * g + 8, :]

        put_y(0, (jnp.ones_like(lr), jnp.zeros_like(lr)))
        y = z8
        put_y(1, y)
        for j in range(2, 16):
            y = _cmul(y, z8)
            put_y(j, y)
        v = w
        for b in range(8):
            if b:
                v = _cmul(v, z1)
            t = v
            for k in range(8):
                if (128 * k + b) in HI:
                    if k:
                        t = _cmul(t, z128)
                    put_x(HI.index(128 * k + b), t)
        t = _cmul(w, z1024)
        for k in range(8, 17):
            if k > 8:
                t = _cmul(t, z128)
            put_x(HI.index(128 * k), t)
        for g in range(CH // 8):
            o = (_dot_nt(_bf(xr_v[g]), _bf(yr_v[g])) + _dot_nt(_bf(xi_v[g]), _bf(yi_v[g])))
            for i in range(NHI):
                o_v[i, pl.ds(pl.multiple_of(r0 + 8 * g, 8), 8), :] = o[8 * i:8 * i + 8, :]
        return carry

    with jax.named_scope('p_kgen'):
        lax.fori_loop(0, D // CH, kgen, 0)

    rid = lax.broadcasted_iota(jnp.int32, (D, 128), 0)
    lid = lax.broadcasted_iota(jnp.int32, (D, 128), 1)
    keep = (rid % 8) == (lid % 8)
    keep_last = keep & (lid < 8)
    sel = sel_ref[...]
    with jax.named_scope('p_sel'):
        for i in range(NHI):
            oi = jnp.where(keep_last if HI[i] == 2048 else keep, o_v[i], 0.0)
            kd_v[16 * i:16 * i + 16, :] = _dot_nt(sel, _bf(oi))

    copies[2].wait()
    off = 0
    for dl in range(NB):
        s0, ln = WIN[dl]
        kt_v[dl] = _dot(g_v[:, off:off + ln], _bf(kd_v[s0:s0 + ln, :]))
        off += ln

    copies[0].wait()
    copies[1].wait()
    h_v[0:8, :] = jnp.zeros((8, D), jnp.float32)
    h_v[8 + L:16 + L, :] = jnp.zeros((8, D), jnp.float32)

    def phase1(b, carry):
        r0 = pl.multiple_of(b * RB, RB)
        x = x_v[pl.ds(r0, RB), :].astype(jnp.float32)
        xn = _bf(_layernorm(x))
        xn_v[pl.ds(r0, RB), :] = xn
        h = _gelu(_dot(xn, w1_v[...]))
        h_v[pl.ds(pl.multiple_of(r0 + 8, 8), RB), :] = h
        for k in range(RB // J):
            u_v[b * (RB // J) + k] = _dot(ffwd_ref[...], xn[k * J:(k + 1) * J, :])
        return carry

    with jax.named_scope('p_phase1'):
        lax.fori_loop(0, L // RB, phase1, 0)

    def zphase(t, carry):
        f0 = pl.multiple_of((t // 4) * 8, 8)
        re = pl.ds(f0, 8)
        im = pl.ds(pl.multiple_of(f0 + J, 8), 8)
        cs = pl.ds(pl.multiple_of((t % 4) * 128, 128), 128)
        GZ = 4
        for i0 in range(0, NB, GZ):
            acc = {}
            uc = {}
            for dl in range(i0 + GZ):
                kr = kt_v[dl, re, cs]
                ki = kt_v[dl, im, cs]
                ks = kr + ki
                for i in range(max(i0, dl), i0 + GZ):
                    src = i - dl
                    if src not in uc:
                        ur = u_v[src, re, cs]
                        ui = u_v[src, im, cs]
                        uc[src] = (ur, ui, ur + ui)
                    ur, ui, us = uc[src]
                    p = (kr * ur, ki * ui, ks * us)
                    acc[i] = p if i not in acc else tuple(x + y for x, y in zip(acc[i], p))
            for i in range(i0, i0 + GZ):
                s1, s2, s3 = acc[i]
                z_v[i, re, cs] = s1 - s2
                z_v[i, im, cs] = s3 - (s1 + s2)
        return carry

    with jax.named_scope('p_z'):
        lax.fori_loop(0, 64, zphase, 0)

    copies[3].wait()
    copies[4].wait()
    copies[5].wait()
    dsk = dsk_ref[...].astype(jnp.float32).reshape(1, D)

    def out_copy(b):
        r0 = pl.multiple_of(b * RB, RB)
        return pltpu.make_async_copy(out_v.at[pl.ds(r0, RB), :],
                                     out_hbm.at[pl.ds(r0, RB), :], sem_out.at[b])

    def phase2(b, carry):
        r0 = pl.multiple_of(b * RB, RB)
        ext = RB + 16
        parts = []
        for gi, sh in enumerate((1, -1, 2, -2)):
            hv = h_v[pl.ds(r0, ext), gi * 128:(gi + 1) * 128]
            hv = pltpu.roll(hv, sh % ext, 0)
            parts.append(_bf(hv[8:8 + RB, :]))
        hs = _dot(jnp.concatenate(parts, axis=1), w2_v[...])
        xn = xn_v[pl.ds(r0, RB), :].astype(jnp.float32)
        x1 = xn + hs
        a = _dot_nt(_bf(_layernorm2(x1)), w3_v[...])
        h2 = _dot(_bf(_gelu(a)), w4_v[...])
        bb = x1 + h2
        gate = bb * jax.nn.sigmoid(bb)
        ys = [_dot(finv_ref[...], _bf(z_v[b * (RB // J) + k])) for k in range(RB // J)]
        y = jnp.concatenate(ys, axis=0)
        s = y + xn * dsk
        x = x_v[pl.ds(r0, RB), :].astype(jnp.float32)
        out_v[pl.ds(r0, RB), :] = _bf(x + s * gate)
        out_copy(b).start()
        return carry

    with jax.named_scope('p_phase2'):
        lax.fori_loop(0, L // RB, phase2, 0)
    for b in range(L // RB):
        out_copy(b).wait()


@jax.jit
def pallas_recurrent_scan__ssm_conv_s4__mixer_s_mlp__prompt_kernel(
    A_u: jax.Array,
    A_A_re: jax.Array,
    A_A_im: jax.Array,
    A_B_re: jax.Array,
    A_B_im: jax.Array,
    A_C_re: jax.Array,
    A_C_im: jax.Array,
    A_log_dt: jax.Array,
    A_Dskip: jax.Array,
    B_x: jax.Array,
    B_w1: jax.Array,
    B_w2: jax.Array,
    B_w3: jax.Array,
    B_w4: jax.Array,
):
    bf16 = jnp.bfloat16
    f32 = jnp.float32
    x = A_u.reshape(L, D)
    vm = pl.BlockSpec(memory_space=pltpu.VMEM)
    hbm = pl.BlockSpec(memory_space=pltpu.HBM)
    out = pl.pallas_call(
        _kernel,
        out_shape=jax.ShapeDtypeStruct((L, D), bf16),
        in_specs=[vm] * 11 + [hbm] * 6,
        out_specs=hbm,
        scratch_shapes=[
            pltpu.VMEM((L, D), bf16),
            pltpu.VMEM((D, D), bf16),
            pltpu.VMEM((D, D), bf16),
            pltpu.VMEM((FF, D), bf16),
            pltpu.VMEM((FF, D), bf16),
            pltpu.VMEM((2 * J, GW), bf16),
            pltpu.VMEM((L, D), bf16),
            pltpu.VMEM((L, D), bf16),
            pltpu.VMEM((L + 16, D), f32),
            pltpu.VMEM((NB, 2 * J, D), f32),
            pltpu.VMEM((NB, 2 * J, D), f32),
            pltpu.VMEM((NB, 2 * J, D), f32),
            pltpu.VMEM((CH // 8, 128, N), f32),
            pltpu.VMEM((CH // 8, 128, N), f32),
            pltpu.VMEM((CH // 8, 8 * NHI, N), f32),
            pltpu.VMEM((CH // 8, 8 * NHI, N), f32),
            pltpu.VMEM((NHI, D, 128), f32),
            pltpu.VMEM((NQ, D), f32),
            pltpu.VMEM((D, N), f32),
            pltpu.SemaphoreType.DMA((6,)),
            pltpu.SemaphoreType.DMA((L // RB,)),
        ],
        compiler_params=pltpu.CompilerParams(vmem_limit_bytes=100 * 1024 * 1024),
    )(A_A_re, A_A_im, A_B_re, A_B_im, A_C_re, A_C_im,
      A_log_dt, A_Dskip,
      jnp.asarray(_F_FWD, bf16), jnp.asarray(_F_INV, bf16), jnp.asarray(_SEL, bf16),
      *[pltpu.with_memory_space_constraint(t, pltpu.HBM)
        for t in (x, B_w1, B_w2, B_w3.T, B_w4, jnp.asarray(_G_ALL, bf16))])
    return out.reshape(1, L, D)
```

```python
import functools
import numpy as np
import jax
import jax.numpy as jnp
from jax import lax
import jax.experimental.pallas as pl
import jax.experimental.pallas.tpu as pltpu

L = 2048
D = 512
N = 128
FF = 1376
J = 128
NB = L // J
NQ = 656
_STEP = (1, 1, 2, 2, 4, 4, 4, 4, 8, 8, 8, 8, 8, 8, 8, 8)
HI = tuple(128 * k + b for k in range(16) for b in range(0, 8, _STEP[k])) + (2048,)
NHI = len(HI)
CH = 32
RB = 512
WIN = ((0, 128), (0, 256), (128, 256), (256, 256), (320, 128), (384, 128),
       (384, 128), (448, 128), (448, 128), (512, 128), (512, 128), (512, 128),
       (512, 128), (512, 128), (512, 128), (528, 128))
GW = sum(w[1] for w in WIN)


def _q_of_m(m):
    hi = (m // 128) * 128 + (m % 8)
    return 16 * HI.index(hi) + (m % 128) // 8


def _build_tables():
    pos = np.arange(L, dtype=np.int64)
    rr = np.zeros(L, np.int64)
    for l in range(L):
        if l < 256:
            rr[l] = l
        else:
            step = 1 << (int(l).bit_length() - 8)
            lo = (l // step) * step
            rem = l - lo
            if rem * 2 < step or (rem * 2 == step and (lo // step) % 2 == 0):
                rr[l] = lo
            else:
                rr[l] = lo + step
    w = np.pi * (2 * np.arange(J) + 1) / (2 * J)
    n = np.arange(J)
    f_fwd = np.concatenate([np.cos(np.outer(w, n)), -np.sin(np.outer(w, n))], 0)
    f_inv = np.concatenate([np.cos(np.outer(n, w)), -np.sin(np.outer(n, w))], 1) / J
    g_all = np.zeros((2 * J, GW))
    off = 0
    for dl in range(NB):
        s0, ln = WIN[dl]
        for p in range(-J, J):
            l = dl * J + p
            if 0 <= l < L:
                q = _q_of_m(int(rr[l])) - s0
                assert 0 <= q < ln
                g_all[:J, off + q] += np.cos(w * p)
                g_all[J:, off + q] += -np.sin(w * p)
        off += ln
    sel = np.zeros((16, 128))
    for dd in range(8):
        sel[np.arange(16), np.arange(16) * 8 + dd] = 1.0
    del pos
    return (f_fwd.astype(np.float32), f_inv.astype(np.float32),
            g_all.astype(np.float32), sel.astype(np.float32))


_F_FWD, _F_INV, _G_ALL, _SEL = _build_tables()


def _bf(x):
    return x.astype(jnp.bfloat16)


def _rb(x):
    return x.astype(jnp.bfloat16).astype(jnp.float32)


def _cmul(a, b):
    return (a[0] * b[0] - a[1] * b[1], a[0] * b[1] + a[1] * b[0])


def _sincos(x):
    k = jnp.floor(x * 0.6366197723675814 + 0.5)
    r = x - k * 1.5703125
    r = r - k * 4.837512969970703125e-4
    r = r - k * 7.549789954891882e-8
    r2 = r * r
    sn = r + r * r2 * (-1.6666654611e-1 + r2 * (8.3321608736e-3 + r2 * -1.9515295891e-4))
    cs = 1.0 + r2 * (-0.5 + r2 * (4.166664568298827e-2 + r2 * (-1.388731625493765e-3
                                                             + r2 * 2.443315711809948e-5)))
    q = k - 4.0 * jnp.floor(k * 0.25)
    odd = (q == 1.0) | (q == 3.0)
    s0 = jnp.where(odd, cs, sn)
    c0 = jnp.where(odd, sn, cs)
    s1 = jnp.where(q >= 2.0, -s0, s0)
    c1 = jnp.where((q == 1.0) | (q == 2.0), -c0, c0)
    return s1, c1


def _gelu(x):
    c = 0.7978845608028654
    return 0.5 * x * (1.0 + jnp.tanh(c * (x + 0.044715 * (x * x * x))))


def _layernorm(x):
    m = jnp.mean(x, axis=-1, keepdims=True)
    xc = x - m
    v = jnp.mean(xc * xc, axis=-1, keepdims=True)
    den = _rb(jnp.sqrt(_rb(_rb(v) + 1e-5)))
    return _rb(_rb(x - _rb(m)) / den)


def _layernorm2(x):
    m = jnp.mean(x, axis=-1, keepdims=True)
    xc = x - m
    v = jnp.mean(xc * xc, axis=-1, keepdims=True)
    return xc / jnp.sqrt(v + 1e-5)


def _dot(a, b):
    return jnp.dot(a, b, preferred_element_type=jnp.float32)


def _dot_nt(a, b):
    return lax.dot_general(a, b, (((1,), (1,)), ((), ())),
                           preferred_element_type=jnp.float32)


def _kernel(are_ref, aim_ref, bre_ref, bim_ref, cre_ref, cim_ref, ldt_ref, dsk_ref,
            ffwd_ref, finv_ref, sel_ref,
            x_hbm, w1_hbm, w2_hbm, w3_hbm, w4_hbm, g_hbm,
            out_hbm,
            x_v, w1_v, w2_v, w3_v, w4_v, g_v, out_v,
            xn_v, h_v, u_v, kt_v, z_v,
            yr_v, yi_v, xr_v, xi_v, o_v, kd_v, dt_v,
            sem_in, sem_out):
    copies = [pltpu.make_async_copy(s, d, sem_in.at[k]) for k, (s, d) in enumerate(
        [(x_hbm, x_v), (w1_hbm, w1_v), (g_hbm, g_v), (w2_hbm, w2_v), (w3_hbm, w3_v),
         (w4_hbm, w4_v)])]
    for c in copies:
        c.start()

    dt_row = _rb(jnp.exp(ldt_ref[...].astype(jnp.float32))).reshape(1, D)
    dt_v[...] = jnp.transpose(jnp.broadcast_to(dt_row, (N, D)))

    def kgen_powers(c):
        slot = c % 2
        r0 = pl.multiple_of(c * CH, CH)
        rows = pl.ds(r0, CH)
        f32 = jnp.float32
        dt = dt_v[rows, :]
        lr = dt * are_ref[rows, :].astype(f32)
        li = dt * aim_ref[rows, :].astype(f32)
        dbr = dt * bre_ref[rows, :].astype(f32)
        dbi = dt * bim_ref[rows, :].astype(f32)
        w = _cmul((cre_ref[rows, :].astype(f32), cim_ref[rows, :].astype(f32)), (dbr, dbi))

        def csq(a):
            ab = a[0] * a[1]
            return (a[0] * a[0] - a[1] * a[1], ab + ab)

        e1 = jnp.exp(lr)
        sn, cs = _sincos(li)
        z1 = (e1 * cs, e1 * sn)
        z8 = csq(csq(csq(z1)))
        z128 = csq(csq(csq(csq(z8))))
        z1024 = csq(csq(csq(z128)))

        def put_y(j, v):
            for g in range(CH // 8):
                yr_v[slot, g, 8 * j:8 * j + 8, :] = v[0][8 * g:8 * g + 8, :]
                yi_v[slot, g, 8 * j:8 * j + 8, :] = v[1][8 * g:8 * g + 8, :]

        def put_x(i, v):
            nvi = -v[1]
            for g in range(CH // 8):
                xr_v[slot, g, 8 * i:8 * i + 8, :] = v[0][8 * g:8 * g + 8, :]
                xi_v[slot, g, 8 * i:8 * i + 8, :] = nvi[8 * g:8 * g + 8, :]

        put_y(0, (jnp.ones_like(lr), jnp.zeros_like(lr)))
        y = z8
        put_y(1, y)
        yield
        for j in range(2, 16):
            y = _cmul(y, z8)
            put_y(j, y)
        yield
        v = w
        for b in range(8):
            if b:
                v = _cmul(v, z1)
            t = v
            for k in range(8):
                if (128 * k + b) in HI:
                    if k:
                        t = _cmul(t, z128)
                    put_x(HI.index(128 * k + b), t)
            if b in (0, 3):
                yield
        t = _cmul(w, z1024)
        for k in range(8, 17):
            if k > 8:
                t = _cmul(t, z128)
            put_x(HI.index(128 * k), t)

    def kgen_mm(c, g):
        slot = c % 2
        o = (_dot_nt(_bf(xr_v[slot, g]), _bf(yr_v[slot, g]))
             + _dot_nt(_bf(xi_v[slot, g]), _bf(yi_v[slot, g])))
        for i in range(NHI):
            o_v[i, pl.ds(pl.multiple_of(c * CH + 8 * g, 8), 8), :] = o[8 * i:8 * i + 8, :]

    def kgen(c, carry):
        g = 0
        for _ in kgen_powers(c):
            kgen_mm(c - 1, g)
            g += 1
        assert g == CH // 8
        return carry

    with jax.named_scope('p_kgen'):
        for _ in kgen_powers(0):
            pass
        lax.fori_loop(1, D // CH, kgen, 0)
        for g in range(CH // 8):
            kgen_mm(D // CH - 1, g)

    rid = lax.broadcasted_iota(jnp.int32, (D, 128), 0)
    lid = lax.broadcasted_iota(jnp.int32, (D, 128), 1)
    keep = (rid % 8) == (lid % 8)
    keep_last = keep & (lid < 8)
    sel = sel_ref[...]
    with jax.named_scope('p_sel'):
        for i in range(NHI):
            oi = jnp.where(keep_last if HI[i] == 2048 else keep, o_v[i], 0.0)
            kd_v[16 * i:16 * i + 16, :] = _dot_nt(sel, _bf(oi))

    copies[2].wait()
    off = 0
    for dl in range(NB):
        s0, ln = WIN[dl]
        kt_v[dl] = _dot(g_v[:, off:off + ln], _bf(kd_v[s0:s0 + ln, :]))
        off += ln

    copies[0].wait()
    copies[1].wait()
    h_v[0:8, :] = jnp.zeros((8, D), jnp.float32)
    h_v[8 + L:16 + L, :] = jnp.zeros((8, D), jnp.float32)

    def phase1(b, carry):
        r0 = pl.multiple_of(b * RB, RB)
        x = x_v[pl.ds(r0, RB), :].astype(jnp.float32)
        xn = _bf(_layernorm(x))
        xn_v[pl.ds(r0, RB), :] = xn
        h = _gelu(_dot(xn, w1_v[...]))
        h_v[pl.ds(pl.multiple_of(r0 + 8, 8), RB), :] = h
        for k in range(RB // J):
            u_v[b * (RB // J) + k] = _dot(ffwd_ref[...], xn[k * J:(k + 1) * J, :])
        return carry

    with jax.named_scope('p_phase1'):
        lax.fori_loop(0, L // RB, phase1, 0)

    def zphase(t, carry):
        f0 = pl.multiple_of((t // 4) * 8, 8)
        re = pl.ds(f0, 8)
        im = pl.ds(pl.multiple_of(f0 + J, 8), 8)
        cs = pl.ds(pl.multiple_of((t % 4) * 128, 128), 128)
        GZ = 4
        for i0 in range(0, NB, GZ):
            acc = {}
            uc = {}
            for dl in range(i0 + GZ):
                kr = kt_v[dl, re, cs]
                ki = kt_v[dl, im, cs]
                ks = kr + ki
                for i in range(max(i0, dl), i0 + GZ):
                    src = i - dl
                    if src not in uc:
                        ur = u_v[src, re, cs]
                        ui = u_v[src, im, cs]
                        uc[src] = (ur, ui, ur + ui)
                    ur, ui, us = uc[src]
                    p = (kr * ur, ki * ui, ks * us)
                    acc[i] = p if i not in acc else tuple(x + y for x, y in zip(acc[i], p))
            for i in range(i0, i0 + GZ):
                s1, s2, s3 = acc[i]
                z_v[i, re, cs] = s1 - s2
                z_v[i, im, cs] = s3 - (s1 + s2)
        return carry

    with jax.named_scope('p_z'):
        lax.fori_loop(0, 64, zphase, 0)

    copies[3].wait()
    copies[4].wait()
    copies[5].wait()
    dsk = dsk_ref[...].astype(jnp.float32).reshape(1, D)

    def out_copy(b):
        r0 = pl.multiple_of(b * RB, RB)
        return pltpu.make_async_copy(out_v.at[pl.ds(r0, RB), :],
                                     out_hbm.at[pl.ds(r0, RB), :], sem_out.at[b])

    def phase2(b, carry):
        r0 = pl.multiple_of(b * RB, RB)
        ext = RB + 16
        parts = []
        for gi, sh in enumerate((1, -1, 2, -2)):
            hv = h_v[pl.ds(r0, ext), gi * 128:(gi + 1) * 128]
            hv = pltpu.roll(hv, sh % ext, 0)
            parts.append(_bf(hv[8:8 + RB, :]))
        hs = _dot(jnp.concatenate(parts, axis=1), w2_v[...])
        xn = xn_v[pl.ds(r0, RB), :].astype(jnp.float32)
        x1 = xn + hs
        a = _dot_nt(_bf(_layernorm2(x1)), w3_v[...])
        h2 = _dot(_bf(_gelu(a)), w4_v[...])
        bb = x1 + h2
        gate = bb * jax.nn.sigmoid(bb)
        ys = [_dot(finv_ref[...], _bf(z_v[b * (RB // J) + k])) for k in range(RB // J)]
        y = jnp.concatenate(ys, axis=0)
        s = y + xn * dsk
        x = x_v[pl.ds(r0, RB), :].astype(jnp.float32)
        out_v[pl.ds(r0, RB), :] = _bf(x + s * gate)
        out_copy(b).start()
        return carry

    with jax.named_scope('p_phase2'):
        lax.fori_loop(0, L // RB, phase2, 0)
    for b in range(L // RB):
        out_copy(b).wait()


@jax.jit
def pallas_recurrent_scan__ssm_conv_s4__mixer_s_mlp__prompt_kernel(
    A_u: jax.Array,
    A_A_re: jax.Array,
    A_A_im: jax.Array,
    A_B_re: jax.Array,
    A_B_im: jax.Array,
    A_C_re: jax.Array,
    A_C_im: jax.Array,
    A_log_dt: jax.Array,
    A_Dskip: jax.Array,
    B_x: jax.Array,
    B_w1: jax.Array,
    B_w2: jax.Array,
    B_w3: jax.Array,
    B_w4: jax.Array,
):
    bf16 = jnp.bfloat16
    f32 = jnp.float32
    x = A_u.reshape(L, D)
    vm = pl.BlockSpec(memory_space=pltpu.VMEM)
    hbm = pl.BlockSpec(memory_space=pltpu.HBM)
    out = pl.pallas_call(
        _kernel,
        out_shape=jax.ShapeDtypeStruct((L, D), bf16),
        in_specs=[vm] * 11 + [hbm] * 6,
        out_specs=hbm,
        scratch_shapes=[
            pltpu.VMEM((L, D), bf16),
            pltpu.VMEM((D, D), bf16),
            pltpu.VMEM((D, D), bf16),
            pltpu.VMEM((FF, D), bf16),
            pltpu.VMEM((FF, D), bf16),
            pltpu.VMEM((2 * J, GW), bf16),
            pltpu.VMEM((L, D), bf16),
            pltpu.VMEM((L, D), bf16),
            pltpu.VMEM((L + 16, D), f32),
            pltpu.VMEM((NB, 2 * J, D), f32),
            pltpu.VMEM((NB, 2 * J, D), f32),
            pltpu.VMEM((NB, 2 * J, D), f32),
            pltpu.VMEM((2, CH // 8, 128, N), f32),
            pltpu.VMEM((2, CH // 8, 128, N), f32),
            pltpu.VMEM((2, CH // 8, 8 * NHI, N), f32),
            pltpu.VMEM((2, CH // 8, 8 * NHI, N), f32),
            pltpu.VMEM((NHI, D, 128), f32),
            pltpu.VMEM((NQ, D), f32),
            pltpu.VMEM((D, N), f32),
            pltpu.SemaphoreType.DMA((6,)),
            pltpu.SemaphoreType.DMA((L // RB,)),
        ],
        compiler_params=pltpu.CompilerParams(vmem_limit_bytes=100 * 1024 * 1024),
    )(A_A_re, A_A_im, A_B_re, A_B_im, A_C_re, A_C_im,
      A_log_dt, A_Dskip,
      jnp.asarray(_F_FWD, bf16), jnp.asarray(_F_INV, bf16), jnp.asarray(_SEL, bf16),
      *[pltpu.with_memory_space_constraint(t, pltpu.HBM)
        for t in (x, B_w1, B_w2, B_w3.T, B_w4, jnp.asarray(_G_ALL, bf16))])
    return out.reshape(1, L, D)
```

```python
import functools
import numpy as np
import jax
import jax.numpy as jnp
from jax import lax
import jax.experimental.pallas as pl
import jax.experimental.pallas.tpu as pltpu

L = 2048
D = 512
N = 128
FF = 1376
J = 128
NB = L // J
NQ = 656
_STEP = (1, 1, 2, 2, 4, 4, 4, 4, 8, 8, 8, 8, 8, 8, 8, 8)
HI = tuple(128 * k + b for k in range(16) for b in range(0, 8, _STEP[k])) + (2048,)
NHI = len(HI)
CH = 32
RB = 512
WIN = ((0, 128), (0, 256), (128, 256), (256, 256), (320, 128), (384, 128),
       (384, 128), (448, 128), (448, 128), (512, 128), (512, 128), (512, 128),
       (512, 128), (512, 128), (512, 128), (528, 128))
GW = sum(w[1] for w in WIN)


def _q_of_m(m):
    hi = (m // 128) * 128 + (m % 8)
    return 16 * HI.index(hi) + (m % 128) // 8


def _build_tables():
    pos = np.arange(L, dtype=np.int64)
    rr = np.zeros(L, np.int64)
    for l in range(L):
        if l < 256:
            rr[l] = l
        else:
            step = 1 << (int(l).bit_length() - 8)
            lo = (l // step) * step
            rem = l - lo
            if rem * 2 < step or (rem * 2 == step and (lo // step) % 2 == 0):
                rr[l] = lo
            else:
                rr[l] = lo + step
    w = np.pi * (2 * np.arange(J) + 1) / (2 * J)
    n = np.arange(J)
    f_fwd = np.concatenate([np.cos(np.outer(w, n)), -np.sin(np.outer(w, n))], 0)
    f_inv = np.concatenate([np.cos(np.outer(n, w)), -np.sin(np.outer(n, w))], 1) / J
    g_all = np.zeros((2 * J, GW))
    off = 0
    for dl in range(NB):
        s0, ln = WIN[dl]
        for p in range(-J, J):
            l = dl * J + p
            if 0 <= l < L:
                q = _q_of_m(int(rr[l])) - s0
                assert 0 <= q < ln
                g_all[:J, off + q] += np.cos(w * p)
                g_all[J:, off + q] += -np.sin(w * p)
        off += ln
    sel = np.zeros((16, 128))
    for dd in range(8):
        sel[np.arange(16), np.arange(16) * 8 + dd] = 1.0
    del pos
    return (f_fwd.astype(np.float32), f_inv.astype(np.float32),
            g_all.astype(np.float32), sel.astype(np.float32))


_F_FWD, _F_INV, _G_ALL, _SEL = _build_tables()


def _bf(x):
    return x.astype(jnp.bfloat16)


def _rb(x):
    return x.astype(jnp.bfloat16).astype(jnp.float32)


def _cmul(a, b):
    return (a[0] * b[0] - a[1] * b[1], a[0] * b[1] + a[1] * b[0])


def _sincos(x):
    k = jnp.floor(x * 0.6366197723675814 + 0.5)
    r = x - k * 1.5703125
    r = r - k * 4.837512969970703125e-4
    r = r - k * 7.549789954891882e-8
    r2 = r * r
    sn = r + r * r2 * (-1.6666654611e-1 + r2 * (8.3321608736e-3 + r2 * -1.9515295891e-4))
    cs = 1.0 + r2 * (-0.5 + r2 * (4.166664568298827e-2 + r2 * (-1.388731625493765e-3
                                                             + r2 * 2.443315711809948e-5)))
    q = k - 4.0 * jnp.floor(k * 0.25)
    odd = (q == 1.0) | (q == 3.0)
    s0 = jnp.where(odd, cs, sn)
    c0 = jnp.where(odd, sn, cs)
    s1 = jnp.where(q >= 2.0, -s0, s0)
    c1 = jnp.where((q == 1.0) | (q == 2.0), -c0, c0)
    return s1, c1


def _gelu(x):
    c = 0.7978845608028654
    return 0.5 * x * (1.0 + jnp.tanh(c * (x + 0.044715 * (x * x * x))))


def _layernorm(x):
    m = jnp.mean(x, axis=-1, keepdims=True)
    xc = x - m
    v = jnp.mean(xc * xc, axis=-1, keepdims=True)
    den = _rb(jnp.sqrt(_rb(_rb(v) + 1e-5)))
    return _rb(_rb(x - _rb(m)) / den)


def _layernorm2(x):
    m = jnp.mean(x, axis=-1, keepdims=True)
    xc = x - m
    v = jnp.mean(xc * xc, axis=-1, keepdims=True)
    return xc / jnp.sqrt(v + 1e-5)


def _dot(a, b):
    return jnp.dot(a, b, preferred_element_type=jnp.float32)


def _dot_nt(a, b):
    return lax.dot_general(a, b, (((1,), (1,)), ((), ())),
                           preferred_element_type=jnp.float32)


def _kernel(are_ref, aim_ref, bre_ref, bim_ref, cre_ref, cim_ref, ldt_ref, dsk_ref,
            ffwd_ref, finv_ref, sel_ref,
            x_hbm, w1_hbm, w2_hbm, w3_hbm, w4_hbm, g_hbm,
            out_hbm,
            x_v, w1_v, w2_v, w3_v, w4_v, g_v, out_v,
            xn_v, h_v, u_v, kt_v, z_v,
            yr_v, yi_v, xr_v, xi_v, o_v, kd_v, dt_v,
            sem_in, sem_out):
    copies = [pltpu.make_async_copy(s, d, sem_in.at[k]) for k, (s, d) in enumerate(
        [(x_hbm, x_v), (w1_hbm, w1_v), (g_hbm, g_v), (w2_hbm, w2_v), (w3_hbm, w3_v),
         (w4_hbm, w4_v)])]
    for c in copies:
        c.start()

    dt_row = _rb(jnp.exp(ldt_ref[...].astype(jnp.float32))).reshape(1, D)
    dt_v[...] = jnp.transpose(jnp.broadcast_to(dt_row, (N, D)))

    def kgen(c, carry):
        r0 = pl.multiple_of(c * CH, CH)
        rows = pl.ds(r0, CH)
        f32 = jnp.float32
        dt = dt_v[rows, :]
        lr = dt * are_ref[rows, :].astype(f32)
        li = dt * aim_ref[rows, :].astype(f32)
        dbr = dt * bre_ref[rows, :].astype(f32)
        dbi = dt * bim_ref[rows, :].astype(f32)
        w = _cmul((cre_ref[rows, :].astype(f32), cim_ref[rows, :].astype(f32)), (dbr, dbi))

        def csq(a):
            ab = a[0] * a[1]
            return (a[0] * a[0] - a[1] * a[1], ab + ab)

        e1 = jnp.exp(lr)
        sn, cs = _sincos(li)
        z1 = (e1 * cs, e1 * sn)
        z8 = csq(csq(csq(z1)))
        z128 = csq(csq(csq(csq(z8))))
        z1024 = csq(csq(csq(z128)))

        def put_y(j, v):
            for g in range(CH // 8):
                yr_v[g, 8 * j:8 * j + 8, :] = v[0][8 * g:8 * g + 8, :]
                yi_v[g, 8 * j:8 * j + 8, :] = v[1][8 * g:8 * g + 8, :]

        def put_x(i, v):
            nvi = -v[1]
            for g in range(CH // 8):
                xr_v[g, 8 * i:8 * i + 8, :] = v[0][8 * g:8 * g + 8, :]
                xi_v[g, 8 * i:8 * i + 8, :] = nvi[8 * g:8 * g + 8, :]

        put_y(0, (jnp.ones_like(lr), jnp.zeros_like(lr)))
        y = z8
        put_y(1, y)
        for j in range(2, 16):
            y = _cmul(y, z8)
            put_y(j, y)
        v = w
        for b in range(8):
            if b:
                v = _cmul(v, z1)
            t = v
            for k in range(8):
                if (128 * k + b) in HI:
                    if k:
                        t = _cmul(t, z128)
                    put_x(HI.index(128 * k + b), t)
        t = _cmul(w, z1024)
        for k in range(8, 17):
            if k > 8:
                t = _cmul(t, z128)
            put_x(HI.index(128 * k), t)
        for g in range(CH // 8):
            o = (_dot_nt(_bf(xr_v[g]), _bf(yr_v[g])) + _dot_nt(_bf(xi_v[g]), _bf(yi_v[g])))
            for i in range(NHI):
                o_v[i, pl.ds(pl.multiple_of(r0 + 8 * g, 8), 8), :] = o[8 * i:8 * i + 8, :]
        return carry

    with jax.named_scope('p_kgen'):
        lax.fori_loop(0, D // CH, kgen, 0)

    rid = lax.broadcasted_iota(jnp.int32, (D, 128), 0)
    lid = lax.broadcasted_iota(jnp.int32, (D, 128), 1)
    keep = (rid % 8) == (lid % 8)
    keep_last = keep & (lid < 8)
    sel = sel_ref[...]
    with jax.named_scope('p_sel'):
        for i in range(NHI):
            oi = jnp.where(keep_last if HI[i] == 2048 else keep, o_v[i], 0.0)
            kd_v[16 * i:16 * i + 16, :] = _dot_nt(sel, _bf(oi))

    copies[2].wait()
    off = 0
    for dl in range(NB):
        s0, ln = WIN[dl]
        kt_v[dl] = _dot(g_v[:, off:off + ln], _bf(kd_v[s0:s0 + ln, :]))
        off += ln

    copies[0].wait()
    copies[1].wait()
    h_v[0:8, :] = jnp.zeros((8, D), jnp.float32)
    h_v[8 + L:16 + L, :] = jnp.zeros((8, D), jnp.float32)

    def phase1(b, carry):
        r0 = pl.multiple_of(b * RB, RB)
        xs = []
        for k in range(RB // J):
            rk = pl.multiple_of(r0 + k * J, J)
            xk = _bf(_layernorm(x_v[pl.ds(rk, J), :].astype(jnp.float32)))
            xn_v[pl.ds(rk, J), :] = xk
            u_v[b * (RB // J) + k] = _dot(ffwd_ref[...], xk)
            xs.append(xk)
        h = _gelu(_dot(jnp.concatenate(xs, axis=0), w1_v[...]))
        h_v[pl.ds(pl.multiple_of(r0 + 8, 8), RB), :] = h
        return carry

    with jax.named_scope('p_phase1'):
        lax.fori_loop(0, L // RB, phase1, 0)

    def zphase(t, carry):
        f0 = pl.multiple_of((t // 4) * 8, 8)
        re = pl.ds(f0, 8)
        im = pl.ds(pl.multiple_of(f0 + J, 8), 8)
        cs = pl.ds(pl.multiple_of((t % 4) * 128, 128), 128)
        GZ = 4
        for i0 in range(0, NB, GZ):
            acc = {}
            uc = {}
            for dl in range(i0 + GZ):
                kr = kt_v[dl, re, cs]
                ki = kt_v[dl, im, cs]
                ks = kr + ki
                for i in range(max(i0, dl), i0 + GZ):
                    src = i - dl
                    if src not in uc:
                        ur = u_v[src, re, cs]
                        ui = u_v[src, im, cs]
                        uc[src] = (ur, ui, ur + ui)
                    ur, ui, us = uc[src]
                    p = (kr * ur, ki * ui, ks * us)
                    acc[i] = p if i not in acc else tuple(x + y for x, y in zip(acc[i], p))
            for i in range(i0, i0 + GZ):
                s1, s2, s3 = acc[i]
                z_v[i, re, cs] = s1 - s2
                z_v[i, im, cs] = s3 - (s1 + s2)
        return carry

    with jax.named_scope('p_z'):
        lax.fori_loop(0, 64, zphase, 0)

    copies[3].wait()
    copies[4].wait()
    copies[5].wait()
    dsk = dsk_ref[...].astype(jnp.float32).reshape(1, D)

    def out_copy(b):
        r0 = pl.multiple_of(b * RB, RB)
        return pltpu.make_async_copy(out_v.at[pl.ds(r0, RB), :],
                                     out_hbm.at[pl.ds(r0, RB), :], sem_out.at[b])

    def phase2(b, carry):
        r0 = pl.multiple_of(b * RB, RB)
        ext = RB + 16
        parts = []
        for gi, sh in enumerate((1, -1, 2, -2)):
            hv = h_v[pl.ds(r0, ext), gi * 128:(gi + 1) * 128]
            hv = pltpu.roll(hv, sh % ext, 0)
            parts.append(_bf(hv[8:8 + RB, :]))
        hs = _dot(jnp.concatenate(parts, axis=1), w2_v[...])
        ys = [_dot(finv_ref[...], _bf(z_v[b * (RB // J) + k])) for k in range(RB // J)]
        y = jnp.concatenate(ys, axis=0)
        xn = xn_v[pl.ds(r0, RB), :].astype(jnp.float32)
        x1 = xn + hs
        a = _dot_nt(_bf(_layernorm2(x1)), w3_v[...])
        h2 = _dot(_bf(_gelu(a)), w4_v[...])
        bb = x1 + h2
        gate = bb * jax.nn.sigmoid(bb)
        s = y + xn * dsk
        x = x_v[pl.ds(r0, RB), :].astype(jnp.float32)
        out_v[pl.ds(r0, RB), :] = _bf(x + s * gate)
        out_copy(b).start()
        return carry

    with jax.named_scope('p_phase2'):
        lax.fori_loop(0, L // RB, phase2, 0)
    for b in range(L // RB):
        out_copy(b).wait()


@jax.jit
def pallas_recurrent_scan__ssm_conv_s4__mixer_s_mlp__prompt_kernel(
    A_u: jax.Array,
    A_A_re: jax.Array,
    A_A_im: jax.Array,
    A_B_re: jax.Array,
    A_B_im: jax.Array,
    A_C_re: jax.Array,
    A_C_im: jax.Array,
    A_log_dt: jax.Array,
    A_Dskip: jax.Array,
    B_x: jax.Array,
    B_w1: jax.Array,
    B_w2: jax.Array,
    B_w3: jax.Array,
    B_w4: jax.Array,
):
    bf16 = jnp.bfloat16
    f32 = jnp.float32
    x = A_u.reshape(L, D)
    vm = pl.BlockSpec(memory_space=pltpu.VMEM)
    hbm = pl.BlockSpec(memory_space=pltpu.HBM)
    out = pl.pallas_call(
        _kernel,
        out_shape=jax.ShapeDtypeStruct((L, D), bf16),
        in_specs=[vm] * 11 + [hbm] * 6,
        out_specs=hbm,
        scratch_shapes=[
            pltpu.VMEM((L, D), bf16),
            pltpu.VMEM((D, D), bf16),
            pltpu.VMEM((D, D), bf16),
            pltpu.VMEM((FF, D), bf16),
            pltpu.VMEM((FF, D), bf16),
            pltpu.VMEM((2 * J, GW), bf16),
            pltpu.VMEM((L, D), bf16),
            pltpu.VMEM((L, D), bf16),
            pltpu.VMEM((L + 16, D), f32),
            pltpu.VMEM((NB, 2 * J, D), f32),
            pltpu.VMEM((NB, 2 * J, D), f32),
            pltpu.VMEM((NB, 2 * J, D), f32),
            pltpu.VMEM((CH // 8, 128, N), f32),
            pltpu.VMEM((CH // 8, 128, N), f32),
            pltpu.VMEM((CH // 8, 8 * NHI, N), f32),
            pltpu.VMEM((CH // 8, 8 * NHI, N), f32),
            pltpu.VMEM((NHI, D, 128), f32),
            pltpu.VMEM((NQ, D), f32),
            pltpu.VMEM((D, N), f32),
            pltpu.SemaphoreType.DMA((6,)),
            pltpu.SemaphoreType.DMA((L // RB,)),
        ],
        compiler_params=pltpu.CompilerParams(vmem_limit_bytes=100 * 1024 * 1024),
    )(A_A_re, A_A_im, A_B_re, A_B_im, A_C_re, A_C_im,
      A_log_dt, A_Dskip,
      jnp.asarray(_F_FWD, bf16), jnp.asarray(_F_INV, bf16), jnp.asarray(_SEL, bf16),
      *[pltpu.with_memory_space_constraint(t, pltpu.HBM)
        for t in (x, B_w1, B_w2, B_w3.T, B_w4, jnp.asarray(_G_ALL, bf16))])
    return out.reshape(1, L, D)
```

```python
import functools
import numpy as np
import jax
import jax.numpy as jnp
from jax import lax
import jax.experimental.pallas as pl
import jax.experimental.pallas.tpu as pltpu

L = 2048
D = 512
N = 128
FF = 1376
J = 128
NB = L // J
NQ = 656
_STEP = (1, 1, 2, 2, 4, 4, 4, 4, 8, 8, 8, 8, 8, 8, 8, 8)
HI = tuple(128 * k + b for k in range(16) for b in range(0, 8, _STEP[k])) + (2048,)
NHI = len(HI)
CH = 32
RB = 512
WIN = ((0, 128), (0, 256), (128, 256), (256, 256), (320, 128), (384, 128),
       (384, 128), (448, 128), (448, 128), (512, 128), (512, 128), (512, 128),
       (512, 128), (512, 128), (512, 128), (528, 128))
GW = sum(w[1] for w in WIN)


def _q_of_m(m):
    hi = (m // 128) * 128 + (m % 8)
    return 16 * HI.index(hi) + (m % 128) // 8


def _build_tables():
    pos = np.arange(L, dtype=np.int64)
    rr = np.zeros(L, np.int64)
    for l in range(L):
        if l < 256:
            rr[l] = l
        else:
            step = 1 << (int(l).bit_length() - 8)
            lo = (l // step) * step
            rem = l - lo
            if rem * 2 < step or (rem * 2 == step and (lo // step) % 2 == 0):
                rr[l] = lo
            else:
                rr[l] = lo + step
    w = np.pi * (2 * np.arange(J) + 1) / (2 * J)
    n = np.arange(J)
    f_fwd = np.concatenate([np.cos(np.outer(w, n)), -np.sin(np.outer(w, n))], 0)
    f_inv = np.concatenate([np.cos(np.outer(n, w)), -np.sin(np.outer(n, w))], 1) / J
    g_all = np.zeros((2 * J, GW))
    off = 0
    for dl in range(NB):
        s0, ln = WIN[dl]
        for p in range(-J, J):
            l = dl * J + p
            if 0 <= l < L:
                q = _q_of_m(int(rr[l])) - s0
                assert 0 <= q < ln
                g_all[:J, off + q] += np.cos(w * p)
                g_all[J:, off + q] += -np.sin(w * p)
        off += ln
    sel = np.zeros((16, 128))
    for dd in range(8):
        sel[np.arange(16), np.arange(16) * 8 + dd] = 1.0
    del pos
    return (f_fwd.astype(np.float32), f_inv.astype(np.float32),
            g_all.astype(np.float32), sel.astype(np.float32))


_F_FWD, _F_INV, _G_ALL, _SEL = _build_tables()


def _bf(x):
    return x.astype(jnp.bfloat16)


def _rb(x):
    return x.astype(jnp.bfloat16).astype(jnp.float32)


def _cmul(a, b):
    return (a[0] * b[0] - a[1] * b[1], a[0] * b[1] + a[1] * b[0])


def _sincos(x):
    k = jnp.floor(x * 0.6366197723675814 + 0.5)
    r = x - k * 1.5703125
    r = r - k * 4.837512969970703125e-4
    r = r - k * 7.549789954891882e-8
    r2 = r * r
    sn = r + r * r2 * (-1.6666654611e-1 + r2 * (8.3321608736e-3 + r2 * -1.9515295891e-4))
    cs = 1.0 + r2 * (-0.5 + r2 * (4.166664568298827e-2 + r2 * (-1.388731625493765e-3
                                                             + r2 * 2.443315711809948e-5)))
    q = k - 4.0 * jnp.floor(k * 0.25)
    odd = (q == 1.0) | (q == 3.0)
    s0 = jnp.where(odd, cs, sn)
    c0 = jnp.where(odd, sn, cs)
    s1 = jnp.where(q >= 2.0, -s0, s0)
    c1 = jnp.where((q == 1.0) | (q == 2.0), -c0, c0)
    return s1, c1


def _gelu(x):
    c = 0.7978845608028654
    return 0.5 * x * (1.0 + jnp.tanh(c * (x + 0.044715 * (x * x * x))))


def _layernorm(x):
    m = jnp.mean(x, axis=-1, keepdims=True)
    xc = x - m
    v = jnp.mean(xc * xc, axis=-1, keepdims=True)
    den = _rb(jnp.sqrt(_rb(_rb(v) + 1e-5)))
    return _rb(_rb(x - _rb(m)) / den)


def _layernorm2(x):
    m = jnp.mean(x, axis=-1, keepdims=True)
    xc = x - m
    v = jnp.mean(xc * xc, axis=-1, keepdims=True)
    return xc / jnp.sqrt(v + 1e-5)


def _dot(a, b):
    return jnp.dot(a, b, preferred_element_type=jnp.float32)


def _dot_nt(a, b):
    return lax.dot_general(a, b, (((1,), (1,)), ((), ())),
                           preferred_element_type=jnp.float32)


def _kernel(are_ref, aim_ref, bre_ref, bim_ref, cre_ref, cim_ref, ldt_ref, dsk_ref,
            ffwd_ref, finv_ref, sel_ref,
            x_hbm, w1_hbm, w2_hbm, w3_hbm, w4_hbm, g_hbm,
            out_hbm,
            x_v, w1_v, w2_v, w3_v, w4_v, g_v, out_v,
            xn_v, h_v, u_v, kt_v, z_v,
            yr_v, yi_v, xr_v, xi_v, o_v, kd_v, dt_v, gate_v,
            sem_in, sem_out):
    copies = [pltpu.make_async_copy(s, d, sem_in.at[k]) for k, (s, d) in enumerate(
        [(x_hbm, x_v), (w1_hbm, w1_v), (g_hbm, g_v), (w2_hbm, w2_v), (w3_hbm, w3_v),
         (w4_hbm, w4_v)])]
    for c in copies:
        c.start()

    dt_row = _rb(jnp.exp(ldt_ref[...].astype(jnp.float32))).reshape(1, D)
    dt_v[...] = jnp.transpose(jnp.broadcast_to(dt_row, (N, D)))

    def kgen(c, carry):
        r0 = pl.multiple_of(c * CH, CH)
        rows = pl.ds(r0, CH)
        f32 = jnp.float32
        dt = dt_v[rows, :]
        lr = dt * are_ref[rows, :].astype(f32)
        li = dt * aim_ref[rows, :].astype(f32)
        dbr = dt * bre_ref[rows, :].astype(f32)
        dbi = dt * bim_ref[rows, :].astype(f32)
        w = _cmul((cre_ref[rows, :].astype(f32), cim_ref[rows, :].astype(f32)), (dbr, dbi))

        def csq(a):
            ab = a[0] * a[1]
            return (a[0] * a[0] - a[1] * a[1], ab + ab)

        e1 = jnp.exp(lr)
        sn, cs = _sincos(li)
        z1 = (e1 * cs, e1 * sn)
        z8 = csq(csq(csq(z1)))
        z128 = csq(csq(csq(csq(z8))))
        z1024 = csq(csq(csq(z128)))

        def put_y(j, v):
            for g in range(CH // 8):
                yr_v[g, 8 * j:8 * j + 8, :] = v[0][8 * g:8 * g + 8, :]
                yi_v[g, 8 * j:8 * j + 8, :] = v[1][8 * g:8 * g + 8, :]

        def put_x(i, v):
            nvi = -v[1]
            for g in range(CH // 8):
                xr_v[g, 8 * i:8 * i + 8, :] = v[0][8 * g:8 * g + 8, :]
                xi_v[g, 8 * i:8 * i + 8, :] = nvi[8 * g:8 * g + 8, :]

        put_y(0, (jnp.ones_like(lr), jnp.zeros_like(lr)))
        y = z8
        put_y(1, y)
        for j in range(2, 16):
            y = _cmul(y, z8)
            put_y(j, y)
        v = w
        for b in range(8):
            if b:
                v = _cmul(v, z1)
            t = v
            for k in range(8):
                if (128 * k + b) in HI:
                    if k:
                        t = _cmul(t, z128)
                    put_x(HI.index(128 * k + b), t)
        t = _cmul(w, z1024)
        for k in range(8, 17):
            if k > 8:
                t = _cmul(t, z128)
            put_x(HI.index(128 * k), t)
        for g in range(CH // 8):
            o = (_dot_nt(_bf(xr_v[g]), _bf(yr_v[g])) + _dot_nt(_bf(xi_v[g]), _bf(yi_v[g])))
            for i in range(NHI):
                o_v[i, pl.ds(pl.multiple_of(r0 + 8 * g, 8), 8), :] = o[8 * i:8 * i + 8, :]
        return carry

    with jax.named_scope('p_kgen'):
        lax.fori_loop(0, D // CH, kgen, 0)

    rid = lax.broadcasted_iota(jnp.int32, (D, 128), 0)
    lid = lax.broadcasted_iota(jnp.int32, (D, 128), 1)
    keep = (rid % 8) == (lid % 8)
    keep_last = keep & (lid < 8)
    sel = sel_ref[...]
    with jax.named_scope('p_sel'):
        for i in range(NHI):
            oi = jnp.where(keep_last if HI[i] == 2048 else keep, o_v[i], 0.0)
            kd_v[16 * i:16 * i + 16, :] = _dot_nt(sel, _bf(oi))

    copies[2].wait()
    off = 0
    for dl in range(NB):
        s0, ln = WIN[dl]
        kt_v[dl] = _dot(g_v[:, off:off + ln], _bf(kd_v[s0:s0 + ln, :]))
        off += ln

    copies[0].wait()
    copies[1].wait()
    h_v[0:8, :] = jnp.zeros((8, D), jnp.float32)
    h_v[8 + L:16 + L, :] = jnp.zeros((8, D), jnp.float32)

    def phase1(b, carry):
        r0 = pl.multiple_of(b * RB, RB)
        xs = []
        for k in range(RB // J):
            rk = pl.multiple_of(r0 + k * J, J)
            xk = _bf(_layernorm(x_v[pl.ds(rk, J), :].astype(jnp.float32)))
            xn_v[pl.ds(rk, J), :] = xk
            u_v[b * (RB // J) + k] = _dot(ffwd_ref[...], xk)
            xs.append(xk)
        h = _gelu(_dot(jnp.concatenate(xs, axis=0), w1_v[...]))
        h_v[pl.ds(pl.multiple_of(r0 + 8, 8), RB), :] = h
        return carry

    with jax.named_scope('p_phase1'):
        lax.fori_loop(0, L // RB, phase1, 0)

    def ztile(t):
        f0 = pl.multiple_of((t // 4) * 8, 8)
        re = pl.ds(f0, 8)
        im = pl.ds(pl.multiple_of(f0 + J, 8), 8)
        cs = pl.ds(pl.multiple_of((t % 4) * 128, 128), 128)
        GZ = 4
        for i0 in range(0, NB, GZ):
            acc = {}
            uc = {}
            for dl in range(i0 + GZ):
                kr = kt_v[dl, re, cs]
                ki = kt_v[dl, im, cs]
                ks = kr + ki
                for i in range(max(i0, dl), i0 + GZ):
                    src = i - dl
                    if src not in uc:
                        ur = u_v[src, re, cs]
                        ui = u_v[src, im, cs]
                        uc[src] = (ur, ui, ur + ui)
                    ur, ui, us = uc[src]
                    p = (kr * ur, ki * ui, ks * us)
                    acc[i] = p if i not in acc else tuple(x + y for x, y in zip(acc[i], p))
            for i in range(i0, i0 + GZ):
                s1, s2, s3 = acc[i]
                z_v[i, re, cs] = s1 - s2
                z_v[i, im, cs] = s3 - (s1 + s2)

    copies[3].wait()
    copies[4].wait()
    copies[5].wait()
    dsk = dsk_ref[...].astype(jnp.float32).reshape(1, D)

    TPB = 64 // (L // RB)

    def phase2(b, carry):
        r0 = pl.multiple_of(b * RB, RB)
        nt = [0]

        def zfill(n):
            for _ in range(n):
                ztile(b * TPB + nt[0])
                nt[0] += 1

        ext = RB + 16
        parts = []
        for gi, sh in enumerate((1, -1, 2, -2)):
            hv = h_v[pl.ds(r0, ext), gi * 128:(gi + 1) * 128]
            hv = pltpu.roll(hv, sh % ext, 0)
            parts.append(_bf(hv[8:8 + RB, :]))
        hs = _dot(jnp.concatenate(parts, axis=1), w2_v[...])
        zfill(TPB // 8)
        xn = xn_v[pl.ds(r0, RB), :].astype(jnp.float32)
        x1 = xn + hs
        ln2 = _bf(_layernorm2(x1))
        gas = []
        for c in range(0, FF, 256):
            n = min(256, FF - c)
            gas.append(_bf(_gelu(_dot_nt(ln2, w3_v[c:c + n, :]))))
            zfill(TPB // 8)
        h2 = _dot(jnp.concatenate(gas, axis=1), w4_v[...])
        zfill(TPB - nt[0])
        bb = x1 + h2
        gate_v[pl.ds(r0, RB), :] = bb * jax.nn.sigmoid(bb)
        return carry

    with jax.named_scope('p_phase2'):
        lax.fori_loop(0, L // RB, phase2, 0)

    R3 = 256

    def out_copy(b):
        r0 = pl.multiple_of(b * R3, R3)
        return pltpu.make_async_copy(out_v.at[pl.ds(r0, R3), :],
                                     out_hbm.at[pl.ds(r0, R3), :], sem_out.at[b])

    def phase3(b, carry):
        r0 = pl.multiple_of(b * R3, R3)
        ys = [_dot(finv_ref[...], _bf(z_v[b * (R3 // J) + k])) for k in range(R3 // J)]
        y = jnp.concatenate(ys, axis=0)
        xn = xn_v[pl.ds(r0, R3), :].astype(jnp.float32)
        s = y + xn * dsk
        x = x_v[pl.ds(r0, R3), :].astype(jnp.float32)
        out_v[pl.ds(r0, R3), :] = _bf(x + s * gate_v[pl.ds(r0, R3), :])
        out_copy(b).start()
        return carry

    with jax.named_scope('p_phase3'):
        lax.fori_loop(0, L // R3, phase3, 0)
    for b in range(L // R3):
        out_copy(b).wait()


@jax.jit
def pallas_recurrent_scan__ssm_conv_s4__mixer_s_mlp__prompt_kernel(
    A_u: jax.Array,
    A_A_re: jax.Array,
    A_A_im: jax.Array,
    A_B_re: jax.Array,
    A_B_im: jax.Array,
    A_C_re: jax.Array,
    A_C_im: jax.Array,
    A_log_dt: jax.Array,
    A_Dskip: jax.Array,
    B_x: jax.Array,
    B_w1: jax.Array,
    B_w2: jax.Array,
    B_w3: jax.Array,
    B_w4: jax.Array,
):
    bf16 = jnp.bfloat16
    f32 = jnp.float32
    x = A_u.reshape(L, D)
    vm = pl.BlockSpec(memory_space=pltpu.VMEM)
    hbm = pl.BlockSpec(memory_space=pltpu.HBM)
    out = pl.pallas_call(
        _kernel,
        out_shape=jax.ShapeDtypeStruct((L, D), bf16),
        in_specs=[vm] * 11 + [hbm] * 6,
        out_specs=hbm,
        scratch_shapes=[
            pltpu.VMEM((L, D), bf16),
            pltpu.VMEM((D, D), bf16),
            pltpu.VMEM((D, D), bf16),
            pltpu.VMEM((FF, D), bf16),
            pltpu.VMEM((FF, D), bf16),
            pltpu.VMEM((2 * J, GW), bf16),
            pltpu.VMEM((L, D), bf16),
            pltpu.VMEM((L, D), bf16),
            pltpu.VMEM((L + 16, D), f32),
            pltpu.VMEM((NB, 2 * J, D), f32),
            pltpu.VMEM((NB, 2 * J, D), f32),
            pltpu.VMEM((NB, 2 * J, D), f32),
            pltpu.VMEM((CH // 8, 128, N), f32),
            pltpu.VMEM((CH // 8, 128, N), f32),
            pltpu.VMEM((CH // 8, 8 * NHI, N), f32),
            pltpu.VMEM((CH // 8, 8 * NHI, N), f32),
            pltpu.VMEM((NHI, D, 128), f32),
            pltpu.VMEM((NQ, D), f32),
            pltpu.VMEM((D, N), f32),
            pltpu.VMEM((L, D), f32),
            pltpu.SemaphoreType.DMA((6,)),
            pltpu.SemaphoreType.DMA((8,)),
        ],
        compiler_params=pltpu.CompilerParams(vmem_limit_bytes=100 * 1024 * 1024),
    )(A_A_re, A_A_im, A_B_re, A_B_im, A_C_re, A_C_im,
      A_log_dt, A_Dskip,
      jnp.asarray(_F_FWD, bf16), jnp.asarray(_F_INV, bf16), jnp.asarray(_SEL, bf16),
      *[pltpu.with_memory_space_constraint(t, pltpu.HBM)
        for t in (x, B_w1, B_w2, B_w3.T, B_w4, jnp.asarray(_G_ALL, bf16))])
    return out.reshape(1, L, D)
```

```python
import functools
import numpy as np
import jax
import jax.numpy as jnp
from jax import lax
import jax.experimental.pallas as pl
import jax.experimental.pallas.tpu as pltpu

L = 2048
D = 512
N = 128
FF = 1376
J = 128
NB = L // J
NQ = 656
_STEP = (1, 1, 2, 2, 4, 4, 4, 4, 8, 8, 8, 8, 8, 8, 8, 8)
HI = tuple(128 * k + b for k in range(16) for b in range(0, 8, _STEP[k])) + (2048,)
NHI = len(HI)
CH = 32
RB = 512
WIN = ((0, 128), (0, 256), (128, 256), (256, 256), (320, 128), (384, 128),
       (384, 128), (448, 128), (448, 128), (512, 128), (512, 128), (512, 128),
       (512, 128), (512, 128), (512, 128), (528, 128))
GW = sum(w[1] for w in WIN)


def _q_of_m(m):
    hi = (m // 128) * 128 + (m % 8)
    return 16 * HI.index(hi) + (m % 128) // 8


def _build_tables():
    pos = np.arange(L, dtype=np.int64)
    rr = np.zeros(L, np.int64)
    for l in range(L):
        if l < 256:
            rr[l] = l
        else:
            step = 1 << (int(l).bit_length() - 8)
            lo = (l // step) * step
            rem = l - lo
            if rem * 2 < step or (rem * 2 == step and (lo // step) % 2 == 0):
                rr[l] = lo
            else:
                rr[l] = lo + step
    w = np.pi * (2 * np.arange(J) + 1) / (2 * J)
    n = np.arange(J)
    f_fwd = np.concatenate([np.cos(np.outer(w, n)), -np.sin(np.outer(w, n))], 0)
    f_inv = np.concatenate([np.cos(np.outer(n, w)), -np.sin(np.outer(n, w))], 1) / J
    g_all = np.zeros((2 * J, GW))
    off = 0
    for dl in range(NB):
        s0, ln = WIN[dl]
        for p in range(-J, J):
            l = dl * J + p
            if 0 <= l < L:
                q = _q_of_m(int(rr[l])) - s0
                assert 0 <= q < ln
                g_all[:J, off + q] += np.cos(w * p)
                g_all[J:, off + q] += -np.sin(w * p)
        off += ln
    sel = np.zeros((16, 128))
    for dd in range(8):
        sel[np.arange(16), np.arange(16) * 8 + dd] = 1.0
    del pos
    return (f_fwd.astype(np.float32), f_inv.astype(np.float32),
            g_all.astype(np.float32), sel.astype(np.float32))


_F_FWD, _F_INV, _G_ALL, _SEL = _build_tables()


def _bf(x):
    return x.astype(jnp.bfloat16)


def _rb(x):
    return x.astype(jnp.bfloat16).astype(jnp.float32)


def _cmul(a, b):
    return (a[0] * b[0] - a[1] * b[1], a[0] * b[1] + a[1] * b[0])


def _sincos(x):
    k = jnp.floor(x * 0.6366197723675814 + 0.5)
    r = x - k * 1.5703125
    r = r - k * 4.837512969970703125e-4
    r = r - k * 7.549789954891882e-8
    r2 = r * r
    sn = r + r * r2 * (-1.6666654611e-1 + r2 * (8.3321608736e-3 + r2 * -1.9515295891e-4))
    cs = 1.0 + r2 * (-0.5 + r2 * (4.166664568298827e-2 + r2 * (-1.388731625493765e-3
                                                             + r2 * 2.443315711809948e-5)))
    q = k - 4.0 * jnp.floor(k * 0.25)
    odd = (q == 1.0) | (q == 3.0)
    s0 = jnp.where(odd, cs, sn)
    c0 = jnp.where(odd, sn, cs)
    s1 = jnp.where(q >= 2.0, -s0, s0)
    c1 = jnp.where((q == 1.0) | (q == 2.0), -c0, c0)
    return s1, c1


def _gelu(x):
    c = 0.7978845608028654
    return 0.5 * x * (1.0 + jnp.tanh(c * (x + 0.044715 * (x * x * x))))


def _layernorm(x):
    m = jnp.mean(x, axis=-1, keepdims=True)
    xc = x - m
    v = jnp.mean(xc * xc, axis=-1, keepdims=True)
    den = _rb(jnp.sqrt(_rb(_rb(v) + 1e-5)))
    return _rb(_rb(x - _rb(m)) / den)


def _layernorm2(x):
    m = jnp.mean(x, axis=-1, keepdims=True)
    xc = x - m
    v = jnp.mean(xc * xc, axis=-1, keepdims=True)
    return xc / jnp.sqrt(v + 1e-5)


def _dot(a, b):
    return jnp.dot(a, b, preferred_element_type=jnp.float32)


def _dot_nt(a, b):
    return lax.dot_general(a, b, (((1,), (1,)), ((), ())),
                           preferred_element_type=jnp.float32)


def _kernel(are_ref, aim_ref, bre_ref, bim_ref, cre_ref, cim_ref, ldt_ref, dsk_ref,
            ffwd_ref, finv_ref, sel_ref,
            x_hbm, w1_hbm, w2_hbm, w3_hbm, w4_hbm, g_hbm,
            out_hbm,
            x_v, w1_v, w2_v, w3_v, w4_v, g_v, out_v,
            xn_v, h_v, u_v, kt_v, z_v,
            yr_v, yi_v, xr_v, xi_v, o_v, kd_v, dt_v, gate_v,
            sem_in, sem_out):
    copies = [pltpu.make_async_copy(s, d, sem_in.at[k]) for k, (s, d) in enumerate(
        [(x_hbm, x_v), (w1_hbm, w1_v), (g_hbm, g_v), (w2_hbm, w2_v), (w3_hbm, w3_v),
         (w4_hbm, w4_v)])]
    for c in copies:
        c.start()

    dt_row = _rb(jnp.exp(ldt_ref[...].astype(jnp.float32))).reshape(1, D)
    dt_v[...] = jnp.transpose(jnp.broadcast_to(dt_row, (N, D)))

    def kgen(c, carry):
        r0 = pl.multiple_of(c * CH, CH)
        rows = pl.ds(r0, CH)
        f32 = jnp.float32
        dt = dt_v[rows, :]
        lr = dt * are_ref[rows, :].astype(f32)
        li = dt * aim_ref[rows, :].astype(f32)
        dbr = dt * bre_ref[rows, :].astype(f32)
        dbi = dt * bim_ref[rows, :].astype(f32)
        w = _cmul((cre_ref[rows, :].astype(f32), cim_ref[rows, :].astype(f32)), (dbr, dbi))

        def csq(a):
            ab = a[0] * a[1]
            return (a[0] * a[0] - a[1] * a[1], ab + ab)

        e1 = jnp.exp(lr)
        sn, cs = _sincos(li)
        z1 = (e1 * cs, e1 * sn)
        z8 = csq(csq(csq(z1)))
        z128 = csq(csq(csq(csq(z8))))
        z1024 = csq(csq(csq(z128)))

        def put_y(j, v):
            for g in range(CH // 8):
                yr_v[g, 8 * j:8 * j + 8, :] = v[0][8 * g:8 * g + 8, :]
                yi_v[g, 8 * j:8 * j + 8, :] = v[1][8 * g:8 * g + 8, :]

        def put_x(i, v):
            nvi = -v[1]
            for g in range(CH // 8):
                xr_v[g, 8 * i:8 * i + 8, :] = v[0][8 * g:8 * g + 8, :]
                xi_v[g, 8 * i:8 * i + 8, :] = nvi[8 * g:8 * g + 8, :]

        put_y(0, (jnp.ones_like(lr), jnp.zeros_like(lr)))
        y = z8
        put_y(1, y)
        for j in range(2, 16):
            y = _cmul(y, z8)
            put_y(j, y)
        v = w
        for b in range(8):
            if b:
                v = _cmul(v, z1)
            t = v
            for k in range(8):
                if (128 * k + b) in HI:
                    if k:
                        t = _cmul(t, z128)
                    put_x(HI.index(128 * k + b), t)
        t = _cmul(w, z1024)
        for k in range(8, 17):
            if k > 8:
                t = _cmul(t, z128)
            put_x(HI.index(128 * k), t)
        for g in range(CH // 8):
            o = (_dot_nt(_bf(xr_v[g]), _bf(yr_v[g])) + _dot_nt(_bf(xi_v[g]), _bf(yi_v[g])))
            for i in range(NHI):
                o_v[i, pl.ds(pl.multiple_of(r0 + 8 * g, 8), 8), :] = o[8 * i:8 * i + 8, :]
        return carry

    with jax.named_scope('p_kgen'):
        lax.fori_loop(0, D // CH, kgen, 0)

    rid = lax.broadcasted_iota(jnp.int32, (D, 128), 0)
    lid = lax.broadcasted_iota(jnp.int32, (D, 128), 1)
    keep = (rid % 8) == (lid % 8)
    keep_last = keep & (lid < 8)
    sel = sel_ref[...]
    with jax.named_scope('p_sel'):
        for i in range(NHI):
            oi = jnp.where(keep_last if HI[i] == 2048 else keep, o_v[i], 0.0)
            kd_v[16 * i:16 * i + 16, :] = _dot_nt(sel, _bf(oi))

    copies[2].wait()
    off = 0
    for dl in range(NB):
        s0, ln = WIN[dl]
        kt_v[dl] = _dot(g_v[:, off:off + ln], _bf(kd_v[s0:s0 + ln, :]))
        off += ln

    copies[0].wait()
    copies[1].wait()
    h_v[0:8, :] = jnp.zeros((8, D), jnp.float32)
    h_v[8 + L:16 + L, :] = jnp.zeros((8, D), jnp.float32)

    def phase1(b, carry):
        r0 = pl.multiple_of(b * RB, RB)
        xs = []
        for k in range(RB // J):
            rk = pl.multiple_of(r0 + k * J, J)
            xk = _bf(_layernorm(x_v[pl.ds(rk, J), :].astype(jnp.float32)))
            xn_v[pl.ds(rk, J), :] = xk
            u_v[b * (RB // J) + k] = _dot(ffwd_ref[...], xk)
            xs.append(xk)
        h = _gelu(_dot(jnp.concatenate(xs, axis=0), w1_v[...]))
        h_v[pl.ds(pl.multiple_of(r0 + 8, 8), RB), :] = h
        return carry

    with jax.named_scope('p_phase1'):
        lax.fori_loop(0, L // RB, phase1, 0)

    def ztile(t):
        f0 = pl.multiple_of((t // 4) * 8, 8)
        re = pl.ds(f0, 8)
        im = pl.ds(pl.multiple_of(f0 + J, 8), 8)
        cs = pl.ds(pl.multiple_of((t % 4) * 128, 128), 128)
        GZ = 4
        for i0 in range(0, NB, GZ):
            acc = {}
            uc = {}
            for dl in range(i0 + GZ):
                kr = kt_v[dl, re, cs]
                ki = kt_v[dl, im, cs]
                ks = kr + ki
                for i in range(max(i0, dl), i0 + GZ):
                    src = i - dl
                    if src not in uc:
                        ur = u_v[src, re, cs]
                        ui = u_v[src, im, cs]
                        uc[src] = (ur, ui, ur + ui)
                    ur, ui, us = uc[src]
                    p = (kr * ur, ki * ui, ks * us)
                    acc[i] = p if i not in acc else tuple(x + y for x, y in zip(acc[i], p))
            for i in range(i0, i0 + GZ):
                s1, s2, s3 = acc[i]
                z_v[i, re, cs] = s1 - s2
                z_v[i, im, cs] = s3 - (s1 + s2)

    copies[3].wait()
    copies[4].wait()
    copies[5].wait()
    dsk = dsk_ref[...].astype(jnp.float32).reshape(1, D)

    TPB = 64 // (L // RB)

    def phase2(b, carry):
        r0 = pl.multiple_of(b * RB, RB)
        nt = [0]

        def zfill(n):
            for _ in range(n):
                ztile(b * TPB + nt[0])
                nt[0] += 1

        ext = RB + 16
        parts = []
        for gi, sh in enumerate((1, -1, 2, -2)):
            hv = h_v[pl.ds(r0, ext), gi * 128:(gi + 1) * 128]
            hv = pltpu.roll(hv, sh % ext, 0)
            parts.append(_bf(hv[8:8 + RB, :]))
        hs = _dot(jnp.concatenate(parts, axis=1), w2_v[...])
        xn = xn_v[pl.ds(r0, RB), :].astype(jnp.float32)
        x1 = xn + hs
        ln2 = _bf(_layernorm2(x1))
        gas = []
        for c in range(0, FF, 256):
            n = min(256, FF - c)
            gas.append(_bf(_gelu(_dot_nt(ln2, w3_v[c:c + n, :]))))
            if n == 256:
                zfill(1)
        ga = jnp.concatenate(gas, axis=1)
        for n in range(4):
            cs = slice(n * 128, (n + 1) * 128)
            zfill(1)
            h2 = _dot(ga, w4_v[:, cs])
            zfill(2 if n < 3 else TPB - nt[0])
            bb = x1[:, cs] + h2
            gate_v[pl.ds(r0, RB), cs] = bb * jax.nn.sigmoid(bb)
        return carry

    with jax.named_scope('p_phase2'):
        lax.fori_loop(0, L // RB, phase2, 0)

    R3 = 256

    def out_copy(b):
        r0 = pl.multiple_of(b * R3, R3)
        return pltpu.make_async_copy(out_v.at[pl.ds(r0, R3), :],
                                     out_hbm.at[pl.ds(r0, R3), :], sem_out.at[b])

    def phase3(b, carry):
        r0 = pl.multiple_of(b * R3, R3)
        ys = [_dot(finv_ref[...], _bf(z_v[b * (R3 // J) + k])) for k in range(R3 // J)]
        y = jnp.concatenate(ys, axis=0)
        xn = xn_v[pl.ds(r0, R3), :].astype(jnp.float32)
        s = y + xn * dsk
        x = x_v[pl.ds(r0, R3), :].astype(jnp.float32)
        out_v[pl.ds(r0, R3), :] = _bf(x + s * gate_v[pl.ds(r0, R3), :])
        out_copy(b).start()
        return carry

    with jax.named_scope('p_phase3'):
        lax.fori_loop(0, L // R3, phase3, 0)
    for b in range(L // R3):
        out_copy(b).wait()


@jax.jit
def pallas_recurrent_scan__ssm_conv_s4__mixer_s_mlp__prompt_kernel(
    A_u: jax.Array,
    A_A_re: jax.Array,
    A_A_im: jax.Array,
    A_B_re: jax.Array,
    A_B_im: jax.Array,
    A_C_re: jax.Array,
    A_C_im: jax.Array,
    A_log_dt: jax.Array,
    A_Dskip: jax.Array,
    B_x: jax.Array,
    B_w1: jax.Array,
    B_w2: jax.Array,
    B_w3: jax.Array,
    B_w4: jax.Array,
):
    bf16 = jnp.bfloat16
    f32 = jnp.float32
    x = A_u.reshape(L, D)
    vm = pl.BlockSpec(memory_space=pltpu.VMEM)
    hbm = pl.BlockSpec(memory_space=pltpu.HBM)
    out = pl.pallas_call(
        _kernel,
        out_shape=jax.ShapeDtypeStruct((L, D), bf16),
        in_specs=[vm] * 11 + [hbm] * 6,
        out_specs=hbm,
        scratch_shapes=[
            pltpu.VMEM((L, D), bf16),
            pltpu.VMEM((D, D), bf16),
            pltpu.VMEM((D, D), bf16),
            pltpu.VMEM((FF, D), bf16),
            pltpu.VMEM((FF, D), bf16),
            pltpu.VMEM((2 * J, GW), bf16),
            pltpu.VMEM((L, D), bf16),
            pltpu.VMEM((L, D), bf16),
            pltpu.VMEM((L + 16, D), f32),
            pltpu.VMEM((NB, 2 * J, D), f32),
            pltpu.VMEM((NB, 2 * J, D), f32),
            pltpu.VMEM((NB, 2 * J, D), f32),
            pltpu.VMEM((CH // 8, 128, N), f32),
            pltpu.VMEM((CH // 8, 128, N), f32),
            pltpu.VMEM((CH // 8, 8 * NHI, N), f32),
            pltpu.VMEM((CH // 8, 8 * NHI, N), f32),
            pltpu.VMEM((NHI, D, 128), f32),
            pltpu.VMEM((NQ, D), f32),
            pltpu.VMEM((D, N), f32),
            pltpu.VMEM((L, D), f32),
            pltpu.SemaphoreType.DMA((6,)),
            pltpu.SemaphoreType.DMA((8,)),
        ],
        compiler_params=pltpu.CompilerParams(vmem_limit_bytes=100 * 1024 * 1024),
    )(A_A_re, A_A_im, A_B_re, A_B_im, A_C_re, A_C_im,
      A_log_dt, A_Dskip,
      jnp.asarray(_F_FWD, bf16), jnp.asarray(_F_INV, bf16), jnp.asarray(_SEL, bf16),
      *[pltpu.with_memory_space_constraint(t, pltpu.HBM)
        for t in (x, B_w1, B_w2, B_w3.T, B_w4, jnp.asarray(_G_ALL, bf16))])
    return out.reshape(1, L, D)
```

```python
import functools
import numpy as np
import jax
import jax.numpy as jnp
from jax import lax
import jax.experimental.pallas as pl
import jax.experimental.pallas.tpu as pltpu

L = 2048
D = 512
N = 128
FF = 1376
J = 128
NB = L // J
NQ = 656
_STEP = (1, 1, 2, 2, 4, 4, 4, 4, 8, 8, 8, 8, 8, 8, 8, 8)
HI = tuple(128 * k + b for k in range(16) for b in range(0, 8, _STEP[k])) + (2048,)
NHI = len(HI)
CH = 32
RB = 512
WIN = ((0, 128), (0, 256), (128, 256), (256, 256), (320, 128), (384, 128),
       (384, 128), (448, 128), (448, 128), (512, 128), (512, 128), (512, 128),
       (512, 128), (512, 128), (512, 128), (528, 128))
GW = sum(w[1] for w in WIN)


def _q_of_m(m):
    hi = (m // 128) * 128 + (m % 8)
    return 16 * HI.index(hi) + (m % 128) // 8


def _build_tables():
    pos = np.arange(L, dtype=np.int64)
    rr = np.zeros(L, np.int64)
    for l in range(L):
        if l < 256:
            rr[l] = l
        else:
            step = 1 << (int(l).bit_length() - 8)
            lo = (l // step) * step
            rem = l - lo
            if rem * 2 < step or (rem * 2 == step and (lo // step) % 2 == 0):
                rr[l] = lo
            else:
                rr[l] = lo + step
    w = np.pi * (2 * np.arange(J) + 1) / (2 * J)
    n = np.arange(J)
    f_fwd = np.concatenate([np.cos(np.outer(w, n)), -np.sin(np.outer(w, n))], 0)
    f_inv = np.concatenate([np.cos(np.outer(n, w)), -np.sin(np.outer(n, w))], 1) / J
    g_all = np.zeros((2 * J, GW))
    off = 0
    for dl in range(NB):
        s0, ln = WIN[dl]
        for p in range(-J, J):
            l = dl * J + p
            if 0 <= l < L:
                q = _q_of_m(int(rr[l])) - s0
                assert 0 <= q < ln
                g_all[:J, off + q] += np.cos(w * p)
                g_all[J:, off + q] += -np.sin(w * p)
        off += ln
    sel = np.zeros((16, 128))
    for dd in range(8):
        sel[np.arange(16), np.arange(16) * 8 + dd] = 1.0
    del pos
    return (f_fwd.astype(np.float32), f_inv.astype(np.float32),
            g_all.astype(np.float32), sel.astype(np.float32))


_F_FWD, _F_INV, _G_ALL, _SEL = _build_tables()


def _bf(x):
    return x.astype(jnp.bfloat16)


def _rb(x):
    return x.astype(jnp.bfloat16).astype(jnp.float32)


def _cmul(a, b):
    return (a[0] * b[0] - a[1] * b[1], a[0] * b[1] + a[1] * b[0])


def _sincos(x):
    k = jnp.floor(x * 0.6366197723675814 + 0.5)
    r = x - k * 1.5703125
    r = r - k * 4.837512969970703125e-4
    r = r - k * 7.549789954891882e-8
    r2 = r * r
    sn = r + r * r2 * (-1.6666654611e-1 + r2 * (8.3321608736e-3 + r2 * -1.9515295891e-4))
    cs = 1.0 + r2 * (-0.5 + r2 * (4.166664568298827e-2 + r2 * (-1.388731625493765e-3
                                                             + r2 * 2.443315711809948e-5)))
    q = k - 4.0 * jnp.floor(k * 0.25)
    odd = (q == 1.0) | (q == 3.0)
    s0 = jnp.where(odd, cs, sn)
    c0 = jnp.where(odd, sn, cs)
    s1 = jnp.where(q >= 2.0, -s0, s0)
    c1 = jnp.where((q == 1.0) | (q == 2.0), -c0, c0)
    return s1, c1


def _gelu(x):
    c = 0.7978845608028654
    return 0.5 * x * (1.0 + jnp.tanh(c * (x + 0.044715 * (x * x * x))))


def _layernorm(x):
    m = jnp.mean(x, axis=-1, keepdims=True)
    xc = x - m
    v = jnp.mean(xc * xc, axis=-1, keepdims=True)
    den = _rb(jnp.sqrt(_rb(_rb(v) + 1e-5)))
    return _rb(_rb(x - _rb(m)) / den)


def _layernorm2(x):
    m = jnp.mean(x, axis=-1, keepdims=True)
    xc = x - m
    v = jnp.mean(xc * xc, axis=-1, keepdims=True)
    return xc / jnp.sqrt(v + 1e-5)


def _dot(a, b):
    return jnp.dot(a, b, preferred_element_type=jnp.float32)


def _dot_nt(a, b):
    return lax.dot_general(a, b, (((1,), (1,)), ((), ())),
                           preferred_element_type=jnp.float32)


def _kernel(are_ref, aim_ref, bre_ref, bim_ref, cre_ref, cim_ref, ldt_ref, dsk_ref,
            ffwd_ref, finv_ref, sel_ref,
            x_hbm, w1_hbm, w2_hbm, w3_hbm, w4_hbm, g_hbm,
            out_hbm,
            x_v, w1_v, w2_v, w3_v, w4_v, g_v, out_v,
            xn_v, h_v, u_v, kt_v, z_v,
            yr_v, yi_v, xr_v, xi_v, o_v, kd_v, dt_v, gate_v,
            sem_in, sem_out):
    copies = [pltpu.make_async_copy(s, d, sem_in.at[k]) for k, (s, d) in enumerate(
        [(x_hbm, x_v), (w1_hbm, w1_v), (g_hbm, g_v), (w2_hbm, w2_v), (w3_hbm, w3_v),
         (w4_hbm, w4_v)])]
    for c in copies:
        c.start()

    dt_row = _rb(jnp.exp(ldt_ref[...].astype(jnp.float32))).reshape(1, D)
    dt_v[...] = jnp.transpose(jnp.broadcast_to(dt_row, (N, D)))

    def kgen(c, carry):
        r0 = pl.multiple_of(c * CH, CH)
        rows = pl.ds(r0, CH)
        f32 = jnp.float32
        dt = dt_v[rows, :]
        lr = dt * are_ref[rows, :].astype(f32)
        li = dt * aim_ref[rows, :].astype(f32)
        dbr = dt * bre_ref[rows, :].astype(f32)
        dbi = dt * bim_ref[rows, :].astype(f32)
        w = _cmul((cre_ref[rows, :].astype(f32), cim_ref[rows, :].astype(f32)), (dbr, dbi))

        def csq(a):
            ab = a[0] * a[1]
            return (a[0] * a[0] - a[1] * a[1], ab + ab)

        e1 = jnp.exp(lr)
        sn, cs = _sincos(li)
        z1 = (e1 * cs, e1 * sn)
        z8 = csq(csq(csq(z1)))
        z128 = csq(csq(csq(csq(z8))))
        z1024 = csq(csq(csq(z128)))

        def put_y(j, v):
            for g in range(CH // 8):
                yr_v[g, 8 * j:8 * j + 8, :] = v[0][8 * g:8 * g + 8, :]
                yi_v[g, 8 * j:8 * j + 8, :] = v[1][8 * g:8 * g + 8, :]

        def put_x(i, v):
            nvi = -v[1]
            for g in range(CH // 8):
                xr_v[g, 8 * i:8 * i + 8, :] = v[0][8 * g:8 * g + 8, :]
                xi_v[g, 8 * i:8 * i + 8, :] = nvi[8 * g:8 * g + 8, :]

        put_y(0, (jnp.ones_like(lr), jnp.zeros_like(lr)))
        y = z8
        put_y(1, y)
        for j in range(2, 16):
            y = _cmul(y, z8)
            put_y(j, y)
        v = w
        for b in range(8):
            if b:
                v = _cmul(v, z1)
            t = v
            for k in range(8):
                if (128 * k + b) in HI:
                    if k:
                        t = _cmul(t, z128)
                    put_x(HI.index(128 * k + b), t)
        t = _cmul(w, z1024)
        for k in range(8, 17):
            if k > 8:
                t = _cmul(t, z128)
            put_x(HI.index(128 * k), t)
        for g in range(CH // 8):
            o = (_dot_nt(_bf(xr_v[g]), _bf(yr_v[g])) + _dot_nt(_bf(xi_v[g]), _bf(yi_v[g])))
            for i in range(NHI):
                o_v[i, pl.ds(pl.multiple_of(r0 + 8 * g, 8), 8), :] = o[8 * i:8 * i + 8, :]
        return carry

    with jax.named_scope('p_kgen'):
        lax.fori_loop(0, D // CH, kgen, 0)

    rid = lax.broadcasted_iota(jnp.int32, (D, 128), 0)
    lid = lax.broadcasted_iota(jnp.int32, (D, 128), 1)
    keep = (rid % 8) == (lid % 8)
    keep_last = keep & (lid < 8)
    sel = sel_ref[...]
    with jax.named_scope('p_sel'):
        for i in range(NHI):
            oi = jnp.where(keep_last if HI[i] == 2048 else keep, o_v[i], 0.0)
            kd_v[16 * i:16 * i + 16, :] = _dot_nt(sel, _bf(oi))

    copies[2].wait()
    off = 0
    for dl in range(NB):
        s0, ln = WIN[dl]
        kt_v[dl] = _dot(g_v[:, off:off + ln], _bf(kd_v[s0:s0 + ln, :]))
        off += ln

    copies[0].wait()
    copies[1].wait()
    h_v[0:8, :] = jnp.zeros((8, D), jnp.float32)
    h_v[8 + L:16 + L, :] = jnp.zeros((8, D), jnp.float32)

    def phase1(b, carry):
        r0 = pl.multiple_of(b * RB, RB)
        xs = []
        for k in range(RB // J):
            rk = pl.multiple_of(r0 + k * J, J)
            xk = _bf(_layernorm(x_v[pl.ds(rk, J), :].astype(jnp.float32)))
            xn_v[pl.ds(rk, J), :] = xk
            u_v[b * (RB // J) + k] = _dot(ffwd_ref[...], xk)
            xs.append(xk)
        h = _gelu(_dot(jnp.concatenate(xs, axis=0), w1_v[...]))
        h_v[pl.ds(pl.multiple_of(r0 + 8, 8), RB), :] = h
        return carry

    with jax.named_scope('p_phase1'):
        lax.fori_loop(0, L // RB, phase1, 0)

    def ztile(t):
        f0 = pl.multiple_of((t // 4) * 8, 8)
        re = pl.ds(f0, 8)
        im = pl.ds(pl.multiple_of(f0 + J, 8), 8)
        cs = pl.ds(pl.multiple_of((t % 4) * 128, 128), 128)
        GZ = 4
        for i0 in range(0, NB, GZ):
            acc = {}
            uc = {}
            for dl in range(i0 + GZ):
                kr = kt_v[dl, re, cs]
                ki = kt_v[dl, im, cs]
                ks = kr + ki
                for i in range(max(i0, dl), i0 + GZ):
                    src = i - dl
                    if src not in uc:
                        ur = u_v[src, re, cs]
                        ui = u_v[src, im, cs]
                        uc[src] = (ur, ui, ur + ui)
                    ur, ui, us = uc[src]
                    p = (kr * ur, ki * ui, ks * us)
                    acc[i] = p if i not in acc else tuple(x + y for x, y in zip(acc[i], p))
            for i in range(i0, i0 + GZ):
                s1, s2, s3 = acc[i]
                z_v[i, re, cs] = s1 - s2
                z_v[i, im, cs] = s3 - (s1 + s2)

    copies[3].wait()
    copies[4].wait()
    copies[5].wait()
    dsk = dsk_ref[...].astype(jnp.float32).reshape(1, D)

    TPB = 64 // (L // RB)

    def phase2(b, carry):
        r0 = pl.multiple_of(b * RB, RB)
        nt = [0]

        never = b > 1000

        def zfill(n, dep):
            tok = jnp.where(never, dep[0, 0].astype(jnp.int32), 0)
            for _ in range(n):
                ztile(b * TPB + nt[0] + tok)
                nt[0] += 1

        ext = RB + 16
        parts = []
        for gi, sh in enumerate((1, -1, 2, -2)):
            hv = h_v[pl.ds(r0, ext), gi * 128:(gi + 1) * 128]
            hv = pltpu.roll(hv, sh % ext, 0)
            parts.append(_bf(hv[8:8 + RB, :]))
        hs = _dot(jnp.concatenate(parts, axis=1), w2_v[...])
        zfill(1, parts[0].astype(jnp.float32))
        xn = xn_v[pl.ds(r0, RB), :].astype(jnp.float32)
        x1 = xn + hs
        ln2f = _layernorm2(x1)
        ln2 = _bf(ln2f)
        dep = ln2f
        gas = []
        for c in range(0, FF, 256):
            n = min(256, FF - c)
            zfill(1, dep)
            dep = _dot_nt(ln2, w3_v[c:c + n, :])
            gas.append(_bf(_gelu(dep)))
        ga = jnp.concatenate(gas, axis=1)
        for n in range(4):
            cs = slice(n * 128, (n + 1) * 128)
            zfill(2 if n < 3 else TPB - nt[0], dep)
            dep = _dot(ga, w4_v[:, cs])
            bb = x1[:, cs] + dep
            gate_v[pl.ds(r0, RB), cs] = bb * jax.nn.sigmoid(bb)
        return carry

    with jax.named_scope('p_phase2'):
        lax.fori_loop(0, L // RB, phase2, 0)

    R3 = 256

    def out_copy(b):
        r0 = pl.multiple_of(b * R3, R3)
        return pltpu.make_async_copy(out_v.at[pl.ds(r0, R3), :],
                                     out_hbm.at[pl.ds(r0, R3), :], sem_out.at[b])

    def phase3(b, carry):
        r0 = pl.multiple_of(b * R3, R3)
        ys = [_dot(finv_ref[...], _bf(z_v[b * (R3 // J) + k])) for k in range(R3 // J)]
        y = jnp.concatenate(ys, axis=0)
        xn = xn_v[pl.ds(r0, R3), :].astype(jnp.float32)
        s = y + xn * dsk
        x = x_v[pl.ds(r0, R3), :].astype(jnp.float32)
        out_v[pl.ds(r0, R3), :] = _bf(x + s * gate_v[pl.ds(r0, R3), :])
        out_copy(b).start()
        return carry

    with jax.named_scope('p_phase3'):
        lax.fori_loop(0, L // R3, phase3, 0)
    for b in range(L // R3):
        out_copy(b).wait()


@jax.jit
def pallas_recurrent_scan__ssm_conv_s4__mixer_s_mlp__prompt_kernel(
    A_u: jax.Array,
    A_A_re: jax.Array,
    A_A_im: jax.Array,
    A_B_re: jax.Array,
    A_B_im: jax.Array,
    A_C_re: jax.Array,
    A_C_im: jax.Array,
    A_log_dt: jax.Array,
    A_Dskip: jax.Array,
    B_x: jax.Array,
    B_w1: jax.Array,
    B_w2: jax.Array,
    B_w3: jax.Array,
    B_w4: jax.Array,
):
    bf16 = jnp.bfloat16
    f32 = jnp.float32
    x = A_u.reshape(L, D)
    vm = pl.BlockSpec(memory_space=pltpu.VMEM)
    hbm = pl.BlockSpec(memory_space=pltpu.HBM)
    out = pl.pallas_call(
        _kernel,
        out_shape=jax.ShapeDtypeStruct((L, D), bf16),
        in_specs=[vm] * 11 + [hbm] * 6,
        out_specs=hbm,
        scratch_shapes=[
            pltpu.VMEM((L, D), bf16),
            pltpu.VMEM((D, D), bf16),
            pltpu.VMEM((D, D), bf16),
            pltpu.VMEM((FF, D), bf16),
            pltpu.VMEM((FF, D), bf16),
            pltpu.VMEM((2 * J, GW), bf16),
            pltpu.VMEM((L, D), bf16),
            pltpu.VMEM((L, D), bf16),
            pltpu.VMEM((L + 16, D), f32),
            pltpu.VMEM((NB, 2 * J, D), f32),
            pltpu.VMEM((NB, 2 * J, D), f32),
            pltpu.VMEM((NB, 2 * J, D), f32),
            pltpu.VMEM((CH // 8, 128, N), f32),
            pltpu.VMEM((CH // 8, 128, N), f32),
            pltpu.VMEM((CH // 8, 8 * NHI, N), f32),
            pltpu.VMEM((CH // 8, 8 * NHI, N), f32),
            pltpu.VMEM((NHI, D, 128), f32),
            pltpu.VMEM((NQ, D), f32),
            pltpu.VMEM((D, N), f32),
            pltpu.VMEM((L, D), f32),
            pltpu.SemaphoreType.DMA((6,)),
            pltpu.SemaphoreType.DMA((8,)),
        ],
        compiler_params=pltpu.CompilerParams(vmem_limit_bytes=100 * 1024 * 1024),
    )(A_A_re, A_A_im, A_B_re, A_B_im, A_C_re, A_C_im,
      A_log_dt, A_Dskip,
      jnp.asarray(_F_FWD, bf16), jnp.asarray(_F_INV, bf16), jnp.asarray(_SEL, bf16),
      *[pltpu.with_memory_space_constraint(t, pltpu.HBM)
        for t in (x, B_w1, B_w2, B_w3.T, B_w4, jnp.asarray(_G_ALL, bf16))])
    return out.reshape(1, L, D)
```

```python
import functools
import numpy as np
import jax
import jax.numpy as jnp
from jax import lax
import jax.experimental.pallas as pl
import jax.experimental.pallas.tpu as pltpu

L = 2048
D = 512
N = 128
FF = 1376
J = 128
NB = L // J
NQ = 656
_STEP = (1, 1, 2, 2, 4, 4, 4, 4, 8, 8, 8, 8, 8, 8, 8, 8)
HI = tuple(128 * k + b for k in range(16) for b in range(0, 8, _STEP[k])) + (2048,)
NHI = len(HI)
CH = 32
RB = 512
WIN = ((0, 128), (0, 256), (128, 256), (256, 256), (320, 128), (384, 128),
       (384, 128), (448, 128), (448, 128), (512, 128), (512, 128), (512, 128),
       (512, 128), (512, 128), (512, 128), (528, 128))
GW = sum(w[1] for w in WIN)


def _q_of_m(m):
    hi = (m // 128) * 128 + (m % 8)
    return 16 * HI.index(hi) + (m % 128) // 8


def _build_tables():
    pos = np.arange(L, dtype=np.int64)
    rr = np.zeros(L, np.int64)
    for l in range(L):
        if l < 256:
            rr[l] = l
        else:
            step = 1 << (int(l).bit_length() - 8)
            lo = (l // step) * step
            rem = l - lo
            if rem * 2 < step or (rem * 2 == step and (lo // step) % 2 == 0):
                rr[l] = lo
            else:
                rr[l] = lo + step
    w = np.pi * (2 * np.arange(J) + 1) / (2 * J)
    n = np.arange(J)
    f_fwd = np.concatenate([np.cos(np.outer(w, n)), -np.sin(np.outer(w, n))], 0)
    f_inv = np.concatenate([np.cos(np.outer(n, w)), -np.sin(np.outer(n, w))], 1) / J
    g_all = np.zeros((2 * J, GW))
    off = 0
    for dl in range(NB):
        s0, ln = WIN[dl]
        for p in range(-J, J):
            l = dl * J + p
            if 0 <= l < L:
                q = _q_of_m(int(rr[l])) - s0
                assert 0 <= q < ln
                g_all[:J, off + q] += np.cos(w * p)
                g_all[J:, off + q] += -np.sin(w * p)
        off += ln
    sel = np.zeros((16, 128))
    for dd in range(8):
        sel[np.arange(16), np.arange(16) * 8 + dd] = 1.0
    del pos
    return (f_fwd.astype(np.float32), f_inv.astype(np.float32),
            g_all.astype(np.float32), sel.astype(np.float32))


_F_FWD, _F_INV, _G_ALL, _SEL = _build_tables()


def _bf(x):
    return x.astype(jnp.bfloat16)


def _rb(x):
    return x.astype(jnp.bfloat16).astype(jnp.float32)


def _cmul(a, b):
    return (a[0] * b[0] - a[1] * b[1], a[0] * b[1] + a[1] * b[0])


def _sincos(x):
    k = jnp.floor(x * 0.6366197723675814 + 0.5)
    r = x - k * 1.5703125
    r = r - k * 4.837512969970703125e-4
    r = r - k * 7.549789954891882e-8
    r2 = r * r
    sn = r + r * r2 * (-1.6666654611e-1 + r2 * (8.3321608736e-3 + r2 * -1.9515295891e-4))
    cs = 1.0 + r2 * (-0.5 + r2 * (4.166664568298827e-2 + r2 * (-1.388731625493765e-3
                                                             + r2 * 2.443315711809948e-5)))
    q = k - 4.0 * jnp.floor(k * 0.25)
    odd = (q == 1.0) | (q == 3.0)
    s0 = jnp.where(odd, cs, sn)
    c0 = jnp.where(odd, sn, cs)
    s1 = jnp.where(q >= 2.0, -s0, s0)
    c1 = jnp.where((q == 1.0) | (q == 2.0), -c0, c0)
    return s1, c1


def _gelu(x):
    c = 0.7978845608028654
    return 0.5 * x * (1.0 + jnp.tanh(c * (x + 0.044715 * (x * x * x))))


def _layernorm(x):
    m = jnp.mean(x, axis=-1, keepdims=True)
    xc = x - m
    v = jnp.mean(xc * xc, axis=-1, keepdims=True)
    den = _rb(jnp.sqrt(_rb(_rb(v) + 1e-5)))
    return _rb(_rb(x - _rb(m)) / den)


def _layernorm2(x):
    m = jnp.mean(x, axis=-1, keepdims=True)
    xc = x - m
    v = jnp.mean(xc * xc, axis=-1, keepdims=True)
    return xc / jnp.sqrt(v + 1e-5)


def _dot(a, b):
    return jnp.dot(a, b, preferred_element_type=jnp.float32)


def _dot_nt(a, b):
    return lax.dot_general(a, b, (((1,), (1,)), ((), ())),
                           preferred_element_type=jnp.float32)


def _kernel(are_ref, aim_ref, bre_ref, bim_ref, cre_ref, cim_ref, ldt_ref, dsk_ref,
            ffwd_ref, finv_ref, sel_ref,
            x_hbm, w1_hbm, w2_hbm, w3_hbm, w4_hbm, g_hbm,
            out_hbm,
            x_v, w1_v, w2_v, w3_v, w4_v, g_v, out_v,
            xn_v, h_v, u_v, kt_v, z_v,
            yr_v, yi_v, xr_v, xi_v, o_v, kd_v, dt_v, gate_v,
            sem_in, sem_out):
    copies = [pltpu.make_async_copy(s, d, sem_in.at[k]) for k, (s, d) in enumerate(
        [(x_hbm, x_v), (w1_hbm, w1_v), (g_hbm, g_v), (w2_hbm, w2_v), (w3_hbm, w3_v),
         (w4_hbm, w4_v)])]
    for c in copies:
        c.start()

    dt_row = _rb(jnp.exp(ldt_ref[...].astype(jnp.float32))).reshape(1, D)
    dt_v[...] = jnp.transpose(jnp.broadcast_to(dt_row, (N, D)))

    def kgen(c, carry):
        r0 = pl.multiple_of(c * CH, CH)
        rows = pl.ds(r0, CH)
        f32 = jnp.float32
        dt = dt_v[rows, :]
        lr = dt * are_ref[rows, :].astype(f32)
        li = dt * aim_ref[rows, :].astype(f32)
        dbr = dt * bre_ref[rows, :].astype(f32)
        dbi = dt * bim_ref[rows, :].astype(f32)
        w = _cmul((cre_ref[rows, :].astype(f32), cim_ref[rows, :].astype(f32)), (dbr, dbi))

        def csq(a):
            ab = a[0] * a[1]
            return (a[0] * a[0] - a[1] * a[1], ab + ab)

        e1 = jnp.exp(lr)
        sn, cs = _sincos(li)
        z1 = (e1 * cs, e1 * sn)
        z8 = csq(csq(csq(z1)))
        z128 = csq(csq(csq(csq(z8))))
        z1024 = csq(csq(csq(z128)))

        def put_y(j, v):
            for g in range(CH // 8):
                yr_v[g, 8 * j:8 * j + 8, :] = v[0][8 * g:8 * g + 8, :]
                yi_v[g, 8 * j:8 * j + 8, :] = v[1][8 * g:8 * g + 8, :]

        def put_x(i, v):
            nvi = -v[1]
            for g in range(CH // 8):
                xr_v[g, 8 * i:8 * i + 8, :] = v[0][8 * g:8 * g + 8, :]
                xi_v[g, 8 * i:8 * i + 8, :] = nvi[8 * g:8 * g + 8, :]

        put_y(0, (jnp.ones_like(lr), jnp.zeros_like(lr)))
        y = z8
        put_y(1, y)
        for j in range(2, 16):
            y = _cmul(y, z8)
            put_y(j, y)
        v = w
        for b in range(8):
            if b:
                v = _cmul(v, z1)
            t = v
            for k in range(8):
                if (128 * k + b) in HI:
                    if k:
                        t = _cmul(t, z128)
                    put_x(HI.index(128 * k + b), t)
        t = _cmul(w, z1024)
        for k in range(8, 17):
            if k > 8:
                t = _cmul(t, z128)
            put_x(HI.index(128 * k), t)
        for g in range(CH // 8):
            o = (_dot_nt(_bf(xr_v[g]), _bf(yr_v[g])) + _dot_nt(_bf(xi_v[g]), _bf(yi_v[g])))
            for i in range(NHI):
                o_v[i, pl.ds(pl.multiple_of(r0 + 8 * g, 8), 8), :] = o[8 * i:8 * i + 8, :]
        return carry

    with jax.named_scope('p_kgen'):
        lax.fori_loop(0, D // CH, kgen, 0)

    rid = lax.broadcasted_iota(jnp.int32, (D, 128), 0)
    lid = lax.broadcasted_iota(jnp.int32, (D, 128), 1)
    keep = (rid % 8) == (lid % 8)
    keep_last = keep & (lid < 8)
    sel = sel_ref[...]
    with jax.named_scope('p_sel'):
        for i in range(NHI):
            oi = jnp.where(keep_last if HI[i] == 2048 else keep, o_v[i], 0.0)
            kd_v[16 * i:16 * i + 16, :] = _dot_nt(sel, _bf(oi))

    copies[2].wait()
    off = 0
    for dl in range(NB):
        s0, ln = WIN[dl]
        kt_v[dl] = _dot(g_v[:, off:off + ln], _bf(kd_v[s0:s0 + ln, :]))
        off += ln

    copies[0].wait()
    copies[1].wait()
    h_v[0:8, :] = jnp.zeros((8, D), jnp.float32)
    h_v[8 + L:16 + L, :] = jnp.zeros((8, D), jnp.float32)

    def phase1(b, carry):
        r0 = pl.multiple_of(b * RB, RB)
        xs = []
        for k in range(RB // J):
            rk = pl.multiple_of(r0 + k * J, J)
            xk = _bf(_layernorm(x_v[pl.ds(rk, J), :].astype(jnp.float32)))
            xn_v[pl.ds(rk, J), :] = xk
            u_v[b * (RB // J) + k] = _dot(ffwd_ref[...], xk)
            xs.append(xk)
        h = _gelu(_dot(jnp.concatenate(xs, axis=0), w1_v[...]))
        h_v[pl.ds(pl.multiple_of(r0 + 8, 8), RB), :] = h
        return carry

    with jax.named_scope('p_phase1'):
        lax.fori_loop(0, L // RB, phase1, 0)

    GZ = 4

    def zgroup(t, i0):
        f0 = pl.multiple_of((t // 4) * 8, 8)
        re = pl.ds(f0, 8)
        im = pl.ds(pl.multiple_of(f0 + J, 8), 8)
        cs = pl.ds(pl.multiple_of((t % 4) * 128, 128), 128)
        for _once in range(1):
            acc = {}
            uc = {}
            for dl in range(i0 + GZ):
                kr = kt_v[dl, re, cs]
                ki = kt_v[dl, im, cs]
                ks = kr + ki
                for i in range(max(i0, dl), i0 + GZ):
                    src = i - dl
                    if src not in uc:
                        ur = u_v[src, re, cs]
                        ui = u_v[src, im, cs]
                        uc[src] = (ur, ui, ur + ui)
                    ur, ui, us = uc[src]
                    p = (kr * ur, ki * ui, ks * us)
                    acc[i] = p if i not in acc else tuple(x + y for x, y in zip(acc[i], p))
            for i in range(i0, i0 + GZ):
                s1, s2, s3 = acc[i]
                z_v[i, re, cs] = s1 - s2
                z_v[i, im, cs] = s3 - (s1 + s2)

    copies[3].wait()
    copies[4].wait()
    copies[5].wait()
    dsk = dsk_ref[...].astype(jnp.float32).reshape(1, D)

    TPB = 64 // (L // RB)

    def phase2(b, carry):
        r0 = pl.multiple_of(b * RB, RB)
        nt = [0]

        never = b > 1000
        work = [(tt, i0) for tt in range(TPB) for i0 in range(0, NB, GZ)]

        def zfill(n, dep):
            tok = jnp.where(never, dep[0, 0].astype(jnp.int32), 0)
            for _ in range(n):
                if work:
                    tt, i0 = work.pop(0)
                    zgroup(b * TPB + tt + tok, i0)

        ext = RB + 16
        parts = []
        for gi, sh in enumerate((1, -1, 2, -2)):
            hv = h_v[pl.ds(r0, ext), gi * 128:(gi + 1) * 128]
            hv = pltpu.roll(hv, sh % ext, 0)
            parts.append(_bf(hv[8:8 + RB, :]))
        hs = _dot(jnp.concatenate(parts, axis=1), w2_v[...])
        xn = xn_v[pl.ds(r0, RB), :].astype(jnp.float32)
        x1 = xn + hs
        ln2f = _layernorm2(x1)
        ln2 = _bf(ln2f)
        dep = ln2f
        gas = []
        for c in range(0, FF, 128):
            n = min(128, FF - c)
            zfill(2, dep)
            dep = _dot_nt(ln2, w3_v[c:c + n, :])
            gas.append(_bf(_gelu(dep)))
        for n in range(4):
            cs = slice(n * 128, (n + 1) * 128)
            h2 = None
            for kc, c in enumerate(range(0, FF, 128)):
                zfill(1, dep)
                t2 = _dot(gas[kc], w4_v[c:min(c + 128, FF), cs])
                h2 = t2 if h2 is None else h2 + t2
                dep = h2
            bb = x1[:, cs] + h2
            gate_v[pl.ds(r0, RB), cs] = bb * jax.nn.sigmoid(bb)
        assert not work
        return carry

    with jax.named_scope('p_phase2'):
        lax.fori_loop(0, L // RB, phase2, 0)

    R3 = 256

    def out_copy(b):
        r0 = pl.multiple_of(b * R3, R3)
        return pltpu.make_async_copy(out_v.at[pl.ds(r0, R3), :],
                                     out_hbm.at[pl.ds(r0, R3), :], sem_out.at[b])

    def phase3(b, carry):
        r0 = pl.multiple_of(b * R3, R3)
        ys = [_dot(finv_ref[...], _bf(z_v[b * (R3 // J) + k])) for k in range(R3 // J)]
        y = jnp.concatenate(ys, axis=0)
        xn = xn_v[pl.ds(r0, R3), :].astype(jnp.float32)
        s = y + xn * dsk
        x = x_v[pl.ds(r0, R3), :].astype(jnp.float32)
        out_v[pl.ds(r0, R3), :] = _bf(x + s * gate_v[pl.ds(r0, R3), :])
        out_copy(b).start()
        return carry

    with jax.named_scope('p_phase3'):
        lax.fori_loop(0, L // R3, phase3, 0)
    for b in range(L // R3):
        out_copy(b).wait()


@jax.jit
def pallas_recurrent_scan__ssm_conv_s4__mixer_s_mlp__prompt_kernel(
    A_u: jax.Array,
    A_A_re: jax.Array,
    A_A_im: jax.Array,
    A_B_re: jax.Array,
    A_B_im: jax.Array,
    A_C_re: jax.Array,
    A_C_im: jax.Array,
    A_log_dt: jax.Array,
    A_Dskip: jax.Array,
    B_x: jax.Array,
    B_w1: jax.Array,
    B_w2: jax.Array,
    B_w3: jax.Array,
    B_w4: jax.Array,
):
    bf16 = jnp.bfloat16
    f32 = jnp.float32
    x = A_u.reshape(L, D)
    vm = pl.BlockSpec(memory_space=pltpu.VMEM)
    hbm = pl.BlockSpec(memory_space=pltpu.HBM)
    out = pl.pallas_call(
        _kernel,
        out_shape=jax.ShapeDtypeStruct((L, D), bf16),
        in_specs=[vm] * 11 + [hbm] * 6,
        out_specs=hbm,
        scratch_shapes=[
            pltpu.VMEM((L, D), bf16),
            pltpu.VMEM((D, D), bf16),
            pltpu.VMEM((D, D), bf16),
            pltpu.VMEM((FF, D), bf16),
            pltpu.VMEM((FF, D), bf16),
            pltpu.VMEM((2 * J, GW), bf16),
            pltpu.VMEM((L, D), bf16),
            pltpu.VMEM((L, D), bf16),
            pltpu.VMEM((L + 16, D), f32),
            pltpu.VMEM((NB, 2 * J, D), f32),
            pltpu.VMEM((NB, 2 * J, D), f32),
            pltpu.VMEM((NB, 2 * J, D), f32),
            pltpu.VMEM((CH // 8, 128, N), f32),
            pltpu.VMEM((CH // 8, 128, N), f32),
            pltpu.VMEM((CH // 8, 8 * NHI, N), f32),
            pltpu.VMEM((CH // 8, 8 * NHI, N), f32),
            pltpu.VMEM((NHI, D, 128), f32),
            pltpu.VMEM((NQ, D), f32),
            pltpu.VMEM((D, N), f32),
            pltpu.VMEM((L, D), f32),
            pltpu.SemaphoreType.DMA((6,)),
            pltpu.SemaphoreType.DMA((8,)),
        ],
        compiler_params=pltpu.CompilerParams(vmem_limit_bytes=100 * 1024 * 1024),
    )(A_A_re, A_A_im, A_B_re, A_B_im, A_C_re, A_C_im,
      A_log_dt, A_Dskip,
      jnp.asarray(_F_FWD, bf16), jnp.asarray(_F_INV, bf16), jnp.asarray(_SEL, bf16),
      *[pltpu.with_memory_space_constraint(t, pltpu.HBM)
        for t in (x, B_w1, B_w2, B_w3.T, B_w4, jnp.asarray(_G_ALL, bf16))])
    return out.reshape(1, L, D)
```

```python
import functools
import numpy as np
import jax
import jax.numpy as jnp
from jax import lax
import jax.experimental.pallas as pl
import jax.experimental.pallas.tpu as pltpu

L = 2048
D = 512
N = 128
FF = 1376
J = 128
NB = L // J
NQ = 656
_STEP = (1, 1, 2, 2, 4, 4, 4, 4, 8, 8, 8, 8, 8, 8, 8, 8)
HI = tuple(128 * k + b for k in range(16) for b in range(0, 8, _STEP[k])) + (2048,)
NHI = len(HI)
CH = 32
RB = 512
WIN = ((0, 128), (0, 256), (128, 256), (256, 256), (320, 128), (384, 128),
       (384, 128), (448, 128), (448, 128), (512, 128), (512, 128), (512, 128),
       (512, 128), (512, 128), (512, 128), (528, 128))
GW = sum(w[1] for w in WIN)


def _q_of_m(m):
    hi = (m // 128) * 128 + (m % 8)
    return 16 * HI.index(hi) + (m % 128) // 8


def _build_tables():
    pos = np.arange(L, dtype=np.int64)
    rr = np.zeros(L, np.int64)
    for l in range(L):
        if l < 256:
            rr[l] = l
        else:
            step = 1 << (int(l).bit_length() - 8)
            lo = (l // step) * step
            rem = l - lo
            if rem * 2 < step or (rem * 2 == step and (lo // step) % 2 == 0):
                rr[l] = lo
            else:
                rr[l] = lo + step
    w = np.pi * (2 * np.arange(J) + 1) / (2 * J)
    n = np.arange(J)
    f_fwd = np.concatenate([np.cos(np.outer(w, n)), -np.sin(np.outer(w, n))], 0)
    f_inv = np.concatenate([np.cos(np.outer(n, w)), -np.sin(np.outer(n, w))], 1) / J
    g_all = np.zeros((2 * J, GW))
    off = 0
    for dl in range(NB):
        s0, ln = WIN[dl]
        for p in range(-J, J):
            l = dl * J + p
            if 0 <= l < L:
                q = _q_of_m(int(rr[l])) - s0
                assert 0 <= q < ln
                g_all[:J, off + q] += np.cos(w * p)
                g_all[J:, off + q] += -np.sin(w * p)
        off += ln
    sel = np.zeros((16, 128))
    for dd in range(8):
        sel[np.arange(16), np.arange(16) * 8 + dd] = 1.0
    del pos
    return (f_fwd.astype(np.float32), f_inv.astype(np.float32),
            g_all.astype(np.float32), sel.astype(np.float32))


_F_FWD, _F_INV, _G_ALL, _SEL = _build_tables()


def _bf(x):
    return x.astype(jnp.bfloat16)


def _rb(x):
    return x.astype(jnp.bfloat16).astype(jnp.float32)


def _cmul(a, b):
    return (a[0] * b[0] - a[1] * b[1], a[0] * b[1] + a[1] * b[0])


def _sincos(x):
    k = jnp.floor(x * 0.6366197723675814 + 0.5)
    r = x - k * 1.5703125
    r = r - k * 4.837512969970703125e-4
    r = r - k * 7.549789954891882e-8
    r2 = r * r
    sn = r + r * r2 * (-1.6666654611e-1 + r2 * (8.3321608736e-3 + r2 * -1.9515295891e-4))
    cs = 1.0 + r2 * (-0.5 + r2 * (4.166664568298827e-2 + r2 * (-1.388731625493765e-3
                                                             + r2 * 2.443315711809948e-5)))
    q = k - 4.0 * jnp.floor(k * 0.25)
    odd = (q == 1.0) | (q == 3.0)
    s0 = jnp.where(odd, cs, sn)
    c0 = jnp.where(odd, sn, cs)
    s1 = jnp.where(q >= 2.0, -s0, s0)
    c1 = jnp.where((q == 1.0) | (q == 2.0), -c0, c0)
    return s1, c1


def _gelu(x):
    c = 0.7978845608028654
    return 0.5 * x * (1.0 + jnp.tanh(c * (x + 0.044715 * (x * x * x))))


def _layernorm(x):
    m = jnp.mean(x, axis=-1, keepdims=True)
    xc = x - m
    v = jnp.mean(xc * xc, axis=-1, keepdims=True)
    den = _rb(jnp.sqrt(_rb(_rb(v) + 1e-5)))
    return _rb(_rb(x - _rb(m)) / den)


def _layernorm2(x):
    m = jnp.mean(x, axis=-1, keepdims=True)
    xc = x - m
    v = jnp.mean(xc * xc, axis=-1, keepdims=True)
    return xc / jnp.sqrt(v + 1e-5)


def _dot(a, b):
    return jnp.dot(a, b, preferred_element_type=jnp.float32)


def _dot_nt(a, b):
    return lax.dot_general(a, b, (((1,), (1,)), ((), ())),
                           preferred_element_type=jnp.float32)


def _kernel(are_ref, aim_ref, bre_ref, bim_ref, cre_ref, cim_ref, ldt_ref, dsk_ref,
            ffwd_ref, finv_ref, sel_ref,
            x_hbm, w1_hbm, w2_hbm, w3_hbm, w4_hbm, g_hbm,
            out_hbm,
            x_v, w1_v, w2_v, w3_v, w4_v, g_v, out_v,
            xn_v, h_v, u_v, kt_v, z_v,
            yr_v, yi_v, xr_v, xi_v, o_v, kd_v, dt_v, gate_v,
            sem_in, sem_out):
    copies = [pltpu.make_async_copy(s, d, sem_in.at[k]) for k, (s, d) in enumerate(
        [(x_hbm, x_v), (w1_hbm, w1_v), (g_hbm, g_v), (w2_hbm, w2_v), (w3_hbm, w3_v),
         (w4_hbm, w4_v)])]
    for c in copies:
        c.start()

    dt_row = _rb(jnp.exp(ldt_ref[...].astype(jnp.float32))).reshape(1, D)
    dt_v[...] = jnp.transpose(jnp.broadcast_to(dt_row, (N, D)))

    def kgen(c, carry):
        r0 = pl.multiple_of(c * CH, CH)
        rows = pl.ds(r0, CH)
        f32 = jnp.float32
        dt = dt_v[rows, :]
        lr = dt * are_ref[rows, :].astype(f32)
        li = dt * aim_ref[rows, :].astype(f32)
        dbr = dt * bre_ref[rows, :].astype(f32)
        dbi = dt * bim_ref[rows, :].astype(f32)
        w = _cmul((cre_ref[rows, :].astype(f32), cim_ref[rows, :].astype(f32)), (dbr, dbi))

        def csq(a):
            ab = a[0] * a[1]
            return (a[0] * a[0] - a[1] * a[1], ab + ab)

        e1 = jnp.exp(lr)
        sn, cs = _sincos(li)
        z1 = (e1 * cs, e1 * sn)
        z8 = csq(csq(csq(z1)))
        z128 = csq(csq(csq(csq(z8))))
        z1024 = csq(csq(csq(z128)))

        def put_y(j, v):
            for g in range(CH // 8):
                yr_v[g, 8 * j:8 * j + 8, :] = v[0][8 * g:8 * g + 8, :]
                yi_v[g, 8 * j:8 * j + 8, :] = v[1][8 * g:8 * g + 8, :]

        def put_x(i, v):
            nvi = -v[1]
            for g in range(CH // 8):
                xr_v[g, 8 * i:8 * i + 8, :] = v[0][8 * g:8 * g + 8, :]
                xi_v[g, 8 * i:8 * i + 8, :] = nvi[8 * g:8 * g + 8, :]

        put_y(0, (jnp.ones_like(lr), jnp.zeros_like(lr)))
        y = z8
        put_y(1, y)
        for j in range(2, 16):
            y = _cmul(y, z8)
            put_y(j, y)
        v = w
        for b in range(8):
            if b:
                v = _cmul(v, z1)
            t = v
            for k in range(8):
                if (128 * k + b) in HI:
                    if k:
                        t = _cmul(t, z128)
                    put_x(HI.index(128 * k + b), t)
        t = _cmul(w, z1024)
        for k in range(8, 17):
            if k > 8:
                t = _cmul(t, z128)
            put_x(HI.index(128 * k), t)
        for g in range(CH // 8):
            o = (_dot_nt(_bf(xr_v[g]), _bf(yr_v[g])) + _dot_nt(_bf(xi_v[g]), _bf(yi_v[g])))
            for i in range(NHI):
                o_v[i, pl.ds(pl.multiple_of(r0 + 8 * g, 8), 8), :] = o[8 * i:8 * i + 8, :]
        return carry

    with jax.named_scope('p_kgen'):
        lax.fori_loop(0, D // CH, kgen, 0)

    rid = lax.broadcasted_iota(jnp.int32, (D, 128), 0)
    lid = lax.broadcasted_iota(jnp.int32, (D, 128), 1)
    keep = (rid % 8) == (lid % 8)
    keep_last = keep & (lid < 8)
    sel = sel_ref[...]
    with jax.named_scope('p_sel'):
        for i in range(NHI):
            oi = jnp.where(keep_last if HI[i] == 2048 else keep, o_v[i], 0.0)
            kd_v[16 * i:16 * i + 16, :] = _dot_nt(sel, _bf(oi))

    copies[2].wait()
    off = 0
    for dl in range(NB):
        s0, ln = WIN[dl]
        kt_v[dl] = _dot(g_v[:, off:off + ln], _bf(kd_v[s0:s0 + ln, :]))
        off += ln

    copies[0].wait()
    copies[1].wait()
    h_v[0:8, :] = jnp.zeros((8, D), jnp.float32)
    h_v[8 + L:16 + L, :] = jnp.zeros((8, D), jnp.float32)

    def phase1(b, carry):
        r0 = pl.multiple_of(b * RB, RB)
        xs = []
        for k in range(RB // J):
            rk = pl.multiple_of(r0 + k * J, J)
            xk = _bf(_layernorm(x_v[pl.ds(rk, J), :].astype(jnp.float32)))
            xn_v[pl.ds(rk, J), :] = xk
            u_v[b * (RB // J) + k] = _dot(ffwd_ref[...], xk)
            xs.append(xk)
        h = _gelu(_dot(jnp.concatenate(xs, axis=0), w1_v[...]))
        h_v[pl.ds(pl.multiple_of(r0 + 8, 8), RB), :] = h
        return carry

    with jax.named_scope('p_phase1'):
        lax.fori_loop(0, L // RB, phase1, 0)

    GZ = 1

    def zgroup(t, i0):
        f0 = pl.multiple_of((t // 4) * 8, 8)
        re = pl.ds(f0, 8)
        im = pl.ds(pl.multiple_of(f0 + J, 8), 8)
        cs = pl.ds(pl.multiple_of((t % 4) * 128, 128), 128)
        for _once in range(1):
            acc = {}
            uc = {}
            for dl in range(i0 + GZ):
                kr = kt_v[dl, re, cs]
                ki = kt_v[dl, im, cs]
                ks = kr + ki
                for i in range(max(i0, dl), i0 + GZ):
                    src = i - dl
                    if src not in uc:
                        ur = u_v[src, re, cs]
                        ui = u_v[src, im, cs]
                        uc[src] = (ur, ui, ur + ui)
                    ur, ui, us = uc[src]
                    p = (kr * ur, ki * ui, ks * us)
                    acc[i] = p if i not in acc else tuple(x + y for x, y in zip(acc[i], p))
            for i in range(i0, i0 + GZ):
                s1, s2, s3 = acc[i]
                z_v[i, re, cs] = s1 - s2
                z_v[i, im, cs] = s3 - (s1 + s2)
        return s1

    copies[3].wait()
    copies[4].wait()
    copies[5].wait()
    dsk = dsk_ref[...].astype(jnp.float32).reshape(1, D)

    TPB = 64 // (L // RB)

    def phase2(b, carry):
        r0 = pl.multiple_of(b * RB, RB)
        nt = [0]

        never = b > 1000
        work = [(tt, i0) for tt in range(TPB) for i0 in range(0, NB, GZ)]
        last = [None]

        def zfill(n, dep):
            tok = jnp.where(never, dep[0, 0].astype(jnp.int32), 0)
            for _ in range(n):
                if work:
                    tt, i0 = work.pop(0)
                    if last[0] is not None:
                        tok = jnp.where(never, last[0][0, 0].astype(jnp.int32), tok)
                    last[0] = zgroup(b * TPB + tt + tok, i0)

        ext = RB + 16
        parts = []
        for gi, sh in enumerate((1, -1, 2, -2)):
            hv = h_v[pl.ds(r0, ext), gi * 128:(gi + 1) * 128]
            hv = pltpu.roll(hv, sh % ext, 0)
            parts.append(_bf(hv[8:8 + RB, :]))
        hs = _dot(jnp.concatenate(parts, axis=1), w2_v[...])
        xn = xn_v[pl.ds(r0, RB), :].astype(jnp.float32)
        x1 = xn + hs
        ln2f = _layernorm2(x1)
        ln2 = _bf(ln2f)
        dep = ln2f
        gas = []
        for c in range(0, FF, 128):
            n = min(128, FF - c)
            zfill(8, dep)
            dep = _dot_nt(ln2, w3_v[c:c + n, :])
            gas.append(_bf(_gelu(dep)))
        for n in range(4):
            cs = slice(n * 128, (n + 1) * 128)
            h2 = None
            for kc, c in enumerate(range(0, FF, 128)):
                zfill(4, dep)
                t2 = _dot(gas[kc], w4_v[c:min(c + 128, FF), cs])
                h2 = t2 if h2 is None else h2 + t2
                dep = h2
            bb = x1[:, cs] + h2
            gate_v[pl.ds(r0, RB), cs] = bb * jax.nn.sigmoid(bb)
        assert not work
        return carry

    with jax.named_scope('p_phase2'):
        lax.fori_loop(0, L // RB, phase2, 0)

    R3 = 256

    def out_copy(b):
        r0 = pl.multiple_of(b * R3, R3)
        return pltpu.make_async_copy(out_v.at[pl.ds(r0, R3), :],
                                     out_hbm.at[pl.ds(r0, R3), :], sem_out.at[b])

    def phase3(b, carry):
        r0 = pl.multiple_of(b * R3, R3)
        ys = [_dot(finv_ref[...], _bf(z_v[b * (R3 // J) + k])) for k in range(R3 // J)]
        y = jnp.concatenate(ys, axis=0)
        xn = xn_v[pl.ds(r0, R3), :].astype(jnp.float32)
        s = y + xn * dsk
        x = x_v[pl.ds(r0, R3), :].astype(jnp.float32)
        out_v[pl.ds(r0, R3), :] = _bf(x + s * gate_v[pl.ds(r0, R3), :])
        out_copy(b).start()
        return carry

    with jax.named_scope('p_phase3'):
        lax.fori_loop(0, L // R3, phase3, 0)
    for b in range(L // R3):
        out_copy(b).wait()


@jax.jit
def pallas_recurrent_scan__ssm_conv_s4__mixer_s_mlp__prompt_kernel(
    A_u: jax.Array,
    A_A_re: jax.Array,
    A_A_im: jax.Array,
    A_B_re: jax.Array,
    A_B_im: jax.Array,
    A_C_re: jax.Array,
    A_C_im: jax.Array,
    A_log_dt: jax.Array,
    A_Dskip: jax.Array,
    B_x: jax.Array,
    B_w1: jax.Array,
    B_w2: jax.Array,
    B_w3: jax.Array,
    B_w4: jax.Array,
):
    bf16 = jnp.bfloat16
    f32 = jnp.float32
    x = A_u.reshape(L, D)
    vm = pl.BlockSpec(memory_space=pltpu.VMEM)
    hbm = pl.BlockSpec(memory_space=pltpu.HBM)
    out = pl.pallas_call(
        _kernel,
        out_shape=jax.ShapeDtypeStruct((L, D), bf16),
        in_specs=[vm] * 11 + [hbm] * 6,
        out_specs=hbm,
        scratch_shapes=[
            pltpu.VMEM((L, D), bf16),
            pltpu.VMEM((D, D), bf16),
            pltpu.VMEM((D, D), bf16),
            pltpu.VMEM((FF, D), bf16),
            pltpu.VMEM((FF, D), bf16),
            pltpu.VMEM((2 * J, GW), bf16),
            pltpu.VMEM((L, D), bf16),
            pltpu.VMEM((L, D), bf16),
            pltpu.VMEM((L + 16, D), f32),
            pltpu.VMEM((NB, 2 * J, D), f32),
            pltpu.VMEM((NB, 2 * J, D), f32),
            pltpu.VMEM((NB, 2 * J, D), f32),
            pltpu.VMEM((CH // 8, 128, N), f32),
            pltpu.VMEM((CH // 8, 128, N), f32),
            pltpu.VMEM((CH // 8, 8 * NHI, N), f32),
            pltpu.VMEM((CH // 8, 8 * NHI, N), f32),
            pltpu.VMEM((NHI, D, 128), f32),
            pltpu.VMEM((NQ, D), f32),
            pltpu.VMEM((D, N), f32),
            pltpu.VMEM((L, D), f32),
            pltpu.SemaphoreType.DMA((6,)),
            pltpu.SemaphoreType.DMA((8,)),
        ],
        compiler_params=pltpu.CompilerParams(vmem_limit_bytes=100 * 1024 * 1024),
    )(A_A_re, A_A_im, A_B_re, A_B_im, A_C_re, A_C_im,
      A_log_dt, A_Dskip,
      jnp.asarray(_F_FWD, bf16), jnp.asarray(_F_INV, bf16), jnp.asarray(_SEL, bf16),
      *[pltpu.with_memory_space_constraint(t, pltpu.HBM)
        for t in (x, B_w1, B_w2, B_w3.T, B_w4, jnp.asarray(_G_ALL, bf16))])
    return out.reshape(1, L, D)
```

```python
import functools
import numpy as np
import jax
import jax.numpy as jnp
from jax import lax
import jax.experimental.pallas as pl
import jax.experimental.pallas.tpu as pltpu

L = 2048
D = 512
N = 128
FF = 1376
J = 128
NB = L // J
NQ = 656
_STEP = (1, 1, 2, 2, 4, 4, 4, 4, 8, 8, 8, 8, 8, 8, 8, 8)
HI = tuple(128 * k + b for k in range(16) for b in range(0, 8, _STEP[k])) + (2048,)
NHI = len(HI)
CH = 32
RB = 512
WIN = ((0, 128), (0, 256), (128, 256), (256, 256), (320, 128), (384, 128),
       (384, 128), (448, 128), (448, 128), (512, 128), (512, 128), (512, 128),
       (512, 128), (512, 128), (512, 128), (528, 128))
GW = sum(w[1] for w in WIN)


def _q_of_m(m):
    hi = (m // 128) * 128 + (m % 8)
    return 16 * HI.index(hi) + (m % 128) // 8


def _build_tables():
    pos = np.arange(L, dtype=np.int64)
    rr = np.zeros(L, np.int64)
    for l in range(L):
        if l < 256:
            rr[l] = l
        else:
            step = 1 << (int(l).bit_length() - 8)
            lo = (l // step) * step
            rem = l - lo
            if rem * 2 < step or (rem * 2 == step and (lo // step) % 2 == 0):
                rr[l] = lo
            else:
                rr[l] = lo + step
    w = np.pi * (2 * np.arange(J) + 1) / (2 * J)
    n = np.arange(J)
    f_fwd = np.concatenate([np.cos(np.outer(w, n)), -np.sin(np.outer(w, n))], 0)
    f_inv = np.concatenate([np.cos(np.outer(n, w)), -np.sin(np.outer(n, w))], 1) / J
    g_all = np.zeros((2 * J, GW))
    off = 0
    for dl in range(NB):
        s0, ln = WIN[dl]
        for p in range(-J, J):
            l = dl * J + p
            if 0 <= l < L:
                q = _q_of_m(int(rr[l])) - s0
                assert 0 <= q < ln
                g_all[:J, off + q] += np.cos(w * p)
                g_all[J:, off + q] += -np.sin(w * p)
        off += ln
    sel = np.zeros((16, 128))
    for dd in range(8):
        sel[np.arange(16), np.arange(16) * 8 + dd] = 1.0
    del pos
    return (f_fwd.astype(np.float32), f_inv.astype(np.float32),
            g_all.astype(np.float32), sel.astype(np.float32))


_F_FWD, _F_INV, _G_ALL, _SEL = _build_tables()


def _bf(x):
    return x.astype(jnp.bfloat16)


def _rb(x):
    return x.astype(jnp.bfloat16).astype(jnp.float32)


def _cmul(a, b):
    return (a[0] * b[0] - a[1] * b[1], a[0] * b[1] + a[1] * b[0])


def _sincos(x):
    k = jnp.floor(x * 0.6366197723675814 + 0.5)
    r = x - k * 1.5703125
    r = r - k * 4.837512969970703125e-4
    r = r - k * 7.549789954891882e-8
    r2 = r * r
    sn = r + r * r2 * (-1.6666654611e-1 + r2 * (8.3321608736e-3 + r2 * -1.9515295891e-4))
    cs = 1.0 + r2 * (-0.5 + r2 * (4.166664568298827e-2 + r2 * (-1.388731625493765e-3
                                                             + r2 * 2.443315711809948e-5)))
    q = k - 4.0 * jnp.floor(k * 0.25)
    odd = (q == 1.0) | (q == 3.0)
    s0 = jnp.where(odd, cs, sn)
    c0 = jnp.where(odd, sn, cs)
    s1 = jnp.where(q >= 2.0, -s0, s0)
    c1 = jnp.where((q == 1.0) | (q == 2.0), -c0, c0)
    return s1, c1


def _gelu(x):
    c = 0.7978845608028654
    return 0.5 * x * (1.0 + jnp.tanh(c * (x + 0.044715 * (x * x * x))))


def _layernorm(x):
    m = jnp.mean(x, axis=-1, keepdims=True)
    xc = x - m
    v = jnp.mean(xc * xc, axis=-1, keepdims=True)
    den = _rb(jnp.sqrt(_rb(_rb(v) + 1e-5)))
    return _rb(_rb(x - _rb(m)) / den)


def _layernorm2(x):
    m = jnp.mean(x, axis=-1, keepdims=True)
    xc = x - m
    v = jnp.mean(xc * xc, axis=-1, keepdims=True)
    return xc / jnp.sqrt(v + 1e-5)


def _dot(a, b):
    return jnp.dot(a, b, preferred_element_type=jnp.float32)


def _dot_nt(a, b):
    return lax.dot_general(a, b, (((1,), (1,)), ((), ())),
                           preferred_element_type=jnp.float32)


def _kernel(are_hbm, aim_hbm, bre_hbm, bim_hbm, cre_hbm, cim_hbm, ldt_hbm, dsk_hbm,
            ffwd_hbm, finv_hbm, sel_hbm,
            x_hbm, w1_hbm, w2_hbm, w3_hbm, w4_hbm, g_hbm,
            out_hbm,
            p_v, ldt_ref, dsk_ref, ffwd_ref, finv_ref, sel_ref,
            x_v, w1_v, w2_v, w3_v, w4_v, g_v, out_v,
            xn_v, h_v, u_v, kt_v, z_v,
            yr_v, yi_v, xr_v, xi_v, o_v, kd_v, dt_v,
            sem_p, sem_in, sem_out):
    are_ref, aim_ref, bre_ref, bim_ref, cre_ref, cim_ref = [p_v.at[k] for k in range(6)]
    params = (are_hbm, aim_hbm, bre_hbm, bim_hbm, cre_hbm, cim_hbm)
    P0 = 128
    head = [pltpu.make_async_copy(ldt_hbm, ldt_ref, sem_p.at[0])]
    head += [pltpu.make_async_copy(h.at[pl.ds(0, P0), :], p_v.at[k, pl.ds(0, P0), :],
                                   sem_p.at[1 + k]) for k, h in enumerate(params)]
    tail = [pltpu.make_async_copy(h.at[pl.ds(P0, D - P0), :], p_v.at[k, pl.ds(P0, D - P0), :],
                                  sem_p.at[7 + k]) for k, h in enumerate(params)]
    misc = [pltpu.make_async_copy(s, d, sem_p.at[13 + k]) for k, (s, d) in enumerate(
        [(sel_hbm, sel_ref), (ffwd_hbm, ffwd_ref), (finv_hbm, finv_ref), (dsk_hbm, dsk_ref)])]
    copies = [pltpu.make_async_copy(s, d, sem_in.at[k]) for k, (s, d) in enumerate(
        [(x_hbm, x_v), (w1_hbm, w1_v), (g_hbm, g_v), (w2_hbm, w2_v), (w3_hbm, w3_v),
         (w4_hbm, w4_v)])]
    for c in head + tail + misc + copies:
        c.start()
    for c in head:
        c.wait()

    dt_row = _rb(jnp.exp(ldt_ref[...].astype(jnp.float32))).reshape(1, D)
    dt_v[...] = jnp.transpose(jnp.broadcast_to(dt_row, (N, D)))

    def kgen(c, carry):
        @pl.when(c == P0 // CH)
        def _():
            for cp in tail:
                cp.wait()

        r0 = pl.multiple_of(c * CH, CH)
        rows = pl.ds(r0, CH)
        f32 = jnp.float32
        dt = dt_v[rows, :]
        lr = dt * are_ref[rows, :].astype(f32)
        li = dt * aim_ref[rows, :].astype(f32)
        dbr = dt * bre_ref[rows, :].astype(f32)
        dbi = dt * bim_ref[rows, :].astype(f32)
        w = _cmul((cre_ref[rows, :].astype(f32), cim_ref[rows, :].astype(f32)), (dbr, dbi))

        def csq(a):
            ab = a[0] * a[1]
            return (a[0] * a[0] - a[1] * a[1], ab + ab)

        e1 = jnp.exp(lr)
        sn, cs = _sincos(li)
        z1 = (e1 * cs, e1 * sn)
        z8 = csq(csq(csq(z1)))
        z128 = csq(csq(csq(csq(z8))))
        z1024 = csq(csq(csq(z128)))

        def put_y(j, v):
            for g in range(CH // 8):
                yr_v[g, 8 * j:8 * j + 8, :] = v[0][8 * g:8 * g + 8, :]
                yi_v[g, 8 * j:8 * j + 8, :] = v[1][8 * g:8 * g + 8, :]

        def put_x(i, v):
            nvi = -v[1]
            for g in range(CH // 8):
                xr_v[g, 8 * i:8 * i + 8, :] = v[0][8 * g:8 * g + 8, :]
                xi_v[g, 8 * i:8 * i + 8, :] = nvi[8 * g:8 * g + 8, :]

        put_y(0, (jnp.ones_like(lr), jnp.zeros_like(lr)))
        y = z8
        put_y(1, y)
        for j in range(2, 16):
            y = _cmul(y, z8)
            put_y(j, y)
        v = w
        for b in range(8):
            if b:
                v = _cmul(v, z1)
            t = v
            for k in range(8):
                if (128 * k + b) in HI:
                    if k:
                        t = _cmul(t, z128)
                    put_x(HI.index(128 * k + b), t)
        t = _cmul(w, z1024)
        for k in range(8, 17):
            if k > 8:
                t = _cmul(t, z128)
            put_x(HI.index(128 * k), t)
        for g in range(CH // 8):
            o = (_dot_nt(_bf(xr_v[g]), _bf(yr_v[g])) + _dot_nt(_bf(xi_v[g]), _bf(yi_v[g])))
            for i in range(NHI):
                o_v[i, pl.ds(pl.multiple_of(r0 + 8 * g, 8), 8), :] = o[8 * i:8 * i + 8, :]
        return carry

    with jax.named_scope('p_kgen'):
        lax.fori_loop(0, D // CH, kgen, 0)

    rid = lax.broadcasted_iota(jnp.int32, (D, 128), 0)
    lid = lax.broadcasted_iota(jnp.int32, (D, 128), 1)
    keep = (rid % 8) == (lid % 8)
    keep_last = keep & (lid < 8)
    for cp in misc:
        cp.wait()
    sel = sel_ref[...]
    with jax.named_scope('p_sel'):
        for i in range(NHI):
            oi = jnp.where(keep_last if HI[i] == 2048 else keep, o_v[i], 0.0)
            kd_v[16 * i:16 * i + 16, :] = _dot_nt(sel, _bf(oi))

    copies[2].wait()
    off = 0
    for dl in range(NB):
        s0, ln = WIN[dl]
        kt_v[dl] = _dot(g_v[:, off:off + ln], _bf(kd_v[s0:s0 + ln, :]))
        off += ln

    copies[0].wait()
    copies[1].wait()
    h_v[0:8, :] = jnp.zeros((8, D), jnp.float32)
    h_v[8 + L:16 + L, :] = jnp.zeros((8, D), jnp.float32)

    def phase1(b, carry):
        r0 = pl.multiple_of(b * RB, RB)
        xs = []
        for k in range(RB // J):
            rk = pl.multiple_of(r0 + k * J, J)
            xk = _bf(_layernorm(x_v[pl.ds(rk, J), :].astype(jnp.float32)))
            xn_v[pl.ds(rk, J), :] = xk
            u_v[b * (RB // J) + k] = _dot(ffwd_ref[...], xk)
            xs.append(xk)
        h = _gelu(_dot(jnp.concatenate(xs, axis=0), w1_v[...]))
        h_v[pl.ds(pl.multiple_of(r0 + 8, 8), RB), :] = h
        return carry

    with jax.named_scope('p_phase1'):
        lax.fori_loop(0, L // RB, phase1, 0)

    def zphase(t, carry):
        f0 = pl.multiple_of((t // 4) * 8, 8)
        re = pl.ds(f0, 8)
        im = pl.ds(pl.multiple_of(f0 + J, 8), 8)
        cs = pl.ds(pl.multiple_of((t % 4) * 128, 128), 128)
        GZ = 4
        for i0 in range(0, NB, GZ):
            acc = {}
            uc = {}
            for dl in range(i0 + GZ):
                kr = kt_v[dl, re, cs]
                ki = kt_v[dl, im, cs]
                ks = kr + ki
                for i in range(max(i0, dl), i0 + GZ):
                    src = i - dl
                    if src not in uc:
                        ur = u_v[src, re, cs]
                        ui = u_v[src, im, cs]
                        uc[src] = (ur, ui, ur + ui)
                    ur, ui, us = uc[src]
                    p = (kr * ur, ki * ui, ks * us)
                    acc[i] = p if i not in acc else tuple(x + y for x, y in zip(acc[i], p))
            for i in range(i0, i0 + GZ):
                s1, s2, s3 = acc[i]
                z_v[i, re, cs] = s1 - s2
                z_v[i, im, cs] = s3 - (s1 + s2)
        return carry

    with jax.named_scope('p_z'):
        lax.fori_loop(0, 64, zphase, 0)

    copies[3].wait()
    copies[4].wait()
    copies[5].wait()
    dsk = dsk_ref[...].astype(jnp.float32).reshape(1, D)

    def out_copy(b):
        r0 = pl.multiple_of(b * RB, RB)
        return pltpu.make_async_copy(out_v.at[pl.ds(r0, RB), :],
                                     out_hbm.at[pl.ds(r0, RB), :], sem_out.at[b])

    def phase2(b, carry):
        r0 = pl.multiple_of(b * RB, RB)
        ext = RB + 16
        parts = []
        for gi, sh in enumerate((1, -1, 2, -2)):
            hv = h_v[pl.ds(r0, ext), gi * 128:(gi + 1) * 128]
            hv = pltpu.roll(hv, sh % ext, 0)
            parts.append(_bf(hv[8:8 + RB, :]))
        hs = _dot(jnp.concatenate(parts, axis=1), w2_v[...])
        ys = [_dot(finv_ref[...], _bf(z_v[b * (RB // J) + k])) for k in range(RB // J)]
        y = jnp.concatenate(ys, axis=0)
        xn = xn_v[pl.ds(r0, RB), :].astype(jnp.float32)
        x1 = xn + hs
        a = _dot_nt(_bf(_layernorm2(x1)), w3_v[...])
        h2 = _dot(_bf(_gelu(a)), w4_v[...])
        bb = x1 + h2
        gate = bb * jax.nn.sigmoid(bb)
        s = y + xn * dsk
        x = x_v[pl.ds(r0, RB), :].astype(jnp.float32)
        out_v[pl.ds(r0, RB), :] = _bf(x + s * gate)
        out_copy(b).start()
        return carry

    with jax.named_scope('p_phase2'):
        lax.fori_loop(0, L // RB, phase2, 0)
    for b in range(L // RB):
        out_copy(b).wait()


@jax.jit
def pallas_recurrent_scan__ssm_conv_s4__mixer_s_mlp__prompt_kernel(
    A_u: jax.Array,
    A_A_re: jax.Array,
    A_A_im: jax.Array,
    A_B_re: jax.Array,
    A_B_im: jax.Array,
    A_C_re: jax.Array,
    A_C_im: jax.Array,
    A_log_dt: jax.Array,
    A_Dskip: jax.Array,
    B_x: jax.Array,
    B_w1: jax.Array,
    B_w2: jax.Array,
    B_w3: jax.Array,
    B_w4: jax.Array,
):
    bf16 = jnp.bfloat16
    f32 = jnp.float32
    x = A_u.reshape(L, D)
    hbm = pl.BlockSpec(memory_space=pltpu.HBM)
    out = pl.pallas_call(
        _kernel,
        out_shape=jax.ShapeDtypeStruct((L, D), bf16),
        in_specs=[hbm] * 17,
        out_specs=hbm,
        scratch_shapes=[
            pltpu.VMEM((6, D, N), bf16),
            pltpu.VMEM((D,), bf16),
            pltpu.VMEM((D,), bf16),
            pltpu.VMEM((2 * J, J), bf16),
            pltpu.VMEM((J, 2 * J), bf16),
            pltpu.VMEM((16, 128), bf16),
            pltpu.VMEM((L, D), bf16),
            pltpu.VMEM((D, D), bf16),
            pltpu.VMEM((D, D), bf16),
            pltpu.VMEM((FF, D), bf16),
            pltpu.VMEM((FF, D), bf16),
            pltpu.VMEM((2 * J, GW), bf16),
            pltpu.VMEM((L, D), bf16),
            pltpu.VMEM((L, D), bf16),
            pltpu.VMEM((L + 16, D), f32),
            pltpu.VMEM((NB, 2 * J, D), f32),
            pltpu.VMEM((NB, 2 * J, D), f32),
            pltpu.VMEM((NB, 2 * J, D), f32),
            pltpu.VMEM((CH // 8, 128, N), f32),
            pltpu.VMEM((CH // 8, 128, N), f32),
            pltpu.VMEM((CH // 8, 8 * NHI, N), f32),
            pltpu.VMEM((CH // 8, 8 * NHI, N), f32),
            pltpu.VMEM((NHI, D, 128), f32),
            pltpu.VMEM((NQ, D), f32),
            pltpu.VMEM((D, N), f32),
            pltpu.SemaphoreType.DMA((17,)),
            pltpu.SemaphoreType.DMA((6,)),
            pltpu.SemaphoreType.DMA((L // RB,)),
        ],
        compiler_params=pltpu.CompilerParams(vmem_limit_bytes=100 * 1024 * 1024),
    )(*[pltpu.with_memory_space_constraint(t, pltpu.HBM)
        for t in (A_A_re, A_A_im, A_B_re, A_B_im, A_C_re, A_C_im, A_log_dt, A_Dskip,
                  jnp.asarray(_F_FWD, bf16), jnp.asarray(_F_INV, bf16), jnp.asarray(_SEL, bf16),
                  x, B_w1, B_w2, B_w3.T, B_w4, jnp.asarray(_G_ALL, bf16))])
    return out.reshape(1, L, D)
```

```python
import functools
import numpy as np
import jax
import jax.numpy as jnp
from jax import lax
import jax.experimental.pallas as pl
import jax.experimental.pallas.tpu as pltpu

L = 2048
D = 512
N = 128
FF = 1376
J = 128
NB = L // J
NQ = 656
_STEP = (1, 1, 2, 2, 4, 4, 4, 4, 8, 8, 8, 8, 8, 8, 8, 8)
HI = tuple(128 * k + b for k in range(16) for b in range(0, 8, _STEP[k])) + (2048,)
NHI = len(HI)
CH = 32
RB = 512
WIN = ((0, 128), (0, 256), (128, 256), (256, 256), (320, 128), (384, 128),
       (384, 128), (448, 128), (448, 128), (512, 128), (512, 128), (512, 128),
       (512, 128), (512, 128), (512, 128), (528, 128))
GW = sum(w[1] for w in WIN)


def _q_of_m(m):
    hi = (m // 128) * 128 + (m % 8)
    return 16 * HI.index(hi) + (m % 128) // 8


def _build_tables():
    pos = np.arange(L, dtype=np.int64)
    rr = np.zeros(L, np.int64)
    for l in range(L):
        if l < 256:
            rr[l] = l
        else:
            step = 1 << (int(l).bit_length() - 8)
            lo = (l // step) * step
            rem = l - lo
            if rem * 2 < step or (rem * 2 == step and (lo // step) % 2 == 0):
                rr[l] = lo
            else:
                rr[l] = lo + step
    w = np.pi * (2 * np.arange(J) + 1) / (2 * J)
    n = np.arange(J)
    f_fwd = np.concatenate([np.cos(np.outer(w, n)), -np.sin(np.outer(w, n))], 0)
    f_inv = np.concatenate([np.cos(np.outer(n, w)), -np.sin(np.outer(n, w))], 1) / J
    g_all = np.zeros((2 * J, GW))
    off = 0
    for dl in range(NB):
        s0, ln = WIN[dl]
        for p in range(-J, J):
            l = dl * J + p
            if 0 <= l < L:
                q = _q_of_m(int(rr[l])) - s0
                assert 0 <= q < ln
                g_all[:J, off + q] += np.cos(w * p)
                g_all[J:, off + q] += -np.sin(w * p)
        off += ln
    sel = np.zeros((16, 128))
    for dd in range(8):
        sel[np.arange(16), np.arange(16) * 8 + dd] = 1.0
    del pos
    return (f_fwd.astype(np.float32), f_inv.astype(np.float32),
            g_all.astype(np.float32), sel.astype(np.float32))


_F_FWD, _F_INV, _G_ALL, _SEL = _build_tables()


def _bf(x):
    return x.astype(jnp.bfloat16)


def _rb(x):
    return x.astype(jnp.bfloat16).astype(jnp.float32)


def _cmul(a, b):
    return (a[0] * b[0] - a[1] * b[1], a[0] * b[1] + a[1] * b[0])


def _sincos(x):
    k = jnp.floor(x * 0.6366197723675814 + 0.5)
    r = x - k * 1.5703125
    r = r - k * 4.837512969970703125e-4
    r = r - k * 7.549789954891882e-8
    r2 = r * r
    sn = r + r * r2 * (-1.6666654611e-1 + r2 * (8.3321608736e-3 + r2 * -1.9515295891e-4))
    cs = 1.0 + r2 * (-0.5 + r2 * (4.166664568298827e-2 + r2 * (-1.388731625493765e-3
                                                             + r2 * 2.443315711809948e-5)))
    q = k - 4.0 * jnp.floor(k * 0.25)
    odd = (q == 1.0) | (q == 3.0)
    s0 = jnp.where(odd, cs, sn)
    c0 = jnp.where(odd, sn, cs)
    s1 = jnp.where(q >= 2.0, -s0, s0)
    c1 = jnp.where((q == 1.0) | (q == 2.0), -c0, c0)
    return s1, c1


def _gelu(x):
    c = 0.7978845608028654
    return 0.5 * x * (1.0 + jnp.tanh(c * (x + 0.044715 * (x * x * x))))


def _layernorm(x):
    m = jnp.mean(x, axis=-1, keepdims=True)
    xc = x - m
    v = jnp.mean(xc * xc, axis=-1, keepdims=True)
    den = _rb(jnp.sqrt(_rb(_rb(v) + 1e-5)))
    return _rb(_rb(x - _rb(m)) / den)


def _layernorm2(x):
    m = jnp.mean(x, axis=-1, keepdims=True)
    xc = x - m
    v = jnp.mean(xc * xc, axis=-1, keepdims=True)
    return xc / jnp.sqrt(v + 1e-5)


def _dot(a, b):
    return jnp.dot(a, b, preferred_element_type=jnp.float32)


def _dot_nt(a, b):
    return lax.dot_general(a, b, (((1,), (1,)), ((), ())),
                           preferred_element_type=jnp.float32)


def _kernel(are_ref, aim_ref, bre_ref, bim_ref, cre_ref, cim_ref, ldt_ref, dsk_ref,
            ffwd_ref, finv_ref, sel_ref,
            x_hbm, w1_hbm, w2_hbm, w3_hbm, w4_hbm, g_hbm,
            out_hbm,
            x_v, w1_v, w2_v, w3_v, w4_v, g_v, out_v,
            xn_v, h_v, u_v, kt_v, z_v,
            yr_v, yi_v, xr_v, xi_v, o_v, kd_v, dt_v,
            sem_in, sem_out):
    copies = [pltpu.make_async_copy(s, d, sem_in.at[k]) for k, (s, d) in enumerate(
        [(x_hbm, x_v), (w1_hbm, w1_v), (g_hbm, g_v), (w2_hbm, w2_v), (w3_hbm, w3_v),
         (w4_hbm, w4_v)])]
    for c in copies:
        c.start()

    dt_row = _rb(jnp.exp(ldt_ref[...].astype(jnp.float32))).reshape(1, D)
    dt_v[...] = jnp.transpose(jnp.broadcast_to(dt_row, (N, D)))

    def kgen(c, carry):
        r0 = pl.multiple_of(c * CH, CH)
        rows = pl.ds(r0, CH)
        f32 = jnp.float32
        dt = dt_v[rows, :]
        lr = dt * are_ref[rows, :].astype(f32)
        li = dt * aim_ref[rows, :].astype(f32)
        dbr = dt * bre_ref[rows, :].astype(f32)
        dbi = dt * bim_ref[rows, :].astype(f32)
        w = _cmul((cre_ref[rows, :].astype(f32), cim_ref[rows, :].astype(f32)), (dbr, dbi))

        def csq(a):
            ab = a[0] * a[1]
            return (a[0] * a[0] - a[1] * a[1], ab + ab)

        e1 = jnp.exp(lr)
        sn, cs = _sincos(li)
        z1 = (e1 * cs, e1 * sn)
        z8 = csq(csq(csq(z1)))
        z128 = csq(csq(csq(csq(z8))))
        z1024 = csq(csq(csq(z128)))

        def put_y(j, v):
            for g in range(CH // 8):
                yr_v[g, 8 * j:8 * j + 8, :] = v[0][8 * g:8 * g + 8, :]
                yi_v[g, 8 * j:8 * j + 8, :] = v[1][8 * g:8 * g + 8, :]

        def put_x(i, v):
            nvi = -v[1]
            for g in range(CH // 8):
                xr_v[g, 8 * i:8 * i + 8, :] = v[0][8 * g:8 * g + 8, :]
                xi_v[g, 8 * i:8 * i + 8, :] = nvi[8 * g:8 * g + 8, :]

        put_y(0, (jnp.ones_like(lr), jnp.zeros_like(lr)))
        y = z8
        put_y(1, y)
        for j in range(2, 16):
            y = _cmul(y, z8)
            put_y(j, y)
        v = w
        for b in range(8):
            if b:
                v = _cmul(v, z1)
            t = v
            for k in range(8):
                if (128 * k + b) in HI:
                    if k:
                        t = _cmul(t, z128)
                    put_x(HI.index(128 * k + b), t)
        t = _cmul(w, z1024)
        for k in range(8, 17):
            if k > 8:
                t = _cmul(t, z128)
            put_x(HI.index(128 * k), t)
        for g in range(CH // 8):
            o = (_dot_nt(_bf(xr_v[g]), _bf(yr_v[g])) + _dot_nt(_bf(xi_v[g]), _bf(yi_v[g])))
            for i in range(NHI):
                o_v[i, pl.ds(pl.multiple_of(r0 + 8 * g, 8), 8), :] = o[8 * i:8 * i + 8, :]
        return carry

    with jax.named_scope('p_kgen'):
        lax.fori_loop(0, D // CH, kgen, 0)

    rid = lax.broadcasted_iota(jnp.int32, (D, 128), 0)
    lid = lax.broadcasted_iota(jnp.int32, (D, 128), 1)
    keep = (rid % 8) == (lid % 8)
    keep_last = keep & (lid < 8)
    sel = sel_ref[...]
    with jax.named_scope('p_sel'):
        for i in range(NHI):
            oi = jnp.where(keep_last if HI[i] == 2048 else keep, o_v[i], 0.0)
            kd_v[16 * i:16 * i + 16, :] = _dot_nt(sel, _bf(oi))

    copies[2].wait()
    off = 0
    for dl in range(NB):
        s0, ln = WIN[dl]
        kt_v[dl] = _dot(g_v[:, off:off + ln], _bf(kd_v[s0:s0 + ln, :]))
        off += ln

    copies[0].wait()
    copies[1].wait()
    h_v[0:8, :] = jnp.zeros((8, D), jnp.float32)
    h_v[8 + L:16 + L, :] = jnp.zeros((8, D), jnp.float32)

    def phase1(b, carry):
        r0 = pl.multiple_of(b * RB, RB)
        xs = []
        for k in range(RB // J):
            rk = pl.multiple_of(r0 + k * J, J)
            xk = _bf(_layernorm(x_v[pl.ds(rk, J), :].astype(jnp.float32)))
            xn_v[pl.ds(rk, J), :] = xk
            u_v[b * (RB // J) + k] = _dot(ffwd_ref[...], xk)
            xs.append(xk)
        h = _gelu(_dot(jnp.concatenate(xs, axis=0), w1_v[...]))
        h_v[pl.ds(pl.multiple_of(r0 + 8, 8), RB), :] = h
        return carry

    with jax.named_scope('p_phase1'):
        lax.fori_loop(0, L // RB, phase1, 0)

    def zphase(t, carry):
        f0 = pl.multiple_of((t // 4) * 8, 8)
        re = pl.ds(f0, 8)
        im = pl.ds(pl.multiple_of(f0 + J, 8), 8)
        cs = pl.ds(pl.multiple_of((t % 4) * 128, 128), 128)
        GZ = 4
        for i0 in range(0, NB, GZ):
            acc = {}
            uc = {}
            for dl in range(i0 + GZ):
                kr = kt_v[dl, re, cs]
                ki = kt_v[dl, im, cs]
                ks = kr + ki
                for i in range(max(i0, dl), i0 + GZ):
                    src = i - dl
                    if src not in uc:
                        ur = u_v[src, re, cs]
                        ui = u_v[src, im, cs]
                        uc[src] = (ur, ui, ur + ui)
                    ur, ui, us = uc[src]
                    p = (kr * ur, ki * ui, ks * us)
                    acc[i] = p if i not in acc else tuple(x + y for x, y in zip(acc[i], p))
            for i in range(i0, i0 + GZ):
                s1, s2, s3 = acc[i]
                z_v[i, re, cs] = s1 - s2
                z_v[i, im, cs] = s3 - (s1 + s2)
        return carry

    with jax.named_scope('p_z'):
        lax.fori_loop(0, 64, zphase, 0)

    copies[3].wait()
    copies[4].wait()
    copies[5].wait()
    dsk = dsk_ref[...].astype(jnp.float32).reshape(1, D)

    HB = RB // 2

    def out_copy(b):
        r0 = pl.multiple_of(b * HB, HB)
        return pltpu.make_async_copy(out_v.at[pl.ds(r0, HB), :],
                                     out_hbm.at[pl.ds(r0, HB), :], sem_out.at[b])

    def phase2(b, carry):
        r0 = pl.multiple_of(b * RB, RB)
        ext = RB + 16
        parts = []
        for gi, sh in enumerate((1, -1, 2, -2)):
            hv = h_v[pl.ds(r0, ext), gi * 128:(gi + 1) * 128]
            hv = pltpu.roll(hv, sh % ext, 0)
            parts.append(_bf(hv[8:8 + RB, :]))
        hs = _dot(jnp.concatenate(parts, axis=1), w2_v[...])
        ys = [_dot(finv_ref[...], _bf(z_v[b * (RB // J) + k])) for k in range(RB // J)]
        y = jnp.concatenate(ys, axis=0)
        xn = xn_v[pl.ds(r0, RB), :].astype(jnp.float32)
        x1 = xn + hs
        a = _dot_nt(_bf(_layernorm2(x1)), w3_v[...])
        for hf in range(2):
            sl = slice(hf * HB, (hf + 1) * HB)
            rh = pl.multiple_of(r0 + hf * HB, HB)
            bb = x1[sl] + _dot(_bf(_gelu(a[sl])), w4_v[...])
            gate = bb * jax.nn.sigmoid(bb)
            s = y[sl] + xn[sl] * dsk
            x = x_v[pl.ds(rh, HB), :].astype(jnp.float32)
            out_v[pl.ds(rh, HB), :] = _bf(x + s * gate)
            out_copy(2 * b + hf).start()
        return carry

    with jax.named_scope('p_phase2'):
        lax.fori_loop(0, L // RB, phase2, 0)
    for b in range(L // HB):
        out_copy(b).wait()


@jax.jit
def pallas_recurrent_scan__ssm_conv_s4__mixer_s_mlp__prompt_kernel(
    A_u: jax.Array,
    A_A_re: jax.Array,
    A_A_im: jax.Array,
    A_B_re: jax.Array,
    A_B_im: jax.Array,
    A_C_re: jax.Array,
    A_C_im: jax.Array,
    A_log_dt: jax.Array,
    A_Dskip: jax.Array,
    B_x: jax.Array,
    B_w1: jax.Array,
    B_w2: jax.Array,
    B_w3: jax.Array,
    B_w4: jax.Array,
):
    bf16 = jnp.bfloat16
    f32 = jnp.float32
    x = A_u.reshape(L, D)
    vm = pl.BlockSpec(memory_space=pltpu.VMEM)
    hbm = pl.BlockSpec(memory_space=pltpu.HBM)
    out = pl.pallas_call(
        _kernel,
        out_shape=jax.ShapeDtypeStruct((L, D), bf16),
        in_specs=[vm] * 11 + [hbm] * 6,
        out_specs=hbm,
        scratch_shapes=[
            pltpu.VMEM((L, D), bf16),
            pltpu.VMEM((D, D), bf16),
            pltpu.VMEM((D, D), bf16),
            pltpu.VMEM((FF, D), bf16),
            pltpu.VMEM((FF, D), bf16),
            pltpu.VMEM((2 * J, GW), bf16),
            pltpu.VMEM((L, D), bf16),
            pltpu.VMEM((L, D), bf16),
            pltpu.VMEM((L + 16, D), f32),
            pltpu.VMEM((NB, 2 * J, D), f32),
            pltpu.VMEM((NB, 2 * J, D), f32),
            pltpu.VMEM((NB, 2 * J, D), f32),
            pltpu.VMEM((CH // 8, 128, N), f32),
            pltpu.VMEM((CH // 8, 128, N), f32),
            pltpu.VMEM((CH // 8, 8 * NHI, N), f32),
            pltpu.VMEM((CH // 8, 8 * NHI, N), f32),
            pltpu.VMEM((NHI, D, 128), f32),
            pltpu.VMEM((NQ, D), f32),
            pltpu.VMEM((D, N), f32),
            pltpu.SemaphoreType.DMA((6,)),
            pltpu.SemaphoreType.DMA((2 * L // RB,)),
        ],
        compiler_params=pltpu.CompilerParams(vmem_limit_bytes=100 * 1024 * 1024),
    )(A_A_re, A_A_im, A_B_re, A_B_im, A_C_re, A_C_im,
      A_log_dt, A_Dskip,
      jnp.asarray(_F_FWD, bf16), jnp.asarray(_F_INV, bf16), jnp.asarray(_SEL, bf16),
      *[pltpu.with_memory_space_constraint(t, pltpu.HBM)
        for t in (x, B_w1, B_w2, B_w3.T, B_w4, jnp.asarray(_G_ALL, bf16))])
    return out.reshape(1, L, D)
```

```python
import functools
import numpy as np
import jax
import jax.numpy as jnp
from jax import lax
import jax.experimental.pallas as pl
import jax.experimental.pallas.tpu as pltpu

L = 2048
D = 512
N = 128
FF = 1376
J = 128
NB = L // J
NQ = 656
_STEP = (1, 1, 2, 2, 4, 4, 4, 4, 8, 8, 8, 8, 8, 8, 8, 8)
HI = tuple(128 * k + b for k in range(16) for b in range(0, 8, _STEP[k])) + (2048,)
NHI = len(HI)
CH = 32
RB = 512
WIN = ((0, 128), (0, 256), (128, 256), (256, 256), (320, 128), (384, 128),
       (384, 128), (448, 128), (448, 128), (512, 128), (512, 128), (512, 128),
       (512, 128), (512, 128), (512, 128), (528, 128))
GW = sum(w[1] for w in WIN)


def _q_of_m(m):
    hi = (m // 128) * 128 + (m % 8)
    return 16 * HI.index(hi) + (m % 128) // 8


def _build_tables():
    pos = np.arange(L, dtype=np.int64)
    rr = np.zeros(L, np.int64)
    for l in range(L):
        if l < 256:
            rr[l] = l
        else:
            step = 1 << (int(l).bit_length() - 8)
            lo = (l // step) * step
            rem = l - lo
            if rem * 2 < step or (rem * 2 == step and (lo // step) % 2 == 0):
                rr[l] = lo
            else:
                rr[l] = lo + step
    w = np.pi * (2 * np.arange(J) + 1) / (2 * J)
    n = np.arange(J)
    f_fwd = np.concatenate([np.cos(np.outer(w, n)), -np.sin(np.outer(w, n))], 0)
    f_inv = np.concatenate([np.cos(np.outer(n, w)), -np.sin(np.outer(n, w))], 1) / J
    g_all = np.zeros((2 * J, GW))
    off = 0
    for dl in range(NB):
        s0, ln = WIN[dl]
        for p in range(-J, J):
            l = dl * J + p
            if 0 <= l < L:
                q = _q_of_m(int(rr[l])) - s0
                assert 0 <= q < ln
                g_all[:J, off + q] += np.cos(w * p)
                g_all[J:, off + q] += -np.sin(w * p)
        off += ln
    sel = np.zeros((16, 128))
    for dd in range(8):
        sel[np.arange(16), np.arange(16) * 8 + dd] = 1.0
    del pos
    return (f_fwd.astype(np.float32), f_inv.astype(np.float32),
            g_all.astype(np.float32), sel.astype(np.float32))


_F_FWD, _F_INV, _G_ALL, _SEL = _build_tables()


def _bf(x):
    return x.astype(jnp.bfloat16)


def _rb(x):
    return x.astype(jnp.bfloat16).astype(jnp.float32)


def _cmul(a, b):
    return (a[0] * b[0] - a[1] * b[1], a[0] * b[1] + a[1] * b[0])


def _sincos(x):
    k = jnp.floor(x * 0.6366197723675814 + 0.5)
    r = x - k * 1.5703125
    r = r - k * 4.837512969970703125e-4
    r = r - k * 7.549789954891882e-8
    r2 = r * r
    sn = r + r * r2 * (-1.6666654611e-1 + r2 * (8.3321608736e-3 + r2 * -1.9515295891e-4))
    cs = 1.0 + r2 * (-0.5 + r2 * (4.166664568298827e-2 + r2 * (-1.388731625493765e-3
                                                             + r2 * 2.443315711809948e-5)))
    q = k - 4.0 * jnp.floor(k * 0.25)
    odd = (q == 1.0) | (q == 3.0)
    s0 = jnp.where(odd, cs, sn)
    c0 = jnp.where(odd, sn, cs)
    s1 = jnp.where(q >= 2.0, -s0, s0)
    c1 = jnp.where((q == 1.0) | (q == 2.0), -c0, c0)
    return s1, c1


def _gelu(x):
    c = 0.7978845608028654
    return 0.5 * x * (1.0 + jnp.tanh(c * (x + 0.044715 * (x * x * x))))


def _layernorm(x):
    m = jnp.mean(x, axis=-1, keepdims=True)
    xc = x - m
    v = jnp.mean(xc * xc, axis=-1, keepdims=True)
    den = _rb(jnp.sqrt(_rb(_rb(v) + 1e-5)))
    return _rb(_rb(x - _rb(m)) / den)


def _layernorm2(x):
    m = jnp.mean(x, axis=-1, keepdims=True)
    xc = x - m
    v = jnp.mean(xc * xc, axis=-1, keepdims=True)
    return xc / jnp.sqrt(v + 1e-5)


def _dot(a, b):
    return jnp.dot(a, b, preferred_element_type=jnp.float32)


def _dot_nt(a, b):
    return lax.dot_general(a, b, (((1,), (1,)), ((), ())),
                           preferred_element_type=jnp.float32)


def _kernel(are_ref, aim_ref, bre_ref, bim_ref, cre_ref, cim_ref, ldt_ref, dsk_ref,
            ffwd_ref, finv_ref, sel_ref,
            x_hbm, w1_hbm, w2_hbm, w3_hbm, w4_hbm, g_hbm,
            out_hbm,
            x_v, w1_v, w2_v, w3_v, w4_v, g_v, out_v,
            xn_v, h_v, u_v, kt_v, z_v,
            yr_v, yi_v, xr_v, xi_v, o_v, kd_v, dt_v,
            sem_in, sem_out):
    copies = [pltpu.make_async_copy(s, d, sem_in.at[k]) for k, (s, d) in enumerate(
        [(x_hbm, x_v), (w1_hbm, w1_v), (g_hbm, g_v), (w2_hbm, w2_v), (w3_hbm, w3_v),
         (w4_hbm, w4_v)])]
    for c in copies:
        c.start()

    dt_row = _rb(jnp.exp(ldt_ref[...].astype(jnp.float32))).reshape(1, D)
    dt_v[...] = jnp.transpose(jnp.broadcast_to(dt_row, (N, D)))

    def kgen(c, carry):
        r0 = pl.multiple_of(c * CH, CH)
        rows = pl.ds(r0, CH)
        f32 = jnp.float32
        dt = dt_v[rows, :]
        lr = dt * are_ref[rows, :].astype(f32)
        li = dt * aim_ref[rows, :].astype(f32)
        dbr = dt * bre_ref[rows, :].astype(f32)
        dbi = dt * bim_ref[rows, :].astype(f32)
        w = _cmul((cre_ref[rows, :].astype(f32), cim_ref[rows, :].astype(f32)), (dbr, dbi))

        def csq(a):
            ab = a[0] * a[1]
            return (a[0] * a[0] - a[1] * a[1], ab + ab)

        e1 = jnp.exp(lr)
        sn, cs = _sincos(li)
        z1 = (e1 * cs, e1 * sn)
        z8 = csq(csq(csq(z1)))
        z128 = csq(csq(csq(csq(z8))))
        z1024 = csq(csq(csq(z128)))

        def put_y(j, v):
            for g in range(CH // 8):
                yr_v[g, 8 * j:8 * j + 8, :] = v[0][8 * g:8 * g + 8, :]
                yi_v[g, 8 * j:8 * j + 8, :] = v[1][8 * g:8 * g + 8, :]

        def put_x(i, v):
            nvi = -v[1]
            for g in range(CH // 8):
                xr_v[g, 8 * i:8 * i + 8, :] = v[0][8 * g:8 * g + 8, :]
                xi_v[g, 8 * i:8 * i + 8, :] = nvi[8 * g:8 * g + 8, :]

        put_y(0, (jnp.ones_like(lr), jnp.zeros_like(lr)))
        y = z8
        put_y(1, y)
        for j in range(2, 16):
            y = _cmul(y, z8)
            put_y(j, y)
        v = w
        for b in range(8):
            if b:
                v = _cmul(v, z1)
            t = v
            for k in range(8):
                if (128 * k + b) in HI:
                    if k:
                        t = _cmul(t, z128)
                    put_x(HI.index(128 * k + b), t)
        t = _cmul(w, z1024)
        for k in range(8, 17):
            if k > 8:
                t = _cmul(t, z128)
            put_x(HI.index(128 * k), t)
        for g in range(CH // 8):
            o = (_dot_nt(_bf(xr_v[g]), _bf(yr_v[g])) + _dot_nt(_bf(xi_v[g]), _bf(yi_v[g])))
            for i in range(NHI):
                o_v[i, pl.ds(pl.multiple_of(r0 + 8 * g, 8), 8), :] = o[8 * i:8 * i + 8, :]
        return carry

    with jax.named_scope('p_kgen'):
        lax.fori_loop(0, D // CH, kgen, 0)

    rid = lax.broadcasted_iota(jnp.int32, (D, 128), 0)
    lid = lax.broadcasted_iota(jnp.int32, (D, 128), 1)
    keep = (rid % 8) == (lid % 8)
    keep_last = keep & (lid < 8)
    sel = sel_ref[...]
    with jax.named_scope('p_sel'):
        for i in range(NHI):
            oi = jnp.where(keep_last if HI[i] == 2048 else keep, o_v[i], 0.0)
            kd_v[16 * i:16 * i + 16, :] = _dot_nt(sel, _bf(oi))

    copies[2].wait()
    off = 0
    for dl in range(NB):
        s0, ln = WIN[dl]
        kt_v[dl] = _dot(g_v[:, off:off + ln], _bf(kd_v[s0:s0 + ln, :]))
        off += ln

    copies[0].wait()
    copies[1].wait()
    h_v[0:8, :] = jnp.zeros((8, D), jnp.float32)
    h_v[8 + L:16 + L, :] = jnp.zeros((8, D), jnp.float32)

    def phase1(b, carry):
        r0 = pl.multiple_of(b * RB, RB)
        xs = []
        for k in range(RB // J):
            rk = pl.multiple_of(r0 + k * J, J)
            xk = _bf(_layernorm(x_v[pl.ds(rk, J), :].astype(jnp.float32)))
            xn_v[pl.ds(rk, J), :] = xk
            u_v[b * (RB // J) + k] = _dot(ffwd_ref[...], xk)
            xs.append(xk)
        h = _gelu(_dot(jnp.concatenate(xs, axis=0), w1_v[...]))
        h_v[pl.ds(pl.multiple_of(r0 + 8, 8), RB), :] = h
        return carry

    with jax.named_scope('p_phase1'):
        lax.fori_loop(0, L // RB, phase1, 0)

    def zphase(t, carry):
        f0 = pl.multiple_of((t // 4) * 8, 8)
        re = pl.ds(f0, 8)
        im = pl.ds(pl.multiple_of(f0 + J, 8), 8)
        cs = pl.ds(pl.multiple_of((t % 4) * 128, 128), 128)
        GZ = 4
        for i0 in range(0, NB, GZ):
            acc = {}
            uc = {}
            for dl in range(i0 + GZ):
                kr = kt_v[dl, re, cs]
                ki = kt_v[dl, im, cs]
                ks = kr + ki
                for i in range(max(i0, dl), i0 + GZ):
                    src = i - dl
                    if src not in uc:
                        ur = u_v[src, re, cs]
                        ui = u_v[src, im, cs]
                        uc[src] = (ur, ui, ur + ui)
                    ur, ui, us = uc[src]
                    p = (kr * ur, ki * ui, ks * us)
                    acc[i] = p if i not in acc else tuple(x + y for x, y in zip(acc[i], p))
            for i in range(i0, i0 + GZ):
                s1, s2, s3 = acc[i]
                z_v[i, re, cs] = s1 - s2
                z_v[i, im, cs] = s3 - (s1 + s2)
        return carry

    with jax.named_scope('p_z'):
        lax.fori_loop(0, 64, zphase, 0)

    copies[3].wait()
    copies[4].wait()
    copies[5].wait()
    dsk = dsk_ref[...].astype(jnp.float32).reshape(1, D)

    HB = RB // 4

    def out_copy(b):
        r0 = pl.multiple_of(b * HB, HB)
        return pltpu.make_async_copy(out_v.at[pl.ds(r0, HB), :],
                                     out_hbm.at[pl.ds(r0, HB), :], sem_out.at[b])

    def phase2(b, carry):
        r0 = pl.multiple_of(b * RB, RB)
        ext = RB + 16
        parts = []
        for gi, sh in enumerate((1, -1, 2, -2)):
            hv = h_v[pl.ds(r0, ext), gi * 128:(gi + 1) * 128]
            hv = pltpu.roll(hv, sh % ext, 0)
            parts.append(_bf(hv[8:8 + RB, :]))
        hs = _dot(jnp.concatenate(parts, axis=1), w2_v[...])
        ys = [_dot(finv_ref[...], _bf(z_v[b * (RB // J) + k])) for k in range(RB // J)]
        y = jnp.concatenate(ys, axis=0)
        xn = xn_v[pl.ds(r0, RB), :].astype(jnp.float32)
        x1 = xn + hs
        a = _dot_nt(_bf(_layernorm2(x1)), w3_v[...])
        for hf in range(4):
            sl = slice(hf * HB, (hf + 1) * HB)
            rh = pl.multiple_of(r0 + hf * HB, HB)
            bb = x1[sl] + _dot(_bf(_gelu(a[sl])), w4_v[...])
            gate = bb * jax.nn.sigmoid(bb)
            s = y[sl] + xn[sl] * dsk
            x = x_v[pl.ds(rh, HB), :].astype(jnp.float32)
            out_v[pl.ds(rh, HB), :] = _bf(x + s * gate)
            out_copy(4 * b + hf).start()
        return carry

    with jax.named_scope('p_phase2'):
        lax.fori_loop(0, L // RB, phase2, 0)
    for b in range(L // HB):
        out_copy(b).wait()


@jax.jit
def pallas_recurrent_scan__ssm_conv_s4__mixer_s_mlp__prompt_kernel(
    A_u: jax.Array,
    A_A_re: jax.Array,
    A_A_im: jax.Array,
    A_B_re: jax.Array,
    A_B_im: jax.Array,
    A_C_re: jax.Array,
    A_C_im: jax.Array,
    A_log_dt: jax.Array,
    A_Dskip: jax.Array,
    B_x: jax.Array,
    B_w1: jax.Array,
    B_w2: jax.Array,
    B_w3: jax.Array,
    B_w4: jax.Array,
):
    bf16 = jnp.bfloat16
    f32 = jnp.float32
    x = A_u.reshape(L, D)
    vm = pl.BlockSpec(memory_space=pltpu.VMEM)
    hbm = pl.BlockSpec(memory_space=pltpu.HBM)
    out = pl.pallas_call(
        _kernel,
        out_shape=jax.ShapeDtypeStruct((L, D), bf16),
        in_specs=[vm] * 11 + [hbm] * 6,
        out_specs=hbm,
        scratch_shapes=[
            pltpu.VMEM((L, D), bf16),
            pltpu.VMEM((D, D), bf16),
            pltpu.VMEM((D, D), bf16),
            pltpu.VMEM((FF, D), bf16),
            pltpu.VMEM((FF, D), bf16),
            pltpu.VMEM((2 * J, GW), bf16),
            pltpu.VMEM((L, D), bf16),
            pltpu.VMEM((L, D), bf16),
            pltpu.VMEM((L + 16, D), f32),
            pltpu.VMEM((NB, 2 * J, D), f32),
            pltpu.VMEM((NB, 2 * J, D), f32),
            pltpu.VMEM((NB, 2 * J, D), f32),
            pltpu.VMEM((CH // 8, 128, N), f32),
            pltpu.VMEM((CH // 8, 128, N), f32),
            pltpu.VMEM((CH // 8, 8 * NHI, N), f32),
            pltpu.VMEM((CH // 8, 8 * NHI, N), f32),
            pltpu.VMEM((NHI, D, 128), f32),
            pltpu.VMEM((NQ, D), f32),
            pltpu.VMEM((D, N), f32),
            pltpu.SemaphoreType.DMA((6,)),
            pltpu.SemaphoreType.DMA((4 * L // RB,)),
        ],
        compiler_params=pltpu.CompilerParams(vmem_limit_bytes=100 * 1024 * 1024),
    )(A_A_re, A_A_im, A_B_re, A_B_im, A_C_re, A_C_im,
      A_log_dt, A_Dskip,
      jnp.asarray(_F_FWD, bf16), jnp.asarray(_F_INV, bf16), jnp.asarray(_SEL, bf16),
      *[pltpu.with_memory_space_constraint(t, pltpu.HBM)
        for t in (x, B_w1, B_w2, B_w3.T, B_w4, jnp.asarray(_G_ALL, bf16))])
    return out.reshape(1, L, D)
```

```python
import functools
import numpy as np
import jax
import jax.numpy as jnp
from jax import lax
import jax.experimental.pallas as pl
import jax.experimental.pallas.tpu as pltpu

L = 2048
D = 512
N = 128
FF = 1376
J = 128
NB = L // J
NQ = 656
_STEP = (1, 1, 2, 2, 4, 4, 4, 4, 8, 8, 8, 8, 8, 8, 8, 8)
HI = tuple(128 * k + b for k in range(16) for b in range(0, 8, _STEP[k])) + (2048,)
NHI = len(HI)
CH = 32
RB = 512
WIN = ((0, 128), (0, 256), (128, 256), (256, 256), (320, 128), (384, 128),
       (384, 128), (448, 128), (448, 128), (512, 128), (512, 128), (512, 128),
       (512, 128), (512, 128), (512, 128), (528, 128))
GW = sum(w[1] for w in WIN)


def _q_of_m(m):
    hi = (m // 128) * 128 + (m % 8)
    return 16 * HI.index(hi) + (m % 128) // 8


def _build_tables():
    pos = np.arange(L, dtype=np.int64)
    rr = np.zeros(L, np.int64)
    for l in range(L):
        if l < 256:
            rr[l] = l
        else:
            step = 1 << (int(l).bit_length() - 8)
            lo = (l // step) * step
            rem = l - lo
            if rem * 2 < step or (rem * 2 == step and (lo // step) % 2 == 0):
                rr[l] = lo
            else:
                rr[l] = lo + step
    w = np.pi * (2 * np.arange(J) + 1) / (2 * J)
    n = np.arange(J)
    f_fwd = np.concatenate([np.cos(np.outer(w, n)), -np.sin(np.outer(w, n))], 0)
    f_inv = np.concatenate([np.cos(np.outer(n, w)), -np.sin(np.outer(n, w))], 1) / J
    g_all = np.zeros((2 * J, GW))
    off = 0
    for dl in range(NB):
        s0, ln = WIN[dl]
        for p in range(-J, J):
            l = dl * J + p
            if 0 <= l < L:
                q = _q_of_m(int(rr[l])) - s0
                assert 0 <= q < ln
                g_all[:J, off + q] += np.cos(w * p)
                g_all[J:, off + q] += -np.sin(w * p)
        off += ln
    sel = np.zeros((16, 128))
    for dd in range(8):
        sel[np.arange(16), np.arange(16) * 8 + dd] = 1.0
    del pos
    return (f_fwd.astype(np.float32), f_inv.astype(np.float32),
            g_all.astype(np.float32), sel.astype(np.float32))


_F_FWD, _F_INV, _G_ALL, _SEL = _build_tables()


def _bf(x):
    return x.astype(jnp.bfloat16)


def _rb(x):
    return x.astype(jnp.bfloat16).astype(jnp.float32)


def _cmul(a, b):
    return (a[0] * b[0] - a[1] * b[1], a[0] * b[1] + a[1] * b[0])


def _sincos(x):
    k = jnp.floor(x * 0.6366197723675814 + 0.5)
    r = x - k * 1.5703125
    r = r - k * 4.837512969970703125e-4
    r = r - k * 7.549789954891882e-8
    r2 = r * r
    sn = r + r * r2 * (-1.6666654611e-1 + r2 * (8.3321608736e-3 + r2 * -1.9515295891e-4))
    cs = 1.0 + r2 * (-0.5 + r2 * (4.166664568298827e-2 + r2 * (-1.388731625493765e-3
                                                             + r2 * 2.443315711809948e-5)))
    q = k - 4.0 * jnp.floor(k * 0.25)
    odd = (q == 1.0) | (q == 3.0)
    s0 = jnp.where(odd, cs, sn)
    c0 = jnp.where(odd, sn, cs)
    s1 = jnp.where(q >= 2.0, -s0, s0)
    c1 = jnp.where((q == 1.0) | (q == 2.0), -c0, c0)
    return s1, c1


def _gelu(x):
    c = 0.7978845608028654
    return 0.5 * x * (1.0 + jnp.tanh(c * (x + 0.044715 * (x * x * x))))


def _layernorm(x):
    m = jnp.mean(x, axis=-1, keepdims=True)
    xc = x - m
    v = jnp.mean(xc * xc, axis=-1, keepdims=True)
    den = _rb(jnp.sqrt(_rb(_rb(v) + 1e-5)))
    return _rb(_rb(x - _rb(m)) / den)


def _layernorm2(x):
    m = jnp.mean(x, axis=-1, keepdims=True)
    xc = x - m
    v = jnp.mean(xc * xc, axis=-1, keepdims=True)
    return xc / jnp.sqrt(v + 1e-5)


def _dot(a, b):
    return jnp.dot(a, b, preferred_element_type=jnp.float32)


def _dot_nt(a, b):
    return lax.dot_general(a, b, (((1,), (1,)), ((), ())),
                           preferred_element_type=jnp.float32)


def _kernel(are_ref, aim_ref, bre_ref, bim_ref, cre_ref, cim_ref, ldt_ref, dsk_ref,
            ffwd_ref, finv_ref, sel_ref,
            x_hbm, w1_hbm, w2_hbm, w3_hbm, w4_hbm, g_hbm,
            out_hbm,
            x_v, w1_v, w2_v, w3_v, w4_v, g_v, out_v,
            xn_v, h_v, u_v, kt_v, z_v,
            yr_v, yi_v, xr_v, xi_v, o_v, kd_v, dt_v,
            sem_in, sem_out):
    copies = [pltpu.make_async_copy(s, d, sem_in.at[k]) for k, (s, d) in enumerate(
        [(x_hbm, x_v), (w1_hbm, w1_v), (g_hbm, g_v), (w2_hbm, w2_v), (w3_hbm, w3_v),
         (w4_hbm, w4_v)])]
    for c in copies:
        c.start()

    dt_row = _rb(jnp.exp(ldt_ref[...].astype(jnp.float32))).reshape(1, D)
    dt_v[...] = jnp.transpose(jnp.broadcast_to(dt_row, (N, D)))

    def kgen(c, carry):
        r0 = pl.multiple_of(c * CH, CH)
        rows = pl.ds(r0, CH)
        f32 = jnp.float32
        dt = dt_v[rows, :]
        lr = dt * are_ref[rows, :].astype(f32)
        li = dt * aim_ref[rows, :].astype(f32)
        dbr = dt * bre_ref[rows, :].astype(f32)
        dbi = dt * bim_ref[rows, :].astype(f32)
        w = _cmul((cre_ref[rows, :].astype(f32), cim_ref[rows, :].astype(f32)), (dbr, dbi))

        def csq(a):
            ab = a[0] * a[1]
            return (a[0] * a[0] - a[1] * a[1], ab + ab)

        e1 = jnp.exp(lr)
        sn, cs = _sincos(li)
        z1 = (e1 * cs, e1 * sn)
        z8 = csq(csq(csq(z1)))
        z128 = csq(csq(csq(csq(z8))))
        z1024 = csq(csq(csq(z128)))

        def put_y(j, v):
            for g in range(CH // 8):
                yr_v[g, 8 * j:8 * j + 8, :] = v[0][8 * g:8 * g + 8, :]
                yi_v[g, 8 * j:8 * j + 8, :] = v[1][8 * g:8 * g + 8, :]

        def put_x(i, v):
            nvi = -v[1]
            for g in range(CH // 8):
                xr_v[g, 8 * i:8 * i + 8, :] = v[0][8 * g:8 * g + 8, :]
                xi_v[g, 8 * i:8 * i + 8, :] = nvi[8 * g:8 * g + 8, :]

        put_y(0, (jnp.ones_like(lr), jnp.zeros_like(lr)))
        y = z8
        put_y(1, y)
        for j in range(2, 16):
            y = _cmul(y, z8)
            put_y(j, y)
        v = w
        for b in range(8):
            if b:
                v = _cmul(v, z1)
            t = v
            for k in range(8):
                if (128 * k + b) in HI:
                    if k:
                        t = _cmul(t, z128)
                    put_x(HI.index(128 * k + b), t)
        t = _cmul(w, z1024)
        for k in range(8, 17):
            if k > 8:
                t = _cmul(t, z128)
            put_x(HI.index(128 * k), t)
        for g in range(CH // 8):
            o = (_dot_nt(_bf(xr_v[g]), _bf(yr_v[g])) + _dot_nt(_bf(xi_v[g]), _bf(yi_v[g])))
            for i in range(NHI):
                o_v[i, pl.ds(pl.multiple_of(r0 + 8 * g, 8), 8), :] = o[8 * i:8 * i + 8, :]
        return carry

    with jax.named_scope('p_kgen'):
        lax.fori_loop(0, D // CH, kgen, 0)

    rid = lax.broadcasted_iota(jnp.int32, (D, 128), 0)
    lid = lax.broadcasted_iota(jnp.int32, (D, 128), 1)
    keep = (rid % 8) == (lid % 8)
    keep_last = keep & (lid < 8)
    sel = sel_ref[...]
    with jax.named_scope('p_sel'):
        for i in range(NHI):
            oi = jnp.where(keep_last if HI[i] == 2048 else keep, o_v[i], 0.0)
            kd_v[16 * i:16 * i + 16, :] = _dot_nt(sel, _bf(oi))

    copies[2].wait()
    off = 0
    for dl in range(NB):
        s0, ln = WIN[dl]
        kt_v[dl] = _dot(g_v[:, off:off + ln], _bf(kd_v[s0:s0 + ln, :]))
        off += ln

    copies[0].wait()
    copies[1].wait()
    h_v[0:8, :] = jnp.zeros((8, D), jnp.float32)
    h_v[8 + L:16 + L, :] = jnp.zeros((8, D), jnp.float32)

    def phase1(b, carry):
        r0 = pl.multiple_of(b * RB, RB)
        xs = []
        for k in range(RB // J):
            rk = pl.multiple_of(r0 + k * J, J)
            xk = _bf(_layernorm(x_v[pl.ds(rk, J), :].astype(jnp.float32)))
            xn_v[pl.ds(rk, J), :] = xk
            u_v[b * (RB // J) + k] = _dot(ffwd_ref[...], xk)
            xs.append(xk)
        h = _gelu(_dot(jnp.concatenate(xs, axis=0), w1_v[...]))
        h_v[pl.ds(pl.multiple_of(r0 + 8, 8), RB), :] = h
        return carry

    with jax.named_scope('p_phase1'):
        lax.fori_loop(0, L // RB, phase1, 0)

    def zphase(t, carry):
        f0 = pl.multiple_of((t // 4) * 8, 8)
        re = pl.ds(f0, 8)
        im = pl.ds(pl.multiple_of(f0 + J, 8), 8)
        cs = pl.ds(pl.multiple_of((t % 4) * 128, 128), 128)
        GZ = 4
        for i0 in range(0, NB, GZ):
            acc = {}
            uc = {}
            for dl in range(i0 + GZ):
                kr = kt_v[dl, re, cs]
                ki = kt_v[dl, im, cs]
                ks = kr + ki
                for i in range(max(i0, dl), i0 + GZ):
                    src = i - dl
                    if src not in uc:
                        ur = u_v[src, re, cs]
                        ui = u_v[src, im, cs]
                        uc[src] = (ur, ui, ur + ui)
                    ur, ui, us = uc[src]
                    p = (kr * ur, ki * ui, ks * us)
                    acc[i] = p if i not in acc else tuple(x + y for x, y in zip(acc[i], p))
            for i in range(i0, i0 + GZ):
                s1, s2, s3 = acc[i]
                z_v[i, re, cs] = s1 - s2
                z_v[i, im, cs] = s3 - (s1 + s2)
        return carry

    with jax.named_scope('p_z'):
        lax.fori_loop(0, 64, zphase, 0)

    copies[3].wait()
    copies[4].wait()
    copies[5].wait()
    dsk = dsk_ref[...].astype(jnp.float32).reshape(1, D)

    HB = RB // 2

    def out_copy(b):
        r0 = pl.multiple_of(b * HB, HB)
        return pltpu.make_async_copy(out_v.at[pl.ds(r0, HB), :],
                                     out_hbm.at[pl.ds(r0, HB), :], sem_out.at[b])

    def phase2(b, carry):
        r0 = pl.multiple_of(b * RB, RB)
        ext = RB + 16
        parts = []
        for gi, sh in enumerate((1, -1, 2, -2)):
            hv = h_v[pl.ds(r0, ext), gi * 128:(gi + 1) * 128]
            hv = pltpu.roll(hv, sh % ext, 0)
            parts.append(_bf(hv[8:8 + RB, :]))
        hs = _dot(jnp.concatenate(parts, axis=1), w2_v[...])
        ys = [_dot(finv_ref[...], _bf(z_v[b * (RB // J) + k])) for k in range(RB // J)]
        y = jnp.concatenate(ys, axis=0)
        xn = xn_v[pl.ds(r0, RB), :].astype(jnp.float32)
        x1 = xn + hs
        for hf in range(2):
            sl = slice(hf * HB, (hf + 1) * HB)
            rh = pl.multiple_of(r0 + hf * HB, HB)
            a = _dot_nt(_bf(_layernorm2(x1[sl])), w3_v[...])
            bb = x1[sl] + _dot(_bf(_gelu(a)), w4_v[...])
            gate = bb * jax.nn.sigmoid(bb)
            s = y[sl] + xn[sl] * dsk
            x = x_v[pl.ds(rh, HB), :].astype(jnp.float32)
            out_v[pl.ds(rh, HB), :] = _bf(x + s * gate)
            out_copy(2 * b + hf).start()
        return carry

    with jax.named_scope('p_phase2'):
        lax.fori_loop(0, L // RB, phase2, 0)
    for b in range(L // HB):
        out_copy(b).wait()


@jax.jit
def pallas_recurrent_scan__ssm_conv_s4__mixer_s_mlp__prompt_kernel(
    A_u: jax.Array,
    A_A_re: jax.Array,
    A_A_im: jax.Array,
    A_B_re: jax.Array,
    A_B_im: jax.Array,
    A_C_re: jax.Array,
    A_C_im: jax.Array,
    A_log_dt: jax.Array,
    A_Dskip: jax.Array,
    B_x: jax.Array,
    B_w1: jax.Array,
    B_w2: jax.Array,
    B_w3: jax.Array,
    B_w4: jax.Array,
):
    bf16 = jnp.bfloat16
    f32 = jnp.float32
    x = A_u.reshape(L, D)
    vm = pl.BlockSpec(memory_space=pltpu.VMEM)
    hbm = pl.BlockSpec(memory_space=pltpu.HBM)
    out = pl.pallas_call(
        _kernel,
        out_shape=jax.ShapeDtypeStruct((L, D), bf16),
        in_specs=[vm] * 11 + [hbm] * 6,
        out_specs=hbm,
        scratch_shapes=[
            pltpu.VMEM((L, D), bf16),
            pltpu.VMEM((D, D), bf16),
            pltpu.VMEM((D, D), bf16),
            pltpu.VMEM((FF, D), bf16),
            pltpu.VMEM((FF, D), bf16),
            pltpu.VMEM((2 * J, GW), bf16),
            pltpu.VMEM((L, D), bf16),
            pltpu.VMEM((L, D), bf16),
            pltpu.VMEM((L + 16, D), f32),
            pltpu.VMEM((NB, 2 * J, D), f32),
            pltpu.VMEM((NB, 2 * J, D), f32),
            pltpu.VMEM((NB, 2 * J, D), f32),
            pltpu.VMEM((CH // 8, 128, N), f32),
            pltpu.VMEM((CH // 8, 128, N), f32),
            pltpu.VMEM((CH // 8, 8 * NHI, N), f32),
            pltpu.VMEM((CH // 8, 8 * NHI, N), f32),
            pltpu.VMEM((NHI, D, 128), f32),
            pltpu.VMEM((NQ, D), f32),
            pltpu.VMEM((D, N), f32),
            pltpu.SemaphoreType.DMA((6,)),
            pltpu.SemaphoreType.DMA((2 * L // RB,)),
        ],
        compiler_params=pltpu.CompilerParams(vmem_limit_bytes=100 * 1024 * 1024),
    )(A_A_re, A_A_im, A_B_re, A_B_im, A_C_re, A_C_im,
      A_log_dt, A_Dskip,
      jnp.asarray(_F_FWD, bf16), jnp.asarray(_F_INV, bf16), jnp.asarray(_SEL, bf16),
      *[pltpu.with_memory_space_constraint(t, pltpu.HBM)
        for t in (x, B_w1, B_w2, B_w3.T, B_w4, jnp.asarray(_G_ALL, bf16))])
    return out.reshape(1, L, D)
```

```python
import functools
import numpy as np
import jax
import jax.numpy as jnp
from jax import lax
import jax.experimental.pallas as pl
import jax.experimental.pallas.tpu as pltpu

L = 2048
D = 512
N = 128
FF = 1376
J = 128
NB = L // J
NQ = 656
_STEP = (1, 1, 2, 2, 4, 4, 4, 4, 8, 8, 8, 8, 8, 8, 8, 8)
HI = tuple(128 * k + b for k in range(16) for b in range(0, 8, _STEP[k])) + (2048,)
NHI = len(HI)
CH = 32
RB = 512
WIN = ((0, 128), (0, 256), (128, 256), (256, 256), (320, 128), (384, 128),
       (384, 128), (448, 128), (448, 128), (512, 128), (512, 128), (512, 128),
       (512, 128), (512, 128), (512, 128), (528, 128))
GW = sum(w[1] for w in WIN)


def _q_of_m(m):
    hi = (m // 128) * 128 + (m % 8)
    return 16 * HI.index(hi) + (m % 128) // 8


def _build_tables():
    pos = np.arange(L, dtype=np.int64)
    rr = np.zeros(L, np.int64)
    for l in range(L):
        if l < 256:
            rr[l] = l
        else:
            step = 1 << (int(l).bit_length() - 8)
            lo = (l // step) * step
            rem = l - lo
            if rem * 2 < step or (rem * 2 == step and (lo // step) % 2 == 0):
                rr[l] = lo
            else:
                rr[l] = lo + step
    w = np.pi * (2 * np.arange(J) + 1) / (2 * J)
    n = np.arange(J)
    f_fwd = np.concatenate([np.cos(np.outer(w, n)), -np.sin(np.outer(w, n))], 0)
    f_inv = np.concatenate([np.cos(np.outer(n, w)), -np.sin(np.outer(n, w))], 1) / J
    g_all = np.zeros((2 * J, GW))
    off = 0
    for dl in range(NB):
        s0, ln = WIN[dl]
        for p in range(-J, J):
            l = dl * J + p
            if 0 <= l < L:
                q = _q_of_m(int(rr[l])) - s0
                assert 0 <= q < ln
                g_all[:J, off + q] += np.cos(w * p)
                g_all[J:, off + q] += -np.sin(w * p)
        off += ln
    sel = np.zeros((16, 128))
    for dd in range(8):
        sel[np.arange(16), np.arange(16) * 8 + dd] = 1.0
    del pos
    return (f_fwd.astype(np.float32), f_inv.astype(np.float32),
            g_all.astype(np.float32), sel.astype(np.float32))


_F_FWD, _F_INV, _G_ALL, _SEL = _build_tables()


def _bf(x):
    return x.astype(jnp.bfloat16)


def _rb(x):
    return x.astype(jnp.bfloat16).astype(jnp.float32)


def _cmul(a, b):
    return (a[0] * b[0] - a[1] * b[1], a[0] * b[1] + a[1] * b[0])


def _sincos(x):
    k = jnp.floor(x * 0.6366197723675814 + 0.5)
    r = x - k * 1.5703125
    r = r - k * 4.837512969970703125e-4
    r = r - k * 7.549789954891882e-8
    r2 = r * r
    sn = r + r * r2 * (-1.6666654611e-1 + r2 * (8.3321608736e-3 + r2 * -1.9515295891e-4))
    cs = 1.0 + r2 * (-0.5 + r2 * (4.166664568298827e-2 + r2 * (-1.388731625493765e-3
                                                             + r2 * 2.443315711809948e-5)))
    q = k - 4.0 * jnp.floor(k * 0.25)
    odd = (q == 1.0) | (q == 3.0)
    s0 = jnp.where(odd, cs, sn)
    c0 = jnp.where(odd, sn, cs)
    s1 = jnp.where(q >= 2.0, -s0, s0)
    c1 = jnp.where((q == 1.0) | (q == 2.0), -c0, c0)
    return s1, c1


def _gelu(x):
    c = 0.7978845608028654
    return 0.5 * x * (1.0 + jnp.tanh(c * (x + 0.044715 * (x * x * x))))


def _layernorm(x):
    m = jnp.mean(x, axis=-1, keepdims=True)
    xc = x - m
    v = jnp.mean(xc * xc, axis=-1, keepdims=True)
    den = _rb(jnp.sqrt(_rb(_rb(v) + 1e-5)))
    return _rb(_rb(x - _rb(m)) / den)


def _layernorm2(x):
    m = jnp.mean(x, axis=-1, keepdims=True)
    xc = x - m
    v = jnp.mean(xc * xc, axis=-1, keepdims=True)
    return xc / jnp.sqrt(v + 1e-5)


def _dot(a, b):
    return jnp.dot(a, b, preferred_element_type=jnp.float32)


def _dot_nt(a, b):
    return lax.dot_general(a, b, (((1,), (1,)), ((), ())),
                           preferred_element_type=jnp.float32)


def _kernel(are_ref, aim_ref, bre_ref, bim_ref, cre_ref, cim_ref, ldt_ref, dsk_ref,
            ffwd_ref, finv_ref, sel_ref,
            x_hbm, w1_hbm, w2_hbm, w3_hbm, w4_hbm, g_hbm,
            out_hbm,
            x_v, w1_v, w2_v, w3_v, w4_v, g_v, out_v,
            xn_v, h_v, u_v, kt_v, z_v,
            yr_v, yi_v, xr_v, xi_v, o_v, kd_v, dt_v,
            sem_in, sem_out):
    copies = [pltpu.make_async_copy(s, d, sem_in.at[k]) for k, (s, d) in enumerate(
        [(x_hbm, x_v), (w1_hbm, w1_v), (g_hbm, g_v), (w2_hbm, w2_v), (w3_hbm, w3_v),
         (w4_hbm, w4_v)])]
    for c in copies:
        c.start()

    dt_row = _rb(jnp.exp(ldt_ref[...].astype(jnp.float32))).reshape(1, D)
    dt_v[...] = jnp.transpose(jnp.broadcast_to(dt_row, (N, D)))

    def kgen(c, carry):
        r0 = pl.multiple_of(c * CH, CH)
        rows = pl.ds(r0, CH)
        f32 = jnp.float32
        dt = dt_v[rows, :]
        lr = dt * are_ref[rows, :].astype(f32)
        li = dt * aim_ref[rows, :].astype(f32)
        dbr = dt * bre_ref[rows, :].astype(f32)
        dbi = dt * bim_ref[rows, :].astype(f32)
        w = _cmul((cre_ref[rows, :].astype(f32), cim_ref[rows, :].astype(f32)), (dbr, dbi))

        def csq(a):
            ab = a[0] * a[1]
            return (a[0] * a[0] - a[1] * a[1], ab + ab)

        e1 = jnp.exp(lr)
        sn, cs = _sincos(li)
        z1 = (e1 * cs, e1 * sn)
        z8 = csq(csq(csq(z1)))
        z128 = csq(csq(csq(csq(z8))))
        z1024 = csq(csq(csq(z128)))

        def put_pair(re_v, im_v, p, a, b):
            for g in range(CH // 8):
                sl = slice(8 * g, 8 * g + 8)
                re_v[g, 16 * p:16 * p + 16, :] = _bf(jnp.concatenate([a[0][sl], b[0][sl]], axis=0))
                im_v[g, 16 * p:16 * p + 16, :] = _bf(jnp.concatenate([a[1][sl], b[1][sl]], axis=0))

        y_prev = (jnp.ones_like(lr), jnp.zeros_like(lr))
        y = z8
        put_pair(yr_v, yi_v, 0, y_prev, y)
        for j in range(2, 16):
            y_prev = y
            y = _cmul(y, z8)
            if j % 2:
                put_pair(yr_v, yi_v, j // 2, y_prev, y)
        order = []
        pend = []

        def put_x(i, v):
            order.append(i)
            pend.append((v[0], -v[1]))
            if len(pend) == 2:
                put_pair(xr_v, xi_v, len(order) // 2 - 1, pend[0], pend[1])
                pend.clear()

        v = w
        for b in range(8):
            if b:
                v = _cmul(v, z1)
            t = v
            for k in range(8):
                if (128 * k + b) in HI:
                    if k:
                        t = _cmul(t, z128)
                    put_x(HI.index(128 * k + b), t)
        t = _cmul(w, z1024)
        for k in range(8, 17):
            if k > 8:
                t = _cmul(t, z128)
            put_x(HI.index(128 * k), t)
        put_x(NHI - 1, t)
        for g in range(CH // 8):
            o = _dot_nt(xr_v[g], yr_v[g]) + _dot_nt(xi_v[g], yi_v[g])
            for pos in range(NHI):
                o_v[order[pos], pl.ds(pl.multiple_of(r0 + 8 * g, 8), 8), :] = (
                    o[8 * pos:8 * pos + 8, :])
        return carry

    with jax.named_scope('p_kgen'):
        lax.fori_loop(0, D // CH, kgen, 0)

    rid = lax.broadcasted_iota(jnp.int32, (D, 128), 0)
    lid = lax.broadcasted_iota(jnp.int32, (D, 128), 1)
    keep = (rid % 8) == (lid % 8)
    keep_last = keep & (lid < 8)
    sel = sel_ref[...]
    with jax.named_scope('p_sel'):
        for i in range(NHI):
            oi = jnp.where(keep_last if HI[i] == 2048 else keep, o_v[i], 0.0)
            kd_v[16 * i:16 * i + 16, :] = _dot_nt(sel, _bf(oi))

    copies[2].wait()
    off = 0
    for dl in range(NB):
        s0, ln = WIN[dl]
        kt_v[dl] = _dot(g_v[:, off:off + ln], _bf(kd_v[s0:s0 + ln, :]))
        off += ln

    copies[0].wait()
    copies[1].wait()
    h_v[0:8, :] = jnp.zeros((8, D), jnp.float32)
    h_v[8 + L:16 + L, :] = jnp.zeros((8, D), jnp.float32)

    def phase1(b, carry):
        r0 = pl.multiple_of(b * RB, RB)
        xs = []
        for k in range(RB // J):
            rk = pl.multiple_of(r0 + k * J, J)
            xk = _bf(_layernorm(x_v[pl.ds(rk, J), :].astype(jnp.float32)))
            xn_v[pl.ds(rk, J), :] = xk
            u_v[b * (RB // J) + k] = _dot(ffwd_ref[...], xk)
            xs.append(xk)
        h = _gelu(_dot(jnp.concatenate(xs, axis=0), w1_v[...]))
        h_v[pl.ds(pl.multiple_of(r0 + 8, 8), RB), :] = h
        return carry

    with jax.named_scope('p_phase1'):
        lax.fori_loop(0, L // RB, phase1, 0)

    def zphase(t, carry):
        f0 = pl.multiple_of((t // 4) * 8, 8)
        re = pl.ds(f0, 8)
        im = pl.ds(pl.multiple_of(f0 + J, 8), 8)
        cs = pl.ds(pl.multiple_of((t % 4) * 128, 128), 128)
        GZ = 4
        for i0 in range(0, NB, GZ):
            acc = {}
            uc = {}
            for dl in range(i0 + GZ):
                kr = kt_v[dl, re, cs]
                ki = kt_v[dl, im, cs]
                ks = kr + ki
                for i in range(max(i0, dl), i0 + GZ):
                    src = i - dl
                    if src not in uc:
                        ur = u_v[src, re, cs]
                        ui = u_v[src, im, cs]
                        uc[src] = (ur, ui, ur + ui)
                    ur, ui, us = uc[src]
                    p = (kr * ur, ki * ui, ks * us)
                    acc[i] = p if i not in acc else tuple(x + y for x, y in zip(acc[i], p))
            for i in range(i0, i0 + GZ):
                s1, s2, s3 = acc[i]
                z_v[i, re, cs] = s1 - s2
                z_v[i, im, cs] = s3 - (s1 + s2)
        return carry

    with jax.named_scope('p_z'):
        lax.fori_loop(0, 64, zphase, 0)

    copies[3].wait()
    copies[4].wait()
    copies[5].wait()
    dsk = dsk_ref[...].astype(jnp.float32).reshape(1, D)

    HB = RB // 2

    def out_copy(b):
        r0 = pl.multiple_of(b * HB, HB)
        return pltpu.make_async_copy(out_v.at[pl.ds(r0, HB), :],
                                     out_hbm.at[pl.ds(r0, HB), :], sem_out.at[b])

    def phase2(b, carry):
        r0 = pl.multiple_of(b * RB, RB)
        ext = RB + 16
        parts = []
        for gi, sh in enumerate((1, -1, 2, -2)):
            hv = h_v[pl.ds(r0, ext), gi * 128:(gi + 1) * 128]
            hv = pltpu.roll(hv, sh % ext, 0)
            parts.append(_bf(hv[8:8 + RB, :]))
        hs = _dot(jnp.concatenate(parts, axis=1), w2_v[...])
        ys = [_dot(finv_ref[...], _bf(z_v[b * (RB // J) + k])) for k in range(RB // J)]
        y = jnp.concatenate(ys, axis=0)
        xn = xn_v[pl.ds(r0, RB), :].astype(jnp.float32)
        x1 = xn + hs
        a = _dot_nt(_bf(_layernorm2(x1)), w3_v[...])
        for hf in range(2):
            sl = slice(hf * HB, (hf + 1) * HB)
            rh = pl.multiple_of(r0 + hf * HB, HB)
            bb = x1[sl] + _dot(_bf(_gelu(a[sl])), w4_v[...])
            gate = bb * jax.nn.sigmoid(bb)
            s = y[sl] + xn[sl] * dsk
            x = x_v[pl.ds(rh, HB), :].astype(jnp.float32)
            out_v[pl.ds(rh, HB), :] = _bf(x + s * gate)
            out_copy(2 * b + hf).start()
        return carry

    with jax.named_scope('p_phase2'):
        lax.fori_loop(0, L // RB, phase2, 0)
    for b in range(L // HB):
        out_copy(b).wait()


@jax.jit
def pallas_recurrent_scan__ssm_conv_s4__mixer_s_mlp__prompt_kernel(
    A_u: jax.Array,
    A_A_re: jax.Array,
    A_A_im: jax.Array,
    A_B_re: jax.Array,
    A_B_im: jax.Array,
    A_C_re: jax.Array,
    A_C_im: jax.Array,
    A_log_dt: jax.Array,
    A_Dskip: jax.Array,
    B_x: jax.Array,
    B_w1: jax.Array,
    B_w2: jax.Array,
    B_w3: jax.Array,
    B_w4: jax.Array,
):
    bf16 = jnp.bfloat16
    f32 = jnp.float32
    x = A_u.reshape(L, D)
    vm = pl.BlockSpec(memory_space=pltpu.VMEM)
    hbm = pl.BlockSpec(memory_space=pltpu.HBM)
    out = pl.pallas_call(
        _kernel,
        out_shape=jax.ShapeDtypeStruct((L, D), bf16),
        in_specs=[vm] * 11 + [hbm] * 6,
        out_specs=hbm,
        scratch_shapes=[
            pltpu.VMEM((L, D), bf16),
            pltpu.VMEM((D, D), bf16),
            pltpu.VMEM((D, D), bf16),
            pltpu.VMEM((FF, D), bf16),
            pltpu.VMEM((FF, D), bf16),
            pltpu.VMEM((2 * J, GW), bf16),
            pltpu.VMEM((L, D), bf16),
            pltpu.VMEM((L, D), bf16),
            pltpu.VMEM((L + 16, D), f32),
            pltpu.VMEM((NB, 2 * J, D), f32),
            pltpu.VMEM((NB, 2 * J, D), f32),
            pltpu.VMEM((NB, 2 * J, D), f32),
            pltpu.VMEM((CH // 8, 128, N), bf16),
            pltpu.VMEM((CH // 8, 128, N), bf16),
            pltpu.VMEM((CH // 8, 8 * NHI + 8, N), bf16),
            pltpu.VMEM((CH // 8, 8 * NHI + 8, N), bf16),
            pltpu.VMEM((NHI, D, 128), f32),
            pltpu.VMEM((NQ, D), f32),
            pltpu.VMEM((D, N), f32),
            pltpu.SemaphoreType.DMA((6,)),
            pltpu.SemaphoreType.DMA((2 * L // RB,)),
        ],
        compiler_params=pltpu.CompilerParams(vmem_limit_bytes=100 * 1024 * 1024),
    )(A_A_re, A_A_im, A_B_re, A_B_im, A_C_re, A_C_im,
      A_log_dt, A_Dskip,
      jnp.asarray(_F_FWD, bf16), jnp.asarray(_F_INV, bf16), jnp.asarray(_SEL, bf16),
      *[pltpu.with_memory_space_constraint(t, pltpu.HBM)
        for t in (x, B_w1, B_w2, B_w3.T, B_w4, jnp.asarray(_G_ALL, bf16))])
    return out.reshape(1, L, D)
```

```python
import functools
import numpy as np
import jax
import jax.numpy as jnp
from jax import lax
import jax.experimental.pallas as pl
import jax.experimental.pallas.tpu as pltpu

L = 2048
D = 512
N = 128
FF = 1376
J = 128
NB = L // J
NQ = 656
_STEP = (1, 1, 2, 2, 4, 4, 4, 4, 8, 8, 8, 8, 8, 8, 8, 8)
HI = tuple(128 * k + b for k in range(16) for b in range(0, 8, _STEP[k])) + (2048,)
NHI = len(HI)
CH = 32
RB = 512
WIN = ((0, 128), (0, 256), (128, 256), (256, 256), (320, 128), (384, 128),
       (384, 128), (448, 128), (448, 128), (512, 128), (512, 128), (512, 128),
       (512, 128), (512, 128), (512, 128), (528, 128))
GW = sum(w[1] for w in WIN)


def _q_of_m(m):
    hi = (m // 128) * 128 + (m % 8)
    return 16 * HI.index(hi) + (m % 128) // 8


def _build_tables():
    pos = np.arange(L, dtype=np.int64)
    rr = np.zeros(L, np.int64)
    for l in range(L):
        if l < 256:
            rr[l] = l
        else:
            step = 1 << (int(l).bit_length() - 8)
            lo = (l // step) * step
            rem = l - lo
            if rem * 2 < step or (rem * 2 == step and (lo // step) % 2 == 0):
                rr[l] = lo
            else:
                rr[l] = lo + step
    w = np.pi * (2 * np.arange(J) + 1) / (2 * J)
    n = np.arange(J)
    f_fwd = np.concatenate([np.cos(np.outer(w, n)), -np.sin(np.outer(w, n))], 0)
    f_inv = np.concatenate([np.cos(np.outer(n, w)), -np.sin(np.outer(n, w))], 1) / J
    g_all = np.zeros((2 * J, GW))
    off = 0
    for dl in range(NB):
        s0, ln = WIN[dl]
        for p in range(-J, J):
            l = dl * J + p
            if 0 <= l < L:
                q = _q_of_m(int(rr[l])) - s0
                assert 0 <= q < ln
                g_all[:J, off + q] += np.cos(w * p)
                g_all[J:, off + q] += -np.sin(w * p)
        off += ln
    sel = np.zeros((16, 128))
    for dd in range(8):
        sel[np.arange(16), np.arange(16) * 8 + dd] = 1.0
    del pos
    return (f_fwd.astype(np.float32), f_inv.astype(np.float32),
            g_all.astype(np.float32), sel.astype(np.float32))


_F_FWD, _F_INV, _G_ALL, _SEL = _build_tables()


def _bf(x):
    return x.astype(jnp.bfloat16)


def _rb(x):
    return x.astype(jnp.bfloat16).astype(jnp.float32)


def _cmul(a, b):
    return (a[0] * b[0] - a[1] * b[1], a[0] * b[1] + a[1] * b[0])


def _sincos(x):
    k = jnp.floor(x * 0.6366197723675814 + 0.5)
    r = x - k * 1.5703125
    r = r - k * 4.837512969970703125e-4
    r = r - k * 7.549789954891882e-8
    r2 = r * r
    sn = r + r * r2 * (-1.6666654611e-1 + r2 * (8.3321608736e-3 + r2 * -1.9515295891e-4))
    cs = 1.0 + r2 * (-0.5 + r2 * (4.166664568298827e-2 + r2 * (-1.388731625493765e-3
                                                             + r2 * 2.443315711809948e-5)))
    q = k - 4.0 * jnp.floor(k * 0.25)
    odd = (q == 1.0) | (q == 3.0)
    s0 = jnp.where(odd, cs, sn)
    c0 = jnp.where(odd, sn, cs)
    s1 = jnp.where(q >= 2.0, -s0, s0)
    c1 = jnp.where((q == 1.0) | (q == 2.0), -c0, c0)
    return s1, c1


def _gelu(x):
    c = 0.7978845608028654
    return 0.5 * x * (1.0 + jnp.tanh(c * (x + 0.044715 * (x * x * x))))


def _layernorm(x):
    m = jnp.mean(x, axis=-1, keepdims=True)
    xc = x - m
    v = jnp.mean(xc * xc, axis=-1, keepdims=True)
    den = _rb(jnp.sqrt(_rb(_rb(v) + 1e-5)))
    return _rb(_rb(x - _rb(m)) / den)


def _layernorm2(x):
    m = jnp.mean(x, axis=-1, keepdims=True)
    xc = x - m
    v = jnp.mean(xc * xc, axis=-1, keepdims=True)
    return xc / jnp.sqrt(v + 1e-5)


def _dot(a, b):
    return jnp.dot(a, b, preferred_element_type=jnp.float32)


def _dot_nt(a, b):
    return lax.dot_general(a, b, (((1,), (1,)), ((), ())),
                           preferred_element_type=jnp.float32)


def _kernel(are_ref, aim_ref, bre_ref, bim_ref, cre_ref, cim_ref, ldt_ref, dsk_ref,
            ffwd_ref, finv_ref, sel_ref,
            x_hbm, w1_hbm, w2_hbm, w3_hbm, w4_hbm, g_hbm,
            out_hbm,
            x_v, w1_v, w2_v, w3_v, w4_v, g_v, out_v,
            xn_v, h_v, u_v, kt_v, z_v,
            yr_v, yi_v, xr_v, xi_v, o_v, kd_v, dt_v,
            sem_in, sem_out):
    copies = [pltpu.make_async_copy(s, d, sem_in.at[k]) for k, (s, d) in enumerate(
        [(x_hbm, x_v), (w1_hbm, w1_v), (g_hbm, g_v), (w2_hbm, w2_v), (w3_hbm, w3_v),
         (w4_hbm, w4_v)])]
    for c in copies:
        c.start()

    dt_row = _rb(jnp.exp(ldt_ref[...].astype(jnp.float32))).reshape(1, D)
    dt_v[...] = jnp.transpose(jnp.broadcast_to(dt_row, (N, D)))

    def kgen(c, carry):
        r0 = pl.multiple_of(c * CH, CH)
        rows = pl.ds(r0, CH)
        f32 = jnp.float32
        dt = dt_v[rows, :]
        lr = dt * are_ref[rows, :].astype(f32)
        li = dt * aim_ref[rows, :].astype(f32)
        dbr = dt * bre_ref[rows, :].astype(f32)
        dbi = dt * bim_ref[rows, :].astype(f32)
        w = _cmul((cre_ref[rows, :].astype(f32), cim_ref[rows, :].astype(f32)), (dbr, dbi))

        def csq(a):
            ab = a[0] * a[1]
            return (a[0] * a[0] - a[1] * a[1], ab + ab)

        e1 = jnp.exp(lr)
        sn, cs = _sincos(li)
        z1 = (e1 * cs, e1 * sn)
        z8 = csq(csq(csq(z1)))
        z128 = csq(csq(csq(csq(z8))))
        z1024 = csq(csq(csq(z128)))

        def put_y(j, v):
            for g in range(CH // 8):
                yr_v[g, 8 * j:8 * j + 8, :] = v[0][8 * g:8 * g + 8, :]
                yi_v[g, 8 * j:8 * j + 8, :] = v[1][8 * g:8 * g + 8, :]

        def put_x(i, v):
            for g in range(CH // 8):
                xr_v[g, 8 * i:8 * i + 8, :] = v[0][8 * g:8 * g + 8, :]
                xi_v[g, 8 * i:8 * i + 8, :] = v[1][8 * g:8 * g + 8, :]

        put_y(0, (jnp.ones_like(lr), jnp.zeros_like(lr)))
        y = z8
        put_y(1, y)
        for j in range(2, 16):
            y = _cmul(y, z8)
            put_y(j, y)
        v = w
        for b in range(8):
            if b:
                v = _cmul(v, z1)
            t = v
            for k in range(8):
                if (128 * k + b) in HI:
                    if k:
                        t = _cmul(t, z128)
                    put_x(HI.index(128 * k + b), t)
        t = _cmul(w, z1024)
        for k in range(8, 17):
            if k > 8:
                t = _cmul(t, z128)
            put_x(HI.index(128 * k), t)
        for g in range(CH // 8):
            o = (_dot_nt(_bf(xr_v[g]), _bf(yr_v[g])) - _dot_nt(_bf(xi_v[g]), _bf(yi_v[g])))
            for i in range(NHI):
                o_v[i, pl.ds(pl.multiple_of(r0 + 8 * g, 8), 8), :] = o[8 * i:8 * i + 8, :]
        return carry

    with jax.named_scope('p_kgen'):
        lax.fori_loop(0, D // CH, kgen, 0)

    rid = lax.broadcasted_iota(jnp.int32, (D, 128), 0)
    lid = lax.broadcasted_iota(jnp.int32, (D, 128), 1)
    keep = (rid % 8) == (lid % 8)
    keep_last = keep & (lid < 8)
    sel = sel_ref[...]
    with jax.named_scope('p_sel'):
        for i in range(NHI):
            oi = jnp.where(keep_last if HI[i] == 2048 else keep, o_v[i], 0.0)
            kd_v[16 * i:16 * i + 16, :] = _dot_nt(sel, _bf(oi))

    copies[2].wait()
    off = 0
    for dl in range(NB):
        s0, ln = WIN[dl]
        kt_v[dl] = _dot(g_v[:, off:off + ln], _bf(kd_v[s0:s0 + ln, :]))
        off += ln

    copies[0].wait()
    copies[1].wait()
    h_v[0:8, :] = jnp.zeros((8, D), jnp.float32)
    h_v[8 + L:16 + L, :] = jnp.zeros((8, D), jnp.float32)

    def phase1(b, carry):
        r0 = pl.multiple_of(b * RB, RB)
        xs = []
        for k in range(RB // J):
            rk = pl.multiple_of(r0 + k * J, J)
            xk = _bf(_layernorm(x_v[pl.ds(rk, J), :].astype(jnp.float32)))
            xn_v[pl.ds(rk, J), :] = xk
            u_v[b * (RB // J) + k] = _dot(ffwd_ref[...], xk)
            xs.append(xk)
        h = _gelu(_dot(jnp.concatenate(xs, axis=0), w1_v[...]))
        h_v[pl.ds(pl.multiple_of(r0 + 8, 8), RB), :] = h
        return carry

    with jax.named_scope('p_phase1'):
        lax.fori_loop(0, L // RB, phase1, 0)

    def zphase(t, carry):
        f0 = pl.multiple_of((t // 4) * 8, 8)
        re = pl.ds(f0, 8)
        im = pl.ds(pl.multiple_of(f0 + J, 8), 8)
        cs = pl.ds(pl.multiple_of((t % 4) * 128, 128), 128)
        GZ = 4
        for i0 in range(0, NB, GZ):
            acc = {}
            uc = {}
            for dl in range(i0 + GZ):
                kr = kt_v[dl, re, cs]
                ki = kt_v[dl, im, cs]
                ks = kr + ki
                for i in range(max(i0, dl), i0 + GZ):
                    src = i - dl
                    if src not in uc:
                        ur = u_v[src, re, cs]
                        ui = u_v[src, im, cs]
                        uc[src] = (ur, ui, ur + ui)
                    ur, ui, us = uc[src]
                    p = (kr * ur, ki * ui, ks * us)
                    acc[i] = p if i not in acc else tuple(x + y for x, y in zip(acc[i], p))
            for i in range(i0, i0 + GZ):
                s1, s2, s3 = acc[i]
                z_v[i, re, cs] = s1 - s2
                z_v[i, im, cs] = s3 - (s1 + s2)
        return carry

    with jax.named_scope('p_z'):
        lax.fori_loop(0, 64, zphase, 0)

    copies[3].wait()
    copies[4].wait()
    copies[5].wait()
    dsk = dsk_ref[...].astype(jnp.float32).reshape(1, D)

    HB = RB // 2

    def out_copy(b):
        r0 = pl.multiple_of(b * HB, HB)
        return pltpu.make_async_copy(out_v.at[pl.ds(r0, HB), :],
                                     out_hbm.at[pl.ds(r0, HB), :], sem_out.at[b])

    def phase2(b, carry):
        r0 = pl.multiple_of(b * RB, RB)
        ext = RB + 16
        parts = []
        for gi, sh in enumerate((1, -1, 2, -2)):
            hv = h_v[pl.ds(r0, ext), gi * 128:(gi + 1) * 128]
            hv = pltpu.roll(hv, sh % ext, 0)
            parts.append(_bf(hv[8:8 + RB, :]))
        hs = _dot(jnp.concatenate(parts, axis=1), w2_v[...])
        ys = [_dot(finv_ref[...], _bf(z_v[b * (RB // J) + k])) for k in range(RB // J)]
        y = jnp.concatenate(ys, axis=0)
        xn = xn_v[pl.ds(r0, RB), :].astype(jnp.float32)
        x1 = xn + hs
        a = _dot_nt(_bf(_layernorm2(x1)), w3_v[...])
        for hf in range(2):
            sl = slice(hf * HB, (hf + 1) * HB)
            rh = pl.multiple_of(r0 + hf * HB, HB)
            bb = x1[sl] + _dot(_bf(_gelu(a[sl])), w4_v[...])
            gate = bb * jax.nn.sigmoid(bb)
            s = y[sl] + xn[sl] * dsk
            x = x_v[pl.ds(rh, HB), :].astype(jnp.float32)
            out_v[pl.ds(rh, HB), :] = _bf(x + s * gate)
            out_copy(2 * b + hf).start()
        return carry

    with jax.named_scope('p_phase2'):
        lax.fori_loop(0, L // RB, phase2, 0)
    for b in range(L // HB):
        out_copy(b).wait()


@jax.jit
def pallas_recurrent_scan__ssm_conv_s4__mixer_s_mlp__prompt_kernel(
    A_u: jax.Array,
    A_A_re: jax.Array,
    A_A_im: jax.Array,
    A_B_re: jax.Array,
    A_B_im: jax.Array,
    A_C_re: jax.Array,
    A_C_im: jax.Array,
    A_log_dt: jax.Array,
    A_Dskip: jax.Array,
    B_x: jax.Array,
    B_w1: jax.Array,
    B_w2: jax.Array,
    B_w3: jax.Array,
    B_w4: jax.Array,
):
    bf16 = jnp.bfloat16
    f32 = jnp.float32
    x = A_u.reshape(L, D)
    vm = pl.BlockSpec(memory_space=pltpu.VMEM)
    hbm = pl.BlockSpec(memory_space=pltpu.HBM)
    out = pl.pallas_call(
        _kernel,
        out_shape=jax.ShapeDtypeStruct((L, D), bf16),
        in_specs=[vm] * 11 + [hbm] * 6,
        out_specs=hbm,
        scratch_shapes=[
            pltpu.VMEM((L, D), bf16),
            pltpu.VMEM((D, D), bf16),
            pltpu.VMEM((D, D), bf16),
            pltpu.VMEM((FF, D), bf16),
            pltpu.VMEM((FF, D), bf16),
            pltpu.VMEM((2 * J, GW), bf16),
            pltpu.VMEM((L, D), bf16),
            pltpu.VMEM((L, D), bf16),
            pltpu.VMEM((L + 16, D), f32),
            pltpu.VMEM((NB, 2 * J, D), f32),
            pltpu.VMEM((NB, 2 * J, D), f32),
            pltpu.VMEM((NB, 2 * J, D), f32),
            pltpu.VMEM((CH // 8, 128, N), f32),
            pltpu.VMEM((CH // 8, 128, N), f32),
            pltpu.VMEM((CH // 8, 8 * NHI, N), f32),
            pltpu.VMEM((CH // 8, 8 * NHI, N), f32),
            pltpu.VMEM((NHI, D, 128), f32),
            pltpu.VMEM((NQ, D), f32),
            pltpu.VMEM((D, N), f32),
            pltpu.SemaphoreType.DMA((6,)),
            pltpu.SemaphoreType.DMA((2 * L // RB,)),
        ],
        compiler_params=pltpu.CompilerParams(vmem_limit_bytes=100 * 1024 * 1024),
    )(A_A_re, A_A_im, A_B_re, A_B_im, A_C_re, A_C_im,
      A_log_dt, A_Dskip,
      jnp.asarray(_F_FWD, bf16), jnp.asarray(_F_INV, bf16), jnp.asarray(_SEL, bf16),
      *[pltpu.with_memory_space_constraint(t, pltpu.HBM)
        for t in (x, B_w1, B_w2, B_w3.T, B_w4, jnp.asarray(_G_ALL, bf16))])
    return out.reshape(1, L, D)
```

```python
import functools
import numpy as np
import jax
import jax.numpy as jnp
from jax import lax
import jax.experimental.pallas as pl
import jax.experimental.pallas.tpu as pltpu

L = 2048
D = 512
N = 128
FF = 1376
J = 128
NB = L // J
NQ = 656
_STEP = (1, 1, 2, 2, 4, 4, 4, 4, 8, 8, 8, 8, 8, 8, 8, 8)
HI = tuple(128 * k + b for k in range(16) for b in range(0, 8, _STEP[k])) + (2048,)
NHI = len(HI)
CH = 32
RB = 512
WIN = ((0, 128), (0, 256), (128, 256), (256, 256), (320, 128), (384, 128),
       (384, 128), (448, 128), (448, 128), (512, 128), (512, 128), (512, 128),
       (512, 128), (512, 128), (512, 128), (528, 128))
GW = sum(w[1] for w in WIN)


def _q_of_m(m):
    hi = (m // 128) * 128 + (m % 8)
    return 16 * HI.index(hi) + (m % 128) // 8


def _build_tables():
    pos = np.arange(L, dtype=np.int64)
    rr = np.zeros(L, np.int64)
    for l in range(L):
        if l < 256:
            rr[l] = l
        else:
            step = 1 << (int(l).bit_length() - 8)
            lo = (l // step) * step
            rem = l - lo
            if rem * 2 < step or (rem * 2 == step and (lo // step) % 2 == 0):
                rr[l] = lo
            else:
                rr[l] = lo + step
    w = np.pi * (2 * np.arange(J) + 1) / (2 * J)
    n = np.arange(J)
    f_fwd = np.concatenate([np.cos(np.outer(w, n)), -np.sin(np.outer(w, n))], 0)
    f_inv = np.concatenate([np.cos(np.outer(n, w)), -np.sin(np.outer(n, w))], 1) / J
    g_all = np.zeros((2 * J, GW))
    off = 0
    for dl in range(NB):
        s0, ln = WIN[dl]
        for p in range(-J, J):
            l = dl * J + p
            if 0 <= l < L:
                q = _q_of_m(int(rr[l])) - s0
                assert 0 <= q < ln
                g_all[:J, off + q] += np.cos(w * p)
                g_all[J:, off + q] += -np.sin(w * p)
        off += ln
    sel = np.zeros((16, 128))
    for dd in range(8):
        sel[np.arange(16), np.arange(16) * 8 + dd] = 1.0
    del pos
    return (f_fwd.astype(np.float32), f_inv.astype(np.float32),
            g_all.astype(np.float32), sel.astype(np.float32))


_F_FWD, _F_INV, _G_ALL, _SEL = _build_tables()


def _bf(x):
    return x.astype(jnp.bfloat16)


def _rb(x):
    return x.astype(jnp.bfloat16).astype(jnp.float32)


def _cmul(a, b):
    return (a[0] * b[0] - a[1] * b[1], a[0] * b[1] + a[1] * b[0])


def _sincos(x):
    k = jnp.floor(x * 0.6366197723675814 + 0.5)
    r = x - k * 1.5703125
    r = r - k * 4.837512969970703125e-4
    r = r - k * 7.549789954891882e-8
    r2 = r * r
    sn = r + r * r2 * (-1.6666654611e-1 + r2 * (8.3321608736e-3 + r2 * -1.9515295891e-4))
    cs = 1.0 + r2 * (-0.5 + r2 * (4.166664568298827e-2 + r2 * (-1.388731625493765e-3
                                                             + r2 * 2.443315711809948e-5)))
    q = k - 4.0 * jnp.floor(k * 0.25)
    odd = (q == 1.0) | (q == 3.0)
    s0 = jnp.where(odd, cs, sn)
    c0 = jnp.where(odd, sn, cs)
    s1 = jnp.where(q >= 2.0, -s0, s0)
    c1 = jnp.where((q == 1.0) | (q == 2.0), -c0, c0)
    return s1, c1


def _gelu(x):
    c = 0.7978845608028654
    return 0.5 * x * (1.0 + jnp.tanh(c * (x + 0.044715 * (x * x * x))))


def _layernorm(x):
    m = jnp.mean(x, axis=-1, keepdims=True)
    xc = x - m
    v = jnp.mean(xc * xc, axis=-1, keepdims=True)
    den = _rb(jnp.sqrt(_rb(_rb(v) + 1e-5)))
    return _rb(_rb(x - _rb(m)) / den)


def _layernorm2(x):
    m = jnp.mean(x, axis=-1, keepdims=True)
    xc = x - m
    v = jnp.mean(xc * xc, axis=-1, keepdims=True)
    return xc / jnp.sqrt(v + 1e-5)


def _dot(a, b):
    return jnp.dot(a, b, preferred_element_type=jnp.float32)


def _dot_nt(a, b):
    return lax.dot_general(a, b, (((1,), (1,)), ((), ())),
                           preferred_element_type=jnp.float32)


def _kernel(are_ref, aim_ref, bre_ref, bim_ref, cre_ref, cim_ref, ldt_ref, dsk_ref,
            ffwd_ref, finv_ref, sel_ref,
            x_hbm, w1_hbm, w2_hbm, w3_hbm, w4_hbm, g_hbm,
            out_hbm,
            x_v, w1_v, w2_v, w3_v, w4_v, g_v, out_v,
            xn_v, h_v, u_v, kt_v, z_v,
            yr_v, yi_v, xr_v, xi_v, o_v, kd_v, dt_v, pw_v,
            sem_in, sem_out):
    copies = [pltpu.make_async_copy(s, d, sem_in.at[k]) for k, (s, d) in enumerate(
        [(x_hbm, x_v), (w1_hbm, w1_v), (g_hbm, g_v), (w2_hbm, w2_v), (w3_hbm, w3_v),
         (w4_hbm, w4_v)])]
    for c in copies:
        c.start()

    dt_row = _rb(jnp.exp(ldt_ref[...].astype(jnp.float32))).reshape(1, D)
    dt_v[...] = jnp.transpose(jnp.broadcast_to(dt_row, (N, D)))

    NCH = D // CH
    f32 = jnp.float32

    def csq(a):
        ab = a[0] * a[1]
        return (a[0] * a[0] - a[1] * a[1], ab + ab)

    def kprep(c):
        rows = pl.ds(pl.multiple_of(c * CH, CH), CH)
        dt = dt_v[rows, :]
        lr = dt * are_ref[rows, :].astype(f32)
        li = dt * aim_ref[rows, :].astype(f32)
        dbr = dt * bre_ref[rows, :].astype(f32)
        dbi = dt * bim_ref[rows, :].astype(f32)
        w = _cmul((cre_ref[rows, :].astype(f32), cim_ref[rows, :].astype(f32)), (dbr, dbi))
        e1 = jnp.exp(lr)
        sn, cs = _sincos(li)
        z1 = (e1 * cs, e1 * sn)
        z8 = csq(csq(csq(z1)))
        z128 = csq(csq(csq(csq(z8))))
        z1024 = csq(csq(csq(z128)))
        for k, v in enumerate((w, z1, z128, z1024)):
            pw_v[2 * k] = v[0]
            pw_v[2 * k + 1] = v[1]

        def put_y(j, v):
            for g in range(CH // 8):
                yr_v[g, 8 * j:8 * j + 8, :] = v[0][8 * g:8 * g + 8, :]
                yi_v[g, 8 * j:8 * j + 8, :] = v[1][8 * g:8 * g + 8, :]

        put_y(0, (jnp.ones_like(lr), jnp.zeros_like(lr)))
        y = z8
        put_y(1, y)
        for j in range(2, 16):
            y = _cmul(y, z8)
            put_y(j, y)

    def kgen(c, carry):
        r0 = pl.multiple_of(c * CH, CH)
        w, z1, z128, z1024 = [(pw_v[2 * k], pw_v[2 * k + 1]) for k in range(4)]
        ys = [(_bf(yr_v[g]), _bf(yi_v[g])) for g in range(CH // 8)]

        def put_x(i, v):
            for g in range(CH // 8):
                xr_v[g, 8 * i:8 * i + 8, :] = v[0][8 * g:8 * g + 8, :]
                xi_v[g, 8 * i:8 * i + 8, :] = v[1][8 * g:8 * g + 8, :]

        v = w
        for b in range(8):
            if b:
                v = _cmul(v, z1)
            t = v
            for k in range(8):
                if (128 * k + b) in HI:
                    if k:
                        t = _cmul(t, z128)
                    put_x(HI.index(128 * k + b), t)
        t = _cmul(w, z1024)
        for k in range(8, 17):
            if k > 8:
                t = _cmul(t, z128)
            put_x(HI.index(128 * k), t)
        for g in range(CH // 8):
            o = _dot_nt(_bf(xr_v[g]), ys[g][0]) - _dot_nt(_bf(xi_v[g]), ys[g][1])
            for i in range(NHI):
                o_v[i, pl.ds(pl.multiple_of(r0 + 8 * g, 8), 8), :] = o[8 * i:8 * i + 8, :]
        kprep(jnp.minimum(c + 1, NCH - 1))
        return carry

    with jax.named_scope('p_kgen'):
        kprep(0)
        lax.fori_loop(0, NCH, kgen, 0, unroll=16)

    rid = lax.broadcasted_iota(jnp.int32, (D, 128), 0)
    lid = lax.broadcasted_iota(jnp.int32, (D, 128), 1)
    keep = (rid % 8) == (lid % 8)
    keep_last = keep & (lid < 8)
    sel = sel_ref[...]
    with jax.named_scope('p_sel'):
        for i in range(NHI):
            oi = jnp.where(keep_last if HI[i] == 2048 else keep, o_v[i], 0.0)
            kd_v[16 * i:16 * i + 16, :] = _dot_nt(sel, _bf(oi))

    copies[2].wait()
    off = 0
    for dl in range(NB):
        s0, ln = WIN[dl]
        kt_v[dl] = _dot(g_v[:, off:off + ln], _bf(kd_v[s0:s0 + ln, :]))
        off += ln

    copies[0].wait()
    copies[1].wait()
    h_v[0:8, :] = jnp.zeros((8, D), jnp.float32)
    h_v[8 + L:16 + L, :] = jnp.zeros((8, D), jnp.float32)

    def phase1(b, carry):
        r0 = pl.multiple_of(b * RB, RB)
        xs = []
        for k in range(RB // J):
            rk = pl.multiple_of(r0 + k * J, J)
            xk = _bf(_layernorm(x_v[pl.ds(rk, J), :].astype(jnp.float32)))
            xn_v[pl.ds(rk, J), :] = xk
            u_v[b * (RB // J) + k] = _dot(ffwd_ref[...], xk)
            xs.append(xk)
        h = _gelu(_dot(jnp.concatenate(xs, axis=0), w1_v[...]))
        h_v[pl.ds(pl.multiple_of(r0 + 8, 8), RB), :] = h
        return carry

    with jax.named_scope('p_phase1'):
        lax.fori_loop(0, L // RB, phase1, 0)

    def zphase(t, carry):
        f0 = pl.multiple_of((t // 4) * 8, 8)
        re = pl.ds(f0, 8)
        im = pl.ds(pl.multiple_of(f0 + J, 8), 8)
        cs = pl.ds(pl.multiple_of((t % 4) * 128, 128), 128)
        GZ = 4
        for i0 in range(0, NB, GZ):
            acc = {}
            uc = {}
            for dl in range(i0 + GZ):
                kr = kt_v[dl, re, cs]
                ki = kt_v[dl, im, cs]
                ks = kr + ki
                for i in range(max(i0, dl), i0 + GZ):
                    src = i - dl
                    if src not in uc:
                        ur = u_v[src, re, cs]
                        ui = u_v[src, im, cs]
                        uc[src] = (ur, ui, ur + ui)
                    ur, ui, us = uc[src]
                    p = (kr * ur, ki * ui, ks * us)
                    acc[i] = p if i not in acc else tuple(x + y for x, y in zip(acc[i], p))
            for i in range(i0, i0 + GZ):
                s1, s2, s3 = acc[i]
                z_v[i, re, cs] = s1 - s2
                z_v[i, im, cs] = s3 - (s1 + s2)
        return carry

    with jax.named_scope('p_z'):
        lax.fori_loop(0, 64, zphase, 0)

    copies[3].wait()
    copies[4].wait()
    copies[5].wait()
    dsk = dsk_ref[...].astype(jnp.float32).reshape(1, D)

    HB = RB // 2

    def out_copy(b):
        r0 = pl.multiple_of(b * HB, HB)
        return pltpu.make_async_copy(out_v.at[pl.ds(r0, HB), :],
                                     out_hbm.at[pl.ds(r0, HB), :], sem_out.at[b])

    def phase2(b, carry):
        r0 = pl.multiple_of(b * RB, RB)
        ext = RB + 16
        parts = []
        for gi, sh in enumerate((1, -1, 2, -2)):
            hv = h_v[pl.ds(r0, ext), gi * 128:(gi + 1) * 128]
            hv = pltpu.roll(hv, sh % ext, 0)
            parts.append(_bf(hv[8:8 + RB, :]))
        hs = _dot(jnp.concatenate(parts, axis=1), w2_v[...])
        ys = [_dot(finv_ref[...], _bf(z_v[b * (RB // J) + k])) for k in range(RB // J)]
        y = jnp.concatenate(ys, axis=0)
        xn = xn_v[pl.ds(r0, RB), :].astype(jnp.float32)
        x1 = xn + hs
        a = _dot_nt(_bf(_layernorm2(x1)), w3_v[...])
        for hf in range(2):
            sl = slice(hf * HB, (hf + 1) * HB)
            rh = pl.multiple_of(r0 + hf * HB, HB)
            bb = x1[sl] + _dot(_bf(_gelu(a[sl])), w4_v[...])
            gate = bb * jax.nn.sigmoid(bb)
            s = y[sl] + xn[sl] * dsk
            x = x_v[pl.ds(rh, HB), :].astype(jnp.float32)
            out_v[pl.ds(rh, HB), :] = _bf(x + s * gate)
            out_copy(2 * b + hf).start()
        return carry

    with jax.named_scope('p_phase2'):
        lax.fori_loop(0, L // RB, phase2, 0)
    for b in range(L // HB):
        out_copy(b).wait()


@jax.jit
def pallas_recurrent_scan__ssm_conv_s4__mixer_s_mlp__prompt_kernel(
    A_u: jax.Array,
    A_A_re: jax.Array,
    A_A_im: jax.Array,
    A_B_re: jax.Array,
    A_B_im: jax.Array,
    A_C_re: jax.Array,
    A_C_im: jax.Array,
    A_log_dt: jax.Array,
    A_Dskip: jax.Array,
    B_x: jax.Array,
    B_w1: jax.Array,
    B_w2: jax.Array,
    B_w3: jax.Array,
    B_w4: jax.Array,
):
    bf16 = jnp.bfloat16
    f32 = jnp.float32
    x = A_u.reshape(L, D)
    vm = pl.BlockSpec(memory_space=pltpu.VMEM)
    hbm = pl.BlockSpec(memory_space=pltpu.HBM)
    out = pl.pallas_call(
        _kernel,
        out_shape=jax.ShapeDtypeStruct((L, D), bf16),
        in_specs=[vm] * 11 + [hbm] * 6,
        out_specs=hbm,
        scratch_shapes=[
            pltpu.VMEM((L, D), bf16),
            pltpu.VMEM((D, D), bf16),
            pltpu.VMEM((D, D), bf16),
            pltpu.VMEM((FF, D), bf16),
            pltpu.VMEM((FF, D), bf16),
            pltpu.VMEM((2 * J, GW), bf16),
            pltpu.VMEM((L, D), bf16),
            pltpu.VMEM((L, D), bf16),
            pltpu.VMEM((L + 16, D), f32),
            pltpu.VMEM((NB, 2 * J, D), f32),
            pltpu.VMEM((NB, 2 * J, D), f32),
            pltpu.VMEM((NB, 2 * J, D), f32),
            pltpu.VMEM((CH // 8, 128, N), f32),
            pltpu.VMEM((CH // 8, 128, N), f32),
            pltpu.VMEM((CH // 8, 8 * NHI, N), f32),
            pltpu.VMEM((CH // 8, 8 * NHI, N), f32),
            pltpu.VMEM((NHI, D, 128), f32),
            pltpu.VMEM((NQ, D), f32),
            pltpu.VMEM((D, N), f32),
            pltpu.VMEM((8, CH, N), f32),
            pltpu.SemaphoreType.DMA((6,)),
            pltpu.SemaphoreType.DMA((2 * L // RB,)),
        ],
        compiler_params=pltpu.CompilerParams(vmem_limit_bytes=100 * 1024 * 1024),
    )(A_A_re, A_A_im, A_B_re, A_B_im, A_C_re, A_C_im,
      A_log_dt, A_Dskip,
      jnp.asarray(_F_FWD, bf16), jnp.asarray(_F_INV, bf16), jnp.asarray(_SEL, bf16),
      *[pltpu.with_memory_space_constraint(t, pltpu.HBM)
        for t in (x, B_w1, B_w2, B_w3.T, B_w4, jnp.asarray(_G_ALL, bf16))])
    return out.reshape(1, L, D)
```

```python
import functools
import numpy as np
import jax
import jax.numpy as jnp
from jax import lax
import jax.experimental.pallas as pl
import jax.experimental.pallas.tpu as pltpu

L = 2048
D = 512
N = 128
FF = 1376
J = 128
NB = L // J
NQ = 656
_STEP = (1, 1, 2, 2, 4, 4, 4, 4, 8, 8, 8, 8, 8, 8, 8, 8)
HI = tuple(128 * k + b for k in range(16) for b in range(0, 8, _STEP[k])) + (2048,)
NHI = len(HI)
WAITC = 14
CH = 32
RB = 512
WIN = ((0, 128), (0, 256), (128, 256), (256, 256), (320, 128), (384, 128),
       (384, 128), (448, 128), (448, 128), (512, 128), (512, 128), (512, 128),
       (512, 128), (512, 128), (512, 128), (528, 128))
GW = sum(w[1] for w in WIN)


def _q_of_m(m):
    hi = (m // 128) * 128 + (m % 8)
    return 16 * HI.index(hi) + (m % 128) // 8


def _build_tables():
    pos = np.arange(L, dtype=np.int64)
    rr = np.zeros(L, np.int64)
    for l in range(L):
        if l < 256:
            rr[l] = l
        else:
            step = 1 << (int(l).bit_length() - 8)
            lo = (l // step) * step
            rem = l - lo
            if rem * 2 < step or (rem * 2 == step and (lo // step) % 2 == 0):
                rr[l] = lo
            else:
                rr[l] = lo + step
    w = np.pi * (2 * np.arange(J) + 1) / (2 * J)
    n = np.arange(J)
    f_fwd = np.concatenate([np.cos(np.outer(w, n)), -np.sin(np.outer(w, n))], 0)
    f_inv = np.concatenate([np.cos(np.outer(n, w)), -np.sin(np.outer(n, w))], 1) / J
    g_all = np.zeros((2 * J, GW))
    off = 0
    for dl in range(NB):
        s0, ln = WIN[dl]
        for p in range(-J, J):
            l = dl * J + p
            if 0 <= l < L:
                q = _q_of_m(int(rr[l])) - s0
                assert 0 <= q < ln
                g_all[:J, off + q] += np.cos(w * p)
                g_all[J:, off + q] += -np.sin(w * p)
        off += ln
    sel = np.zeros((16, 128))
    for dd in range(8):
        sel[np.arange(16), np.arange(16) * 8 + dd] = 1.0
    del pos
    return (f_fwd.astype(np.float32), f_inv.astype(np.float32),
            g_all.astype(np.float32), sel.astype(np.float32))


_F_FWD, _F_INV, _G_ALL, _SEL = _build_tables()


def _bf(x):
    return x.astype(jnp.bfloat16)


def _rb(x):
    return x.astype(jnp.bfloat16).astype(jnp.float32)


def _cmul(a, b):
    return (a[0] * b[0] - a[1] * b[1], a[0] * b[1] + a[1] * b[0])


def _sincos(x):
    k = jnp.floor(x * 0.6366197723675814 + 0.5)
    r = x - k * 1.5703125
    r = r - k * 4.837512969970703125e-4
    r = r - k * 7.549789954891882e-8
    r2 = r * r
    sn = r + r * r2 * (-1.6666654611e-1 + r2 * (8.3321608736e-3 + r2 * -1.9515295891e-4))
    cs = 1.0 + r2 * (-0.5 + r2 * (4.166664568298827e-2 + r2 * (-1.388731625493765e-3
                                                             + r2 * 2.443315711809948e-5)))
    q = k - 4.0 * jnp.floor(k * 0.25)
    odd = (q == 1.0) | (q == 3.0)
    s0 = jnp.where(odd, cs, sn)
    c0 = jnp.where(odd, sn, cs)
    s1 = jnp.where(q >= 2.0, -s0, s0)
    c1 = jnp.where((q == 1.0) | (q == 2.0), -c0, c0)
    return s1, c1


def _gelu(x):
    c = 0.7978845608028654
    return 0.5 * x * (1.0 + jnp.tanh(c * (x + 0.044715 * (x * x * x))))


def _layernorm(x):
    m = jnp.mean(x, axis=-1, keepdims=True)
    xc = x - m
    v = jnp.mean(xc * xc, axis=-1, keepdims=True)
    den = _rb(jnp.sqrt(_rb(_rb(v) + 1e-5)))
    return _rb(_rb(x - _rb(m)) / den)


def _layernorm2(x):
    m = jnp.mean(x, axis=-1, keepdims=True)
    xc = x - m
    v = jnp.mean(xc * xc, axis=-1, keepdims=True)
    return xc / jnp.sqrt(v + 1e-5)


def _dot(a, b):
    return jnp.dot(a, b, preferred_element_type=jnp.float32)


def _dot_nt(a, b):
    return lax.dot_general(a, b, (((1,), (1,)), ((), ())),
                           preferred_element_type=jnp.float32)


def _kernel(are_ref, aim_ref, bre_ref, bim_ref, cre_ref, cim_ref, ldt_ref, dsk_ref,
            ffwd_ref, finv_ref, sel_ref,
            x_hbm, w1_hbm, w2_hbm, w3_hbm, w4_hbm, g_hbm,
            out_hbm,
            x_v, w1_v, w2_v, w3_v, w4_v, g_v, out_v,
            xn_v, h_v, u_v, kt_v, z_v,
            yr_v, yi_v, xr_v, xi_v, o_v, kd_v, dt_v, pw_v,
            sem_in, sem_out):
    copies = [pltpu.make_async_copy(s, d, sem_in.at[k]) for k, (s, d) in enumerate(
        [(x_hbm, x_v), (w1_hbm, w1_v), (g_hbm, g_v), (w2_hbm, w2_v), (w3_hbm, w3_v),
         (w4_hbm, w4_v)])]
    for c in copies:
        c.start()

    dt_row = _rb(jnp.exp(ldt_ref[...].astype(jnp.float32))).reshape(1, D)
    dt_v[...] = jnp.transpose(jnp.broadcast_to(dt_row, (N, D)))

    NCH = D // CH
    f32 = jnp.float32

    def csq(a):
        ab = a[0] * a[1]
        return (a[0] * a[0] - a[1] * a[1], ab + ab)

    def kprep(c):
        rows = pl.ds(c * CH, CH)
        dt = dt_v[rows, :]
        lr = dt * are_ref[rows, :].astype(f32)
        li = dt * aim_ref[rows, :].astype(f32)
        dbr = dt * bre_ref[rows, :].astype(f32)
        dbi = dt * bim_ref[rows, :].astype(f32)
        w = _cmul((cre_ref[rows, :].astype(f32), cim_ref[rows, :].astype(f32)), (dbr, dbi))
        e1 = jnp.exp(lr)
        sn, cs = _sincos(li)
        z1 = (e1 * cs, e1 * sn)
        z8 = csq(csq(csq(z1)))
        z128 = csq(csq(csq(csq(z8))))
        z1024 = csq(csq(csq(z128)))
        for k, v in enumerate((w, z1, z128, z1024)):
            pw_v[2 * k] = v[0]
            pw_v[2 * k + 1] = v[1]

        def put_y(j, v):
            for g in range(CH // 8):
                yr_v[g, 8 * j:8 * j + 8, :] = v[0][8 * g:8 * g + 8, :]
                yi_v[g, 8 * j:8 * j + 8, :] = v[1][8 * g:8 * g + 8, :]

        put_y(0, (jnp.ones_like(lr), jnp.zeros_like(lr)))
        y = z8
        put_y(1, y)
        for j in range(2, 16):
            y = _cmul(y, z8)
            put_y(j, y)

    def kgen(c):
        r0 = c * CH
        w, z1, z128, z1024 = [(pw_v[2 * k], pw_v[2 * k + 1]) for k in range(4)]
        ys = [(_bf(yr_v[g]), _bf(yi_v[g])) for g in range(CH // 8)]

        def put_x(i, v):
            for g in range(CH // 8):
                xr_v[g, 8 * i:8 * i + 8, :] = v[0][8 * g:8 * g + 8, :]
                xi_v[g, 8 * i:8 * i + 8, :] = v[1][8 * g:8 * g + 8, :]

        v = w
        for b in range(8):
            if b:
                v = _cmul(v, z1)
            t = v
            for k in range(8):
                if (128 * k + b) in HI:
                    if k:
                        t = _cmul(t, z128)
                    put_x(HI.index(128 * k + b), t)
        t = _cmul(w, z1024)
        for k in range(8, 17):
            if k > 8:
                t = _cmul(t, z128)
            put_x(HI.index(128 * k), t)
        for g in range(CH // 8):
            o = _dot_nt(_bf(xr_v[g]), ys[g][0]) - _dot_nt(_bf(xi_v[g]), ys[g][1])
            for i in range(NHI):
                o_v[i, pl.ds(r0 + 8 * g, 8), :] = o[8 * i:8 * i + 8, :]
        if c + 1 < NCH:
            kprep(c + 1)

    with jax.named_scope('p_kgen'):
        kprep(0)
        for c in range(NCH):
            if c == WAITC:
                copies[2].wait()
                copies[0].wait()
                copies[1].wait()
            kgen(c)

    rid = lax.broadcasted_iota(jnp.int32, (D, 128), 0)
    lid = lax.broadcasted_iota(jnp.int32, (D, 128), 1)
    keep = (rid % 8) == (lid % 8)
    keep_last = keep & (lid < 8)
    sel = sel_ref[...]
    with jax.named_scope('p_sel'):
        for i in range(NHI):
            oi = jnp.where(keep_last if HI[i] == 2048 else keep, o_v[i], 0.0)
            kd_v[16 * i:16 * i + 16, :] = _dot_nt(sel, _bf(oi))

    off = 0
    for dl in range(NB):
        s0, ln = WIN[dl]
        kt_v[dl] = _dot(g_v[:, off:off + ln], _bf(kd_v[s0:s0 + ln, :]))
        off += ln

    h_v[0:8, :] = jnp.zeros((8, D), jnp.float32)
    h_v[8 + L:16 + L, :] = jnp.zeros((8, D), jnp.float32)

    def phase1(b, carry):
        r0 = pl.multiple_of(b * RB, RB)
        xs = []
        for k in range(RB // J):
            rk = pl.multiple_of(r0 + k * J, J)
            xk = _bf(_layernorm(x_v[pl.ds(rk, J), :].astype(jnp.float32)))
            xn_v[pl.ds(rk, J), :] = xk
            u_v[b * (RB // J) + k] = _dot(ffwd_ref[...], xk)
            xs.append(xk)
        h = _gelu(_dot(jnp.concatenate(xs, axis=0), w1_v[...]))
        h_v[pl.ds(pl.multiple_of(r0 + 8, 8), RB), :] = h
        return carry

    with jax.named_scope('p_phase1'):
        lax.fori_loop(0, L // RB, phase1, 0, unroll=4)

    def zphase(t, carry):
        f0 = pl.multiple_of((t // 4) * 8, 8)
        re = pl.ds(f0, 8)
        im = pl.ds(pl.multiple_of(f0 + J, 8), 8)
        cs = pl.ds(pl.multiple_of((t % 4) * 128, 128), 128)
        GZ = 4
        for i0 in range(0, NB, GZ):
            acc = {}
            uc = {}
            for dl in range(i0 + GZ):
                kr = kt_v[dl, re, cs]
                ki = kt_v[dl, im, cs]
                ks = kr + ki
                for i in range(max(i0, dl), i0 + GZ):
                    src = i - dl
                    if src not in uc:
                        ur = u_v[src, re, cs]
                        ui = u_v[src, im, cs]
                        uc[src] = (ur, ui, ur + ui)
                    ur, ui, us = uc[src]
                    p = (kr * ur, ki * ui, ks * us)
                    acc[i] = p if i not in acc else tuple(x + y for x, y in zip(acc[i], p))
            for i in range(i0, i0 + GZ):
                s1, s2, s3 = acc[i]
                z_v[i, re, cs] = s1 - s2
                z_v[i, im, cs] = s3 - (s1 + s2)
        return carry

    with jax.named_scope('p_z'):
        lax.fori_loop(0, 64, zphase, 0, unroll=8)

    copies[3].wait()
    copies[4].wait()
    copies[5].wait()
    dsk = dsk_ref[...].astype(jnp.float32).reshape(1, D)

    HB = RB // 2

    def out_copy(b):
        r0 = pl.multiple_of(b * HB, HB)
        return pltpu.make_async_copy(out_v.at[pl.ds(r0, HB), :],
                                     out_hbm.at[pl.ds(r0, HB), :], sem_out.at[b])

    def phase2(b, carry):
        r0 = pl.multiple_of(b * RB, RB)
        ext = RB + 16
        parts = []
        for gi, sh in enumerate((1, -1, 2, -2)):
            hv = h_v[pl.ds(r0, ext), gi * 128:(gi + 1) * 128]
            hv = pltpu.roll(hv, sh % ext, 0)
            parts.append(_bf(hv[8:8 + RB, :]))
        hs = _dot(jnp.concatenate(parts, axis=1), w2_v[...])
        ys = [_dot(finv_ref[...], _bf(z_v[b * (RB // J) + k])) for k in range(RB // J)]
        y = jnp.concatenate(ys, axis=0)
        xn = xn_v[pl.ds(r0, RB), :].astype(jnp.float32)
        x1 = xn + hs
        a = _dot_nt(_bf(_layernorm2(x1)), w3_v[...])
        for hf in range(2):
            sl = slice(hf * HB, (hf + 1) * HB)
            rh = pl.multiple_of(r0 + hf * HB, HB)
            bb = x1[sl] + _dot(_bf(_gelu(a[sl])), w4_v[...])
            gate = bb * jax.nn.sigmoid(bb)
            s = y[sl] + xn[sl] * dsk
            x = x_v[pl.ds(rh, HB), :].astype(jnp.float32)
            out_v[pl.ds(rh, HB), :] = _bf(x + s * gate)
            out_copy(2 * b + hf).start()
        return carry

    with jax.named_scope('p_phase2'):
        lax.fori_loop(0, L // RB, phase2, 0, unroll=2)
    for b in range(L // HB):
        out_copy(b).wait()


@jax.jit
def pallas_recurrent_scan__ssm_conv_s4__mixer_s_mlp__prompt_kernel(
    A_u: jax.Array,
    A_A_re: jax.Array,
    A_A_im: jax.Array,
    A_B_re: jax.Array,
    A_B_im: jax.Array,
    A_C_re: jax.Array,
    A_C_im: jax.Array,
    A_log_dt: jax.Array,
    A_Dskip: jax.Array,
    B_x: jax.Array,
    B_w1: jax.Array,
    B_w2: jax.Array,
    B_w3: jax.Array,
    B_w4: jax.Array,
):
    bf16 = jnp.bfloat16
    f32 = jnp.float32
    x = A_u.reshape(L, D)
    vm = pl.BlockSpec(memory_space=pltpu.VMEM)
    hbm = pl.BlockSpec(memory_space=pltpu.HBM)
    out = pl.pallas_call(
        _kernel,
        out_shape=jax.ShapeDtypeStruct((L, D), bf16),
        in_specs=[vm] * 11 + [hbm] * 6,
        out_specs=hbm,
        scratch_shapes=[
            pltpu.VMEM((L, D), bf16),
            pltpu.VMEM((D, D), bf16),
            pltpu.VMEM((D, D), bf16),
            pltpu.VMEM((FF, D), bf16),
            pltpu.VMEM((FF, D), bf16),
            pltpu.VMEM((2 * J, GW), bf16),
            pltpu.VMEM((L, D), bf16),
            pltpu.VMEM((L, D), bf16),
            pltpu.VMEM((L + 16, D), f32),
            pltpu.VMEM((NB, 2 * J, D), f32),
            pltpu.VMEM((NB, 2 * J, D), f32),
            pltpu.VMEM((NB, 2 * J, D), f32),
            pltpu.VMEM((CH // 8, 128, N), f32),
            pltpu.VMEM((CH // 8, 128, N), f32),
            pltpu.VMEM((CH // 8, 8 * NHI, N), f32),
            pltpu.VMEM((CH // 8, 8 * NHI, N), f32),
            pltpu.VMEM((NHI, D, 128), f32),
            pltpu.VMEM((NQ, D), f32),
            pltpu.VMEM((D, N), f32),
            pltpu.VMEM((8, CH, N), f32),
            pltpu.SemaphoreType.DMA((6,)),
            pltpu.SemaphoreType.DMA((2 * L // RB,)),
        ],
        compiler_params=pltpu.CompilerParams(vmem_limit_bytes=100 * 1024 * 1024),
    )(A_A_re, A_A_im, A_B_re, A_B_im, A_C_re, A_C_im,
      A_log_dt, A_Dskip,
      jnp.asarray(_F_FWD, bf16), jnp.asarray(_F_INV, bf16), jnp.asarray(_SEL, bf16),
      *[pltpu.with_memory_space_constraint(t, pltpu.HBM)
        for t in (x, B_w1, B_w2, B_w3.T, B_w4, jnp.asarray(_G_ALL, bf16))])
    return out.reshape(1, L, D)
```
